```python
import jax
import jax.numpy as jnp

def _softmax(x, axis=-1):
    return jax.nn.softmax(x, axis=axis)

def _gelu(x):
    return jax.nn.gelu(x, approximate=True)

def _silu(x):
    return jax.nn.silu(x)

def _sigmoid(x):
    return jax.nn.sigmoid(x)

def _layernorm(x, axis=-1, eps=1e-05):
    m = jnp.mean(x, axis=axis, keepdims=True)
    v = jnp.var(x, axis=axis, keepdims=True)
    return (x - m) / jnp.sqrt(v + eps)

def _scatter_add(tgt, idx, src, axis=0):
    return tgt.at[idx].add(src)

def _segment_sum(src, seg, n):
    return jax.ops.segment_sum(src, seg, n)

class _Rng:

    def __init__(self, key):
        self._k = key

    def _next(self):
        self._k, sub = jax.random.split(self._k)
        return sub

    def normal(self, shape):
        return jax.random.normal(self._next(), shape, dtype=jnp.bfloat16)

    def randint(self, lo, hi, shape):
        return jax.random.randint(self._next(), shape, lo, hi, dtype=jnp.int32)

    def uniform(self, shape, lo=0.0, hi=1.0):
        return jax.random.uniform(self._next(), shape, jnp.bfloat16, lo, hi)

    def permutation(self, n):
        return jax.random.permutation(self._next(), n)
kernel_name = 'standalone__conformer_family_branchformer__speech'

def setup_inputs():
    _rng = _Rng(jax.random.key(int.from_bytes(__import__("os").urandom(4), "little")))
    _w = lambda a: (lambda t: t.astype(jnp.bfloat16) if jnp.issubdtype(t.dtype, jnp.floating) else t)(jnp.asarray(a))
    B, T, D, K = (2, 4000, 512, 31)
    s = float(D) ** (-0.5)
    return {'x': _w((lambda *s: _rng.normal(s) * 0.05)(B, T, D)), 'w_q': _w((lambda *s: _rng.normal(s) * 0.05)(D, D) * s), 'w_k': _w((lambda *s: _rng.normal(s) * 0.05)(D, D) * s), 'w_v': _w((lambda *s: _rng.normal(s) * 0.05)(D, D) * s), 'w_ao': _w((lambda *s: _rng.normal(s) * 0.05)(D, D) * s), 'w_up': _w((lambda *s: _rng.normal(s) * 0.05)(D, 2 * D) * s), 'dw': _w((lambda *s: _rng.normal(s) * 0.05)(K, D) * (1.0 / K)), 'w_dn': _w((lambda *s: _rng.normal(s) * 0.05)(D, D) * s), 'w_merge': _w((lambda *s: _rng.normal(s) * 0.05)(2 * D, D) * s)}

def reference(x, w_q, w_k, w_v, w_ao, w_up, dw, w_dn, w_merge):
    B, T, D = x.shape
    K = dw.shape[0]
    xa = _layernorm(x, axis=-1)
    q = jnp.einsum('btd,de->bte', xa, w_q)
    k = jnp.einsum('btd,de->bte', xa, w_k)
    v = jnp.einsum('btd,de->bte', xa, w_v)
    logits = jnp.einsum('btd,bsd->bts', q, k) * float(D) ** (-0.5)
    attn = _softmax(logits, axis=-1)
    ya = jnp.einsum('bts,bsd->btd', attn, v)
    ya = jnp.einsum('btd,de->bte', ya, w_ao)
    xc = _layernorm(x, axis=-1)
    h = _gelu(jnp.einsum('btd,de->bte', xc, w_up))
    u = h[..., :D].copy()
    g = _layernorm(h[..., D:], axis=-1)
    pad = K // 2
    gp = jnp.pad(g, ((0, 0), (pad, pad), (0, 0)))
    conv = jnp.zeros_like(g)
    for i in range(K):
        conv = conv + gp[:, i:i + T, :] * dw[i][None, None, :]
    yc = jnp.einsum('btd,de->bte', u * conv, w_dn)
    merged = jnp.concatenate([ya, yc], axis=-1)
    out = jnp.einsum('btf,fd->btd', merged, w_merge)
    return x + out
```

```python
import functools
import math

import jax
import jax.numpy as jnp
from jax import lax
import jax.experimental.pallas as pl
import jax.experimental.pallas.tpu as pltpu

LANES = 128
EPS = 1e-05
F32 = jnp.float32
BF16 = jnp.bfloat16
NT = (((1,), (1,)), ((), ()))
HALO = 16


def _ln(x, eps):
    d = x.shape[-1]
    m = jnp.sum(x, axis=-1, keepdims=True) * (1.0 / d)
    xc = x - m
    v = jnp.sum(xc * xc, axis=-1, keepdims=True) * (1.0 / d)
    return xc * lax.rsqrt(v + eps)


def _gelu2(x):
    c1 = math.sqrt(2.0 / math.pi)
    c2 = c1 * 0.044715
    t = jnp.tanh(x * (c1 + c2 * (x * x)))
    return x + x * t


def _kernel(x_ref, wq_ref, wk_ref, wv_ref, wao_ref, wup_ref, dw_ref, wdn_ref, wm_ref,
            o_ref,
            xa_s, wa_s, wo_s, dwb_s, s_s, m_s, u_s, g_s,
            *, B, T, D, K, TQ, TK, TP):
    NQ = T // TQ
    N = B * NQ
    NKV = TP // TK
    NC = D // LANES
    CPK = TK // LANES
    GP = T + 2 * HALO
    PAD = K // 2
    step = pl.program_id(0)

    def prologue():
        scale = float(D) ** (-0.5) * math.log2(math.e)
        mqk = lax.dot_general(wq_ref[...], wk_ref[...], NT, preferred_element_type=F32)
        wa_s[:, 0:D] = (mqk * scale).astype(BF16)
        wa_s[:, D:3 * D] = wup_ref[...]
        wva = jnp.dot(wv_ref[...], wao_ref[...], preferred_element_type=F32).astype(BF16)
        wo_s[0:D, :] = jnp.dot(wva, wm_ref[0:D, :], preferred_element_type=F32).astype(BF16)
        wo_s[D:2 * D, :] = (0.5 * jnp.dot(wdn_ref[...], wm_ref[D:2 * D, :],
                                          preferred_element_type=F32)).astype(BF16)
        dwf = dw_ref[...].astype(F32)
        for k in range(K):
            dwb_s[k] = jnp.broadcast_to(dwf[k:k + 1, :], (8, D))
        for b in range(B):
            xa_s[b, T:TP, :] = jnp.zeros((TP - T, D), BF16)
            for c in range(NC):
                g_s[c, b * GP:b * GP + HALO, :] = jnp.zeros((HALO, LANES), F32)
                g_s[c, b * GP + HALO + T:(b + 1) * GP, :] = jnp.zeros((HALO, LANES), F32)
        R = 80

        def ln_body(r, carry):
            for b in range(B):
                src = pl.multiple_of(b * T + r * R, 16)
                dst = pl.multiple_of(r * R, 16)
                xa_s[b, pl.ds(dst, R), :] = _ln(x_ref[pl.ds(src, R), :].astype(F32), EPS).astype(BF16)
            return carry

        lax.fori_loop(0, T // R, ln_body, 0)

    def body(do_a, do_b):
        if do_a:
            ba = step // NQ
            ia = step % NQ
            xq = xa_s[ba, pl.ds(pl.multiple_of(ia * TQ, 16), TQ), :]
        if do_b:
            sb = step - 1
            bb = sb // NQ
            ib = sb % NQ
            m_old = m_s[...]

            def probs(j):
                tiles = []
                lsum = None
                for c in range(CPK):
                    col = j * TK + c * LANES
                    p = jnp.exp2(s_s[:, col:col + LANES] - m_old)
                    lsum = p if lsum is None else lsum + p
                    tiles.append(p.astype(BF16))
                return jnp.concatenate(tiles, axis=1), lsum

            p_cur, l_acc = probs(0)

        if do_a:
            q = jnp.dot(xq, wa_s[:, 0:D], preferred_element_type=F32).astype(BF16)
            hg = _gelu2(jnp.dot(xq, wa_s[:, 2 * D:3 * D], preferred_element_type=F32))
            g = _ln(hg, 4.0 * EPS)
            grow = pl.multiple_of(ba * GP + HALO + ia * TQ, 8)
            for c in range(NC):
                g_s[c, pl.ds(grow, TQ), :] = g[:, c * LANES:(c + 1) * LANES]
            hu = _gelu2(jnp.dot(xq, wa_s[:, D:2 * D], preferred_element_type=F32))
            u_s[step % 2] = hu

        if do_b:
            gbase = pl.multiple_of(bb * GP + ib * TQ, 8)
            uslot = sb % 2

            def conv_rows(r0, R):
                cols = []
                for c in range(NC):
                    acc = None
                    for k in range(K):
                        off = r0 + HALO - PAD + k
                        gv = g_s[c, pl.ds(gbase + off, R), :].reshape(R // 8, 8, LANES)
                        term = gv * dwb_s[k, :, c * LANES:(c + 1) * LANES][None]
                        acc = term if acc is None else acc + term
                    cols.append(acc.reshape(R, LANES))
                conv = jnp.concatenate(cols, axis=1)
                return (u_s[uslot, r0:r0 + R, :] * conv).astype(BF16)

            ng = TQ // 16
            bounds = [16 * ((ng * j) // NKV) for j in range(NKV + 1)]
            yc_parts = []

        mx = None
        acc = None
        for j in range(NKV):
            def qk():
                nonlocal mx
                kj = xa_s[ba, j * TK:(j + 1) * TK, :]
                s = lax.dot_general(q, kj, NT, preferred_element_type=F32)
                for c in range(CPK):
                    col = j * TK + c * LANES
                    st = s[:, c * LANES:(c + 1) * LANES]
                    if col + LANES > T:
                        lane = lax.broadcasted_iota(jnp.int32, (TQ, LANES), 1)
                        st = jnp.where(lane < T - col, st, -jnp.inf)
                    s_s[:, col:col + LANES] = st
                    mx = st if mx is None else jnp.maximum(mx, st)

            def pv(p):
                nonlocal acc
                vj = xa_s[bb, j * TK:(j + 1) * TK, :]
                o = jnp.dot(p, vj, preferred_element_type=F32)
                acc = o if acc is None else acc + o

            if do_b:
                p_this = p_cur
                if j + 1 < NKV:
                    p_cur, l_new = probs(j + 1)
                    l_acc = l_acc + l_new
                pv(p_this)
                yc_parts.append(conv_rows(bounds[j], bounds[j + 1] - bounds[j]))
            if do_a:
                qk()

        if do_b:
            l = jnp.sum(l_acc, axis=-1, keepdims=True)
            ya = (acc * (1.0 / l)).astype(BF16)
            yc = jnp.concatenate(yc_parts, axis=0)
            out = jnp.dot(yc, wo_s[D:2 * D, :], preferred_element_type=F32)
            out = out + jnp.dot(ya, wo_s[0:D, :], preferred_element_type=F32)
            xr = x_ref[pl.ds(pl.multiple_of(sb * TQ, 16), TQ), :].astype(F32)
            o_ref[...] = (xr + out).astype(o_ref.dtype)
        if do_a:
            m_s[...] = jnp.broadcast_to(jnp.max(mx, axis=-1, keepdims=True), (TQ, LANES))

    @pl.when(step == 0)
    def _():
        prologue()
        body(True, False)

    @pl.when(jnp.logical_and(step > 0, step < N))
    def _():
        body(True, True)

    @pl.when(step == N)
    def _():
        body(False, True)


@jax.jit
def pallas_standalone__conformer_family_branchformer__speech_kernel(
    x: jax.Array,
    w_q: jax.Array,
    w_k: jax.Array,
    w_v: jax.Array,
    w_ao: jax.Array,
    w_up: jax.Array,
    dw: jax.Array,
    w_dn: jax.Array,
    w_merge: jax.Array,
):
    B, T, D = x.shape
    K = dw.shape[0]
    TQ = 400
    TK = 512
    TP = -(-T // TK) * TK
    assert T % TQ == 0 and TQ % 16 == 0 and D % LANES == 0 and K // 2 < HALO
    N = B * (T // TQ)
    x2 = x.reshape(B * T, D)

    def whole(a):
        nd = a.ndim
        return pl.BlockSpec(a.shape, lambda s: (0,) * nd, pipeline_mode=pl.Buffered(1))

    kern = functools.partial(_kernel, B=B, T=T, D=D, K=K, TQ=TQ, TK=TK, TP=TP)
    ins = (x2, w_q, w_k, w_v, w_ao, w_up, dw, w_dn, w_merge)
    out = pl.pallas_call(
        kern,
        grid=(N + 1,),
        in_specs=[whole(a) for a in ins],
        out_specs=pl.BlockSpec((TQ, D), lambda s: (jnp.maximum(s - 1, 0), 0)),
        out_shape=jax.ShapeDtypeStruct((B * T, D), x.dtype),
        scratch_shapes=[
            pltpu.VMEM((B, TP, D), BF16),
            pltpu.VMEM((D, 3 * D), BF16),
            pltpu.VMEM((2 * D, D), BF16),
            pltpu.VMEM((K, 8, D), F32),
            pltpu.VMEM((TQ, TP), F32),
            pltpu.VMEM((TQ, LANES), F32),
            pltpu.VMEM((2, TQ, D), F32),
            pltpu.VMEM((D // LANES, B * (T + 2 * HALO), LANES), F32),
        ],
        compiler_params=pltpu.CompilerParams(
            dimension_semantics=("arbitrary",),
            vmem_limit_bytes=100 * 1024 * 1024,
        ),
    )(*ins)
    return out.reshape(B, T, D)
```

```python
import functools
import math

import jax
import jax.numpy as jnp
from jax import lax
import jax.experimental.pallas as pl
import jax.experimental.pallas.tpu as pltpu

LANES = 128
EPS = 1e-05
F32 = jnp.float32
BF16 = jnp.bfloat16
U32 = jnp.uint32
NT = (((1,), (1,)), ((), ()))
CG = 16
LNJ = 3
TIER = 0
TIEC = 2
HALO = 16


def _ln(x, eps):
    d = x.shape[-1]
    m = jnp.sum(x, axis=-1, keepdims=True) * (1.0 / d)
    xc = x - m
    v = jnp.sum(xc * xc, axis=-1, keepdims=True) * (1.0 / d)
    return xc * lax.rsqrt(v + eps)


def _gelu2(x):
    c1 = math.sqrt(2.0 / math.pi)
    c2 = c1 * 0.044715
    t = jnp.tanh(x * (c1 + c2 * (x * x)))
    return x + x * t


def _pack(x):
    return pltpu.bitcast(x.astype(BF16), U32)


def _unpack(x):
    return pltpu.bitcast(x, BF16)


def _dot(a, b):
    return jnp.dot(a, b, preferred_element_type=F32)


def _dot_nt(a, b):
    return lax.dot_general(a, b, NT, preferred_element_type=F32)


def _kernel(x_hbm, wq_hbm, wk_hbm, wv_hbm, wao_hbm, wup_hbm, dw_hbm, wdn_hbm, wm_hbm,
            o_ref,
            x_s, wq_s, wk_s, wv_s, wao_s, wup_s, dw_s, wdn_s, wm_s, sems,
            xa_s, wa_s, wo_s, dwb_s, s_s, m_s, u_s, g_s, gn_s, q_s, p_s, acc_s, l_s, yc_s, z_s,
            *, B, T, D, K, TQ, TK, TP):
    NQ = T // TQ
    N = B * NQ
    NKV = TP // TK
    NC = D // LANES
    CPK = TK // LANES
    PAD = K // 2
    H = 2
    step = pl.program_id(0)

    def keys(b, j):
        start = b * (TP // H) + j * (TK // H)
        if not isinstance(start, int):
            start = pl.multiple_of(start, 8)
        return _unpack(xa_s[pl.ds(start, TK // H), :])

    def ln_rows(src, dst, rows):
        if not isinstance(src, int):
            src = pl.multiple_of(src, 16)
        dsth = dst // H
        if not isinstance(dsth, int):
            dsth = pl.multiple_of(dsth, 8)
        xa_s[pl.ds(dsth, rows // H), :] = _pack(_ln(x_s[pl.ds(src, rows), :].astype(F32), EPS))

    def qk_chunk(q, b, j, last, tok=None):
        s = _dot_nt(q, keys(b, j))
        if tok is not None:
            tok[0] = s
        mx = None
        for c in range(CPK):
            st = s[:, c * LANES:(c + 1) * LANES]
            if last:
                valid = T - (NKV - 1) * TK - c * LANES
                if valid < LANES:
                    lane = lax.broadcasted_iota(jnp.int32, (TQ, LANES), 1)
                    st = jnp.where(lane < valid, st, -jnp.inf)
            s_s[j, :, c * LANES:(c + 1) * LANES] = st
            mx = st if mx is None else jnp.maximum(mx, st)
        return mx

    def probs(j, m):
        tiles = []
        lsum = None
        for c in range(CPK):
            p = jnp.exp2(s_s[j, :, c * LANES:(c + 1) * LANES] - m)
            lsum = p if lsum is None else lsum + p
            tiles.append(p.astype(BF16))
        return jnp.concatenate(tiles, axis=1), lsum

    def up_g(xq):
        return _ln(_gelu2(_dot(xq, _unpack(wa_s[:, 2 * D:3 * D]))), 4.0 * EPS)

    def up_u(xq):
        return _gelu2(_dot(xq, _unpack(wa_s[:, D:2 * D])))

    def store_g(ref, row, g):
        for c in range(NC):
            ref[c, row:row + g.shape[0], :] = g[:, c * LANES:(c + 1) * LANES]

    def shift_g(seq_start):
        for c in range(NC):
            g_s[c, 0:HALO, :] = jnp.where(seq_start, 0.0, g_s[c, TQ:TQ + HALO, :])
            g_s[c, HALO:HALO + TQ, :] = gn_s[c]

    def conv_rows(r0, R, chain=None):
        G = R if chain is None else CG
        rows = []
        for rr in range(0, R, G):
            cols = []
            for c in range(NC):
                acc = None
                for k in range(K):
                    off = HALO - PAD + k
                    gv = g_s[c, pl.ds(r0 + rr + off, G), :].reshape(G // 8, 8, LANES)
                    term = gv * dwb_s[k, :, c * LANES:(c + 1) * LANES][None]
                    if acc is None:
                        if chain is not None and chain[1] is not None:
                            term = jnp.where(chain[0], chain[1], term)
                        acc = term
                    else:
                        acc = acc + term
                if chain is not None:
                    chain[1] = acc
                cols.append(acc.reshape(G, LANES))
            rows.append(jnp.concatenate(cols, axis=1))
        return jnp.concatenate(rows, axis=0)

    def finish(sb, acc, l_acc, yc):
        l = jnp.sum(l_acc, axis=-1, keepdims=True)
        ya = (acc * (1.0 / l)).astype(BF16)
        out = _dot(yc, _unpack(wo_s[D // H:2 * D // H, :]))
        out = out + _dot(ya, _unpack(wo_s[0:D // H, :]))
        row = sb * TQ
        if not isinstance(row, int):
            row = pl.multiple_of(row, 16)
        xr = x_s[pl.ds(row, TQ), :].astype(F32)
        o_ref[...] = (xr + out).astype(o_ref.dtype)

    def store_max(mx):
        m_s[...] = jnp.broadcast_to(jnp.max(mx, axis=-1, keepdims=True), (TQ, LANES))

    def first_step():
        NW = 8
        wcopies = {}
        for i, (name, src, dst) in enumerate((
                ('wq', wq_hbm, wq_s), ('wk', wk_hbm, wk_s), ('wv', wv_hbm, wv_s), ('wao', wao_hbm, wao_s),
                ('wup', wup_hbm, wup_s), ('dw', dw_hbm, dw_s), ('wm', wm_hbm, wm_s), ('wdn', wdn_hbm, wdn_s))):
            wcopies[name] = pltpu.make_async_copy(src, dst, sems.at[i])

        def xcopy(c):
            rows = TK if not (isinstance(c, int) and c == NKV - 1) else T - (NKV - 1) * TK
            start = c * TK
            if not isinstance(start, int):
                start = pl.multiple_of(start, TK)
            return pltpu.make_async_copy(x_hbm.at[pl.ds(start, rows), :], x_s.at[pl.ds(start, rows), :],
                                         sems.at[NW + c])

        xrest = pltpu.make_async_copy(x_hbm.at[pl.ds(T, (B - 1) * T), :], x_s.at[pl.ds(T, (B - 1) * T), :],
                                      sems.at[NW + NKV])
        wcopies['wq'].start()
        wcopies['wk'].start()
        xcopy(0).start()
        wcopies['wv'].start()
        wcopies['wao'].start()
        for c in range(1, NKV):
            xcopy(c).start()
        for name in ('wup', 'dw', 'wm', 'wdn'):
            wcopies[name].start()
        xrest.start()

        z_s[0] = 0
        z_s[1] = 0
        z_s[2] = 0
        for b in range(B):
            xa_s[(b * TP + T) // H:(b + 1) * TP // H, :] = jnp.zeros(((TP - T) // H, D), U32)
        store_g(g_s, TQ, jnp.zeros((HALO, D), F32))
        m_s[...] = jnp.full((TQ, LANES), -jnp.inf, F32)

        wcopies['wq'].wait()
        wcopies['wk'].wait()
        xcopy(0).wait()
        scale = float(D) ** (-0.5) * math.log2(math.e)
        mqk = _pack(_dot_nt(wq_s[...], wk_s[...]) * scale)
        wa_s[:, 0:D] = mqk
        ln_rows(0, 0, TK)
        xq = _unpack(xa_s[0:TQ // H, :])
        q_s[...] = _pack(_dot(xq, _unpack(mqk)))
        wcopies['wv'].wait()
        wcopies['wao'].wait()
        wv_s[...] = _dot(wv_s[...], wao_s[...]).astype(BF16)

        def loop(c, carry):
            xcopy(c + 1).wait()
            mx = qk_chunk(_unpack(q_s[...]), 0, c, False)
            m_s[...] = jnp.maximum(m_s[...], mx)
            ln_rows((c + 1) * TK, (c + 1) * TK, TK)
            return carry

        lax.fori_loop(0, NKV - 2, loop, 0)

        xcopy(NKV - 1).wait()
        wcopies['wup'].wait()
        wcopies['dw'].wait()
        q = _unpack(q_s[...])
        mx = jnp.maximum(m_s[...], qk_chunk(q, 0, NKV - 2, False))
        ln_rows((NKV - 1) * TK, (NKV - 1) * TK, T - (NKV - 1) * TK)
        wa_s[:, D:3 * D] = _pack(wup_s[...])
        xq = _unpack(xa_s[0:TQ // H, :])
        store_g(gn_s, 0, up_g(xq))
        u_s[0] = up_u(xq)
        mx = jnp.maximum(mx, qk_chunk(q, 0, NKV - 1, True))
        store_max(mx)
        dwf = dw_s[...].astype(F32)
        for k in range(K):
            dwb_s[k] = jnp.broadcast_to(dwf[k:k + 1, :], (8, D))
        wcopies['wm'].wait()
        wcopies['wdn'].wait()
        xrest.wait()
        wo_s[0:D // H, :] = _pack(_dot(wv_s[...], wm_s[0:D, :]))
        wo_s[D // H:2 * D // H, :] = _pack(0.5 * _dot(wdn_s[...], wm_s[D:2 * D, :]))
        ln_rows(T, TP, TQ)

    def main_step():
        ba = step // NQ
        ia = step % NQ
        sb = step - 1
        bb = sb // NQ
        sa = step % 2
        so = 1 - sa
        shift_g(sb % NQ == 0)
        never = z_s[0] > 0
        never2 = z_s[1] > 0
        never3 = z_s[2] > 0
        tok = [None]

        def after(lhs):
            dep = tok[0]
            if dep is None:
                return _unpack(lhs)
            n = TQ // H
            r0 = TIER
            d = pltpu.bitcast(dep[r0:r0 + n, TIEC * LANES:(TIEC + 1) * LANES], U32)
            head = jnp.where(never3, d, lhs[:, 0:LANES])
            return _unpack(jnp.concatenate([head, lhs[:, LANES:]], axis=1))

        def mm(lhs, rhs):
            tok[0] = _dot(after(lhs), rhs)
            return tok[0]

        m_old = m_s[...]
        xq = xa_s[pl.ds(pl.multiple_of(ba * (TP // H) + ia * (TQ // H), 8), TQ // H), :]
        p_cur, l_acc = probs(0, m_old)
        qp = _pack(mm(xq, _unpack(wa_s[:, 0:D])))
        g_new = _ln(_gelu2(mm(xq, _unpack(wa_s[:, 2 * D:3 * D]))), 4.0 * EPS)
        store_g(gn_s, 0, g_new)
        store_g(g_s, HALO + TQ, jnp.where(ia == 0, 0.0, g_new[0:HALO, :]))
        u_s[sa] = _gelu2(mm(xq, _unpack(wa_s[:, D:2 * D])))
        nxt = jnp.minimum(step + NQ, N - 1)
        xn = _pack(_ln(x_s[pl.ds(pl.multiple_of(nxt * TQ, 16), TQ), :].astype(F32), EPS))
        conv = conv_rows(0, TQ, [never, None])
        yc = _pack(u_s[so] * conv)
        mx = None
        acc = None
        for j in range(NKV):
            p_this = p_cur
            if j + 1 < NKV:
                m_use = m_old
                if mx is not None:
                    m_use = jnp.where(never, mx, m_use)
                p_cur, l_new = probs(j + 1, m_use)
                l_acc = l_acc + l_new
            o = mm(pltpu.bitcast(p_this, U32), keys(bb, j))
            acc = o if acc is None else acc + o
            qj = qp
            if j == LNJ:
                qj = jnp.where(never2, xn, qp)
            mj = qk_chunk(after(qj), ba, j, j == NKV - 1, tok)
            mx = mj if mx is None else jnp.maximum(mx, mj)
        l = jnp.sum(l_acc, axis=-1, keepdims=True)
        ya = _pack(acc * (1.0 / l))
        out = mm(yc, _unpack(wo_s[D // H:2 * D // H, :]))
        out = out + mm(ya, _unpack(wo_s[0:D // H, :]))
        xr = x_s[pl.ds(pl.multiple_of(sb * TQ, 16), TQ), :].astype(F32)
        o_ref[...] = (xr + out).astype(o_ref.dtype)
        store_max(mx)
        dst = pl.multiple_of((nxt // NQ) * (TP // H) + (nxt % NQ) * (TQ // H), 8)
        late = pltpu.bitcast(mx[0:TQ // H, :], U32)
        for c in range(NC):
            xa_s[pl.ds(dst, TQ // H), c * LANES:(c + 1) * LANES] = jnp.where(
                never, late, xn[:, c * LANES:(c + 1) * LANES])

    def last_step():
        sb = N - 1
        bb = B - 1
        uslot = sb % 2
        shift_g(NQ == 1)
        store_g(g_s, HALO + TQ, jnp.zeros((HALO, D), F32))
        RL = 48
        p0, l0 = probs(0, m_s[...])
        p_s[...] = pltpu.bitcast(p0, U32)
        l_s[...] = l0
        acc_s[...] = jnp.zeros((TQ, D), F32)

        def loop(j, carry):
            p_this = _unpack(p_s[...])
            p_next, l_new = probs(j + 1, m_s[...])
            acc_s[...] += _dot(p_this, keys(bb, j))
            p_s[...] = pltpu.bitcast(p_next, U32)
            l_s[...] += l_new
            r0 = pl.multiple_of(j * RL, 16)
            yc = u_s[uslot, pl.ds(r0, RL), :] * conv_rows(r0, RL)
            yc_s[pl.ds(pl.multiple_of(j * (RL // H), 8), RL // H), :] = _pack(yc)
            return carry

        lax.fori_loop(0, NKV - 1, loop, 0)
        acc = acc_s[...] + _dot(_unpack(p_s[...]), keys(bb, NKV - 1))
        r0 = (NKV - 1) * RL
        yc_s[r0 // H:TQ // H, :] = _pack(u_s[uslot, r0:TQ, :] * conv_rows(r0, TQ - r0))
        finish(sb, acc, l_s[...], _unpack(yc_s[...]))

    @pl.when(step == 0)
    def _():
        with jax.named_scope("first_step"):
            first_step()

    @pl.when(jnp.logical_and(step > 0, step < N))
    def _():
        with jax.named_scope("main_step"):
            main_step()

    @pl.when(step == N)
    def _():
        with jax.named_scope("last_step"):
            last_step()


@jax.jit
def pallas_standalone__conformer_family_branchformer__speech_kernel(
    x: jax.Array,
    w_q: jax.Array,
    w_k: jax.Array,
    w_v: jax.Array,
    w_ao: jax.Array,
    w_up: jax.Array,
    dw: jax.Array,
    w_dn: jax.Array,
    w_merge: jax.Array,
):
    B, T, D = x.shape
    K = dw.shape[0]
    TQ = 400
    TK = 512
    TP = -(-T // TK) * TK
    NKV = TP // TK
    assert T % TQ == 0 and TQ % 16 == 0 and D % LANES == 0 and K // 2 < HALO
    assert TQ <= TK and B >= 2 and NKV >= 3 and T % 16 == 0
    N = B * (T // TQ)
    x2 = x.reshape(B * T, D)

    kern = functools.partial(_kernel, B=B, T=T, D=D, K=K, TQ=TQ, TK=TK, TP=TP)
    ins = (x2, w_q, w_k, w_v, w_ao, w_up, dw, w_dn, w_merge)
    out = pl.pallas_call(
        kern,
        grid=(N + 1,),
        in_specs=[pl.BlockSpec(memory_space=pl.ANY) for _ in ins],
        out_specs=pl.BlockSpec((TQ, D), lambda s: (jnp.maximum(s - 1, 0), 0)),
        out_shape=jax.ShapeDtypeStruct((B * T, D), x.dtype),
        scratch_shapes=[pltpu.VMEM(a.shape, a.dtype) for a in ins] + [
            pltpu.SemaphoreType.DMA((8 + NKV + 1,)),
            pltpu.VMEM((B * TP // 2, D), U32),
            pltpu.VMEM((D // 2, 3 * D), U32),
            pltpu.VMEM((D, D), U32),
            pltpu.VMEM((K, 8, D), F32),
            pltpu.VMEM((NKV, TQ, TK), F32),
            pltpu.VMEM((TQ, LANES), F32),
            pltpu.VMEM((2, TQ, D), F32),
            pltpu.VMEM((D // LANES, TQ + 2 * HALO, LANES), F32),
            pltpu.VMEM((D // LANES, TQ, LANES), F32),
            pltpu.VMEM((TQ // 2, D), U32),
            pltpu.VMEM((TQ // 2, TK), U32),
            pltpu.VMEM((TQ, D), F32),
            pltpu.VMEM((TQ, LANES), F32),
            pltpu.VMEM((TQ // 2, D), U32),
            pltpu.SMEM((3,), jnp.int32),
        ],
        compiler_params=pltpu.CompilerParams(
            dimension_semantics=("arbitrary",),
            vmem_limit_bytes=100 * 1024 * 1024,
        ),
    )(*ins)
    return out.reshape(B, T, D)
```

```python
import functools
import math

import jax
import jax.numpy as jnp
from jax import lax
import jax.experimental.pallas as pl
import jax.experimental.pallas.tpu as pltpu

LANES = 128
EPS = 1e-05
F32 = jnp.float32
BF16 = jnp.bfloat16
U32 = jnp.uint32
NT = (((1,), (1,)), ((), ()))
CG = 16
LNJ = 3
TIER = 0
TIEC = 2
TIEN = 200
GJ = 4
LCG = 16
HALO = 16


def _ln(x, eps):
    d = x.shape[-1]
    m = jnp.sum(x, axis=-1, keepdims=True) * (1.0 / d)
    xc = x - m
    v = jnp.sum(xc * xc, axis=-1, keepdims=True) * (1.0 / d)
    return xc * lax.rsqrt(v + eps)


def _gelu2(x):
    c1 = math.sqrt(2.0 / math.pi)
    c2 = c1 * 0.044715
    t = jnp.tanh(x * (c1 + c2 * (x * x)))
    return x + x * t


def _pack(x):
    return pltpu.bitcast(x.astype(BF16), U32)


def _unpack(x):
    return pltpu.bitcast(x, BF16)


def _dot(a, b):
    return jnp.dot(a, b, preferred_element_type=F32)


def _dot_nt(a, b):
    return lax.dot_general(a, b, NT, preferred_element_type=F32)


def _kernel(x_hbm, wq_hbm, wk_hbm, wv_hbm, wao_hbm, wup_hbm, dw_hbm, wdn_hbm, wm_hbm,
            o_ref,
            x_s, wq_s, wk_s, wv_s, wao_s, wup_s, dw_s, wdn_s, wm_s, sems,
            xa_s, wa_s, wo_s, dwb_s, s_s, m_s, u_s, g_s, gn_s, acc_s, l_s, yc_s, z_s,
            *, B, T, D, K, TQ, TK, TP):
    NQ = T // TQ
    N = B * NQ
    NKV = TP // TK
    NC = D // LANES
    CPK = TK // LANES
    PAD = K // 2
    H = 2
    step = pl.program_id(0)

    def keys(b, j):
        start = b * (TP // H) + j * (TK // H)
        if not isinstance(start, int):
            start = pl.multiple_of(start, 8)
        return _unpack(xa_s[pl.ds(start, TK // H), :])

    def ln_rows(src, dst, rows):
        if not isinstance(src, int):
            src = pl.multiple_of(src, 16)
        dsth = dst // H
        if not isinstance(dsth, int):
            dsth = pl.multiple_of(dsth, 8)
        xa_s[pl.ds(dsth, rows // H), :] = _pack(_ln(x_s[pl.ds(src, rows), :].astype(F32), EPS))

    def qk_chunk(q, b, j, last, tok=None):
        s = _dot_nt(q, keys(b, j))
        if tok is not None:
            tok[0] = s
        mx = None
        for c in range(CPK):
            st = s[:, c * LANES:(c + 1) * LANES]
            if last:
                valid = T - (NKV - 1) * TK - c * LANES
                if valid < LANES:
                    lane = lax.broadcasted_iota(jnp.int32, (TQ, LANES), 1)
                    st = jnp.where(lane < valid, st, -jnp.inf)
            s_s[j, :, c * LANES:(c + 1) * LANES] = st
            mx = st if mx is None else jnp.maximum(mx, st)
        return mx

    def probs(j, m, raw=False):
        tiles = []
        lsum = None
        for c in range(CPK):
            p = jnp.exp2(s_s[j, :, c * LANES:(c + 1) * LANES] - m)
            lsum = p if lsum is None else lsum + p
            tiles.append(p)
        if raw:
            return tiles, lsum
        return jnp.concatenate(tiles, axis=1).astype(BF16), lsum

    def up_g(xq):
        return _ln(_gelu2(_dot(xq, _unpack(wa_s[:, 2 * D:3 * D]))), 4.0 * EPS)

    def up_u(xq):
        return _gelu2(_dot(xq, _unpack(wa_s[:, D:2 * D])))

    def store_g(ref, row, g):
        for c in range(NC):
            ref[c, row:row + g.shape[0], :] = g[:, c * LANES:(c + 1) * LANES]

    def shift_g(seq_start):
        for c in range(NC):
            g_s[c, 0:HALO, :] = jnp.where(seq_start, 0.0, g_s[c, TQ:TQ + HALO, :])
            g_s[c, HALO:HALO + TQ, :] = gn_s[c, HALO:HALO + TQ, :]

    def conv_rows(r0, R, chain=None, cg=None):
        G = R if chain is None else (cg or CG)
        rows = []
        for rr in range(0, R, G):
            cols = []
            for c in range(NC):
                acc = None
                for k in range(K):
                    off = HALO - PAD + k
                    gv = g_s[c, pl.ds(r0 + rr + off, G), :].reshape(G // 8, 8, LANES)
                    term = gv * dwb_s[k, :, c * LANES:(c + 1) * LANES][None]
                    if acc is None:
                        if chain is not None and chain[1] is not None:
                            term = jnp.where(chain[0], chain[1], term)
                        acc = term
                    else:
                        acc = acc + term
                if chain is not None:
                    chain[1] = acc
                cols.append(acc.reshape(G, LANES))
            rows.append(jnp.concatenate(cols, axis=1))
        return jnp.concatenate(rows, axis=0)

    def finish(sb, acc, l_acc, yc):
        l = jnp.sum(l_acc, axis=-1, keepdims=True)
        ya = (acc * (1.0 / l)).astype(BF16)
        out = _dot(yc, _unpack(wo_s[D // H:2 * D // H, :]))
        out = out + _dot(ya, _unpack(wo_s[0:D // H, :]))
        row = sb * TQ
        if not isinstance(row, int):
            row = pl.multiple_of(row, 16)
        xr = x_s[pl.ds(row, TQ), :].astype(F32)
        o_ref[...] = (xr + out).astype(o_ref.dtype)

    def store_max(mx):
        m_s[...] = jnp.broadcast_to(jnp.max(mx, axis=-1, keepdims=True), (TQ, LANES))

    def tie(flag, dep, val, n):
        if n == val.shape[0]:
            return jnp.where(flag, dep[0:n], val)
        return jnp.concatenate([jnp.where(flag, dep[0:n], val[0:n]), val[n:]], axis=0)

    def tie_bf16(flag, dep, val):
        head = pltpu.bitcast(val[0:16, 0:LANES], U32)
        head = _unpack(jnp.where(flag, pltpu.bitcast(dep, U32), head))
        top = jnp.concatenate([head, val[0:16, LANES:]], axis=1)
        return jnp.concatenate([top, val[16:, :]], axis=0)

    def first_step():
        NA = 2
        copies = {}
        plan = (
            ('wq', wq_hbm, wq_s), ('wk', wk_hbm, wk_s),
            ('xa', x_hbm.at[pl.ds(0, NA * TK), :], x_s.at[pl.ds(0, NA * TK), :]),
            ('xb', x_hbm.at[pl.ds(NA * TK, T - NA * TK), :], x_s.at[pl.ds(NA * TK, T - NA * TK), :]),
            ('wup', wup_hbm, wup_s), ('dw', dw_hbm, dw_s),
            ('xc', x_hbm.at[pl.ds(T, TQ), :], x_s.at[pl.ds(T, TQ), :]),
            ('wv', wv_hbm, wv_s), ('wao', wao_hbm, wao_s), ('wdn', wdn_hbm, wdn_s), ('wm', wm_hbm, wm_s),
            ('xd', x_hbm.at[pl.ds(T + TQ, (B - 1) * T - TQ), :], x_s.at[pl.ds(T + TQ, (B - 1) * T - TQ), :]),
        )
        for i, (name, src, dst) in enumerate(plan):
            copies[name] = pltpu.make_async_copy(src, dst, sems.at[i])
            copies[name].start()

        z_s[0] = 0
        z_s[1] = 0
        z_s[2] = 0
        for b in range(B):
            xa_s[(b * TP + T) // H:(b + 1) * TP // H, :] = jnp.zeros(((TP - T) // H, D), U32)
        store_g(g_s, TQ, jnp.zeros((HALO, D), F32))
        acc_s[...] = jnp.zeros((TQ, D), F32)
        l_s[...] = jnp.zeros((TQ, LANES), F32)

        def ln_chunk(c):
            ln_rows(c * TK, c * TK, min(TK, T - c * TK))

        copies['wq'].wait()
        copies['wk'].wait()
        scale = float(D) ** (-0.5) * math.log2(math.e)
        wa_s[:, 0:D] = _pack(_dot_nt(wq_s[...], wk_s[...]) * scale)

        copies['xa'].wait()
        ln_chunk(0)
        q = _dot(_unpack(xa_s[0:TQ // H, :]), _unpack(wa_s[:, 0:D])).astype(BF16)
        mx = None
        for c in range(NA):
            if c > 0:
                ln_chunk(c)
            mj = qk_chunk(q, 0, c, False)
            mx = mj if mx is None else jnp.maximum(mx, mj)

        copies['xb'].wait()
        for c in range(NA, NKV):
            ln_chunk(c)
            mx = jnp.maximum(mx, qk_chunk(q, 0, c, c == NKV - 1))

        for name in ('wup', 'dw', 'xc', 'wv', 'wao', 'wdn', 'wm'):
            copies[name].wait()
        never = z_s[0] > 0
        zero = pl.multiple_of(z_s[0], 8)
        store_max(mx)
        xq = _unpack(xa_s[0:TQ // H, :])
        store_g(gn_s, HALO, _ln(_gelu2(_dot(xq, wup_s[:, D:2 * D])), 4.0 * EPS))
        u_s[0] = _gelu2(_dot(xq, wup_s[:, 0:D]))
        wa_s[:, D:3 * D] = _pack(wup_s[...])
        dwf = dw_s[...].astype(F32)
        for k in range(K):
            dwb_s[k] = jnp.broadcast_to(dwf[k:k + 1, :], (8, D))
        ln_rows(T, TP, TQ)
        wva = _dot(tie_bf16(never, gn_s[0, pl.ds(zero + HALO, 8), :], wv_s[...]), wao_s[...]).astype(BF16)
        lhs = tie_bf16(never, u_s[0, pl.ds(zero, 8), 0:LANES], wdn_s[...])
        wo_s[D // H:2 * D // H, :] = _pack(0.5 * _dot(lhs, wm_s[D:2 * D, :]))
        lhs = tie_bf16(never, xa_s[pl.ds(zero, 8), 0:LANES], wva)
        wo_s[0:D // H, :] = _pack(_dot(lhs, wm_s[0:D, :]))
        copies['xd'].wait()

    def main_step():
        ba = step // NQ
        ia = step % NQ
        sb = step - 1
        bb = sb // NQ
        sa = step % 2
        so = 1 - sa
        shift_g(sb % NQ == 0)
        never = z_s[0] > 0
        never2 = z_s[1] > 0
        never3 = z_s[2] > 0
        tok = [None]

        def prev_tile():
            return tok[0][TIER:, TIEC * LANES:(TIEC + 1) * LANES]

        def after_packed(lhs):
            if tok[0] is None:
                return _unpack(lhs)
            head = tie(never3, pltpu.bitcast(prev_tile(), U32), lhs[:, 0:LANES], min(TIEN, TQ // H))
            return _unpack(jnp.concatenate([head, lhs[:, LANES:]], axis=1))

        def after_tiles(tiles):
            tiles = list(tiles)
            tiles[1] = tie(never3, prev_tile(), tiles[1], TIEN)
            return jnp.concatenate(tiles, axis=1).astype(BF16)

        def split(v):
            return [v[:, c * LANES:(c + 1) * LANES] for c in range(v.shape[1] // LANES)]

        def mm(lhs, rhs):
            tok[0] = _dot(lhs, rhs)
            return tok[0]

        m_old = m_s[...]
        xq = xa_s[pl.ds(pl.multiple_of(ba * (TP // H) + ia * (TQ // H), 8), TQ // H), :]
        qp = _pack(mm(after_packed(xq), _unpack(wa_s[:, 0:D])))
        g_new = _ln(_gelu2(mm(after_packed(xq), _unpack(wa_s[:, 2 * D:3 * D]))), 4.0 * EPS)
        store_g(gn_s, HALO, g_new)
        store_g(g_s, HALO + TQ, jnp.where(ia == 0, 0.0, g_new[0:HALO, :]))
        u_s[sa] = _gelu2(mm(after_packed(xq), _unpack(wa_s[:, D:2 * D])))
        nxt = jnp.minimum(step + NQ, N - 1)
        xn = _pack(_ln(x_s[pl.ds(pl.multiple_of(nxt * TQ, 16), TQ), :].astype(F32), EPS))
        conv = conv_rows(0, TQ, [never, None])
        yc = u_s[so] * conv
        mx = None
        mx_prev = None
        acc = None
        l_acc = None
        for j in range(NKV):
            m_use = m_old
            if mx_prev is not None:
                m_use = jnp.where(never, mx_prev, m_use)
            tiles, l_new = probs(j, m_use, raw=True)
            l_acc = l_new if l_acc is None else l_acc + l_new
            tiles[0] = jnp.where(never2, l_acc, tiles[0])
            o = mm(after_tiles(tiles), keys(bb, j))
            acc = o if acc is None else acc + o
            qj = qp
            if j == LNJ:
                qj = jnp.where(never2, xn, qp)
            if j == GJ:
                gdep = gn_s[0, pl.ds(pl.multiple_of(z_s[0] + HALO, 8), 8), :]
                qj = jnp.concatenate([qj[:, 0:LANES], tie(never2, pltpu.bitcast(gdep, U32), qj[:, LANES:2 * LANES], 8), qj[:, 2 * LANES:]], axis=1)
            mx_prev = mx
            mj = qk_chunk(after_packed(qj), ba, j, j == NKV - 1, tok)
            mx = mj if mx is None else jnp.maximum(mx, mj)
        l = jnp.sum(l_acc, axis=-1, keepdims=True)
        ya = acc * (1.0 / l)
        out = mm(after_tiles(split(yc)), _unpack(wo_s[D // H:2 * D // H, :]))
        out = out + mm(after_tiles(split(ya)), _unpack(wo_s[0:D // H, :]))
        xr = x_s[pl.ds(pl.multiple_of(sb * TQ, 16), TQ), :].astype(F32)
        o_ref[...] = (xr + out).astype(o_ref.dtype)
        store_max(mx)
        dst = pl.multiple_of((nxt // NQ) * (TP // H) + (nxt % NQ) * (TQ // H), 8)
        late = pltpu.bitcast(mx[0:TQ // H, :], U32)
        for c in range(NC):
            xa_s[pl.ds(dst, TQ // H), c * LANES:(c + 1) * LANES] = jnp.where(
                never, late, xn[:, c * LANES:(c + 1) * LANES])

    def last_step():
        sb = N - 1
        bb = B - 1
        uslot = sb % 2
        CPI = 2
        NIT = NKV // CPI
        RL = 16 * (-(-TQ // (16 * NIT)))
        never = z_s[0] > 0
        never2 = z_s[1] > 0
        for c in range(NC):
            gn_s[c, 0:HALO, :] = jnp.where(NQ == 1, 0.0, g_s[c, TQ:TQ + HALO, :])
        store_g(gn_s, HALO + TQ, jnp.zeros((HALO, D), F32))

        def attend(j0):
            acc = acc_s[...]
            l_acc = l_s[...]
            for jj in range(CPI):
                tiles, l_new = probs(j0 + jj, m_s[...], raw=True)
                l_acc = l_acc + l_new
                tiles[0] = jnp.where(never2, l_acc, tiles[0])
                acc = acc + _dot(jnp.concatenate(tiles, axis=1).astype(BF16), keys(bb, j0 + jj))
            return acc, l_acc

        def loop(t, carry):
            acc, l_acc = attend(t * CPI)
            acc_s[...] = acc
            l_s[...] = l_acc
            r0 = pl.multiple_of(jnp.minimum(t * RL, TQ - RL), 16)
            for c in range(NC):
                g_s[c, 0:RL + 2 * HALO, :] = gn_s[c, pl.ds(r0, RL + 2 * HALO), :]
            yc = u_s[uslot, pl.ds(r0, RL), :] * conv_rows(0, RL, [never, None], LCG)
            yc_s[pl.ds(pl.multiple_of(r0 // H, 8), RL // H), :] = _pack(yc)
            return carry

        lax.fori_loop(0, NIT, loop, 0)
        finish(sb, acc_s[...], l_s[...], _unpack(yc_s[...]))

    @pl.when(step == 0)
    def _():
        first_step()

    @pl.when(jnp.logical_and(step > 0, step < N))
    def _():
        main_step()

    @pl.when(step == N)
    def _():
        last_step()


@jax.jit
def pallas_standalone__conformer_family_branchformer__speech_kernel(
    x: jax.Array,
    w_q: jax.Array,
    w_k: jax.Array,
    w_v: jax.Array,
    w_ao: jax.Array,
    w_up: jax.Array,
    dw: jax.Array,
    w_dn: jax.Array,
    w_merge: jax.Array,
):
    B, T, D = x.shape
    K = dw.shape[0]
    TQ = 400
    TK = 512
    TP = -(-T // TK) * TK
    NKV = TP // TK
    assert T % TQ == 0 and TQ % 16 == 0 and D % LANES == 0 and K // 2 < HALO
    assert TQ <= TK and B >= 2 and NKV >= 3 and T % 16 == 0
    N = B * (T // TQ)
    x2 = x.reshape(B * T, D)

    kern = functools.partial(_kernel, B=B, T=T, D=D, K=K, TQ=TQ, TK=TK, TP=TP)
    ins = (x2, w_q, w_k, w_v, w_ao, w_up, dw, w_dn, w_merge)
    out = pl.pallas_call(
        kern,
        grid=(N + 1,),
        in_specs=[pl.BlockSpec(memory_space=pl.ANY) for _ in ins],
        out_specs=pl.BlockSpec((TQ, D), lambda s: (jnp.maximum(s - 1, 0), 0)),
        out_shape=jax.ShapeDtypeStruct((B * T, D), x.dtype),
        scratch_shapes=[pltpu.VMEM(a.shape, a.dtype) for a in ins] + [
            pltpu.SemaphoreType.DMA((12,)),
            pltpu.VMEM((B * TP // 2, D), U32),
            pltpu.VMEM((D // 2, 3 * D), U32),
            pltpu.VMEM((D, D), U32),
            pltpu.VMEM((K, 8, D), F32),
            pltpu.VMEM((NKV, TQ, TK), F32),
            pltpu.VMEM((TQ, LANES), F32),
            pltpu.VMEM((2, TQ, D), F32),
            pltpu.VMEM((D // LANES, TQ + 2 * HALO, LANES), F32),
            pltpu.VMEM((D // LANES, TQ + 2 * HALO, LANES), F32),
            pltpu.VMEM((TQ, D), F32),
            pltpu.VMEM((TQ, LANES), F32),
            pltpu.VMEM((TQ // 2, D), U32),
            pltpu.SMEM((3,), jnp.int32),
        ],
        compiler_params=pltpu.CompilerParams(
            dimension_semantics=("arbitrary",),
            vmem_limit_bytes=100 * 1024 * 1024,
        ),
    )(*ins)
    return out.reshape(B, T, D)
```

```python
import functools
import math

import jax
import jax.numpy as jnp
from jax import lax
import jax.experimental.pallas as pl
import jax.experimental.pallas.tpu as pltpu

LANES = 128
EPS = 1e-05
F32 = jnp.float32
BF16 = jnp.bfloat16
U32 = jnp.uint32
NT = (((1,), (1,)), ((), ()))
CG = 16
LNJ = 1
TIER = 0
TIEC = 0
TIEN = 8
GJ = 3
LCG = 16
PG = 8
PW = 1
PLAG = 6
GPOS = -1
UPOS = -1
OUTA = 0
TJ0 = 1
TTC = 2
LCPI = 2
FC2 = 5
FSPLIT = 2
HALO = 16


def _ln(x, eps):
    d = x.shape[-1]
    m = jnp.sum(x, axis=-1, keepdims=True) * (1.0 / d)
    xc = x - m
    v = jnp.sum(xc * xc, axis=-1, keepdims=True) * (1.0 / d)
    return xc * lax.rsqrt(v + eps)


def _gelu2(x):
    c1 = math.sqrt(2.0 / math.pi)
    c2 = c1 * 0.044715
    t = jnp.tanh(x * (c1 + c2 * (x * x)))
    return x + x * t


def _pack(x):
    return pltpu.bitcast(x.astype(BF16), U32)


def _unpack(x):
    return pltpu.bitcast(x, BF16)


def _dot(a, b):
    return jnp.dot(a, b, preferred_element_type=F32)


def _dot_nt(a, b):
    return lax.dot_general(a, b, NT, preferred_element_type=F32)


def _kernel(x_hbm, wq_hbm, wk_hbm, wv_hbm, wao_hbm, wup_hbm, dw_hbm, wdn_hbm, wm_hbm,
            o_ref,
            x_s, wq_s, wk_s, wv_s, wao_s, wup_s, dw_s, wdn_s, wm_s, sems,
            xa_s, wa_s, wo_s, dwb_s, s_s, m_s, u_s, g_s, gn_s, acc_s, l_s, yc_s, vt_s, z_s,
            *, B, T, D, K, TQ, TK, TP):
    NQ = T // TQ
    N = B * NQ
    NKV = TP // TK
    NC = D // LANES
    CPK = TK // LANES
    PAD = K // 2
    H = 2
    TQP = -(-TQ // LANES) * LANES
    step = pl.program_id(0)

    def keys(b, j):
        start = b * (TP // H) + j * (TK // H)
        if not isinstance(start, int):
            start = pl.multiple_of(start, 8)
        return _unpack(xa_s[pl.ds(start, TK // H), :])

    def ln_rows(src, dst, rows):
        if not isinstance(src, int):
            src = pl.multiple_of(src, 16)
        dsth = dst // H
        if not isinstance(dsth, int):
            dsth = pl.multiple_of(dsth, 8)
        xa_s[pl.ds(dsth, rows // H), :] = _pack(_ln(x_s[pl.ds(src, rows), :].astype(F32), EPS))

    def keys_rows(b, r0, n):
        start = b * (TP // H) + r0 // H
        if not isinstance(start, int):
            start = pl.multiple_of(start, 8)
        return _unpack(xa_s[pl.ds(start, n // H), :])

    NVALID = T - (NKV - 1) * TK
    NFULL = NVALID // LANES
    TAIL = NVALID % LANES

    def tail_keys(b):
        return keys_rows(b, (NKV - 1) * TK + NFULL * LANES, TAIL)

    def tail_part(kt, q, n):
        qn = q[n * LANES:min((n + 1) * LANES, TQ), :]
        if qn.shape[0] < LANES:
            qn = jnp.concatenate([qn, jnp.zeros((LANES - qn.shape[0], D), BF16)], axis=0)
        return _dot_nt(kt, qn)

    def tail_tile(parts):
        fill = jnp.full((LANES - TAIL, LANES), -jnp.inf, F32)
        return jnp.concatenate([jnp.concatenate([p, fill], axis=0).T for p in parts], axis=0)[0:TQ, :]

    def qk_chunk(q, b, j, last, tok=None, parts=None):
        if last:
            s = _dot_nt(q, keys_rows(b, j * TK, NFULL * LANES))
            if parts is None:
                kt = tail_keys(b)
                parts = [tail_part(kt, q, n) for n in range(TQP // LANES)]
        else:
            s = _dot_nt(q, keys(b, j))
        if tok is not None:
            tok[0] = s
        mx = None
        for c in range(CPK):
            if last and c >= NFULL:
                st = tail_tile(parts) if c == NFULL else jnp.full((TQ, LANES), -jnp.inf, F32)
            else:
                st = s[:, c * LANES:(c + 1) * LANES]
            s_s[j, :, c * LANES:(c + 1) * LANES] = st
            mx = st if mx is None else jnp.maximum(mx, st)
        return mx

    def probs(j, m, raw=False, ntiles=CPK):
        tiles = []
        lsum = None
        for c in range(ntiles):
            p = jnp.exp2(s_s[j, :, c * LANES:(c + 1) * LANES] - m)
            lsum = p if lsum is None else lsum + p
            tiles.append(p)
        if raw:
            return tiles, lsum
        return jnp.concatenate(tiles, axis=1).astype(BF16), lsum

    def up_g(xq):
        return _ln(_gelu2(_dot(xq, _unpack(wa_s[:, 2 * D:3 * D]))), 4.0 * EPS)

    def up_u(xq):
        return _gelu2(_dot(xq, _unpack(wa_s[:, D:2 * D])))

    def store_g(ref, row, g):
        for c in range(NC):
            ref[c, row:row + g.shape[0], :] = g[:, c * LANES:(c + 1) * LANES]

    def shift_g(seq_start):
        for c in range(NC):
            g_s[c, 0:HALO, :] = jnp.where(seq_start, 0.0, g_s[c, TQ:TQ + HALO, :])
            g_s[c, HALO:HALO + TQ, :] = gn_s[c, HALO:HALO + TQ, :]

    def conv_rows(r0, R, chain=None, cg=None):
        G = R if chain is None else (cg or CG)
        rows = []
        for rr in range(0, R, G):
            cols = []
            for c in range(NC):
                acc = None
                for k in range(K):
                    off = HALO - PAD + k
                    gv = g_s[c, pl.ds(r0 + rr + off, G), :].reshape(G // 8, 8, LANES)
                    term = gv * dwb_s[k, :, c * LANES:(c + 1) * LANES][None]
                    if acc is None:
                        if chain is not None and chain[1] is not None:
                            term = jnp.where(chain[0], chain[1], term)
                        acc = term
                    else:
                        acc = acc + term
                if chain is not None:
                    chain[1] = acc
                cols.append(acc.reshape(G, LANES))
            rows.append(jnp.concatenate(cols, axis=1))
        return jnp.concatenate(rows, axis=0)

    def pv_tail(pt, flag, hist):
        rows = []
        for r in range(0, TQ, PG):
            pr = pt[r:r + PG, :]
            if PLAG and len(hist) >= PLAG:
                pr = jnp.where(flag, hist[-PLAG], pr)
            pb = [jnp.broadcast_to(pr[:, k:k + 1], (PG, LANES)) for k in range(TAIL)]
            cols = []
            for c in range(NC):
                acc = None
                for k in range(TAIL):
                    term = pb[k] * vt_s[k:k + 1, c * LANES:(c + 1) * LANES]
                    if acc is None and len(hist) >= PW:
                        term = jnp.where(flag, hist[-PW], term)
                    acc = term if acc is None else acc + term
                hist.append(acc)
                cols.append(acc)
            rows.append(jnp.concatenate(cols, axis=1))
        return jnp.concatenate(rows, axis=0)

    def finish(sb, acc, l_acc, yc):
        l = jnp.sum(l_acc, axis=-1, keepdims=True)
        ya = (acc * (1.0 / l)).astype(BF16)
        out = _dot(yc, _unpack(wo_s[D // H:2 * D // H, :]))
        out = out + _dot(ya, _unpack(wo_s[0:D // H, :]))
        row = sb * TQ
        if not isinstance(row, int):
            row = pl.multiple_of(row, 16)
        xr = x_s[pl.ds(row, TQ), :].astype(F32)
        o_ref[...] = (xr + out).astype(o_ref.dtype)

    def store_max(mx):
        m_s[...] = jnp.broadcast_to(jnp.max(mx, axis=-1, keepdims=True), (TQ, LANES))

    def tie(flag, dep, val, n):
        if n == val.shape[0]:
            return jnp.where(flag, dep[0:n], val)
        return jnp.concatenate([jnp.where(flag, dep[0:n], val[0:n]), val[n:]], axis=0)

    def tie_bf16(flag, dep, val):
        head = pltpu.bitcast(val[0:16, 0:LANES], U32)
        head = _unpack(jnp.where(flag, pltpu.bitcast(dep, U32), head))
        top = jnp.concatenate([head, val[0:16, LANES:]], axis=1)
        return jnp.concatenate([top, val[16:, :]], axis=0)

    def first_step():
        C2 = FC2

        def xrows(r0, r1):
            return x_hbm.at[pl.ds(r0, r1 - r0), :], x_s.at[pl.ds(r0, r1 - r0), :]

        copies = {}
        plan = (
            ('wq', wq_hbm, wq_s), ('wk', wk_hbm, wk_s),
            ('xa',) + xrows(0, TK), ('xb',) + xrows(TK, C2 * TK), ('xc',) + xrows(C2 * TK, T),
            ('wup', wup_hbm, wup_s), ('dw', dw_hbm, dw_s), ('xd',) + xrows(T, T + TQ),
            ('wv', wv_hbm, wv_s), ('wao', wao_hbm, wao_s), ('wdn', wdn_hbm, wdn_s), ('wm', wm_hbm, wm_s),
            ('xe',) + xrows(T + TQ, B * T),
        )
        for i, (name, src, dst) in enumerate(plan):
            copies[name] = pltpu.make_async_copy(src, dst, sems.at[i])
            copies[name].start()

        z_s[0] = 0
        z_s[1] = 0
        z_s[2] = 0
        for b in range(B):
            xa_s[(b * TP + T) // H:(b + 1) * TP // H, :] = jnp.zeros(((TP - T) // H, D), U32)
        store_g(g_s, TQ, jnp.zeros((HALO, D), F32))
        acc_s[...] = jnp.zeros((TQ, D), F32)
        l_s[...] = jnp.zeros((TQ, LANES), F32)

        def ln_chunk(c):
            ln_rows(c * TK, c * TK, min(TK, T - c * TK))

        scale = float(D) ** (-0.5) * math.log2(math.e)
        DS = FSPLIT * LANES
        copies['wq'].wait()
        copies['wk'].wait()
        wa_s[:, 0:DS] = _pack(_dot_nt(wq_s[...], wk_s[0:DS, :]) * scale)

        never = z_s[0] > 0
        zero = pl.multiple_of(z_s[0], 8)
        copies['xa'].wait()
        wa_s[:, DS:D] = _pack(_dot_nt(wq_s[...], wk_s[DS:D, :]) * scale)
        ln_chunk(0)
        q = _dot(_unpack(xa_s[0:TQ // H, :]), _unpack(wa_s[:, 0:D])).astype(BF16)
        mx = qk_chunk(q, 0, 0, False)

        copies['xb'].wait()
        for c in range(1, C2):
            ln_chunk(c)
            mx = jnp.maximum(mx, qk_chunk(q, 0, c, False))

        for name in ('xc', 'wup', 'dw', 'xd'):
            copies[name].wait()
        xq = _unpack(xa_s[0:TQ // H, :])
        hg = _dot(xq, wup_s[:, D:2 * D])
        hu = _dot(tie_bf16(never, hg[0:8, LANES:2 * LANES], xq), wup_s[:, 0:D])
        store_g(gn_s, HALO, _ln(_gelu2(hg), 4.0 * EPS))
        u_s[0] = _gelu2(hu)
        wa_s[:, D:3 * D] = _pack(wup_s[...])
        dwf = dw_s[...].astype(F32)
        for k in range(K):
            dwb_s[k] = jnp.broadcast_to(dwf[k:k + 1, :], (8, D))
        deps = [hu[0:8, LANES:2 * LANES], gn_s[0, pl.ds(zero + HALO, 8), :], u_s[0, pl.ds(zero, 8), 0:LANES]]
        for c in range(C2, NKV):
            ln_chunk(c)
            qc = tie_bf16(never, deps[c - C2], q) if c - C2 < len(deps) else q
            mx = jnp.maximum(mx, qk_chunk(qc, 0, c, c == NKV - 1))

        for name in ('wv', 'wao', 'wdn', 'wm'):
            copies[name].wait()
        store_max(mx)
        ln_rows(T, TP, TQ)
        wva = _dot(wv_s[...], wao_s[...]).astype(BF16)
        wo_s[D // H:2 * D // H, :] = _pack(0.5 * _dot(wdn_s[...], wm_s[D:2 * D, :]))
        lhs = tie_bf16(never, xa_s[pl.ds(zero, 8), 0:LANES], wva)
        wo_s[0:D // H, :] = _pack(_dot(lhs, wm_s[0:D, :]))
        copies['xe'].wait()

    def main_step():
        ba = step // NQ
        ia = step % NQ
        sb = step - 1
        bb = sb // NQ
        sa = step % 2
        so = 1 - sa
        shift_g(sb % NQ == 0)
        never = z_s[0] > 0
        never2 = z_s[1] > 0
        never3 = z_s[2] > 0
        tok = [None]

        def prev_tile():
            return tok[0][TIER:, TIEC * LANES:(TIEC + 1) * LANES]

        def after_packed(lhs):
            if tok[0] is None:
                return _unpack(lhs)
            head = tie(never3, pltpu.bitcast(prev_tile(), U32), lhs[:, 0:LANES], min(TIEN, TQ // H))
            return _unpack(jnp.concatenate([head, lhs[:, LANES:]], axis=1))

        def after_tiles(tiles):
            tiles = list(tiles)
            tiles[1] = tie(never3, prev_tile(), tiles[1], TIEN)
            return jnp.concatenate(tiles, axis=1).astype(BF16)

        def split(v):
            return [v[:, c * LANES:(c + 1) * LANES] for c in range(v.shape[1] // LANES)]

        def mm(lhs, rhs):
            tok[0] = _dot(lhs, rhs)
            return tok[0]

        m_old = m_s[...]
        xq = xa_s[pl.ds(pl.multiple_of(ba * (TP // H) + ia * (TQ // H), 8), TQ // H), :]
        qp = _pack(mm(after_packed(xq), _unpack(wa_s[:, 0:D])))
        def proj_g():
            g_new = _ln(_gelu2(mm(after_packed(xq), _unpack(wa_s[:, 2 * D:3 * D]))), 4.0 * EPS)
            store_g(gn_s, HALO, g_new)
            store_g(g_s, HALO + TQ, jnp.where(ia == 0, 0.0, g_new[0:HALO, :]))

        def proj_u():
            u_s[sa] = _gelu2(mm(after_packed(xq), _unpack(wa_s[:, D:2 * D])))

        if GPOS < 0:
            proj_g()
        if UPOS < 0:
            proj_u()
        nxt = jnp.minimum(step + NQ, N - 1)
        xn = _pack(_ln(x_s[pl.ds(pl.multiple_of(nxt * TQ, 16), TQ), :].astype(F32), EPS))
        mx = None
        mx_prev = None
        acc = None
        vt_s[...] = tail_keys(bb).astype(F32)
        l_acc = jnp.exp2(s_s[NKV - 1, :, NFULL * LANES:(NFULL + 1) * LANES] - m_old)
        p_tail = l_acc
        parts = []
        for j in range(NKV):
            m_use = m_old
            if mx_prev is not None:
                m_use = jnp.where(never, mx_prev, m_use)
            nt = NFULL if j == NKV - 1 else CPK
            tiles, l_new = probs(j, m_use, raw=True, ntiles=nt)
            l_acc = l_acc + l_new
            tiles[0] = jnp.where(never2, l_acc, tiles[0])
            o = mm(after_tiles(tiles), keys_rows(bb, j * TK, nt * LANES))
            acc = o if acc is None else acc + o
            qj = qp
            if j == LNJ:
                qj = jnp.where(never2, xn, qp)
            if j == GJ and GJ > GPOS:
                gdep = gn_s[0, pl.ds(pl.multiple_of(z_s[0] + HALO, 8), 8), :]
                qj = jnp.concatenate([qj[:, 0:LANES], tie(never2, pltpu.bitcast(gdep, U32), qj[:, LANES:2 * LANES], 8), qj[:, 2 * LANES:]], axis=1)
            n = j - TJ0
            if 0 <= n < TQP // LANES:
                kt = tie_bf16(never3, o[0:8, TTC * LANES:(TTC + 1) * LANES], tail_keys(ba))
                parts.append(tail_part(kt, _unpack(qp), n))
            if 0 <= n - 1 < TQP // LANES:
                dep = pltpu.bitcast(parts[n - 1], U32)
                qj = jnp.concatenate([qj[:, 0:2 * LANES], tie(never2, dep, qj[:, 2 * LANES:3 * LANES], TAIL), qj[:, 3 * LANES:]], axis=1)
            mx_prev = mx
            mj = qk_chunk(after_packed(qj), ba, j, j == NKV - 1, tok, parts if parts else None)
            mx = mj if mx is None else jnp.maximum(mx, mj)
            if j == GPOS:
                proj_g()
            if j == UPOS:
                proj_u()
        yc = u_s[so] * conv_rows(0, TQ, [never, None])
        o_tail = pv_tail(p_tail, never, [])
        l = jnp.sum(l_acc, axis=-1, keepdims=True)
        ya = (acc + o_tail) * (1.0 / l)
        if OUTA:
            out = mm(after_tiles(split(ya)), _unpack(wo_s[0:D // H, :]))
            out = out + mm(after_tiles(split(yc)), _unpack(wo_s[D // H:2 * D // H, :]))
        else:
            out = mm(after_tiles(split(yc)), _unpack(wo_s[D // H:2 * D // H, :]))
            out = out + mm(after_tiles(split(ya)), _unpack(wo_s[0:D // H, :]))
        xr = x_s[pl.ds(pl.multiple_of(sb * TQ, 16), TQ), :].astype(F32)
        o_ref[...] = (xr + out).astype(o_ref.dtype)
        store_max(mx)
        dst = pl.multiple_of((nxt // NQ) * (TP // H) + (nxt % NQ) * (TQ // H), 8)
        late = pltpu.bitcast(mx[0:TQ // H, :], U32)
        for c in range(NC):
            xa_s[pl.ds(dst, TQ // H), c * LANES:(c + 1) * LANES] = jnp.where(
                never, late, xn[:, c * LANES:(c + 1) * LANES])

    def last_step():
        sb = N - 1
        bb = B - 1
        uslot = sb % 2
        CPI = LCPI
        NIT = NKV // CPI
        RL = 16 * (-(-TQ // (16 * NIT)))
        never = z_s[0] > 0
        never2 = z_s[1] > 0
        for c in range(NC):
            gn_s[c, 0:HALO, :] = jnp.where(NQ == 1, 0.0, g_s[c, TQ:TQ + HALO, :])
        store_g(gn_s, HALO + TQ, jnp.zeros((HALO, D), F32))

        def attend(j0):
            acc = acc_s[...]
            l_acc = l_s[...]
            for jj in range(CPI):
                tiles, l_new = probs(j0 + jj, m_s[...], raw=True)
                l_acc = l_acc + l_new
                tiles[0] = jnp.where(never2, l_acc, tiles[0])
                acc = acc + _dot(jnp.concatenate(tiles, axis=1).astype(BF16), keys(bb, j0 + jj))
            return acc, l_acc

        def loop(t, carry):
            acc, l_acc = attend(t * CPI)
            acc_s[...] = acc
            l_s[...] = l_acc
            r0 = pl.multiple_of(jnp.minimum(t * RL, TQ - RL), 16)
            for c in range(NC):
                g_s[c, 0:RL + 2 * HALO, :] = gn_s[c, pl.ds(r0, RL + 2 * HALO), :]
            yc = u_s[uslot, pl.ds(r0, RL), :] * conv_rows(0, RL, [never, None], LCG)
            yc_s[pl.ds(pl.multiple_of(r0 // H, 8), RL // H), :] = _pack(yc)
            return carry

        lax.fori_loop(0, NIT, loop, 0)
        finish(sb, acc_s[...], l_s[...], _unpack(yc_s[...]))

    @pl.when(step == 0)
    def _():
        first_step()

    @pl.when(jnp.logical_and(step > 0, step < N))
    def _():
        main_step()

    @pl.when(step == N)
    def _():
        last_step()


@jax.jit
def pallas_standalone__conformer_family_branchformer__speech_kernel(
    x: jax.Array,
    w_q: jax.Array,
    w_k: jax.Array,
    w_v: jax.Array,
    w_ao: jax.Array,
    w_up: jax.Array,
    dw: jax.Array,
    w_dn: jax.Array,
    w_merge: jax.Array,
):
    B, T, D = x.shape
    K = dw.shape[0]
    TQ = 400
    TK = 512
    TP = -(-T // TK) * TK
    NKV = TP // TK
    assert T % TQ == 0 and TQ % 16 == 0 and D % LANES == 0 and K // 2 < HALO
    assert TQ <= TK and B >= 2 and NKV >= 3 and T % 16 == 0
    N = B * (T // TQ)
    x2 = x.reshape(B * T, D)

    kern = functools.partial(_kernel, B=B, T=T, D=D, K=K, TQ=TQ, TK=TK, TP=TP)
    ins = (x2, w_q, w_k, w_v, w_ao, w_up, dw, w_dn, w_merge)
    out = pl.pallas_call(
        kern,
        grid=(N + 1,),
        in_specs=[pl.BlockSpec(memory_space=pl.ANY) for _ in ins],
        out_specs=pl.BlockSpec((TQ, D), lambda s: (jnp.maximum(s - 1, 0), 0)),
        out_shape=jax.ShapeDtypeStruct((B * T, D), x.dtype),
        scratch_shapes=[pltpu.VMEM(a.shape, a.dtype) for a in ins] + [
            pltpu.SemaphoreType.DMA((13,)),
            pltpu.VMEM((B * TP // 2, D), U32),
            pltpu.VMEM((D // 2, 3 * D), U32),
            pltpu.VMEM((D, D), U32),
            pltpu.VMEM((K, 8, D), F32),
            pltpu.VMEM((NKV, TQ, TK), F32),
            pltpu.VMEM((TQ, LANES), F32),
            pltpu.VMEM((2, TQ, D), F32),
            pltpu.VMEM((D // LANES, TQ + 2 * HALO, LANES), F32),
            pltpu.VMEM((D // LANES, TQ + 2 * HALO, LANES), F32),
            pltpu.VMEM((TQ, D), F32),
            pltpu.VMEM((TQ, LANES), F32),
            pltpu.VMEM((TQ // 2, D), U32),
            pltpu.VMEM((T % LANES, D), F32),
            pltpu.SMEM((3,), jnp.int32),
        ],
        compiler_params=pltpu.CompilerParams(
            dimension_semantics=("arbitrary",),
            vmem_limit_bytes=100 * 1024 * 1024,
        ),
    )(*ins)
    return out.reshape(B, T, D)
```

```python
import functools
import math

import jax
import jax.numpy as jnp
from jax import lax
import jax.experimental.pallas as pl
import jax.experimental.pallas.tpu as pltpu

LANES = 128
EPS = 1e-05
F32 = jnp.float32
BF16 = jnp.bfloat16
U32 = jnp.uint32
NT = (((1,), (1,)), ((), ()))
CG = 16
LNJ = 1
TIER = 0
TIEC = 0
TIEN = 8
GJ = 3
LCG = 16
PG = 8
PW = 1
PLAG = 6
OUTA = 0
TJ0 = 1
TTC = 2
LCPI = 2
FC2 = 5
FSPLIT = 2
UMODE = 1
UFIRST = 1 if UMODE == 2 else 0
HALO = 16


def _ln(x, eps):
    d = x.shape[-1]
    m = jnp.sum(x, axis=-1, keepdims=True) * (1.0 / d)
    xc = x - m
    v = jnp.sum(xc * xc, axis=-1, keepdims=True) * (1.0 / d)
    return xc * lax.rsqrt(v + eps)


def _gelu2(x):
    c1 = math.sqrt(2.0 / math.pi)
    c2 = c1 * 0.044715
    t = jnp.tanh(x * (c1 + c2 * (x * x)))
    return x + x * t


def _center(w):
    return w - jnp.sum(w, axis=0, keepdims=True) * (1.0 / w.shape[0])


def _pack(x):
    return pltpu.bitcast(x.astype(BF16), U32)


def _unpack(x):
    return pltpu.bitcast(x, BF16)


def _dot(a, b):
    return jnp.dot(a, b, preferred_element_type=F32)


def _dot_nt(a, b):
    return lax.dot_general(a, b, NT, preferred_element_type=F32)


def _kernel(x_hbm, wq_hbm, wk_hbm, wv_hbm, wao_hbm, wup_hbm, dw_hbm, wdn_hbm, wm_hbm,
            o_ref,
            x_s, wq_s, wk_s, wv_s, wao_s, wup_s, dw_s, wdn_s, wm_s, sems,
            xa_s, wa_s, wo_s, dwb_s, s_s, m_s, u_s, g_s, gn_s, acc_s, l_s, yc_s, vt_s, z_s,
            *, B, T, D, K, TQ, TK, TP):
    NQ = T // TQ
    N = B * NQ
    NKV = TP // TK
    NC = D // LANES
    CPK = TK // LANES
    PAD = K // 2
    H = 2
    TQP = -(-TQ // LANES) * LANES
    step = pl.program_id(0)

    def keys(b, j):
        start = b * (TP // H) + j * (TK // H)
        if not isinstance(start, int):
            start = pl.multiple_of(start, 8)
        return _unpack(xa_s[pl.ds(start, TK // H), :])

    def ln_rows(src, dst, rows):
        if not isinstance(src, int):
            src = pl.multiple_of(src, 16)
        dsth = dst // H
        if not isinstance(dsth, int):
            dsth = pl.multiple_of(dsth, 8)
        xa_s[pl.ds(dsth, rows // H), :] = _pack(_ln(x_s[pl.ds(src, rows), :].astype(F32), EPS))

    def keys_rows(b, r0, n):
        start = b * (TP // H) + r0 // H
        if not isinstance(start, int):
            start = pl.multiple_of(start, 8)
        return _unpack(xa_s[pl.ds(start, n // H), :])

    NVALID = T - (NKV - 1) * TK
    NFULL = NVALID // LANES
    TAIL = NVALID % LANES

    def tail_keys(b):
        return keys_rows(b, (NKV - 1) * TK + NFULL * LANES, TAIL)

    def tail_part(kt, q, n):
        qn = q[n * LANES:min((n + 1) * LANES, TQ), :]
        if qn.shape[0] < LANES:
            qn = jnp.concatenate([qn, jnp.zeros((LANES - qn.shape[0], D), BF16)], axis=0)
        return _dot_nt(kt, qn)

    def tail_tile(parts):
        fill = jnp.full((LANES - TAIL, LANES), -jnp.inf, F32)
        return jnp.concatenate([jnp.concatenate([p, fill], axis=0).T for p in parts], axis=0)[0:TQ, :]

    def qk_chunk(q, b, j, last, tok=None, parts=None):
        if last:
            s = _dot_nt(q, keys_rows(b, j * TK, NFULL * LANES))
            if parts is None:
                kt = tail_keys(b)
                parts = [tail_part(kt, q, n) for n in range(TQP // LANES)]
        else:
            s = _dot_nt(q, keys(b, j))
        if tok is not None:
            tok[0] = s
        mx = None
        for c in range(CPK):
            if last and c >= NFULL:
                st = tail_tile(parts) if c == NFULL else jnp.full((TQ, LANES), -jnp.inf, F32)
            else:
                st = s[:, c * LANES:(c + 1) * LANES]
            s_s[j, :, c * LANES:(c + 1) * LANES] = st
            mx = st if mx is None else jnp.maximum(mx, st)
        return mx

    def probs(j, m, raw=False, ntiles=CPK):
        tiles = []
        lsum = None
        for c in range(ntiles):
            p = jnp.exp2(s_s[j, :, c * LANES:(c + 1) * LANES] - m)
            lsum = p if lsum is None else lsum + p
            tiles.append(p)
        if raw:
            return tiles, lsum
        return jnp.concatenate(tiles, axis=1).astype(BF16), lsum

    def up_g(xq):
        return _ln(_gelu2(_dot(xq, _unpack(wa_s[:, 2 * D:3 * D]))), 4.0 * EPS)

    def up_u(xq):
        return _gelu2(_dot(xq, _unpack(wa_s[:, D:2 * D])))

    def store_g(ref, row, g):
        for c in range(NC):
            ref[c, row:row + g.shape[0], :] = g[:, c * LANES:(c + 1) * LANES]

    def shift_g(seq_start):
        for c in range(NC):
            g_s[c, 0:HALO, :] = jnp.where(seq_start, 0.0, g_s[c, TQ:TQ + HALO, :])
            g_s[c, HALO:HALO + TQ, :] = gn_s[c, HALO:HALO + TQ, :]

    def conv_rows(r0, R, chain=None, cg=None):
        G = R if chain is None else (cg or CG)
        rows = []
        for rr in range(0, R, G):
            cols = []
            for c in range(NC):
                acc = None
                for k in range(K):
                    off = HALO - PAD + k
                    gv = g_s[c, pl.ds(r0 + rr + off, G), :].reshape(G // 8, 8, LANES)
                    term = gv * dwb_s[k, :, c * LANES:(c + 1) * LANES][None]
                    if acc is None:
                        if chain is not None and chain[1] is not None:
                            term = jnp.where(chain[0], chain[1], term)
                        acc = term
                    else:
                        acc = acc + term
                if chain is not None:
                    chain[1] = acc
                cols.append(acc.reshape(G, LANES))
            rows.append(jnp.concatenate(cols, axis=1))
        return jnp.concatenate(rows, axis=0)

    def pv_tail(pt, flag, hist):
        rows = []
        for r in range(0, TQ, PG):
            pr = pt[r:r + PG, :]
            if PLAG and len(hist) >= PLAG:
                pr = jnp.where(flag, hist[-PLAG], pr)
            pb = [jnp.broadcast_to(pr[:, k:k + 1], (PG, LANES)) for k in range(TAIL)]
            cols = []
            for c in range(NC):
                acc = None
                for k in range(TAIL):
                    term = pb[k] * vt_s[k:k + 1, c * LANES:(c + 1) * LANES]
                    if acc is None and len(hist) >= PW:
                        term = jnp.where(flag, hist[-PW], term)
                    acc = term if acc is None else acc + term
                hist.append(acc)
                cols.append(acc)
            rows.append(jnp.concatenate(cols, axis=1))
        return jnp.concatenate(rows, axis=0)

    def finish(sb, acc, l_acc, yc):
        l = jnp.sum(l_acc, axis=-1, keepdims=True)
        ya = (acc * (1.0 / l)).astype(BF16)
        out = _dot(yc, _unpack(wo_s[D // H:2 * D // H, :]))
        out = out + _dot(ya, _unpack(wo_s[0:D // H, :]))
        row = sb * TQ
        if not isinstance(row, int):
            row = pl.multiple_of(row, 16)
        xr = x_s[pl.ds(row, TQ), :].astype(F32)
        o_ref[...] = (xr + out).astype(o_ref.dtype)

    def store_max(mx):
        m_s[...] = jnp.broadcast_to(jnp.max(mx, axis=-1, keepdims=True), (TQ, LANES))

    def tie(flag, dep, val, n):
        if n == val.shape[0]:
            return jnp.where(flag, dep[0:n], val)
        return jnp.concatenate([jnp.where(flag, dep[0:n], val[0:n]), val[n:]], axis=0)

    def tie_bf16(flag, dep, val):
        head = pltpu.bitcast(val[0:16, 0:LANES], U32)
        head = _unpack(jnp.where(flag, pltpu.bitcast(dep, U32), head))
        top = jnp.concatenate([head, val[0:16, LANES:]], axis=1)
        return jnp.concatenate([top, val[16:, :]], axis=0)

    def first_step():
        C2 = FC2

        def xrows(r0, r1):
            return x_hbm.at[pl.ds(r0, r1 - r0), :], x_s.at[pl.ds(r0, r1 - r0), :]

        copies = {}
        plan = (
            ('wq', wq_hbm, wq_s), ('wk', wk_hbm, wk_s),
            ('xa',) + xrows(0, TK), ('xb',) + xrows(TK, C2 * TK), ('xc',) + xrows(C2 * TK, T),
            ('wup', wup_hbm, wup_s), ('dw', dw_hbm, dw_s), ('xd',) + xrows(T, T + TQ),
            ('wv', wv_hbm, wv_s), ('wao', wao_hbm, wao_s), ('wdn', wdn_hbm, wdn_s), ('wm', wm_hbm, wm_s),
            ('xe',) + xrows(T + TQ, B * T),
        )
        for i, (name, src, dst) in enumerate(plan):
            copies[name] = pltpu.make_async_copy(src, dst, sems.at[i])
            copies[name].start()

        z_s[0] = 0
        z_s[1] = 0
        z_s[2] = 0
        for b in range(B):
            xa_s[(b * TP + T) // H:(b + 1) * TP // H, :] = jnp.zeros(((TP - T) // H, D), U32)
        store_g(g_s, TQ, jnp.zeros((HALO, D), F32))
        acc_s[...] = jnp.zeros((TQ, D), F32)
        l_s[...] = jnp.zeros((TQ, LANES), F32)

        def ln_chunk(c):
            ln_rows(c * TK, c * TK, min(TK, T - c * TK))

        scale = float(D) ** (-0.5) * math.log2(math.e)
        DS = FSPLIT * LANES
        copies['wq'].wait()
        copies['wk'].wait()
        m_lo = _dot_nt(wq_s[...], wk_s[0:DS, :])

        never = z_s[0] > 0
        zero = pl.multiple_of(z_s[0], 8)
        copies['xa'].wait()
        wa_s[:, 0:DS] = _pack(_center(m_lo) * scale)
        wa_s[:, DS:D] = _pack(_center(_dot_nt(wq_s[...], wk_s[DS:D, :])) * scale)
        ln_chunk(0)
        q = _dot(_unpack(xa_s[0:TQ // H, :]), _unpack(wa_s[:, 0:D])).astype(BF16)
        mx = qk_chunk(q, 0, 0, False)

        copies['xb'].wait()
        for c in range(1, C2):
            ln_chunk(c)
            mx = jnp.maximum(mx, qk_chunk(q, 0, c, False))

        for name in ('xc', 'wup', 'dw', 'xd'):
            copies[name].wait()
        xq = _unpack(xa_s[0:TQ // H, :])
        hg = _dot(xq, wup_s[:, D:2 * D])
        hu = _dot(tie_bf16(never, hg[0:8, LANES:2 * LANES], xq), wup_s[:, 0:D])
        store_g(gn_s, HALO, _ln(_gelu2(hg), 4.0 * EPS))
        u_s[UFIRST] = _gelu2(hu)
        wa_s[:, D:3 * D] = _pack(wup_s[...])
        dwf = dw_s[...].astype(F32)
        for k in range(K):
            dwb_s[k] = jnp.broadcast_to(dwf[k:k + 1, :], (8, D))
        deps = [hu[0:8, LANES:2 * LANES], gn_s[0, pl.ds(zero + HALO, 8), :], u_s[UFIRST, pl.ds(zero, 8), 0:LANES]]
        for c in range(C2, NKV):
            ln_chunk(c)
            qc = tie_bf16(never, deps[c - C2], q) if c - C2 < len(deps) else q
            mx = jnp.maximum(mx, qk_chunk(qc, 0, c, c == NKV - 1))

        for name in ('wv', 'wao', 'wdn', 'wm'):
            copies[name].wait()
        store_max(mx)
        ln_rows(T, TP, TQ)
        wva = _center(_dot(wv_s[...], wao_s[...])).astype(BF16)
        wo_s[D // H:2 * D // H, :] = _pack(0.5 * _dot(wdn_s[...], wm_s[D:2 * D, :]))
        lhs = tie_bf16(never, xa_s[pl.ds(zero, 8), 0:LANES], wva)
        wo_s[0:D // H, :] = _pack(_dot(lhs, wm_s[0:D, :]))
        copies['xe'].wait()

    def main_step():
        ba = step // NQ
        ia = step % NQ
        sb = step - 1
        bb = sb // NQ
        sa = step % 2
        so = 1 - sa
        shift_g(sb % NQ == 0)
        never = z_s[0] > 0
        never2 = z_s[1] > 0
        never3 = z_s[2] > 0
        tok = [None]

        def prev_tile():
            return tok[0][TIER:, TIEC * LANES:(TIEC + 1) * LANES]

        def after_packed(lhs):
            if tok[0] is None:
                return _unpack(lhs)
            head = tie(never3, pltpu.bitcast(prev_tile(), U32), lhs[:, 0:LANES], min(TIEN, TQ // H))
            return _unpack(jnp.concatenate([head, lhs[:, LANES:]], axis=1))

        def after_tiles(tiles):
            tiles = list(tiles)
            tiles[1] = tie(never3, prev_tile(), tiles[1], TIEN)
            return jnp.concatenate(tiles, axis=1).astype(BF16)

        def split(v):
            return [v[:, c * LANES:(c + 1) * LANES] for c in range(v.shape[1] // LANES)]

        def mm(lhs, rhs):
            tok[0] = _dot(lhs, rhs)
            return tok[0]

        m_old = m_s[...]
        xq = xa_s[pl.ds(pl.multiple_of(ba * (TP // H) + ia * (TQ // H), 8), TQ // H), :]
        qp = _pack(mm(after_packed(xq), _unpack(wa_s[:, 0:D])))
        def proj_g():
            g_new = _ln(_gelu2(mm(after_packed(xq), _unpack(wa_s[:, 2 * D:3 * D]))), 4.0 * EPS)
            store_g(gn_s, HALO, g_new)
            store_g(g_s, HALO + TQ, jnp.where(ia == 0, 0.0, g_new[0:HALO, :]))

        def proj_u():
            u_s[sa] = _gelu2(mm(after_packed(xq), _unpack(wa_s[:, D:2 * D])))

        proj_g()
        if UMODE == 1:
            sa = so = 0
            u_old = u_s[0]
        elif UMODE == 2:
            sa, so = 1, 0
            u_s[0] = u_s[1]
        proj_u()
        nxt = jnp.minimum(step + NQ, N - 1)
        xn = _pack(_ln(x_s[pl.ds(pl.multiple_of(nxt * TQ, 16), TQ), :].astype(F32), EPS))
        mx = None
        mx_prev = None
        acc = None
        vt_s[...] = tail_keys(bb).astype(F32)
        l_acc = jnp.exp2(s_s[NKV - 1, :, NFULL * LANES:(NFULL + 1) * LANES] - m_old)
        p_tail = l_acc
        parts = []
        for j in range(NKV):
            m_use = m_old
            if mx_prev is not None:
                m_use = jnp.where(never, mx_prev, m_use)
            nt = NFULL if j == NKV - 1 else CPK
            tiles, l_new = probs(j, m_use, raw=True, ntiles=nt)
            l_acc = l_acc + l_new
            tiles[0] = jnp.where(never2, l_acc, tiles[0])
            o = mm(after_tiles(tiles), keys_rows(bb, j * TK, nt * LANES))
            acc = o if acc is None else acc + o
            qj = qp
            if j == LNJ:
                qj = jnp.where(never2, xn, qp)
            if j == GJ:
                gdep = gn_s[0, pl.ds(pl.multiple_of(z_s[0] + HALO, 8), 8), :]
                qj = jnp.concatenate([qj[:, 0:LANES], tie(never2, pltpu.bitcast(gdep, U32), qj[:, LANES:2 * LANES], 8), qj[:, 2 * LANES:]], axis=1)
            n = j - TJ0
            if 0 <= n < TQP // LANES:
                kt = tie_bf16(never3, o[0:8, TTC * LANES:(TTC + 1) * LANES], tail_keys(ba))
                parts.append(tail_part(kt, _unpack(qp), n))
            if 0 <= n - 1 < TQP // LANES:
                dep = pltpu.bitcast(parts[n - 1], U32)
                qj = jnp.concatenate([qj[:, 0:2 * LANES], tie(never2, dep, qj[:, 2 * LANES:3 * LANES], TAIL), qj[:, 3 * LANES:]], axis=1)
            mx_prev = mx
            mj = qk_chunk(after_packed(qj), ba, j, j == NKV - 1, tok, parts if parts else None)
            mx = mj if mx is None else jnp.maximum(mx, mj)
        yc = (u_old if UMODE == 1 else u_s[so]) * conv_rows(0, TQ, [never, None])
        o_tail = pv_tail(p_tail, never, [])
        l = jnp.sum(l_acc, axis=-1, keepdims=True)
        ya = (acc + o_tail) * (1.0 / l)
        if OUTA:
            out = mm(after_tiles(split(ya)), _unpack(wo_s[0:D // H, :]))
            out = out + mm(after_tiles(split(yc)), _unpack(wo_s[D // H:2 * D // H, :]))
        else:
            out = mm(after_tiles(split(yc)), _unpack(wo_s[D // H:2 * D // H, :]))
            out = out + mm(after_tiles(split(ya)), _unpack(wo_s[0:D // H, :]))
        xr = x_s[pl.ds(pl.multiple_of(sb * TQ, 16), TQ), :].astype(F32)
        o_ref[...] = (xr + out).astype(o_ref.dtype)
        store_max(mx)
        dst = pl.multiple_of((nxt // NQ) * (TP // H) + (nxt % NQ) * (TQ // H), 8)
        late = pltpu.bitcast(mx[0:TQ // H, :], U32)
        for c in range(NC):
            xa_s[pl.ds(dst, TQ // H), c * LANES:(c + 1) * LANES] = jnp.where(
                never, late, xn[:, c * LANES:(c + 1) * LANES])

    def last_step():
        sb = N - 1
        bb = B - 1
        uslot = sb % 2 if UMODE == 0 else UFIRST
        CPI = LCPI
        NIT = NKV // CPI
        RL = 16 * (-(-TQ // (16 * NIT)))
        never = z_s[0] > 0
        never2 = z_s[1] > 0
        for c in range(NC):
            gn_s[c, 0:HALO, :] = jnp.where(NQ == 1, 0.0, g_s[c, TQ:TQ + HALO, :])
        store_g(gn_s, HALO + TQ, jnp.zeros((HALO, D), F32))

        def attend(j0):
            acc = acc_s[...]
            l_acc = l_s[...]
            for jj in range(CPI):
                tiles, l_new = probs(j0 + jj, m_s[...], raw=True)
                l_acc = l_acc + l_new
                tiles[0] = jnp.where(never2, l_acc, tiles[0])
                acc = acc + _dot(jnp.concatenate(tiles, axis=1).astype(BF16), keys(bb, j0 + jj))
            return acc, l_acc

        def loop(t, carry):
            acc, l_acc = attend(t * CPI)
            acc_s[...] = acc
            l_s[...] = l_acc
            r0 = pl.multiple_of(jnp.minimum(t * RL, TQ - RL), 16)
            for c in range(NC):
                g_s[c, 0:RL + 2 * HALO, :] = gn_s[c, pl.ds(r0, RL + 2 * HALO), :]
            yc = u_s[uslot, pl.ds(r0, RL), :] * conv_rows(0, RL, [never, None], LCG)
            yc_s[pl.ds(pl.multiple_of(r0 // H, 8), RL // H), :] = _pack(yc)
            return carry

        lax.fori_loop(0, NIT, loop, 0)
        finish(sb, acc_s[...], l_s[...], _unpack(yc_s[...]))

    @pl.when(step == 0)
    def _():
        first_step()

    @pl.when(jnp.logical_and(step > 0, step < N))
    def _():
        main_step()

    @pl.when(step == N)
    def _():
        last_step()


@jax.jit
def pallas_standalone__conformer_family_branchformer__speech_kernel(
    x: jax.Array,
    w_q: jax.Array,
    w_k: jax.Array,
    w_v: jax.Array,
    w_ao: jax.Array,
    w_up: jax.Array,
    dw: jax.Array,
    w_dn: jax.Array,
    w_merge: jax.Array,
):
    B, T, D = x.shape
    K = dw.shape[0]
    TQ = 400
    TK = 512
    TP = -(-T // TK) * TK
    NKV = TP // TK
    assert T % TQ == 0 and TQ % 16 == 0 and D % LANES == 0 and K // 2 < HALO
    assert TQ <= TK and B >= 2 and NKV >= 3 and T % 16 == 0
    N = B * (T // TQ)
    x2 = x.reshape(B * T, D)

    kern = functools.partial(_kernel, B=B, T=T, D=D, K=K, TQ=TQ, TK=TK, TP=TP)
    ins = (x2, w_q, w_k, w_v, w_ao, w_up, dw, w_dn, w_merge)
    out = pl.pallas_call(
        kern,
        grid=(N + 1,),
        in_specs=[pl.BlockSpec(memory_space=pl.ANY) for _ in ins],
        out_specs=pl.BlockSpec((TQ, D), lambda s: (jnp.maximum(s - 1, 0), 0)),
        out_shape=jax.ShapeDtypeStruct((B * T, D), x.dtype),
        scratch_shapes=[pltpu.VMEM(a.shape, a.dtype) for a in ins] + [
            pltpu.SemaphoreType.DMA((13,)),
            pltpu.VMEM((B * TP // 2, D), U32),
            pltpu.VMEM((D // 2, 3 * D), U32),
            pltpu.VMEM((D, D), U32),
            pltpu.VMEM((K, 8, D), F32),
            pltpu.VMEM((NKV, TQ, TK), F32),
            pltpu.VMEM((TQ, LANES), F32),
            pltpu.VMEM((2, TQ, D), F32),
            pltpu.VMEM((D // LANES, TQ + 2 * HALO, LANES), F32),
            pltpu.VMEM((D // LANES, TQ + 2 * HALO, LANES), F32),
            pltpu.VMEM((TQ, D), F32),
            pltpu.VMEM((TQ, LANES), F32),
            pltpu.VMEM((TQ // 2, D), U32),
            pltpu.VMEM((T % LANES, D), F32),
            pltpu.SMEM((3,), jnp.int32),
        ],
        compiler_params=pltpu.CompilerParams(
            dimension_semantics=("arbitrary",),
            vmem_limit_bytes=100 * 1024 * 1024,
            disable_bounds_checks=True,
            disable_semaphore_checks=True,
        ),
    )(*ins)
    return out.reshape(B, T, D)
```

```python
import functools
import math

import jax
import jax.numpy as jnp
from jax import lax
import jax.experimental.pallas as pl
import jax.experimental.pallas.tpu as pltpu

LANES = 128
EPS = 1e-05
F32 = jnp.float32
BF16 = jnp.bfloat16
U32 = jnp.uint32
NT = (((1,), (1,)), ((), ()))
CG = 16
LNJ = 1
TIER = 0
TIEC = 0
TIEN = 8
GJ = 3
LCG = 8
PG = 8
PW = 1
PLAG = 5
OUTA = 1
TJ0 = 0
TTC = 2
LCPI = 2
FC2 = 4
FSPLIT = 2
HOLD = 1
TLAST = 0
R5TIE = 1
GDEP = 1
UDEP = 3
PACE4 = 0
PACE5 = 48
PACE_ALL = 1
CPACE = 64
CSPAN = 3
GPACE = 3
MGP = 3
MLP = 2
EREL = 0
ESPAN = 4
E0 = 0
E1 = 0
LREL = -1
LSPAN = 4
UREL = 4
UJ = -1
GREL = -1
LPACE = 0
LNOL = 0
LORD = 1
LCF = 1
LFLOOR = 1
LFIN = 2
LFC = 16
HALO = 16


def _ln(x, eps):
    d = x.shape[-1]
    m = jnp.sum(x, axis=-1, keepdims=True) * (1.0 / d)
    xc = x - m
    v = jnp.sum(xc * xc, axis=-1, keepdims=True) * (1.0 / d)
    return xc * lax.rsqrt(v + eps)


def _gelu2(x):
    c1 = math.sqrt(2.0 / math.pi)
    c2 = c1 * 0.044715
    t = jnp.tanh(x * (c1 + c2 * (x * x)))
    return x + x * t


def _center(w):
    return w - jnp.sum(w, axis=0, keepdims=True) * (1.0 / w.shape[0])


def _pack(x):
    return pltpu.bitcast(x.astype(BF16), U32)


def _unpack(x):
    return pltpu.bitcast(x, BF16)


def _dot(a, b):
    return jnp.dot(a, b, preferred_element_type=F32)


def _dot_nt(a, b):
    return lax.dot_general(a, b, NT, preferred_element_type=F32)


def _kernel(x_hbm, wq_hbm, wk_hbm, wv_hbm, wao_hbm, wup_hbm, dw_hbm, wdn_hbm, wm_hbm,
            o_ref,
            x_s, wq_s, wk_s, wv_s, wao_s, wup_s, dw_s, wdn_s, wm_s, sems,
            xa_s, wa_s, wo_s, dwb_s, s_s, m_s, u_s, g_s, gn_s, acc_s, l_s, yc_s, vt_s, z_s,
            *, B, T, D, K, TQ, TK, TP):
    NQ = T // TQ
    N = B * NQ
    NKV = TP // TK
    NC = D // LANES
    CPK = TK // LANES
    PAD = K // 2
    H = 2
    TQP = -(-TQ // LANES) * LANES
    step = pl.program_id(0)

    def keys(b, j):
        start = b * (TP // H) + j * (TK // H)
        if not isinstance(start, int):
            start = pl.multiple_of(start, 8)
        return _unpack(xa_s[pl.ds(start, TK // H), :])

    def ln_rows(src, dst, rows):
        if not isinstance(src, int):
            src = pl.multiple_of(src, 16)
        dsth = dst // H
        if not isinstance(dsth, int):
            dsth = pl.multiple_of(dsth, 8)
        xa_s[pl.ds(dsth, rows // H), :] = _pack(_ln(x_s[pl.ds(src, rows), :].astype(F32), EPS))

    def keys_rows(b, r0, n):
        start = b * (TP // H) + r0 // H
        if not isinstance(start, int):
            start = pl.multiple_of(start, 8)
        return _unpack(xa_s[pl.ds(start, n // H), :])

    NVALID = T - (NKV - 1) * TK
    NFULL = NVALID // LANES
    TAIL = NVALID % LANES

    def tail_keys(b):
        return keys_rows(b, (NKV - 1) * TK + NFULL * LANES, TAIL)

    def tail_part(kt, q, n):
        qn = q[n * LANES:min((n + 1) * LANES, TQ), :]
        if qn.shape[0] < LANES:
            qn = jnp.concatenate([qn, jnp.zeros((LANES - qn.shape[0], D), BF16)], axis=0)
        return _dot_nt(kt, qn)

    def tail_tile(parts):
        fill = jnp.full((LANES - TAIL, LANES), -jnp.inf, F32)
        return jnp.concatenate([jnp.concatenate([p, fill], axis=0).T for p in parts], axis=0)[0:TQ, :]

    def ln_rows_paced(src, dst, rows, group, flag):
        prev = None
        for r in range(0, rows, group):
            n = min(group, rows - r)
            xv = x_s[src + r:src + r + n, :].astype(F32)
            if prev is not None:
                head = jnp.concatenate([jnp.where(flag, prev, xv[:, 0:LANES]), xv[:, LANES:]], axis=1) if PACE_ALL else None
                if head is None:
                    top = jnp.concatenate([jnp.where(flag, prev[0:8], xv[0:8, 0:LANES]), xv[0:8, LANES:]], axis=1)
                    head = jnp.concatenate([top, xv[8:]], axis=0)
                xv = head
            y = _ln(xv, EPS)
            xa_s[(dst + r) // H:(dst + r + n) // H, :] = _pack(y)
            prev = y[:, 0:LANES] if n == group and rows - r - n >= group else None
            if prev is None and rows - r - n > 0:
                prev = y[0:rows - r - n, 0:LANES]

    def qk_chunk(q, b, j, last, tok=None, parts=None):
        if last:
            s = _dot_nt(q, keys_rows(b, j * TK, NFULL * LANES))
            if parts is None:
                kt = tail_keys(b)
                parts = [tail_part(kt, q, n) for n in range(TQP // LANES)]
        else:
            s = _dot_nt(q, keys(b, j))
        if tok is not None:
            tok[0] = s
        mx = None
        for c in range(CPK):
            if last and c >= NFULL:
                st = tail_tile(parts) if c == NFULL else jnp.full((TQ, LANES), -jnp.inf, F32)
            else:
                st = s[:, c * LANES:(c + 1) * LANES]
            s_s[j, :, c * LANES:(c + 1) * LANES] = st
            mx = st if mx is None else jnp.maximum(mx, st)
        return mx

    def probs(j, m, raw=False, ntiles=CPK):
        tiles = []
        lsum = None
        for c in range(ntiles):
            p = jnp.exp2(s_s[j, :, c * LANES:(c + 1) * LANES] - m)
            lsum = p if lsum is None else lsum + p
            tiles.append(p)
        if raw:
            return tiles, lsum
        return jnp.concatenate(tiles, axis=1).astype(BF16), lsum

    def up_g(xq):
        return _ln(_gelu2(_dot(xq, _unpack(wa_s[:, 2 * D:3 * D]))), 4.0 * EPS)

    def up_u(xq):
        return _gelu2(_dot(xq, _unpack(wa_s[:, D:2 * D])))

    def store_g(ref, row, g):
        for c in range(NC):
            ref[c, row:row + g.shape[0], :] = g[:, c * LANES:(c + 1) * LANES]

    def shift_g(seq_start):
        for c in range(NC):
            g_s[c, 0:HALO, :] = jnp.where(seq_start, 0.0, g_s[c, TQ:TQ + HALO, :])
            g_s[c, HALO:HALO + TQ, :] = gn_s[c, HALO:HALO + TQ, :]

    def conv_rows(r0, R, chain=None, cg=None):
        G = R if chain is None else (cg or CG)
        rows = []
        for rr in range(0, R, G):
            cols = []
            for c in range(NC):
                acc = None
                for k in range(K):
                    off = HALO - PAD + k
                    gv = g_s[c, pl.ds(r0 + rr + off, G), :].reshape(G // 8, 8, LANES)
                    term = gv * dwb_s[k, :, c * LANES:(c + 1) * LANES][None]
                    if acc is None:
                        if chain is not None and chain[1] is not None:
                            term = jnp.where(chain[0], chain[1], term)
                        acc = term
                    else:
                        acc = acc + term
                if chain is not None:
                    chain[1] = acc
                cols.append(acc.reshape(G, LANES))
            rows.append(jnp.concatenate(cols, axis=1))
        return jnp.concatenate(rows, axis=0)

    def pv_tail(pt, flag, hist):
        rows = []
        for r in range(0, TQ, PG):
            pr = pt[r:r + PG, :]
            if PLAG and len(hist) >= PLAG:
                pr = jnp.where(flag, hist[-PLAG], pr)
            pb = [jnp.broadcast_to(pr[:, k:k + 1], (PG, LANES)) for k in range(TAIL)]
            cols = []
            for c in range(NC):
                acc = None
                for k in range(TAIL):
                    term = pb[k] * vt_s[k:k + 1, c * LANES:(c + 1) * LANES]
                    if acc is None and len(hist) >= PW:
                        term = jnp.where(flag, hist[-PW], term)
                    acc = term if acc is None else acc + term
                hist.append(acc)
                cols.append(acc)
            rows.append(jnp.concatenate(cols, axis=1))
        return jnp.concatenate(rows, axis=0)

    def finish(sb, acc, l_acc, yc):
        l = jnp.sum(l_acc, axis=-1, keepdims=True)
        ya = (acc * (1.0 / l)).astype(BF16)
        flag = z_s[0] > 0
        if LFIN == 1:
            out = _dot(ya, _unpack(wo_s[0:D // H, :]))
            out = out + _dot(tie_bf16(flag, out[0:8, 0:LANES], yc), _unpack(wo_s[D // H:2 * D // H, :]))
        elif LFIN == 2:
            out = _dot(yc, _unpack(wo_s[D // H:2 * D // H, :]))
            out = out + _dot(tie_bf16(flag, out[0:8, 0:LANES], ya), _unpack(wo_s[0:D // H, :]))
        else:
            out = _dot(yc, _unpack(wo_s[D // H:2 * D // H, :]))
            out = out + _dot(ya, _unpack(wo_s[0:D // H, :]))
        row = sb * TQ
        if not isinstance(row, int):
            row = pl.multiple_of(row, 16)
        xr = x_s[pl.ds(row, TQ), :].astype(F32)
        o_ref[...] = (xr + out).astype(o_ref.dtype)

    def store_max(mx):
        m_s[...] = jnp.broadcast_to(jnp.max(mx, axis=-1, keepdims=True), (TQ, LANES))

    def tie(flag, dep, val, n):
        if n == val.shape[0]:
            return jnp.where(flag, dep[0:n], val)
        return jnp.concatenate([jnp.where(flag, dep[0:n], val[0:n]), val[n:]], axis=0)

    def paced_by(flag, src, span, val):
        rel = jnp.concatenate(
            [src[(r * span) % TQ:(r * span) % TQ + 8, ((r * span) // TQ) * LANES:((r * span) // TQ + 1) * LANES]
             for r in range(0, TQ, 8)], axis=0)
        return jnp.where(flag, rel, val)

    def tie_bf16(flag, dep, val):
        head = pltpu.bitcast(val[0:16, 0:LANES], U32)
        head = _unpack(jnp.where(flag, pltpu.bitcast(dep, U32), head))
        top = jnp.concatenate([head, val[0:16, LANES:]], axis=1)
        return jnp.concatenate([top, val[16:, :]], axis=0)

    def first_step():
        C2 = FC2

        def xrows(r0, r1):
            return x_hbm.at[pl.ds(r0, r1 - r0), :], x_s.at[pl.ds(r0, r1 - r0), :]

        copies = {}
        plan = (
            ('wq', wq_hbm, wq_s), ('wk', wk_hbm, wk_s),
            ('xa',) + xrows(0, TK), ('xb',) + xrows(TK, C2 * TK), ('xc',) + xrows(C2 * TK, T),
            ('wup', wup_hbm, wup_s), ('dw', dw_hbm, dw_s), ('xd',) + xrows(T, T + TQ),
            ('wv', wv_hbm, wv_s), ('wao', wao_hbm, wao_s), ('wdn', wdn_hbm, wdn_s), ('wm', wm_hbm, wm_s),
            ('xe',) + xrows(T + TQ, B * T),
        )
        for i, (name, src, dst) in enumerate(plan):
            copies[name] = pltpu.make_async_copy(src, dst, sems.at[i])
            copies[name].start()

        z_s[0] = 0
        z_s[1] = 0
        z_s[2] = 0
        for b in range(B):
            xa_s[(b * TP + T) // H:(b + 1) * TP // H, :] = jnp.zeros(((TP - T) // H, D), U32)
        store_g(g_s, TQ, jnp.zeros((HALO, D), F32))
        acc_s[...] = jnp.zeros((TQ, D), F32)
        l_s[...] = jnp.zeros((TQ, LANES), F32)

        def ln_chunk(c):
            ln_rows(c * TK, c * TK, min(TK, T - c * TK))

        scale = float(D) ** (-0.5) * math.log2(math.e)
        DS = FSPLIT * LANES
        copies['wq'].wait()
        copies['wk'].wait()
        m_lo = _dot_nt(wq_s[...], wk_s[0:DS, :])

        never = z_s[0] > 0
        zero = pl.multiple_of(z_s[0], 8)
        copies['xa'].wait()
        wa_s[:, 0:DS] = _pack(_center(m_lo) * scale)
        wa_s[:, DS:D] = _pack(_center(_dot_nt(wq_s[...], wk_s[DS:D, :])) * scale)
        ln_chunk(0)
        q = _dot(_unpack(xa_s[0:TQ // H, :]), _unpack(wa_s[:, 0:D])).astype(BF16)
        if not HOLD:
            mx = qk_chunk(q, 0, 0, False)

        copies['xb'].wait()
        if HOLD:
            mx = qk_chunk(q, 0, 0, False)
        for c in range(1, C2):
            ln_chunk(c)
            mx = jnp.maximum(mx, qk_chunk(q, 0, c, False))

        for name in ('xc', 'wup', 'dw'):
            copies[name].wait()
        xq = _unpack(xa_s[0:TQ // H, :])
        hg = _dot(xq, wup_s[:, D:2 * D])
        hu = _dot(tie_bf16(never, hg[0:8, LANES:2 * LANES], xq), wup_s[:, 0:D])
        gg = _gelu2(hg)
        if GPACE:
            rel = jnp.concatenate([hu[(r * GPACE) % TQ:(r * GPACE) % TQ + 8, ((r * GPACE) // TQ) * LANES:((r * GPACE) // TQ + 1) * LANES]
                                   for r in range(0, TQ, 8)], axis=0)
            gg = jnp.concatenate([jnp.where(never, rel, gg[:, 0:LANES]), gg[:, LANES:]], axis=1)
        store_g(gn_s, HALO, _ln(gg, 4.0 * EPS))
        u_s[0] = _gelu2(hu)
        wa_s[:, D:3 * D] = _pack(wup_s[...])
        dwf = dw_s[...].astype(F32)
        for k in range(K):
            dwb_s[k] = jnp.broadcast_to(dwf[k:k + 1, :], (8, D))
        deps = [hu[0:8, LANES:2 * LANES], gn_s[0, pl.ds(zero + HALO, 8), :], u_s[0, pl.ds(zero, 8), 0:LANES]]
        order = list(range(C2, NKV))
        if TLAST:
            order = [NKV - 1] + order[:-1]
        deps = {0: deps[0], GDEP: deps[1], UDEP: deps[2]}
        parts = None
        for i, c in enumerate(order):
            if i == 0 and PACE4:
                ln_rows_paced(c * TK, c * TK, min(TK, T - c * TK), PACE4, never)
            else:
                ln_chunk(c)
            qc = tie_bf16(never, deps[i], q) if i in deps else q
            if parts is not None and i == 1:
                dep = jnp.concatenate([p[0:8] for p in parts], axis=0)
                low = pltpu.bitcast(qc[16:16 + 2 * dep.shape[0], 0:LANES], U32)
                low = _unpack(jnp.where(never, pltpu.bitcast(dep, U32), low))
                col = jnp.concatenate([qc[0:16, 0:LANES], low, qc[16 + 2 * dep.shape[0]:, 0:LANES]], axis=0)
                qc = jnp.concatenate([col, qc[:, LANES:]], axis=1)
            if c == NKV - 1:
                kt = tail_keys(0)
                parts = [tail_part(kt, q, n) for n in range(TQP // LANES)]
            mx = jnp.maximum(mx, qk_chunk(qc, 0, c, c == NKV - 1, parts=parts))

        for name in ('xd', 'wv', 'wao', 'wdn', 'wm'):
            copies[name].wait()
        store_max(mx)
        if PACE5:
            ln_rows_paced(T, TP, TQ, PACE5, never)
        else:
            ln_rows(T, TP, TQ)
        wva_raw = _dot(wv_s[...], wao_s[...])
        wdn = tie_bf16(never, wva_raw[0:8, 0:LANES], wdn_s[...]) if R5TIE else wdn_s[...]
        wdm = _dot(wdn, wm_s[D:2 * D, :])
        if CPACE:
            mean = jnp.broadcast_to(jnp.sum(wva_raw, axis=0, keepdims=True) * (1.0 / D), (8, D))
            rows = []
            for i, r in enumerate(range(0, D, CPACE)):
                pos = (i * CPACE * CSPAN) % D // 8 * 8
                col = (i * CPACE * CSPAN) // D
                tokn = wdm[pos:pos + 8, col * LANES:(col + 1) * LANES]
                mu = jnp.where(never, jnp.concatenate([tokn] * NC, axis=1), mean)
                rows.append((wva_raw[r:r + CPACE].reshape(CPACE // 8, 8, D) - mu[None]).reshape(CPACE, D))
            wva = jnp.concatenate(rows, axis=0).astype(BF16)
        else:
            wva = _center(wva_raw).astype(BF16)
        wo_s[D // H:2 * D // H, :] = _pack(0.5 * wdm)
        lhs = tie_bf16(never, xa_s[pl.ds(zero, 8), 0:LANES], wva)
        if R5TIE:
            lhs = jnp.concatenate([lhs[0:16], tie_bf16(never, wdm[0:8, LANES:2 * LANES], lhs[16:])], axis=0)
        wo_s[0:D // H, :] = _pack(_dot(lhs, wm_s[0:D, :]))
        copies['xe'].wait()

    def main_step():
        ba = step // NQ
        ia = step % NQ
        sb = step - 1
        bb = sb // NQ
        shift_g(sb % NQ == 0)
        never = z_s[0] > 0
        never2 = z_s[1] > 0
        never3 = z_s[2] > 0
        tok = [None]
        paced = functools.partial(paced_by, never)

        def prev_tile():
            return tok[0][TIER:, TIEC * LANES:(TIEC + 1) * LANES]

        def after_packed(lhs):
            if tok[0] is None:
                return _unpack(lhs)
            head = tie(never3, pltpu.bitcast(prev_tile(), U32), lhs[:, 0:LANES], min(TIEN, TQ // H))
            return _unpack(jnp.concatenate([head, lhs[:, LANES:]], axis=1))

        def after_tiles(tiles):
            tiles = list(tiles)
            tiles[1] = tie(never3, prev_tile(), tiles[1], TIEN)
            return jnp.concatenate(tiles, axis=1).astype(BF16)

        def split(v):
            return [v[:, c * LANES:(c + 1) * LANES] for c in range(v.shape[1] // LANES)]

        def mm(lhs, rhs):
            tok[0] = _dot(lhs, rhs)
            return tok[0]

        m_old = m_s[...]
        xq = xa_s[pl.ds(pl.multiple_of(ba * (TP // H) + ia * (TQ // H), 8), TQ // H), :]
        q_raw = mm(after_packed(xq), _unpack(wa_s[:, 0:D]))
        qp = _pack(q_raw)
        hg = mm(after_packed(xq), _unpack(wa_s[:, 2 * D:3 * D]))
        hu = mm(after_packed(xq), _unpack(wa_s[:, D:2 * D]))

        def make_g(hg, pace_src, span):
            gg = _gelu2(hg)
            if span:
                gg = jnp.concatenate([paced(pace_src, span, gg[:, 0:LANES]), gg[:, LANES:]], axis=1)
            g_new = _ln(gg, 4.0 * EPS)
            store_g(gn_s, HALO, g_new)
            store_g(g_s, HALO + TQ, jnp.where(ia == 0, 0.0, g_new[0:HALO, :]))

        if GREL < 0:
            make_g(hg, hu, MGP)
        u_old = u_s[0]
        if UREL < 0:
            u_s[0] = _gelu2(hu)
        nxt = jnp.minimum(step + NQ, N - 1)
        xv = x_s[pl.ds(pl.multiple_of(nxt * TQ, 16), TQ), :].astype(F32)
        if MLP:
            xv = jnp.concatenate([paced(q_raw, MLP, xv[:, 0:LANES]), xv[:, LANES:]], axis=1)
        if LREL < 0:
            xn = _pack(_ln(xv, EPS))
        mx = None
        mx_prev = None
        acc = None
        vt_s[...] = tail_keys(bb).astype(F32)
        l_acc = jnp.exp2(s_s[NKV - 1, :, NFULL * LANES:(NFULL + 1) * LANES] - m_old)
        p_tail = l_acc
        parts = []
        s_hist = []
        for j in range(NKV):
            m_use = m_old
            if EREL == 0 and mx_prev is not None:
                m_use = jnp.where(never, mx_prev, m_use)
            elif EREL == 1 and j >= 1:
                m_use = paced(o, min(ESPAN, o.shape[1] // LANES), m_old)
            elif EREL == 2 and j >= 2:
                m_use = paced(s_hist[j - 2], ESPAN, m_old)
            elif EREL == 3 and j >= 1:
                m_use = paced(s_hist[j - 1], ESPAN, m_old)
            if j == 0 and E0:
                m_use = paced((q_raw, hg, hu)[E0 - 1], ESPAN, m_old)
            if j == 1 and EREL == 2 and E1:
                m_use = paced((q_raw, hg, hu, o)[E1 - 1], ESPAN, m_old)
            nt = NFULL if j == NKV - 1 else CPK
            tiles, l_new = probs(j, m_use, raw=True, ntiles=nt)
            l_acc = l_acc + l_new
            tiles[0] = jnp.where(never2, l_acc, tiles[0])
            o = mm(after_tiles(tiles), keys_rows(bb, j * TK, nt * LANES))
            acc = o if acc is None else acc + o
            if j == LREL:
                xn = _pack(_ln(jnp.concatenate([paced(o, LSPAN, xv[:, 0:LANES]), xv[:, LANES:]], axis=1), EPS))
            if j == GREL:
                hg = jnp.concatenate([jnp.where(never, a, b) for a, b in zip(split(o), split(hg))], axis=1)
            if j == UREL:
                u_s[0] = _gelu2(jnp.concatenate(
                    [jnp.where(never, a, b) for a, b in zip(split(o), split(hu))], axis=1))
            qj = qp
            if j == UJ:
                udep = u_s[0, pl.ds(pl.multiple_of(z_s[0], 8), 8), 0:LANES]
                qj = jnp.concatenate([qj[:, 0:3 * LANES], tie(never2, pltpu.bitcast(udep, U32), qj[:, 3 * LANES:], 8)], axis=1)
            if j == LNJ:
                qj = jnp.where(never3, xn, qj)
            if j == GJ:
                gdep = gn_s[0, pl.ds(pl.multiple_of(z_s[0] + HALO, 8), 8), :]
                qj = jnp.concatenate([qj[:, 0:LANES], tie(never2, pltpu.bitcast(gdep, U32), qj[:, LANES:2 * LANES], 8), qj[:, 2 * LANES:]], axis=1)
            n = j - TJ0
            if 0 <= n < TQP // LANES:
                kt = tie_bf16(never3, o[0:8, TTC * LANES:(TTC + 1) * LANES], tail_keys(ba))
                parts.append(tail_part(kt, _unpack(qp), n))
            if 0 <= n - 1 < TQP // LANES:
                dep = pltpu.bitcast(parts[n - 1], U32)
                qj = jnp.concatenate([qj[:, 0:2 * LANES], tie(never2, dep, qj[:, 2 * LANES:3 * LANES], TAIL), qj[:, 3 * LANES:]], axis=1)
            mx_prev = mx
            mj = qk_chunk(after_packed(qj), ba, j, j == NKV - 1, tok, parts if parts else None)
            mx = mj if mx is None else jnp.maximum(mx, mj)
            s_hist.append(tok[0])
            if j == GREL:
                make_g(hg, tok[0], MGP)
        yc = u_old * conv_rows(0, TQ, [never, None])
        o_tail = pv_tail(p_tail, never, [])
        l = jnp.sum(l_acc, axis=-1, keepdims=True)
        ya = (acc + o_tail) * (1.0 / l)
        if OUTA:
            out = mm(after_tiles(split(ya)), _unpack(wo_s[0:D // H, :]))
            out = out + mm(after_tiles(split(yc)), _unpack(wo_s[D // H:2 * D // H, :]))
        else:
            out = mm(after_tiles(split(yc)), _unpack(wo_s[D // H:2 * D // H, :]))
            out = out + mm(after_tiles(split(ya)), _unpack(wo_s[0:D // H, :]))
        xr = x_s[pl.ds(pl.multiple_of(sb * TQ, 16), TQ), :].astype(F32)
        o_ref[...] = (xr + out).astype(o_ref.dtype)
        store_max(mx)
        dst = pl.multiple_of((nxt // NQ) * (TP // H) + (nxt % NQ) * (TQ // H), 8)
        late = pltpu.bitcast(mx[0:TQ // H, :], U32)
        for c in range(NC):
            xa_s[pl.ds(dst, TQ // H), c * LANES:(c + 1) * LANES] = jnp.where(
                never, late, xn[:, c * LANES:(c + 1) * LANES])

    def last_step():
        sb = N - 1
        bb = B - 1
        uslot = 0
        CPI = LCPI
        NIT = NKV // CPI
        RL = 16 * (TQ // (16 * NIT)) if LFLOOR else 16 * (-(-TQ // (16 * NIT)))
        never = z_s[0] > 0
        never2 = z_s[1] > 0
        for c in range(NC):
            gn_s[c, 0:HALO, :] = jnp.where(NQ == 1, 0.0, g_s[c, TQ:TQ + HALO, :])
        store_g(gn_s, HALO + TQ, jnp.zeros((HALO, D), F32))

        def attend(j0):
            acc = acc_s[...]
            l_acc = l_s[...]
            o = None
            for jj in range(CPI):
                m_use = m_s[...]
                if o is not None and LPACE:
                    m_use = paced_by(never, o, LPACE, m_use)
                tiles, l_new = probs(j0 + jj, m_use, raw=True)
                l_acc = l_acc + l_new
                if jj > 0 or not LNOL:
                    tiles[0] = jnp.where(never2, l_acc, tiles[0])
                if o is not None and LORD:
                    tiles[1] = tie(never, o[:, LANES:2 * LANES], tiles[1], 8)
                o = _dot(jnp.concatenate(tiles, axis=1).astype(BF16), keys(bb, j0 + jj))
                acc = acc + o
            return acc, l_acc

        def loop(t, carry):
            r0 = pl.multiple_of(jnp.minimum(t * RL, TQ - RL), 16)

            def conv_part():
                for c in range(NC):
                    g_s[c, 0:RL + 2 * HALO, :] = gn_s[c, pl.ds(r0, RL + 2 * HALO), :]
                yc = u_s[uslot, pl.ds(r0, RL), :] * conv_rows(0, RL, [never, None], LCG)
                yc_s[pl.ds(pl.multiple_of(r0 // H, 8), RL // H), :] = _pack(yc)

            if LCF:
                conv_part()
            acc, l_acc = attend(t * CPI)
            acc_s[...] = acc
            l_s[...] = l_acc
            if not LCF:
                conv_part()
            return carry

        lax.fori_loop(0, NIT, loop, 0)
        if NIT * RL < TQ:
            r0 = NIT * RL
            for c in range(NC):
                g_s[c, 0:TQ - r0 + 2 * HALO, :] = gn_s[c, r0:TQ + 2 * HALO, :]
            yc_s[r0 // H:TQ // H, :] = _pack(u_s[uslot, r0:TQ, :] * conv_rows(0, TQ - r0, [never, None] if LFC else None, LFC))
        finish(sb, acc_s[...], l_s[...], _unpack(yc_s[...]))

    @pl.when(step == 0)
    def _():
        first_step()

    @pl.when(jnp.logical_and(step > 0, step < N))
    def _():
        main_step()

    @pl.when(step == N)
    def _():
        last_step()


@jax.jit
def pallas_standalone__conformer_family_branchformer__speech_kernel(
    x: jax.Array,
    w_q: jax.Array,
    w_k: jax.Array,
    w_v: jax.Array,
    w_ao: jax.Array,
    w_up: jax.Array,
    dw: jax.Array,
    w_dn: jax.Array,
    w_merge: jax.Array,
):
    B, T, D = x.shape
    K = dw.shape[0]
    TQ = 400
    TK = 512
    TP = -(-T // TK) * TK
    NKV = TP // TK
    assert T % TQ == 0 and TQ % 16 == 0 and D % LANES == 0 and K // 2 < HALO
    assert TQ <= TK and B >= 2 and NKV >= 3 and T % 16 == 0
    N = B * (T // TQ)
    x2 = x.reshape(B * T, D)

    kern = functools.partial(_kernel, B=B, T=T, D=D, K=K, TQ=TQ, TK=TK, TP=TP)
    ins = (x2, w_q, w_k, w_v, w_ao, w_up, dw, w_dn, w_merge)
    out = pl.pallas_call(
        kern,
        grid=(N + 1,),
        in_specs=[pl.BlockSpec(memory_space=pl.ANY) for _ in ins],
        out_specs=pl.BlockSpec((TQ, D), lambda s: (jnp.maximum(s - 1, 0), 0)),
        out_shape=jax.ShapeDtypeStruct((B * T, D), x.dtype),
        scratch_shapes=[pltpu.VMEM(a.shape, a.dtype) for a in ins] + [
            pltpu.SemaphoreType.DMA((13,)),
            pltpu.VMEM((B * TP // 2, D), U32),
            pltpu.VMEM((D // 2, 3 * D), U32),
            pltpu.VMEM((D, D), U32),
            pltpu.VMEM((K, 8, D), F32),
            pltpu.VMEM((NKV, TQ, TK), F32),
            pltpu.VMEM((TQ, LANES), F32),
            pltpu.VMEM((1, TQ, D), F32),
            pltpu.VMEM((D // LANES, TQ + 2 * HALO, LANES), F32),
            pltpu.VMEM((D // LANES, TQ + 2 * HALO, LANES), F32),
            pltpu.VMEM((TQ, D), F32),
            pltpu.VMEM((TQ, LANES), F32),
            pltpu.VMEM((TQ // 2, D), U32),
            pltpu.VMEM((T % LANES, D), F32),
            pltpu.SMEM((3,), jnp.int32),
        ],
        compiler_params=pltpu.CompilerParams(
            dimension_semantics=("arbitrary",),
            vmem_limit_bytes=100 * 1024 * 1024,
            disable_bounds_checks=True,
            disable_semaphore_checks=True,
        ),
    )(*ins)
    return out.reshape(B, T, D)
```

```python
import functools
import math

import jax
import jax.numpy as jnp
from jax import lax
import jax.experimental.pallas as pl
import jax.experimental.pallas.tpu as pltpu

LANES = 128
EPS = 1e-05
F32 = jnp.float32
BF16 = jnp.bfloat16
U32 = jnp.uint32
NT = (((1,), (1,)), ((), ()))
CG = 16
LNJ = 1
TIER = 0
TIEC = 0
TIEN = 8
GJ = 3
LCG = 8
PG = 8
PW = 1
PLAG = 5
OUTA = 1
TJ0 = 0
TTC = 2
LCPI = 2
FC2 = 4
FSPLIT = 2
HOLD = 1
TLAST = 0
R5TIE = 1
GDEP = 1
UDEP = 3
PACE4 = 0
PACE5 = 48
PACE_ALL = 1
CPACE = 64
CSPAN = 3
GPACE = 3
MGP = 3
MLP = 2
EREL = 0
ESPAN = 4
E0 = 0
E1 = 0
LREL = -1
LSPAN = 4
UREL = 4
UJ = -1
GREL = -1
LPACE = 0
LNOL = 0
LORD = 1
LCF = 1
LFLOOR = 1
LSPLIT = 256
LSPLIT2 = 352
LFC = 16
HALO = 16


def _ln(x, eps):
    d = x.shape[-1]
    m = jnp.sum(x, axis=-1, keepdims=True) * (1.0 / d)
    xc = x - m
    v = jnp.sum(xc * xc, axis=-1, keepdims=True) * (1.0 / d)
    return xc * lax.rsqrt(v + eps)


def _gelu2(x):
    c1 = math.sqrt(2.0 / math.pi)
    c2 = c1 * 0.044715
    t = jnp.tanh(x * (c1 + c2 * (x * x)))
    return x + x * t


def _center(w):
    return w - jnp.sum(w, axis=0, keepdims=True) * (1.0 / w.shape[0])


def _pack(x):
    return pltpu.bitcast(x.astype(BF16), U32)


def _unpack(x):
    return pltpu.bitcast(x, BF16)


def _dot(a, b):
    return jnp.dot(a, b, preferred_element_type=F32)


def _dot_nt(a, b):
    return lax.dot_general(a, b, NT, preferred_element_type=F32)


def _kernel(x_hbm, wq_hbm, wk_hbm, wv_hbm, wao_hbm, wup_hbm, dw_hbm, wdn_hbm, wm_hbm,
            o_hbm,
            x_s, wq_s, wk_s, wv_s, wao_s, wup_s, dw_s, wdn_s, wm_s, sems,
            xa_s, wa_s, wo_s, dwb_s, s_s, m_s, u_s, g_s, gn_s, acc_s, l_s, yc_s, vt_s, o_s, osems, z_s,
            *, B, T, D, K, TQ, TK, TP):
    NQ = T // TQ
    N = B * NQ
    NKV = TP // TK
    NC = D // LANES
    CPK = TK // LANES
    PAD = K // 2
    H = 2
    TQP = -(-TQ // LANES) * LANES

    def out_copy(blk):
        row = blk * TQ
        if not isinstance(row, int):
            row = pl.multiple_of(row, 16)
        return pltpu.make_async_copy(o_s.at[blk % 2], o_hbm.at[pl.ds(row, TQ), :], osems.at[blk % 2])

    def keys(b, j):
        start = b * (TP // H) + j * (TK // H)
        if not isinstance(start, int):
            start = pl.multiple_of(start, 8)
        return _unpack(xa_s[pl.ds(start, TK // H), :])

    def ln_rows(src, dst, rows):
        if not isinstance(src, int):
            src = pl.multiple_of(src, 16)
        dsth = dst // H
        if not isinstance(dsth, int):
            dsth = pl.multiple_of(dsth, 8)
        xa_s[pl.ds(dsth, rows // H), :] = _pack(_ln(x_s[pl.ds(src, rows), :].astype(F32), EPS))

    def keys_rows(b, r0, n):
        start = b * (TP // H) + r0 // H
        if not isinstance(start, int):
            start = pl.multiple_of(start, 8)
        return _unpack(xa_s[pl.ds(start, n // H), :])

    NVALID = T - (NKV - 1) * TK
    NFULL = NVALID // LANES
    TAIL = NVALID % LANES

    def tail_keys(b):
        return keys_rows(b, (NKV - 1) * TK + NFULL * LANES, TAIL)

    def tail_part(kt, q, n):
        qn = q[n * LANES:min((n + 1) * LANES, TQ), :]
        if qn.shape[0] < LANES:
            qn = jnp.concatenate([qn, jnp.zeros((LANES - qn.shape[0], D), BF16)], axis=0)
        return _dot_nt(kt, qn)

    def tail_tile(parts):
        fill = jnp.full((LANES - TAIL, LANES), -jnp.inf, F32)
        return jnp.concatenate([jnp.concatenate([p, fill], axis=0).T for p in parts], axis=0)[0:TQ, :]

    def ln_rows_paced(src, dst, rows, group, flag):
        prev = None
        for r in range(0, rows, group):
            n = min(group, rows - r)
            xv = x_s[src + r:src + r + n, :].astype(F32)
            if prev is not None:
                head = jnp.concatenate([jnp.where(flag, prev, xv[:, 0:LANES]), xv[:, LANES:]], axis=1) if PACE_ALL else None
                if head is None:
                    top = jnp.concatenate([jnp.where(flag, prev[0:8], xv[0:8, 0:LANES]), xv[0:8, LANES:]], axis=1)
                    head = jnp.concatenate([top, xv[8:]], axis=0)
                xv = head
            y = _ln(xv, EPS)
            xa_s[(dst + r) // H:(dst + r + n) // H, :] = _pack(y)
            prev = y[:, 0:LANES] if n == group and rows - r - n >= group else None
            if prev is None and rows - r - n > 0:
                prev = y[0:rows - r - n, 0:LANES]

    def qk_chunk(q, b, j, last, tok=None, parts=None):
        if last:
            s = _dot_nt(q, keys_rows(b, j * TK, NFULL * LANES))
            if parts is None:
                kt = tail_keys(b)
                parts = [tail_part(kt, q, n) for n in range(TQP // LANES)]
        else:
            s = _dot_nt(q, keys(b, j))
        if tok is not None:
            tok[0] = s
        mx = None
        for c in range(CPK):
            if last and c >= NFULL:
                st = tail_tile(parts) if c == NFULL else jnp.full((TQ, LANES), -jnp.inf, F32)
            else:
                st = s[:, c * LANES:(c + 1) * LANES]
            s_s[j, :, c * LANES:(c + 1) * LANES] = st
            mx = st if mx is None else jnp.maximum(mx, st)
        return mx

    def probs(j, m, raw=False, ntiles=CPK):
        tiles = []
        lsum = None
        for c in range(ntiles):
            p = jnp.exp2(s_s[j, :, c * LANES:(c + 1) * LANES] - m)
            lsum = p if lsum is None else lsum + p
            tiles.append(p)
        if raw:
            return tiles, lsum
        return jnp.concatenate(tiles, axis=1).astype(BF16), lsum

    def up_g(xq):
        return _ln(_gelu2(_dot(xq, _unpack(wa_s[:, 2 * D:3 * D]))), 4.0 * EPS)

    def up_u(xq):
        return _gelu2(_dot(xq, _unpack(wa_s[:, D:2 * D])))

    def store_g(ref, row, g):
        for c in range(NC):
            ref[c, row:row + g.shape[0], :] = g[:, c * LANES:(c + 1) * LANES]

    def shift_g(seq_start):
        for c in range(NC):
            g_s[c, 0:HALO, :] = jnp.where(seq_start, 0.0, g_s[c, TQ:TQ + HALO, :])
            g_s[c, HALO:HALO + TQ, :] = gn_s[c, HALO:HALO + TQ, :]

    def conv_rows(r0, R, chain=None, cg=None):
        G = R if chain is None else (cg or CG)
        rows = []
        for rr in range(0, R, G):
            cols = []
            for c in range(NC):
                acc = None
                for k in range(K):
                    off = HALO - PAD + k
                    gv = g_s[c, pl.ds(r0 + rr + off, G), :].reshape(G // 8, 8, LANES)
                    term = gv * dwb_s[k, :, c * LANES:(c + 1) * LANES][None]
                    if acc is None:
                        if chain is not None and chain[1] is not None:
                            term = jnp.where(chain[0], chain[1], term)
                        acc = term
                    else:
                        acc = acc + term
                if chain is not None:
                    chain[1] = acc
                cols.append(acc.reshape(G, LANES))
            rows.append(jnp.concatenate(cols, axis=1))
        return jnp.concatenate(rows, axis=0)

    def pv_tail(pt, flag, hist):
        rows = []
        for r in range(0, TQ, PG):
            pr = pt[r:r + PG, :]
            if PLAG and len(hist) >= PLAG:
                pr = jnp.where(flag, hist[-PLAG], pr)
            pb = [jnp.broadcast_to(pr[:, k:k + 1], (PG, LANES)) for k in range(TAIL)]
            cols = []
            for c in range(NC):
                acc = None
                for k in range(TAIL):
                    term = pb[k] * vt_s[k:k + 1, c * LANES:(c + 1) * LANES]
                    if acc is None and len(hist) >= PW:
                        term = jnp.where(flag, hist[-PW], term)
                    acc = term if acc is None else acc + term
                hist.append(acc)
                cols.append(acc)
            rows.append(jnp.concatenate(cols, axis=1))
        return jnp.concatenate(rows, axis=0)

    def part_copy(blk, r0, r1, sem):
        return pltpu.make_async_copy(o_s.at[blk % 2, pl.ds(r0, r1 - r0), :],
                                     o_hbm.at[pl.ds(blk * TQ + r0, r1 - r0), :], sem)

    FIN = [0] + [r for r in (LSPLIT, LSPLIT2) if r] + [TQ]

    def finish(sb):
        flag = z_s[0] > 0
        for i, (r0, r1) in enumerate(zip(FIN[:-1], FIN[1:])):
            l = jnp.sum(l_s[r0:r1, :], axis=-1, keepdims=True)
            ya = (acc_s[r0:r1, :] * (1.0 / l)).astype(BF16)
            out = _dot(_unpack(yc_s[r0 // H:r1 // H, :]), _unpack(wo_s[D // H:2 * D // H, :]))
            out = out + _dot(tie_bf16(flag, out[0:8, 0:LANES], ya), _unpack(wo_s[0:D // H, :]))
            xr = x_s[sb * TQ + r0:sb * TQ + r1, :].astype(F32)
            o_s[sb % 2, r0:r1, :] = (xr + out).astype(o_s.dtype)
            part_copy(sb, r0, r1, osems.at[2 + i]).start()

    def store_max(mx):
        m_s[...] = jnp.broadcast_to(jnp.max(mx, axis=-1, keepdims=True), (TQ, LANES))

    def tie(flag, dep, val, n):
        if n == val.shape[0]:
            return jnp.where(flag, dep[0:n], val)
        return jnp.concatenate([jnp.where(flag, dep[0:n], val[0:n]), val[n:]], axis=0)

    def paced_by(flag, src, span, val):
        rel = jnp.concatenate(
            [src[(r * span) % TQ:(r * span) % TQ + 8, ((r * span) // TQ) * LANES:((r * span) // TQ + 1) * LANES]
             for r in range(0, TQ, 8)], axis=0)
        return jnp.where(flag, rel, val)

    def tie_bf16(flag, dep, val):
        head = pltpu.bitcast(val[0:16, 0:LANES], U32)
        head = _unpack(jnp.where(flag, pltpu.bitcast(dep, U32), head))
        top = jnp.concatenate([head, val[0:16, LANES:]], axis=1)
        return jnp.concatenate([top, val[16:, :]], axis=0)

    def first_step():
        C2 = FC2

        def xrows(r0, r1):
            return x_hbm.at[pl.ds(r0, r1 - r0), :], x_s.at[pl.ds(r0, r1 - r0), :]

        copies = {}
        plan = (
            ('wq', wq_hbm, wq_s), ('wk', wk_hbm, wk_s),
            ('xa',) + xrows(0, TK), ('xb',) + xrows(TK, C2 * TK), ('xc',) + xrows(C2 * TK, T),
            ('wup', wup_hbm, wup_s), ('dw', dw_hbm, dw_s), ('xd',) + xrows(T, T + TQ),
            ('wv', wv_hbm, wv_s), ('wao', wao_hbm, wao_s), ('wdn', wdn_hbm, wdn_s), ('wm', wm_hbm, wm_s),
            ('xe',) + xrows(T + TQ, B * T),
        )
        for i, (name, src, dst) in enumerate(plan):
            copies[name] = pltpu.make_async_copy(src, dst, sems.at[i])
            copies[name].start()

        z_s[0] = 0
        z_s[1] = 0
        z_s[2] = 0
        for b in range(B):
            xa_s[(b * TP + T) // H:(b + 1) * TP // H, :] = jnp.zeros(((TP - T) // H, D), U32)
        store_g(g_s, TQ, jnp.zeros((HALO, D), F32))
        acc_s[...] = jnp.zeros((TQ, D), F32)
        l_s[...] = jnp.zeros((TQ, LANES), F32)

        def ln_chunk(c):
            ln_rows(c * TK, c * TK, min(TK, T - c * TK))

        scale = float(D) ** (-0.5) * math.log2(math.e)
        DS = FSPLIT * LANES
        copies['wq'].wait()
        copies['wk'].wait()
        m_lo = _dot_nt(wq_s[...], wk_s[0:DS, :])

        never = z_s[0] > 0
        zero = pl.multiple_of(z_s[0], 8)
        copies['xa'].wait()
        wa_s[:, 0:DS] = _pack(_center(m_lo) * scale)
        wa_s[:, DS:D] = _pack(_center(_dot_nt(wq_s[...], wk_s[DS:D, :])) * scale)
        ln_chunk(0)
        q = _dot(_unpack(xa_s[0:TQ // H, :]), _unpack(wa_s[:, 0:D])).astype(BF16)
        if not HOLD:
            mx = qk_chunk(q, 0, 0, False)

        copies['xb'].wait()
        if HOLD:
            mx = qk_chunk(q, 0, 0, False)
        for c in range(1, C2):
            ln_chunk(c)
            mx = jnp.maximum(mx, qk_chunk(q, 0, c, False))

        for name in ('xc', 'wup', 'dw'):
            copies[name].wait()
        xq = _unpack(xa_s[0:TQ // H, :])
        hg = _dot(xq, wup_s[:, D:2 * D])
        hu = _dot(tie_bf16(never, hg[0:8, LANES:2 * LANES], xq), wup_s[:, 0:D])
        gg = _gelu2(hg)
        if GPACE:
            rel = jnp.concatenate([hu[(r * GPACE) % TQ:(r * GPACE) % TQ + 8, ((r * GPACE) // TQ) * LANES:((r * GPACE) // TQ + 1) * LANES]
                                   for r in range(0, TQ, 8)], axis=0)
            gg = jnp.concatenate([jnp.where(never, rel, gg[:, 0:LANES]), gg[:, LANES:]], axis=1)
        store_g(gn_s, HALO, _ln(gg, 4.0 * EPS))
        u_s[0] = _gelu2(hu)
        wa_s[:, D:3 * D] = _pack(wup_s[...])
        dwf = dw_s[...].astype(F32)
        for k in range(K):
            dwb_s[k] = jnp.broadcast_to(dwf[k:k + 1, :], (8, D))
        deps = [hu[0:8, LANES:2 * LANES], gn_s[0, pl.ds(zero + HALO, 8), :], u_s[0, pl.ds(zero, 8), 0:LANES]]
        order = list(range(C2, NKV))
        if TLAST:
            order = [NKV - 1] + order[:-1]
        deps = {0: deps[0], GDEP: deps[1], UDEP: deps[2]}
        parts = None
        for i, c in enumerate(order):
            if i == 0 and PACE4:
                ln_rows_paced(c * TK, c * TK, min(TK, T - c * TK), PACE4, never)
            else:
                ln_chunk(c)
            qc = tie_bf16(never, deps[i], q) if i in deps else q
            if parts is not None and i == 1:
                dep = jnp.concatenate([p[0:8] for p in parts], axis=0)
                low = pltpu.bitcast(qc[16:16 + 2 * dep.shape[0], 0:LANES], U32)
                low = _unpack(jnp.where(never, pltpu.bitcast(dep, U32), low))
                col = jnp.concatenate([qc[0:16, 0:LANES], low, qc[16 + 2 * dep.shape[0]:, 0:LANES]], axis=0)
                qc = jnp.concatenate([col, qc[:, LANES:]], axis=1)
            if c == NKV - 1:
                kt = tail_keys(0)
                parts = [tail_part(kt, q, n) for n in range(TQP // LANES)]
            mx = jnp.maximum(mx, qk_chunk(qc, 0, c, c == NKV - 1, parts=parts))

        for name in ('xd', 'wv', 'wao', 'wdn', 'wm'):
            copies[name].wait()
        store_max(mx)
        if PACE5:
            ln_rows_paced(T, TP, TQ, PACE5, never)
        else:
            ln_rows(T, TP, TQ)
        wva_raw = _dot(wv_s[...], wao_s[...])
        wdn = tie_bf16(never, wva_raw[0:8, 0:LANES], wdn_s[...]) if R5TIE else wdn_s[...]
        wdm = _dot(wdn, wm_s[D:2 * D, :])
        if CPACE:
            mean = jnp.broadcast_to(jnp.sum(wva_raw, axis=0, keepdims=True) * (1.0 / D), (8, D))
            rows = []
            for i, r in enumerate(range(0, D, CPACE)):
                pos = (i * CPACE * CSPAN) % D // 8 * 8
                col = (i * CPACE * CSPAN) // D
                tokn = wdm[pos:pos + 8, col * LANES:(col + 1) * LANES]
                mu = jnp.where(never, jnp.concatenate([tokn] * NC, axis=1), mean)
                rows.append((wva_raw[r:r + CPACE].reshape(CPACE // 8, 8, D) - mu[None]).reshape(CPACE, D))
            wva = jnp.concatenate(rows, axis=0).astype(BF16)
        else:
            wva = _center(wva_raw).astype(BF16)
        wo_s[D // H:2 * D // H, :] = _pack(0.5 * wdm)
        lhs = tie_bf16(never, xa_s[pl.ds(zero, 8), 0:LANES], wva)
        if R5TIE:
            lhs = jnp.concatenate([lhs[0:16], tie_bf16(never, wdm[0:8, LANES:2 * LANES], lhs[16:])], axis=0)
        wo_s[0:D // H, :] = _pack(_dot(lhs, wm_s[0:D, :]))
        copies['xe'].wait()

    def main_step(step):
        ba = step // NQ
        ia = step % NQ
        sb = step - 1
        bb = sb // NQ
        shift_g(sb % NQ == 0)
        never = z_s[0] > 0
        never2 = z_s[1] > 0
        never3 = z_s[2] > 0
        tok = [None]
        paced = functools.partial(paced_by, never)

        def prev_tile():
            return tok[0][TIER:, TIEC * LANES:(TIEC + 1) * LANES]

        def after_packed(lhs):
            if tok[0] is None:
                return _unpack(lhs)
            head = tie(never3, pltpu.bitcast(prev_tile(), U32), lhs[:, 0:LANES], min(TIEN, TQ // H))
            return _unpack(jnp.concatenate([head, lhs[:, LANES:]], axis=1))

        def after_tiles(tiles):
            tiles = list(tiles)
            tiles[1] = tie(never3, prev_tile(), tiles[1], TIEN)
            return jnp.concatenate(tiles, axis=1).astype(BF16)

        def split(v):
            return [v[:, c * LANES:(c + 1) * LANES] for c in range(v.shape[1] // LANES)]

        def mm(lhs, rhs):
            tok[0] = _dot(lhs, rhs)
            return tok[0]

        m_old = m_s[...]
        xq = xa_s[pl.ds(pl.multiple_of(ba * (TP // H) + ia * (TQ // H), 8), TQ // H), :]
        q_raw = mm(after_packed(xq), _unpack(wa_s[:, 0:D]))
        qp = _pack(q_raw)
        hg = mm(after_packed(xq), _unpack(wa_s[:, 2 * D:3 * D]))
        hu = mm(after_packed(xq), _unpack(wa_s[:, D:2 * D]))

        def make_g(hg, pace_src, span):
            gg = _gelu2(hg)
            if span:
                gg = jnp.concatenate([paced(pace_src, span, gg[:, 0:LANES]), gg[:, LANES:]], axis=1)
            g_new = _ln(gg, 4.0 * EPS)
            store_g(gn_s, HALO, g_new)
            store_g(g_s, HALO + TQ, jnp.where(ia == 0, 0.0, g_new[0:HALO, :]))

        if GREL < 0:
            make_g(hg, hu, MGP)
        u_old = u_s[0]
        if UREL < 0:
            u_s[0] = _gelu2(hu)
        nxt = jnp.minimum(step + NQ, N - 1)
        xv = x_s[pl.ds(pl.multiple_of(nxt * TQ, 16), TQ), :].astype(F32)
        if MLP:
            xv = jnp.concatenate([paced(q_raw, MLP, xv[:, 0:LANES]), xv[:, LANES:]], axis=1)
        if LREL < 0:
            xn = _pack(_ln(xv, EPS))
        mx = None
        mx_prev = None
        acc = None
        vt_s[...] = tail_keys(bb).astype(F32)
        l_acc = jnp.exp2(s_s[NKV - 1, :, NFULL * LANES:(NFULL + 1) * LANES] - m_old)
        p_tail = l_acc
        parts = []
        s_hist = []
        for j in range(NKV):
            m_use = m_old
            if EREL == 0 and mx_prev is not None:
                m_use = jnp.where(never, mx_prev, m_use)
            elif EREL == 1 and j >= 1:
                m_use = paced(o, min(ESPAN, o.shape[1] // LANES), m_old)
            elif EREL == 2 and j >= 2:
                m_use = paced(s_hist[j - 2], ESPAN, m_old)
            elif EREL == 3 and j >= 1:
                m_use = paced(s_hist[j - 1], ESPAN, m_old)
            if j == 0 and E0:
                m_use = paced((q_raw, hg, hu)[E0 - 1], ESPAN, m_old)
            if j == 1 and EREL == 2 and E1:
                m_use = paced((q_raw, hg, hu, o)[E1 - 1], ESPAN, m_old)
            nt = NFULL if j == NKV - 1 else CPK
            tiles, l_new = probs(j, m_use, raw=True, ntiles=nt)
            l_acc = l_acc + l_new
            tiles[0] = jnp.where(never2, l_acc, tiles[0])
            o = mm(after_tiles(tiles), keys_rows(bb, j * TK, nt * LANES))
            acc = o if acc is None else acc + o
            if j == LREL:
                xn = _pack(_ln(jnp.concatenate([paced(o, LSPAN, xv[:, 0:LANES]), xv[:, LANES:]], axis=1), EPS))
            if j == GREL:
                hg = jnp.concatenate([jnp.where(never, a, b) for a, b in zip(split(o), split(hg))], axis=1)
            if j == UREL:
                u_s[0] = _gelu2(jnp.concatenate(
                    [jnp.where(never, a, b) for a, b in zip(split(o), split(hu))], axis=1))
            qj = qp
            if j == UJ:
                udep = u_s[0, pl.ds(pl.multiple_of(z_s[0], 8), 8), 0:LANES]
                qj = jnp.concatenate([qj[:, 0:3 * LANES], tie(never2, pltpu.bitcast(udep, U32), qj[:, 3 * LANES:], 8)], axis=1)
            if j == LNJ:
                qj = jnp.where(never3, xn, qj)
            if j == GJ:
                gdep = gn_s[0, pl.ds(pl.multiple_of(z_s[0] + HALO, 8), 8), :]
                qj = jnp.concatenate([qj[:, 0:LANES], tie(never2, pltpu.bitcast(gdep, U32), qj[:, LANES:2 * LANES], 8), qj[:, 2 * LANES:]], axis=1)
            n = j - TJ0
            if 0 <= n < TQP // LANES:
                kt = tie_bf16(never3, o[0:8, TTC * LANES:(TTC + 1) * LANES], tail_keys(ba))
                parts.append(tail_part(kt, _unpack(qp), n))
            if 0 <= n - 1 < TQP // LANES:
                dep = pltpu.bitcast(parts[n - 1], U32)
                qj = jnp.concatenate([qj[:, 0:2 * LANES], tie(never2, dep, qj[:, 2 * LANES:3 * LANES], TAIL), qj[:, 3 * LANES:]], axis=1)
            mx_prev = mx
            mj = qk_chunk(after_packed(qj), ba, j, j == NKV - 1, tok, parts if parts else None)
            mx = mj if mx is None else jnp.maximum(mx, mj)
            s_hist.append(tok[0])
            if j == GREL:
                make_g(hg, tok[0], MGP)
        yc = u_old * conv_rows(0, TQ, [never, None])
        o_tail = pv_tail(p_tail, never, [])
        l = jnp.sum(l_acc, axis=-1, keepdims=True)
        ya = (acc + o_tail) * (1.0 / l)
        if OUTA:
            out = mm(after_tiles(split(ya)), _unpack(wo_s[0:D // H, :]))
            out = out + mm(after_tiles(split(yc)), _unpack(wo_s[D // H:2 * D // H, :]))
        else:
            out = mm(after_tiles(split(yc)), _unpack(wo_s[D // H:2 * D // H, :]))
            out = out + mm(after_tiles(split(ya)), _unpack(wo_s[0:D // H, :]))
        xr = x_s[pl.ds(pl.multiple_of(sb * TQ, 16), TQ), :].astype(F32)
        o_s[sb % 2] = (xr + out).astype(o_s.dtype)
        store_max(mx)
        dst = pl.multiple_of((nxt // NQ) * (TP // H) + (nxt % NQ) * (TQ // H), 8)
        late = pltpu.bitcast(mx[0:TQ // H, :], U32)
        for c in range(NC):
            xa_s[pl.ds(dst, TQ // H), c * LANES:(c + 1) * LANES] = jnp.where(
                never, late, xn[:, c * LANES:(c + 1) * LANES])

    def last_step():
        sb = N - 1
        bb = B - 1
        uslot = 0
        CPI = LCPI
        NIT = NKV // CPI
        RL = 16 * (TQ // (16 * NIT)) if LFLOOR else 16 * (-(-TQ // (16 * NIT)))
        never = z_s[0] > 0
        never2 = z_s[1] > 0
        for c in range(NC):
            gn_s[c, 0:HALO, :] = jnp.where(NQ == 1, 0.0, g_s[c, TQ:TQ + HALO, :])
        store_g(gn_s, HALO + TQ, jnp.zeros((HALO, D), F32))

        def attend(j0):
            acc = acc_s[...]
            l_acc = l_s[...]
            o = None
            for jj in range(CPI):
                m_use = m_s[...]
                if o is not None and LPACE:
                    m_use = paced_by(never, o, LPACE, m_use)
                tiles, l_new = probs(j0 + jj, m_use, raw=True)
                l_acc = l_acc + l_new
                if jj > 0 or not LNOL:
                    tiles[0] = jnp.where(never2, l_acc, tiles[0])
                if o is not None and LORD:
                    tiles[1] = tie(never, o[:, LANES:2 * LANES], tiles[1], 8)
                o = _dot(jnp.concatenate(tiles, axis=1).astype(BF16), keys(bb, j0 + jj))
                acc = acc + o
            return acc, l_acc

        def loop(t, carry):
            r0 = pl.multiple_of(jnp.minimum(t * RL, TQ - RL), 16)

            def conv_part():
                for c in range(NC):
                    g_s[c, 0:RL + 2 * HALO, :] = gn_s[c, pl.ds(r0, RL + 2 * HALO), :]
                yc = u_s[uslot, pl.ds(r0, RL), :] * conv_rows(0, RL, [never, None], LCG)
                yc_s[pl.ds(pl.multiple_of(r0 // H, 8), RL // H), :] = _pack(yc)

            if LCF:
                conv_part()
            acc, l_acc = attend(t * CPI)
            acc_s[...] = acc
            l_s[...] = l_acc
            if not LCF:
                conv_part()
            return carry

        lax.fori_loop(0, NIT, loop, 0)
        if NIT * RL < TQ:
            r0 = NIT * RL
            for c in range(NC):
                g_s[c, 0:TQ - r0 + 2 * HALO, :] = gn_s[c, r0:TQ + 2 * HALO, :]
            yc_s[r0 // H:TQ // H, :] = _pack(u_s[uslot, r0:TQ, :] * conv_rows(0, TQ - r0, [never, None] if LFC else None, LFC))
        finish(sb)

    first_step()

    def step_fn(step, carry):
        main_step(step)
        out_copy(step - 1).start()

        @pl.when(step >= 2)
        def _():
            out_copy(step - 2).wait()

        return carry

    lax.fori_loop(1, N, step_fn, 0)
    last_step()
    out_copy(N - 2).wait()
    for i, (r0, r1) in enumerate(zip(FIN[:-1], FIN[1:])):
        part_copy(N - 1, r0, r1, osems.at[2 + i]).wait()


@jax.jit
def pallas_standalone__conformer_family_branchformer__speech_kernel(
    x: jax.Array,
    w_q: jax.Array,
    w_k: jax.Array,
    w_v: jax.Array,
    w_ao: jax.Array,
    w_up: jax.Array,
    dw: jax.Array,
    w_dn: jax.Array,
    w_merge: jax.Array,
):
    B, T, D = x.shape
    K = dw.shape[0]
    TQ = 400
    TK = 512
    TP = -(-T // TK) * TK
    NKV = TP // TK
    assert T % TQ == 0 and TQ % 16 == 0 and D % LANES == 0 and K // 2 < HALO
    assert TQ <= TK and B >= 2 and NKV >= 3 and T % 16 == 0
    N = B * (T // TQ)
    x2 = x.reshape(B * T, D)

    kern = functools.partial(_kernel, B=B, T=T, D=D, K=K, TQ=TQ, TK=TK, TP=TP)
    ins = (x2, w_q, w_k, w_v, w_ao, w_up, dw, w_dn, w_merge)
    out = pl.pallas_call(
        kern,
        in_specs=[pl.BlockSpec(memory_space=pl.ANY) for _ in ins],
        out_specs=pl.BlockSpec(memory_space=pl.ANY),
        out_shape=jax.ShapeDtypeStruct((B * T, D), x.dtype),
        scratch_shapes=[pltpu.VMEM(a.shape, a.dtype) for a in ins] + [
            pltpu.SemaphoreType.DMA((13,)),
            pltpu.VMEM((B * TP // 2, D), U32),
            pltpu.VMEM((D // 2, 3 * D), U32),
            pltpu.VMEM((D, D), U32),
            pltpu.VMEM((K, 8, D), F32),
            pltpu.VMEM((NKV, TQ, TK), F32),
            pltpu.VMEM((TQ, LANES), F32),
            pltpu.VMEM((1, TQ, D), F32),
            pltpu.VMEM((D // LANES, TQ + 2 * HALO, LANES), F32),
            pltpu.VMEM((D // LANES, TQ + 2 * HALO, LANES), F32),
            pltpu.VMEM((TQ, D), F32),
            pltpu.VMEM((TQ, LANES), F32),
            pltpu.VMEM((TQ // 2, D), U32),
            pltpu.VMEM((T % LANES, D), F32),
            pltpu.VMEM((2, TQ, D), x.dtype),
            pltpu.SemaphoreType.DMA((5,)),
            pltpu.SMEM((3,), jnp.int32),
        ],
        compiler_params=pltpu.CompilerParams(
            vmem_limit_bytes=100 * 1024 * 1024,
            disable_bounds_checks=True,
            disable_semaphore_checks=True,
        ),
    )(*ins)
    return out.reshape(B, T, D)
```

```python
import functools
import math

import jax
import jax.numpy as jnp
from jax import lax
import jax.experimental.pallas as pl
import jax.experimental.pallas.tpu as pltpu

LANES = 128
EPS = 1e-05
F32 = jnp.float32
BF16 = jnp.bfloat16
U32 = jnp.uint32
NT = (((1,), (1,)), ((), ()))
HALO = 16
H = 2


def _ln(x, eps):
    d = x.shape[-1]
    m = jnp.sum(x, axis=-1, keepdims=True) * (1.0 / d)
    xc = x - m
    v = jnp.sum(xc * xc, axis=-1, keepdims=True) * (1.0 / d)
    return xc * lax.rsqrt(v + eps)


def _gelu2(x):
    c1 = math.sqrt(2.0 / math.pi)
    c2 = c1 * 0.044715
    t = jnp.tanh(x * (c1 + c2 * (x * x)))
    return x + x * t


def _center(w):
    return w - jnp.sum(w, axis=0, keepdims=True) * (1.0 / w.shape[0])


def _pack(x):
    return pltpu.bitcast(x.astype(BF16), U32)


def _unpack(x):
    return pltpu.bitcast(x, BF16)


def _bits(x):
    return pltpu.bitcast(x, U32)


def _dot(a, b):
    return jnp.dot(a, b, preferred_element_type=F32)


def _dot_nt(a, b):
    return lax.dot_general(a, b, NT, preferred_element_type=F32)


def _split(v):
    return [v[:, c * LANES:(c + 1) * LANES] for c in range(v.shape[1] // LANES)]


def _aligned(i, n):
    return i if isinstance(i, int) else pl.multiple_of(i, n)


def _tie(flag, dep, val, n):
    if n == val.shape[0]:
        return jnp.where(flag, dep[0:n], val)
    return jnp.concatenate([jnp.where(flag, dep[0:n], val[0:n]), val[n:]], axis=0)


def _tie_bf16(flag, dep, val):
    head = _bits(val[0:16, 0:LANES])
    head = _unpack(jnp.where(flag, _bits(dep), head))
    top = jnp.concatenate([head, val[0:16, LANES:]], axis=1)
    return jnp.concatenate([top, val[16:, :]], axis=0)


def _paced(flag, src, span, val):
    rows = val.shape[0]
    rel = jnp.concatenate(
        [src[(r * span) % rows:(r * span) % rows + 8,
             ((r * span) // rows) * LANES:((r * span) // rows + 1) * LANES]
         for r in range(0, rows, 8)], axis=0)
    return jnp.concatenate([jnp.where(flag, rel, val[:, 0:LANES]), val[:, LANES:]], axis=1)


def _kernel(x_hbm, wq_hbm, wk_hbm, wv_hbm, wao_hbm, wup_hbm, dw_hbm, wdn_hbm, wm_hbm,
            o_hbm,
            x_s, wq_s, wk_s, wv_s, wao_s, wup_s, dw_s, wdn_s, wm_s, sems,
            xa_s, wa_s, wo_s, dwb_s, s_s, m_s, u_s, g_s, gn_s, acc_s, l_s, yc_s, vt_s, o_s, osems, z_s,
            *, B, T, D, K, TQ, TK, TP, FIN):
    NQ = T // TQ
    N = B * NQ
    NKV = TP // TK
    NC = D // LANES
    CPK = TK // LANES
    PAD = K // 2
    NQT = -(-TQ // LANES)
    NFULL = (T - (NKV - 1) * TK) // LANES
    TAIL = T % LANES

    def out_copy(blk):
        return pltpu.make_async_copy(o_s.at[blk % 2], o_hbm.at[pl.ds(_aligned(blk * TQ, 16), TQ), :],
                                     osems.at[blk % 2])

    def part_copy(blk, i):
        r0, r1 = FIN[i], FIN[i + 1]
        return pltpu.make_async_copy(o_s.at[blk % 2, pl.ds(r0, r1 - r0), :],
                                     o_hbm.at[pl.ds(blk * TQ + r0, r1 - r0), :], osems.at[2 + i])

    def keys(b, r0, n):
        return _unpack(xa_s[pl.ds(_aligned(b * (TP // H) + r0 // H, 8), n // H), :])

    def tail_keys(b):
        return keys(b, T - TAIL, TAIL)

    def tail_part(kt, q, n):
        qn = q[n * LANES:min((n + 1) * LANES, TQ), :]
        if qn.shape[0] < LANES:
            qn = jnp.concatenate([qn, jnp.zeros((LANES - qn.shape[0], D), BF16)], axis=0)
        return _dot_nt(kt, qn)

    def tail_tile(parts):
        fill = jnp.full((LANES - TAIL, LANES), -jnp.inf, F32)
        return jnp.concatenate([jnp.concatenate([p, fill], axis=0).T for p in parts], axis=0)[0:TQ, :]

    def qk_chunk(q, b, j, parts=None):
        last = j == NKV - 1
        s = _dot_nt(q, keys(b, j * TK, (NFULL if last else CPK) * LANES))
        mx = None
        for c in range(CPK):
            st = tail_tile(parts) if last and c == NFULL else s[:, c * LANES:(c + 1) * LANES]
            s_s[j, :, c * LANES:(c + 1) * LANES] = st
            mx = st if mx is None else jnp.maximum(mx, st)
        return s, mx

    def probs(j, m, ntiles):
        tiles = []
        lsum = None
        for c in range(ntiles):
            p = jnp.exp2(s_s[j, :, c * LANES:(c + 1) * LANES] - m)
            lsum = p if lsum is None else lsum + p
            tiles.append(p)
        return tiles, lsum

    def store_g(ref, row, g):
        for c in range(NC):
            ref[c, row:row + g.shape[0], :] = g[:, c * LANES:(c + 1) * LANES]

    def conv_rows(R, G, flag):
        prev = None
        rows = []
        for rr in range(0, R, G):
            cols = []
            for c in range(NC):
                acc = None
                for k in range(K):
                    gv = g_s[c, pl.ds(rr + HALO - PAD + k, G), :].reshape(G // 8, 8, LANES)
                    term = gv * dwb_s[k, :, c * LANES:(c + 1) * LANES][None]
                    if acc is None:
                        acc = term if prev is None else jnp.where(flag, prev, term)
                    else:
                        acc = acc + term
                prev = acc
                cols.append(acc.reshape(G, LANES))
            rows.append(jnp.concatenate(cols, axis=1))
        return jnp.concatenate(rows, axis=0)

    def pv_tail(pt, flag):
        lag = 5
        done = []
        rows = []
        for r in range(0, TQ, 8):
            pr = pt[r:r + 8, :]
            if len(done) >= lag:
                pr = jnp.where(flag, done[-lag], pr)
            pb = [jnp.broadcast_to(pr[:, k:k + 1], (8, LANES)) for k in range(TAIL)]
            cols = []
            for c in range(NC):
                acc = None
                for k in range(TAIL):
                    term = pb[k] * vt_s[k:k + 1, c * LANES:(c + 1) * LANES]
                    if acc is None and done:
                        term = jnp.where(flag, done[-1], term)
                    acc = term if acc is None else acc + term
                done.append(acc)
                cols.append(acc)
            rows.append(jnp.concatenate(cols, axis=1))
        return jnp.concatenate(rows, axis=0)

    def store_max(mx):
        m_s[...] = jnp.broadcast_to(jnp.max(mx, axis=-1, keepdims=True), (TQ, LANES))

    def first_step():
        C2 = NKV // 2

        def xrows(r0, r1):
            return x_hbm.at[pl.ds(r0, r1 - r0), :], x_s.at[pl.ds(r0, r1 - r0), :]

        copies = {}
        plan = (
            ('wq', wq_hbm, wq_s), ('wk', wk_hbm, wk_s),
            ('xa',) + xrows(0, TK), ('xb',) + xrows(TK, C2 * TK), ('xc',) + xrows(C2 * TK, T),
            ('wup', wup_hbm, wup_s), ('dw', dw_hbm, dw_s), ('xd',) + xrows(T, T + TQ),
            ('wv', wv_hbm, wv_s), ('wao', wao_hbm, wao_s), ('wdn', wdn_hbm, wdn_s), ('wm', wm_hbm, wm_s),
            ('xe',) + xrows(T + TQ, B * T),
        )
        for i, (name, src, dst) in enumerate(plan):
            copies[name] = pltpu.make_async_copy(src, dst, sems.at[i])
            copies[name].start()

        z_s[0] = 0
        z_s[1] = 0
        z_s[2] = 0
        for b in range(B):
            xa_s[(b * TP + T) // H:(b + 1) * TP // H, :] = jnp.zeros(((TP - T) // H, D), U32)
        store_g(g_s, TQ, jnp.zeros((HALO, D), F32))
        acc_s[...] = jnp.zeros((TQ, D), F32)
        l_s[...] = jnp.zeros((TQ, LANES), F32)

        def ln_chunk(c):
            r0, r1 = c * TK, min((c + 1) * TK, T)
            xa_s[r0 // H:r1 // H, :] = _pack(_ln(x_s[r0:r1, :].astype(F32), EPS))

        scale = float(D) ** (-0.5) * math.log2(math.e)
        DS = D // 2
        copies['wq'].wait()
        copies['wk'].wait()
        m_lo = _dot_nt(wq_s[...], wk_s[0:DS, :])

        never = z_s[0] > 0
        zero = pl.multiple_of(z_s[0], 8)
        copies['xa'].wait()
        wa_s[:, 0:DS] = _pack(_center(m_lo) * scale)
        wa_s[:, DS:D] = _pack(_center(_dot_nt(wq_s[...], wk_s[DS:D, :])) * scale)
        ln_chunk(0)
        q = _dot(_unpack(xa_s[0:TQ // H, :]), _unpack(wa_s[:, 0:D])).astype(BF16)

        copies['xb'].wait()
        mx = qk_chunk(q, 0, 0)[1]
        for c in range(1, C2):
            ln_chunk(c)
            mx = jnp.maximum(mx, qk_chunk(q, 0, c)[1])

        for name in ('xc', 'wup', 'dw'):
            copies[name].wait()
        xq = _unpack(xa_s[0:TQ // H, :])
        hg = _dot(xq, wup_s[:, D:2 * D])
        hu = _dot(_tie_bf16(never, hg[0:8, LANES:2 * LANES], xq), wup_s[:, 0:D])
        store_g(gn_s, HALO, _ln(_paced(never, hu, 3, _gelu2(hg)), 4.0 * EPS))
        u_s[...] = _gelu2(hu)
        wa_s[:, D:3 * D] = _pack(wup_s[...])
        dwf = dw_s[...].astype(F32)
        for k in range(K):
            dwb_s[k] = jnp.broadcast_to(dwf[k:k + 1, :], (8, D))
        deps = {C2: hu[0:8, LANES:2 * LANES],
                C2 + 1: gn_s[0, pl.ds(zero + HALO, 8), :],
                C2 + 3: u_s[pl.ds(zero, 8), 0:LANES]}
        parts = None
        for c in range(C2, NKV):
            ln_chunk(c)
            qc = _tie_bf16(never, deps[c], q) if c in deps else q
            if c == NKV - 1:
                kt = tail_keys(0)
                parts = [tail_part(kt, q, n) for n in range(NQT)]
            mx = jnp.maximum(mx, qk_chunk(qc, 0, c, parts)[1])

        for name in ('xd', 'wv', 'wao', 'wdn', 'wm'):
            copies[name].wait()
        store_max(mx)
        prev = None
        for r in range(0, TQ, 48):
            n = min(48, TQ - r)
            xv = x_s[T + r:T + r + n, :].astype(F32)
            if prev is not None:
                xv = jnp.concatenate([jnp.where(never, prev[0:n], xv[:, 0:LANES]), xv[:, LANES:]], axis=1)
            y = _ln(xv, EPS)
            xa_s[(TP + r) // H:(TP + r + n) // H, :] = _pack(y)
            prev = y[:, 0:LANES]
        wva_raw = _dot(wv_s[...], wao_s[...])
        wdm = _dot(_tie_bf16(never, wva_raw[0:8, 0:LANES], wdn_s[...]), wm_s[D:2 * D, :])
        mean = jnp.broadcast_to(jnp.sum(wva_raw, axis=0, keepdims=True) * (1.0 / D), (8, D))
        rows = []
        for r in range(0, D, 64):
            tok = wdm[3 * r % D:3 * r % D + 8, (3 * r // D) * LANES:(3 * r // D + 1) * LANES]
            mu = jnp.where(never, jnp.concatenate([tok] * NC, axis=1), mean)
            rows.append((wva_raw[r:r + 64].reshape(8, 8, D) - mu[None]).reshape(64, D))
        wva = jnp.concatenate(rows, axis=0).astype(BF16)
        wo_s[D // H:2 * D // H, :] = _pack(0.5 * wdm)
        lhs = _tie_bf16(never, xa_s[pl.ds(zero, 8), 0:LANES], wva)
        lhs = jnp.concatenate([lhs[0:16], _tie_bf16(never, wdm[0:8, LANES:2 * LANES], lhs[16:])], axis=0)
        wo_s[0:D // H, :] = _pack(_dot(lhs, wm_s[0:D, :]))
        copies['xe'].wait()

    def main_step(step):
        ba = step // NQ
        ia = step % NQ
        sb = step - 1
        bb = sb // NQ
        seq_start = sb % NQ == 0
        for c in range(NC):
            g_s[c, 0:HALO, :] = jnp.where(seq_start, 0.0, g_s[c, TQ:TQ + HALO, :])
            g_s[c, HALO:HALO + TQ, :] = gn_s[c, HALO:HALO + TQ, :]
        never = z_s[0] > 0
        never2 = z_s[1] > 0
        never3 = z_s[2] > 0

        def after_packed(prev, lhs):
            head = _tie(never3, _bits(prev[:, 0:LANES]), lhs[:, 0:LANES], 8)
            return _unpack(jnp.concatenate([head, lhs[:, LANES:]], axis=1))

        def after_tiles(prev, tiles):
            tiles = list(tiles)
            tiles[1] = _tie(never3, prev[:, 0:LANES], tiles[1], 8)
            return jnp.concatenate(tiles, axis=1).astype(BF16)

        m_old = m_s[...]
        xq = xa_s[pl.ds(pl.multiple_of(ba * (TP // H) + ia * (TQ // H), 8), TQ // H), :]
        q_raw = _dot(_unpack(xq), _unpack(wa_s[:, 0:D]))
        qp = _pack(q_raw)
        hg = _dot(after_packed(q_raw, xq), _unpack(wa_s[:, 2 * D:3 * D]))
        hu = _dot(after_packed(hg, xq), _unpack(wa_s[:, D:2 * D]))
        g_new = _ln(_paced(never, hu, 3, _gelu2(hg)), 4.0 * EPS)
        store_g(gn_s, HALO, g_new)
        store_g(g_s, HALO + TQ, jnp.where(ia == 0, 0.0, g_new[0:HALO, :]))
        u_old = u_s[...]
        nxt = jnp.minimum(step + NQ, N - 1)
        xv = x_s[pl.ds(pl.multiple_of(nxt * TQ, 16), TQ), :].astype(F32)
        xn = _pack(_ln(_paced(never, q_raw, 2, xv), EPS))
        vt_s[...] = tail_keys(bb).astype(F32)
        p_tail = jnp.exp2(s_s[NKV - 1, :, NFULL * LANES:(NFULL + 1) * LANES] - m_old)
        l_acc = p_tail
        prev = hu
        mx = None
        mx_prev = None
        acc = None
        parts = []
        for j in range(NKV):
            m_use = m_old if mx_prev is None else jnp.where(never, mx_prev, m_old)
            nt = NFULL if j == NKV - 1 else CPK
            tiles, l_new = probs(j, m_use, nt)
            l_acc = l_acc + l_new
            tiles[0] = jnp.where(never2, l_acc, tiles[0])
            o = _dot(after_tiles(prev, tiles), keys(bb, j * TK, nt * LANES))
            acc = o if acc is None else acc + o
            if j == 4:
                u_s[...] = _gelu2(jnp.concatenate(
                    [jnp.where(never, a, b) for a, b in zip(_split(o), _split(hu))], axis=1))
            qj = qp
            if j == 1:
                qj = jnp.where(never3, xn, qj)
            if j == 3:
                gdep = gn_s[0, pl.ds(pl.multiple_of(z_s[0] + HALO, 8), 8), :]
                qj = jnp.concatenate([qj[:, 0:LANES], _tie(never2, _bits(gdep), qj[:, LANES:2 * LANES], 8),
                                      qj[:, 2 * LANES:]], axis=1)
            if j < NQT:
                kt = _tie_bf16(never3, o[0:8, 2 * LANES:3 * LANES], tail_keys(ba))
                parts.append(tail_part(kt, _unpack(qp), j))
            if 1 <= j <= NQT:
                qj = jnp.concatenate([qj[:, 0:2 * LANES],
                                      _tie(never2, _bits(parts[j - 1]), qj[:, 2 * LANES:3 * LANES], TAIL),
                                      qj[:, 3 * LANES:]], axis=1)
            mx_prev = mx
            prev, mj = qk_chunk(after_packed(o, qj), ba, j, parts)
            mx = mj if mx is None else jnp.maximum(mx, mj)
        yc = u_old * conv_rows(TQ, 16, never)
        o_tail = pv_tail(p_tail, never)
        l = jnp.sum(l_acc, axis=-1, keepdims=True)
        ya = (acc + o_tail) * (1.0 / l)
        out = _dot(after_tiles(prev, _split(ya)), _unpack(wo_s[0:D // H, :]))
        out = out + _dot(after_tiles(out, _split(yc)), _unpack(wo_s[D // H:2 * D // H, :]))
        xr = x_s[pl.ds(pl.multiple_of(sb * TQ, 16), TQ), :].astype(F32)
        o_s[sb % 2] = (xr + out).astype(o_s.dtype)
        store_max(mx)
        dst = pl.multiple_of((nxt // NQ) * (TP // H) + (nxt % NQ) * (TQ // H), 8)
        late = _bits(mx[0:TQ // H, :])
        for c in range(NC):
            xa_s[pl.ds(dst, TQ // H), c * LANES:(c + 1) * LANES] = jnp.where(
                never, late, xn[:, c * LANES:(c + 1) * LANES])

    def last_step():
        bb = B - 1
        CPI = 2
        NIT = NKV // CPI
        RL = 16 * (TQ // (16 * NIT))
        never = z_s[0] > 0
        never2 = z_s[1] > 0
        for c in range(NC):
            gn_s[c, 0:HALO, :] = jnp.where(NQ == 1, 0.0, g_s[c, TQ:TQ + HALO, :])
        store_g(gn_s, HALO + TQ, jnp.zeros((HALO, D), F32))

        def loop(t, carry):
            r0 = pl.multiple_of(jnp.minimum(t * RL, TQ - RL), 16)
            for c in range(NC):
                g_s[c, 0:RL + 2 * HALO, :] = gn_s[c, pl.ds(r0, RL + 2 * HALO), :]
            yc = u_s[pl.ds(r0, RL), :] * conv_rows(RL, 8, never)
            yc_s[pl.ds(pl.multiple_of(r0 // H, 8), RL // H), :] = _pack(yc)
            acc = acc_s[...]
            l_acc = l_s[...]
            o = None
            for jj in range(CPI):
                j = t * CPI + jj
                tiles, l_new = probs(j, m_s[...], CPK)
                l_acc = l_acc + l_new
                tiles[0] = jnp.where(never2, l_acc, tiles[0])
                if o is not None:
                    tiles[1] = _tie(never, o[:, LANES:2 * LANES], tiles[1], 8)
                kj = xa_s[pl.ds(pl.multiple_of(bb * (TP // H) + j * (TK // H), 8), TK // H), :]
                o = _dot(jnp.concatenate(tiles, axis=1).astype(BF16), _unpack(kj))
                acc = acc + o
            acc_s[...] = acc
            l_s[...] = l_acc
            return carry

        lax.fori_loop(0, NIT, loop, 0)
        r0 = NIT * RL
        for c in range(NC):
            g_s[c, 0:TQ - r0 + 2 * HALO, :] = gn_s[c, r0:TQ + 2 * HALO, :]
        yc_s[r0 // H:TQ // H, :] = _pack(u_s[r0:TQ, :] * conv_rows(TQ - r0, 16, never))
        never = z_s[0] > 0
        for i in range(len(FIN) - 1):
            r0, r1 = FIN[i], FIN[i + 1]
            l = jnp.sum(l_s[r0:r1, :], axis=-1, keepdims=True)
            ya = (acc_s[r0:r1, :] * (1.0 / l)).astype(BF16)
            out = _dot(_unpack(yc_s[r0 // H:r1 // H, :]), _unpack(wo_s[D // H:2 * D // H, :]))
            out = out + _dot(_tie_bf16(never, out[0:8, 0:LANES], ya), _unpack(wo_s[0:D // H, :]))
            xr = x_s[(N - 1) * TQ + r0:(N - 1) * TQ + r1, :].astype(F32)
            o_s[(N - 1) % 2, r0:r1, :] = (xr + out).astype(o_s.dtype)
            part_copy(N - 1, i).start()

    first_step()

    def step_fn(step, carry):
        main_step(step)
        out_copy(step - 1).start()

        @pl.when(step >= 2)
        def _():
            out_copy(step - 2).wait()

        return carry

    lax.fori_loop(1, N, step_fn, 0)
    last_step()
    out_copy(N - 2).wait()
    for i in range(len(FIN) - 1):
        part_copy(N - 1, i).wait()


@jax.jit
def pallas_standalone__conformer_family_branchformer__speech_kernel(
    x: jax.Array,
    w_q: jax.Array,
    w_k: jax.Array,
    w_v: jax.Array,
    w_ao: jax.Array,
    w_up: jax.Array,
    dw: jax.Array,
    w_dn: jax.Array,
    w_merge: jax.Array,
):
    B, T, D = x.shape
    K = dw.shape[0]
    TQ = 400
    TK = 512
    FIN = (0, 256, 352, TQ)
    TP = -(-T // TK) * TK
    NKV = TP // TK
    assert B >= 2 and T % TQ == 0 and D == TK and K // 2 < HALO
    assert NKV == 8 and T % LANES in (16, 32, 48, 64) and TP - T < LANES
    x2 = x.reshape(B * T, D)

    kern = functools.partial(_kernel, B=B, T=T, D=D, K=K, TQ=TQ, TK=TK, TP=TP, FIN=FIN)
    ins = (x2, w_q, w_k, w_v, w_ao, w_up, dw, w_dn, w_merge)
    out = pl.pallas_call(
        kern,
        in_specs=[pl.BlockSpec(memory_space=pl.ANY) for _ in ins],
        out_specs=pl.BlockSpec(memory_space=pl.ANY),
        out_shape=jax.ShapeDtypeStruct((B * T, D), x.dtype),
        scratch_shapes=[pltpu.VMEM(a.shape, a.dtype) for a in ins] + [
            pltpu.SemaphoreType.DMA((13,)),
            pltpu.VMEM((B * TP // H, D), U32),
            pltpu.VMEM((D // H, 3 * D), U32),
            pltpu.VMEM((2 * D // H, D), U32),
            pltpu.VMEM((K, 8, D), F32),
            pltpu.VMEM((NKV, TQ, TK), F32),
            pltpu.VMEM((TQ, LANES), F32),
            pltpu.VMEM((TQ, D), F32),
            pltpu.VMEM((D // LANES, TQ + 2 * HALO, LANES), F32),
            pltpu.VMEM((D // LANES, TQ + 2 * HALO, LANES), F32),
            pltpu.VMEM((TQ, D), F32),
            pltpu.VMEM((TQ, LANES), F32),
            pltpu.VMEM((TQ // H, D), U32),
            pltpu.VMEM((T % LANES, D), F32),
            pltpu.VMEM((2, TQ, D), x.dtype),
            pltpu.SemaphoreType.DMA((1 + len(FIN),)),
            pltpu.SMEM((3,), jnp.int32),
        ],
        compiler_params=pltpu.CompilerParams(
            vmem_limit_bytes=100 * 1024 * 1024,
            disable_bounds_checks=True,
            disable_semaphore_checks=True,
        ),
    )(*ins)
    return out.reshape(B, T, D)
```

```python
import functools
import math

import jax
import jax.numpy as jnp
from jax import lax
import jax.experimental.pallas as pl
import jax.experimental.pallas.tpu as pltpu

LANES = 128
EPS = 1e-05
F32 = jnp.float32
BF16 = jnp.bfloat16
U32 = jnp.uint32
NT = (((1,), (1,)), ((), ()))
HALO = 16
H = 2


def _ln(x, eps):
    d = x.shape[-1]
    m = jnp.sum(x, axis=-1, keepdims=True) * (1.0 / d)
    xc = x - m
    v = jnp.sum(xc * xc, axis=-1, keepdims=True) * (1.0 / d)
    return xc * lax.rsqrt(v + eps)


def _gelu2(x):
    c1 = math.sqrt(2.0 / math.pi)
    c2 = c1 * 0.044715
    t = jnp.tanh(x * (c1 + c2 * (x * x)))
    return x + x * t


def _center(w):
    return w - jnp.sum(w, axis=0, keepdims=True) * (1.0 / w.shape[0])


def _pack(x):
    return pltpu.bitcast(x.astype(BF16), U32)


def _unpack(x):
    return pltpu.bitcast(x, BF16)


def _bits(x):
    return pltpu.bitcast(x, U32)


def _dot(a, b):
    return jnp.dot(a, b, preferred_element_type=F32)


def _dot_nt(a, b):
    return lax.dot_general(a, b, NT, preferred_element_type=F32)


def _split(v):
    return [v[:, c * LANES:(c + 1) * LANES] for c in range(v.shape[1] // LANES)]


def _aligned(i, n):
    return i if isinstance(i, int) else pl.multiple_of(i, n)


def _tie(flag, dep, val, n):
    if n == val.shape[0]:
        return jnp.where(flag, dep[0:n], val)
    return jnp.concatenate([jnp.where(flag, dep[0:n], val[0:n]), val[n:]], axis=0)


def _tie_bf16(flag, dep, val):
    head = _bits(val[0:16, 0:LANES])
    head = _unpack(jnp.where(flag, _bits(dep), head))
    top = jnp.concatenate([head, val[0:16, LANES:]], axis=1)
    return jnp.concatenate([top, val[16:, :]], axis=0)


def _tie_vregs(flag, deps, val, row, col):
    cast = _bits if val.dtype == U32 else (lambda v: v if v.dtype == F32 else pltpu.bitcast(v, F32))
    tiles = _split(val)
    t = tiles[col]
    n = 8 * len(deps)
    mid = jnp.where(flag, jnp.concatenate([cast(d) for d in deps], axis=0), t[row:row + n])
    tiles[col] = jnp.concatenate(([t[0:row]] if row else []) + [mid, t[row + n:]], axis=0)
    return jnp.concatenate(tiles, axis=1)


def _to_bf16(v):
    return _unpack(v) if v.dtype == U32 else v.astype(BF16)


def _paced(flag, src, span, val):
    rows = val.shape[0]
    rel = jnp.concatenate(
        [src[(r * span) % rows:(r * span) % rows + 8,
             ((r * span) // rows) * LANES:((r * span) // rows + 1) * LANES]
         for r in range(0, rows, 8)], axis=0)
    return jnp.concatenate([jnp.where(flag, rel, val[:, 0:LANES]), val[:, LANES:]], axis=1)


def _tokens(results):
    out = []
    for s in results:
        ncol = s.shape[1] // LANES
        step = 2 if ncol == 2 else 1
        out += [s[r:r + 8, c * LANES:(c + 1) * LANES] for c in range(0, ncol, step) for r in range(0, s.shape[0], 8)]
    return out


def _released(flag, toks, first, total, val, ntiles=1):
    n = val.shape[0] // 8
    rel = jnp.concatenate([toks[min(first + (i * total) // n, len(toks) - 1)] for i in range(n)], axis=0)
    tiles = _split(val)
    return jnp.concatenate([jnp.where(flag, rel, t) if c < ntiles else t for c, t in enumerate(tiles)], axis=1)


def _kernel(x_hbm, wq_hbm, wk_hbm, wv_hbm, wao_hbm, wup_hbm, dw_hbm, wdn_hbm, wm_hbm,
            o_hbm,
            x_s, wq_s, wk_s, wv_s, wao_s, wup_s, dw_s, wdn_s, wm_s, sems,
            xa_s, wa_s, wo_s, dwb_s, s_s, m_s, u_s, g_s, gn_s, acc_s, l_s, yc_s, vt_s, o_s, osems, tb_s, sx_s, st_s, ssems, wt_s, pl_s, z_s,
            *, B, T, D, K, TQ, TK, TP, FIN):
    NQ = T // TQ
    N = B * NQ
    NKV = TP // TK
    NC = D // LANES
    CPK = TK // LANES
    PAD = K // 2
    NQT = -(-TQ // LANES)
    NFULL = (T - (NKV - 1) * TK) // LANES
    TAIL = T % LANES

    def out_copy(blk):
        return pltpu.make_async_copy(o_s.at[blk % 2], o_hbm.at[pl.ds(_aligned(blk * TQ, 16), TQ), :],
                                     osems.at[blk % 2])

    def part_copy(blk, i):
        r0, r1 = FIN[i], FIN[i + 1]
        return pltpu.make_async_copy(o_s.at[blk % 2, pl.ds(r0, r1 - r0), :],
                                     o_hbm.at[pl.ds(blk * TQ + r0, r1 - r0), :], osems.at[2 + i])

    def keys(b, r0, n):
        return _unpack(xa_s[pl.ds(_aligned(b * (TP // H) + r0 // H, 8), n // H), :])

    def tail_keys(b):
        return keys(b, T - TAIL, TAIL)

    DH = D // 2
    HR = 16 * (-(-TQ // 32))
    R2 = TQ - HR

    def key_tables(y):
        ev = jnp.concatenate([y[t * LANES:(t + 1) * LANES] for t in range(0, CPK, 2)], axis=0)
        od = jnp.concatenate([y[t * LANES:(t + 1) * LANES] for t in range(1, CPK, 2)], axis=0)
        e1, e2, o1, o2 = ev[:, 0:DH], ev[:, DH:], od[:, 0:DH], od[:, DH:]
        return [_pack(v) for v in (e1 + o2, o1 - o2, e2 - e1, e1 + o1, e2 + o2)]

    def row_operands(a, reused=False):
        a11, a12, a21, a22 = a[0:HR, 0:DH], a[0:HR, DH:], a[R2:TQ, 0:DH], a[R2:TQ, DH:]
        return {i: _pack(v) if reused else v
                for i, v in ((1, a11 + a22), (2, a21 + a22), (3, a11), (4, a22),
                             (5, a11 + a12), (6, a21 - a11), (7, a12 - a22))}

    ORDER = (4, 2, 1, 5, 3, 7, 6)

    def weight_tables(mat, w):
        b11, b12, b21, b22 = w[0:DH, 0:DH], w[0:DH, DH:], w[DH:, 0:DH], w[DH:, DH:]
        for i, v in enumerate((b11 + b22, b11, b12 - b22, b21 - b11, b22, b11 + b12, b21 + b22)):
            wt_s[mat, i] = _pack(v)

    def combine(m):
        return {(0, 0): (m[1] + m[4] - m[5]) + m[7], (0, 1): m[3] + m[5],
                (1, 0): m[2] + m[4], (1, 1): (m[1] - m[2] + m[3]) + m[6]}

    def stack(top, bottom):
        return jnp.concatenate([top, bottom[HR - R2:]], axis=0)

    def project(lhs_list, mats, gate):
        m = {}
        for i in ORDER:
            l = jnp.concatenate([lhs[i] for lhs in lhs_list], axis=1)
            m[i] = gate(i, l, lambda v, i=i: _dot(v, _unpack(jnp.concatenate([wt_s[k, i - 1] for k in mats], axis=0))))
        c = combine(m)
        return jnp.concatenate([stack(c[0, 0], c[1, 0]), stack(c[0, 1], c[1, 1])], axis=1)

    def key_operand(b, j, npair, i):
        if i in (2, 5):
            base = _aligned(b * (TP // H) + j * TK // H, 8)
            parity, lo = (0, 0) if i == 2 else (1, DH)
            return _unpack(jnp.concatenate(
                [xa_s[pl.ds(base + (2 * p + parity) * LANES // H, LANES // H), lo:lo + DH] for p in range(npair)],
                axis=0))
        return _unpack(tb_s[b * NKV + j, {1: 0, 3: 1, 4: 2, 6: 3, 7: 4}[i], 0:npair * LANES // H, :])

    def pv_products(tiles, b, j, gate, pend):
        npair = len(tiles) // 2
        ev = jnp.concatenate(tiles[0:2 * npair:2], axis=1)
        od = jnp.concatenate(tiles[1:2 * npair:2], axis=1)
        a11, a12, a21, a22 = ev[0:HR], od[0:HR], ev[R2:TQ], od[R2:TQ]
        ops = {1: (a11 + a22, 1), 2: (a11, 7), 3: (a21 - a22, 2), 4: (a12 - a11, 5),
               5: (a22, 6), 6: (a11 + a21, 4), 7: (a12 + a22, 3)}
        n = {}
        if 0:
            w = npair * LANES
            for i in PVORD:
                pl_s[j % 2, i - 1, :, 0:w] = _pack(ops[i][0])
            if 0 == 1:
                pend.append(pl_s[z_s[0], 0, 0:8, 0:LANES])
            ops = {i: (pl_s[j % 2, i - 1, :, 0:w], ops[i][1]) for i in ops}
        for i in PVORD:
            l, k = ops[i]
            n[i] = gate(i, l, lambda v, k=k: _dot(v, key_operand(b, j, npair, k)),
                        2 if npair == 1 and n else 1)
        return n

    PVORD = (2, 5, 1, 3, 4, 6, 7)

    def qk_chunk2(lhs, q, b, j, gate, parts=None):
        last = j == NKV - 1
        last = last and 1
        npair = (NFULL if last else CPK) // 2
        m = {}
        for i in ORDER:
            m[i] = gate(i, lhs[i], lambda l, i=i: _dot_nt(l, key_operand(b, j, npair, i)), 2 if last and m else 1)
        c = combine(m)
        mx = None
        for t in range(CPK):
            if t < 2 * npair:
                cols = slice((t // 2) * LANES, (t // 2 + 1) * LANES)
                st = stack(c[0, t % 2][:, cols], c[1, t % 2][:, cols])
                if j == NKV - 1 and t == NFULL:
                    st = jnp.where(lax.broadcasted_iota(jnp.int32, st.shape, 1) < TAIL, st, -jnp.inf)
            elif t < NFULL:
                st = gate(0, q, lambda l: _dot_nt(l, keys(b, j * TK + t * LANES, LANES)))
            else:
                st = tail_tile(parts)
            s_s[j, :, t * LANES:(t + 1) * LANES] = st
            mx = st if mx is None else jnp.maximum(mx, st)
        return mx

    def stage_copies(blk, slot):
        row = _aligned(blk * (TK // H), 8)
        return (pltpu.make_async_copy(sx_s.at[slot], xa_s.at[pl.ds(row, TK // H), :], ssems.at[0, slot]),
                pltpu.make_async_copy(st_s.at[slot], tb_s.at[blk], ssems.at[1, slot]))

    def tail_part(kt, q, n):
        qn = q[n * LANES:min((n + 1) * LANES, TQ), :]
        if qn.shape[0] < LANES:
            qn = jnp.concatenate([qn, jnp.zeros((LANES - qn.shape[0], D), BF16)], axis=0)
        return _dot_nt(kt, qn)

    def tail_tile(parts):
        fill = jnp.full((LANES - TAIL, LANES), -jnp.inf, F32)
        return jnp.concatenate([jnp.concatenate([p, fill], axis=0).T for p in parts], axis=0)[0:TQ, :]

    def qk_chunk(q, b, j, parts=None):
        last = j == NKV - 1
        s = _dot_nt(q, keys(b, j * TK, (NFULL if last else CPK) * LANES))
        mx = None
        for c in range(CPK):
            st = tail_tile(parts) if last and c == NFULL else s[:, c * LANES:(c + 1) * LANES]
            s_s[j, :, c * LANES:(c + 1) * LANES] = st
            mx = st if mx is None else jnp.maximum(mx, st)
        return s, mx

    def probs(j, m, ntiles):
        tiles = []
        lsum = None
        for c in range(ntiles):
            p = jnp.exp2(s_s[j, :, c * LANES:(c + 1) * LANES] - m)
            lsum = p if lsum is None else lsum + p
            tiles.append(p)
        return tiles, lsum

    def store_g(ref, row, g):
        for c in range(NC):
            ref[c, row:row + g.shape[0], :] = g[:, c * LANES:(c + 1) * LANES]

    def conv_rows(R, G, flag, prev=None, split2=False):
        rows = []
        for rr in range(0, R, G):
            cols = []
            for c in range(NC):
                acc = None
                acc2 = None
                for k in range(K):
                    gv = g_s[c, pl.ds(rr + HALO - PAD + k, G), :].reshape(G // 8, 8, LANES)
                    term = gv * dwb_s[k, :, c * LANES:(c + 1) * LANES][None]
                    if acc is None:
                        acc = term if prev is None else jnp.where(flag, prev, term)
                    elif split2 and k % 2 == 1:
                        acc2 = term if acc2 is None else acc2 + term
                    else:
                        acc = acc + term
                if acc2 is not None:
                    acc = acc + acc2
                prev = acc
                cols.append(acc.reshape(G, LANES))
            rows.append(jnp.concatenate(cols, axis=1))
        return jnp.concatenate(rows, axis=0)

    def pv_tail(pt, flag, start=None):
        lag, PG, PW = 5, 8, 1
        done = [] if start is None else [jnp.concatenate([start] * (PG // 8), axis=0)] * max(lag, PW)
        rows = []
        for r in range(0, TQ, PG):
            pr = pt[r:r + PG, :]
            if len(done) >= lag:
                pr = jnp.where(flag, done[-lag], pr)
            KG = 16
            cols = [None] * NC
            for k0 in range(0, TAIL, KG):
                if k0 and len(done) >= lag:
                    pr = jnp.where(flag, done[-lag], pt[r:r + PG, :])
                pb = [jnp.broadcast_to(pr[:, k:k + 1], (PG, LANES)) for k in range(k0, k0 + KG)]
                for c in range(NC):
                    acc = cols[c]
                    for k in range(k0, k0 + KG):
                        term = pb[k - k0] * vt_s[k:k + 1, c * LANES:(c + 1) * LANES]
                        if k == k0 and len(done) >= PW:
                            term = jnp.where(flag, done[-PW], term)
                        acc = term if acc is None else acc + term
                    done.append(acc)
                    cols[c] = acc
            rows.append(jnp.concatenate(cols, axis=1))
        return jnp.concatenate(rows, axis=0)

    def store_max(mx):
        m = jnp.max(mx, axis=-1, keepdims=True)
        if 1:
            m = m + jnp.log2(jnp.sum(jnp.exp2(mx - m), axis=-1, keepdims=True))
        m_s[...] = jnp.broadcast_to(m, (TQ, LANES))

    def first_step():
        C2 = NKV // 2

        def xrows(b, r0, r1):
            return x_hbm.at[pl.ds(b * T + r0, r1 - r0), :], x_s.at[pl.ds(b * TP + r0, r1 - r0), :]

        copies = {}
        plan = (
            ('wq', wq_hbm, wq_s), ('wk', wk_hbm, wk_s),
            ('xa',) + xrows(0, 0, TK), ('xb',) + xrows(0, TK, C2 * TK), ('xc',) + xrows(0, C2 * TK, T),
            ('wup', wup_hbm, wup_s), ('dw', dw_hbm, dw_s), ('xd',) + xrows(1, 0, TK),
            ('wv', wv_hbm, wv_s), ('wao', wao_hbm, wao_s), ('wdn', wdn_hbm, wdn_s), ('wm', wm_hbm, wm_s),
            ('xe1',) + xrows(1, TK, T),
        ) + tuple(('xe%d' % b,) + xrows(b, 0, T) for b in range(2, B))
        for i, (name, src, dst) in enumerate(plan):
            copies[name] = pltpu.make_async_copy(src, dst, sems.at[i])
            copies[name].start()

        z_s[0] = 0
        z_s[1] = 0
        z_s[2] = 0
        for b in range(B):
            x_s[b * TP + T:(b + 1) * TP, :] = jnp.zeros((TP - T, D), x_s.dtype)
        store_g(g_s, TQ, jnp.zeros((HALO, D), F32))
        acc_s[...] = jnp.zeros((TQ, D), F32)
        l_s[...] = jnp.zeros((TQ, LANES), F32)

        def ln_chunk(c, t=None, span=100):
            xv = x_s[c * TK:(c + 1) * TK, :].astype(F32)
            if t is not None:
                xv = _released(never, t, 0, len(t) * span // 100, xv)
            y = _ln(xv, EPS)
            xa_s[c * TK // H:(c + 1) * TK // H, :] = _pack(y)
            for i, tbl in enumerate(key_tables(y)):
                tb_s[c, i] = tbl

        scale = float(D) ** (-0.5) * math.log2(math.e)
        DS = D // 2
        FL = 0
        copies['wq'].wait()
        copies['wk'].wait()
        m_lo = _dot_nt(wq_s[...], wk_s[0:DS, :])

        never = z_s[0] > 0
        zero = pl.multiple_of(z_s[0], 8)
        hist = []
        pend = []

        def gate(i, l, run, lag=1):
            if len(hist) >= lag:
                l = _tie_vregs(never, [hist[-lag][0:8, 0:LANES]], l, 0, 0)
            if pend:
                l = _tie_vregs(never, pend, l, 8, 0)
                del pend[:]
            hist.append(run(_to_bf16(l)))
            return hist[-1]

        copies['xa'].wait()
        wa_s[:, 0:DS] = _pack(_center(m_lo) * scale)
        wa_s[:, DS:D] = _pack(_center(_dot_nt(wq_s[...], wk_s[DS:D, :])) * scale)
        ln_chunk(0)
        q_raw = _dot(_unpack(xa_s[0:TQ // H, :]), _unpack(wa_s[:, 0:D]))
        qp = _pack(q_raw)
        q = _unpack(qp)

        copies['xb'].wait()
        FS = 8
        if FS < NKV:
            lhs = row_operands(q_raw, True)
            lhs[3] = qp[0:HR // H, 0:DH]
            lhs[4] = qp[R2 // H:TQ // H, DH:]

        def qk(c, parts=None):
            n0 = len(hist)
            if c >= FS:
                mj = qk_chunk2(lhs, qp, 0, c, gate, parts)
            else:
                res = []
                gate(0, qp, lambda v: res.append(qk_chunk(v, 0, c, parts)) or res[0][0])
                mj = res[0][1]
            return mj, _tokens(hist[n0:]) if FL else None

        mx, t = qk(0)
        for c in range(1, C2):
            ln_chunk(c, t, FL)
            mj, t = qk(c)
            mx = jnp.maximum(mx, mj)

        for name in ('xc', 'wup', 'dw'):
            copies[name].wait()
        del hist[:]
        xq = xa_s[0:TQ // H, :]
        hg = gate(0, xq, lambda v: _dot(v, wup_s[:, D:2 * D]))
        hu = gate(0, xq, lambda v: _dot(v, wup_s[:, 0:D]))
        dwf = dw_s[...].astype(F32)
        for k in range(K):
            dwb_s[k] = jnp.broadcast_to(dwf[k:k + 1, :], (8, D))
        parts = None
        for c in range(C2, NKV):
            ln_chunk(c, (_tokens(hist) if 0 else None) if c == C2 else t, 0 if c == C2 else FL)
            if c == NKV - 1 and 1:
                kt = tail_keys(0)
                parts = [tail_part(kt, q, n) for n in range(NQT)]
            mj, t = qk(c, parts)
            mx = jnp.maximum(mx, mj)

        for name in ('xd', 'wv', 'wao', 'wdn', 'wm'):
            copies[name].wait()
        store_max(mx)
        wva_raw = _dot(wv_s[...], wao_s[...])
        t1 = _tokens([wva_raw])
        wdm = _dot(_tie_bf16(never, wva_raw[0:8, 0:LANES], wdn_s[...]), wm_s[D:2 * D, :])
        t2 = _tokens([wdm])
        t12 = t1 + t2
        n12 = len(t12)

        def rel(v, lo, hi, nt=NC):
            return _released(never, t12, n12 * lo // 100, n12 * (hi - lo) // 100, v, nt)

        store_g(gn_s, HALO, _ln(_gelu2(rel(hg, 0, 30)), 4.0 * EPS))
        u_s[...] = _gelu2(rel(hu, 30, 60))
        y = _ln(rel(x_s[TP:TP + TK, :].astype(F32), 0, 50, 1), EPS)
        xa_s[TP // H:(TP + TK) // H, :] = _pack(y)
        for i, tbl in enumerate(key_tables(y)):
            tb_s[NKV, i] = tbl
        weight_tables(0, rel(_unpack(wa_s[:, 0:D]).astype(F32), 50, 65))
        weight_tables(1, rel(wup_s[:, D:2 * D].astype(F32), 65, 80))
        weight_tables(2, rel(wup_s[:, 0:D].astype(F32), 80, 95))
        mean = jnp.sum(wva_raw, axis=0, keepdims=True) * (1.0 / D)
        wva = (_released(never, t2, 0, len(t2) * 3 // 4, wva_raw, NC) - mean).astype(BF16)
        wo_s[D // H:2 * D // H, :] = _pack(0.5 * wdm)
        deps = [wdm[0:8, LANES:2 * LANES], xa_s[pl.ds(zero, 8), 0:LANES], tb_s[NKV + z_s[0], 4, 0:8, 0:LANES],
                gn_s[0, pl.ds(zero + HALO, 8), :], u_s[pl.ds(zero, 8), 0:LANES]]
        if 1:
            deps.append(wt_s[z_s[0], 0, 0:8, 0:LANES])
        for i, dep in enumerate(deps):
            wva = jnp.concatenate(([wva[0:16 * i]] if i else []) + [_tie_bf16(never, dep, wva[16 * i:])], axis=0)
        wvom = _dot(wva, wm_s[0:D, :])
        t3 = _tokens([wvom])
        weight_tables(4, _released(never, t3, 0, len(t3) // 2, 0.5 * wdm, NC))
        wo_s[0:D // H, :] = _pack(wvom)
        weight_tables(3, wvom)
        for b in range(1, B):
            copies['xe%d' % b].wait()

    def next_chunk(step):
        return jnp.minimum(step // NQ + 1, B - 1) * NKV + jnp.minimum(step % NQ, NKV - 1)

    def has_next(step):
        return jnp.logical_and(step // NQ + 1 < B, step % NQ < NKV)

    def main_step(step):
        ba = step // NQ
        ia = step % NQ
        sb = step - 1
        bb = sb // NQ
        seq_start = sb % NQ == 0
        for c in range(NC):
            g_s[c, 0:HALO, :] = jnp.where(seq_start, 0.0, g_s[c, TQ:TQ + HALO, :])
            g_s[c, HALO:HALO + TQ, :] = gn_s[c, HALO:HALO + TQ, :]
        never = z_s[0] > 0
        never2 = z_s[1] > 0
        never3 = z_s[2] > 0

        hist = []
        pend = []

        def gate(i, l, run, lag=1):
            if hist and (1 == 1 or i in (0, ORDER[0], PVORD[0]) or lag > 1):
                l = _tie_vregs(never3, [hist[-lag][0:8, 0:LANES]], l, 0, 0)
            if pend:
                l = _tie_vregs(never3, pend, l, 8, 0)
                del pend[:]
            hist.append(run(_to_bf16(l)))
            return hist[-1]

        def toks(i0, i1=None):
            return _tokens(hist[i0:i1])

        m_old = m_s[...]
        xq = xa_s[pl.ds(pl.multiple_of(ba * (TP // H) + ia * (TQ // H), 8), TQ // H), :]
        if 1:
            xops = row_operands(_unpack(xq).astype(F32), True)
            xops[3] = xq[0:HR // H, 0:DH]
            xops[4] = xq[R2 // H:TQ // H, DH:]
            q_raw = project([xops], [0], gate)
            hg = project([xops], [1], gate)
            n_u = len(hist)
            hu = project([xops], [2], gate)
        else:
            q_raw = gate(0, xq, lambda v: _dot(v, _unpack(wa_s[:, 0:D])))
            hg = gate(0, xq, lambda v: _dot(v, _unpack(wa_s[:, 2 * D:3 * D])))
            n_u = len(hist)
            hu = gate(0, xq, lambda v: _dot(v, _unpack(wa_s[:, D:2 * D])))
        qp = _pack(q_raw)
        q = _unpack(qp)
        ptok = toks(0)
        NP = len(ptok)
        def make_g(rel1, rel2):
            gg = _gelu2(hg if rel1 is None else _released(never, rel1, 0, len(rel1), hg, NC))
            if rel2 is not None:
                gg = _released(never, rel2, 0, len(rel2) * 75 // 100, gg)
            g_new = _ln(gg, 4.0 * EPS)
            store_g(gn_s, HALO, g_new)
            store_g(g_s, HALO + TQ, jnp.where(ia == 0, 0.0, g_new[0:HALO, :]))

        def make_next(t, first, total):
            slot = step % 2
            xv = x_s[pl.ds(pl.multiple_of(next_chunk(step) * TK, 16), TK), :].astype(F32)
            if total:
                xv = _released(never, t, len(t) * first // 100, len(t) * total // 100, xv)
            y = _ln(xv, EPS)
            sx_s[slot] = _pack(y)
            for i, tbl in enumerate(key_tables(y)):
                st_s[slot, i] = tbl

        if 1 < 0:
            make_g(None, toks(n_u) if 75 else None)
        u_old = u_s[...]
        if 2 < 0:
            make_next(ptok, 0, 60)
        lhs = row_operands(q_raw, True)
        lhs[3] = qp[0:HR // H, 0:DH]
        lhs[4] = qp[R2 // H:TQ // H, DH:]
        l_acc = None
        if 0:
            vt_s[...] = tail_keys(bb).astype(F32)
            p_tail = jnp.exp2(s_s[NKV - 1, :, NFULL * LANES:(NFULL + 1) * LANES] - m_old)
            l_acc = p_tail
        mx = None
        mx_prev = None
        acc = None
        extra = None
        parts = []
        pv0 = None
        cstart = None
        for j in range(NKV):
            m_use = m_old if mx_prev is None else jnp.where(never, mx_prev, m_old)
            if j == 0 and 0:
                m_use = _released(never, ptok, NP * 50 // 100, NP * 0 // 100, m_old)
            if j >= 1 and 60 and (j == 1 or 60 > 0):
                t = toks(pv0, pv1)
                m_use = _released(never, t, 0, len(t) * abs(60) // 100, m_old)
            nt = NFULL if j == NKV - 1 and 0 else CPK
            tiles, l_new = probs(j, m_use, nt)
            l_acc = l_new if l_acc is None else l_acc + l_new
            tiles[0] = jnp.where(never2, l_acc, tiles[0])
            pv0 = len(hist)
            if 1:
                n = pv_products(tiles, bb, j, gate, pend)
                acc = n if acc is None else {i: acc[i] + n[i] for i in n}
                if nt % 2:
                    extra = gate(0, tiles[nt - 1],
                                 lambda v: _dot(v, keys(bb, j * TK + (nt - 1) * LANES, LANES)))
            else:
                o = gate(0, jnp.concatenate(tiles, axis=1),
                         lambda v: _dot(v, keys(bb, j * TK, nt * LANES)))
                acc = o if acc is None else acc + o
            pv1 = len(hist)
            if j == 3:
                t = toks(pv0)
                u_s[...] = _gelu2(_released(never, t, 0, len(t), hu, NC))
            if j == 7:
                pend += [sx_s[z_s[0], 0:8, 0:LANES], st_s[z_s[0], 0, 0:8, 0:LANES]]
            if j == 6:
                pend.append(gn_s[0, pl.ds(pl.multiple_of(z_s[0] + HALO, 8), 8), :])
            if j < NQT and 1:
                t = toks(pv0)
                kt = _tie_bf16(never3, t[len(t) * 3 // 4], tail_keys(ba))
                parts.append(tail_part(kt, q, j))
            if 1 <= j <= NQT and 1:
                pend += [parts[j - 1][r:r + 8] for r in range(0, TAIL if 1 else 8, 8)]
            mx_prev = mx
            mj = qk_chunk2(lhs, qp, ba, j, gate, parts)
            mx = mj if mx is None else jnp.maximum(mx, mj)
            if j == 2:
                make_next(toks(pv0), 0, 60)
            if j == 1:
                make_g(toks(pv0, pv1), toks(pv1))
            if j == -1:
                cstart = jnp.broadcast_to(toks(pv0)[0][None], (16 // 8, 8, LANES))
        yc = u_old * conv_rows(TQ, 16, never, cstart)
        if 1:
            z = combine(acc)
            acc = jnp.concatenate([stack(z[0, 0], z[0, 1]), stack(z[1, 0], z[1, 1])], axis=1)
            if extra is not None:
                acc = acc + extra
        if 0:
            acc = acc + pv_tail(p_tail, never)
        l = jnp.sum(l_acc, axis=-1, keepdims=True)
        ya = acc * (1.0 / l)
        def staged(ops, slot, lo):
            if not 2:
                return ops
            for i in ORDER:
                pl_s[slot, i - 1, :, lo:lo + DH] = _pack(ops[i])
            if 2 == 1:
                pend.append(pl_s[z_s[0], 0, 0:8, 0:LANES])
            return {i: pl_s[slot, i - 1, :, lo:lo + DH] for i in ops}

        if 2 == 1:
            oc = staged(row_operands(yc), 0, DH)
            out = project([staged(row_operands(ya), 1, DH), oc], [3, 4], gate)
        elif 2 == 2:
            out = project([staged(row_operands(yc), 0, DH)], [4], gate)
            out = out + project([staged(row_operands(ya), 1, DH)], [3], gate)
        else:
            out = gate(0, ya, lambda v: _dot(v, _unpack(wo_s[0:D // H, :])))
            out = out + gate(0, yc, lambda v: _dot(v, _unpack(wo_s[D // H:2 * D // H, :])))
        xr = x_s[pl.ds(pl.multiple_of(bb * TP + (sb % NQ) * TQ, 16), TQ), :].astype(F32)
        o_s[sb % 2] = (xr + out).astype(o_s.dtype)
        store_max(mx)

    def last_step():
        bb = B - 1
        CPI = 2
        NIT = NKV // CPI
        RL = 16 * (TQ // (16 * NIT))
        never = z_s[0] > 0
        never2 = z_s[1] > 0
        for c in range(NC):
            gn_s[c, 0:HALO, :] = jnp.where(NQ == 1, 0.0, g_s[c, TQ:TQ + HALO, :])
        store_g(gn_s, HALO + TQ, jnp.zeros((HALO, D), F32))

        def loop(t, carry):
            r0 = pl.multiple_of(jnp.minimum(t * RL, TQ - RL), 16)
            for c in range(NC):
                g_s[c, 0:RL + 2 * HALO, :] = gn_s[c, pl.ds(r0, RL + 2 * HALO), :]
            yc = u_s[pl.ds(r0, RL), :] * conv_rows(RL, 8, never)
            yc_s[pl.ds(pl.multiple_of(r0 // H, 8), RL // H), :] = _pack(yc)
            acc = acc_s[...]
            l_acc = l_s[...]
            o = None
            for jj in range(CPI):
                j = t * CPI + jj
                tiles, l_new = probs(j, m_s[...], CPK)
                l_acc = l_acc + l_new
                tiles[0] = jnp.where(never2, l_acc, tiles[0])
                if o is not None:
                    tiles[1] = _tie(never, o[:, LANES:2 * LANES], tiles[1], 8)
                kj = xa_s[pl.ds(pl.multiple_of(bb * (TP // H) + j * (TK // H), 8), TK // H), :]
                o = _dot(jnp.concatenate(tiles, axis=1).astype(BF16), _unpack(kj))
                acc = acc + o
            acc_s[...] = acc
            l_s[...] = l_acc
            return carry

        lax.fori_loop(0, NIT, loop, 0)
        r0 = NIT * RL
        for c in range(NC):
            g_s[c, 0:TQ - r0 + 2 * HALO, :] = gn_s[c, r0:TQ + 2 * HALO, :]
        yc_s[r0 // H:TQ // H, :] = _pack(u_s[r0:TQ, :] * conv_rows(TQ - r0, 16, never))
        never = z_s[0] > 0
        for i in range(len(FIN) - 1):
            r0, r1 = FIN[i], FIN[i + 1]
            l = jnp.sum(l_s[r0:r1, :], axis=-1, keepdims=True)
            ya = (acc_s[r0:r1, :] * (1.0 / l)).astype(BF16)
            out = _dot(_unpack(yc_s[r0 // H:r1 // H, :]), _unpack(wo_s[D // H:2 * D // H, :]))
            out = out + _dot(_tie_bf16(never, out[0:8, 0:LANES], ya), _unpack(wo_s[0:D // H, :]))
            xr = x_s[bb * TP + T - TQ + r0:bb * TP + T - TQ + r1, :].astype(F32)
            o_s[(N - 1) % 2, r0:r1, :] = (xr + out).astype(o_s.dtype)
            part_copy(N - 1, i).start()

    first_step()

    def step_fn(step, carry):
        main_step(step)
        out_copy(step - 1).start()

        @pl.when(has_next(step))
        def _():
            for c in stage_copies(next_chunk(step), step % 2):
                c.start()

        @pl.when(step >= 2)
        def _():
            out_copy(step - 2).wait()

        @pl.when(jnp.logical_and(step >= 2, has_next(step - 1)))
        def _():
            for c in stage_copies(next_chunk(step - 1), (step - 1) % 2):
                c.wait()

        return carry

    lax.fori_loop(1, N, step_fn, 0)
    last_step()
    out_copy(N - 2).wait()
    for i in range(len(FIN) - 1):
        part_copy(N - 1, i).wait()


@jax.jit
def pallas_standalone__conformer_family_branchformer__speech_kernel(
    x: jax.Array,
    w_q: jax.Array,
    w_k: jax.Array,
    w_v: jax.Array,
    w_ao: jax.Array,
    w_up: jax.Array,
    dw: jax.Array,
    w_dn: jax.Array,
    w_merge: jax.Array,
):
    B, T, D = x.shape
    K = dw.shape[0]
    TQ = 400
    TK = 512
    FIN = (0, 256, 352, TQ)
    TP = -(-T // TK) * TK
    NKV = TP // TK
    assert B >= 2 and T % TQ == 0 and D == TK and K // 2 < HALO
    assert NKV + 1 < T // TQ and NKV == 8 and T % LANES in (16, 32, 48, 64) and TP - T < LANES
    x2 = x.reshape(B * T, D)

    kern = functools.partial(_kernel, B=B, T=T, D=D, K=K, TQ=TQ, TK=TK, TP=TP, FIN=FIN)
    ins = (x2, w_q, w_k, w_v, w_ao, w_up, dw, w_dn, w_merge)
    out = pl.pallas_call(
        kern,
        in_specs=[pl.BlockSpec(memory_space=pl.ANY) for _ in ins],
        out_specs=pl.BlockSpec(memory_space=pl.ANY),
        out_shape=jax.ShapeDtypeStruct((B * T, D), x.dtype),
        scratch_shapes=[pltpu.VMEM((B * TP, D), x.dtype)] + [pltpu.VMEM(a.shape, a.dtype) for a in ins[1:]] + [
            pltpu.SemaphoreType.DMA((11 + B,)),
            pltpu.VMEM((B * TP // H, D), U32),
            pltpu.VMEM((D // H, D), U32),
            pltpu.VMEM((2 * D // H, D), U32),
            pltpu.VMEM((K, 8, D), F32),
            pltpu.VMEM((NKV, TQ, TK), F32),
            pltpu.VMEM((TQ, LANES), F32),
            pltpu.VMEM((TQ, D), F32),
            pltpu.VMEM((D // LANES, TQ + 2 * HALO, LANES), F32),
            pltpu.VMEM((D // LANES, TQ + 2 * HALO, LANES), F32),
            pltpu.VMEM((TQ, D), F32),
            pltpu.VMEM((TQ, LANES), F32),
            pltpu.VMEM((TQ // H, D), U32),
            pltpu.VMEM((T % LANES, D), F32),
            pltpu.VMEM((2, TQ, D), x.dtype),
            pltpu.SemaphoreType.DMA((1 + len(FIN),)),
            pltpu.VMEM((B * NKV, 5, TK // 2 // H, D // 2), U32),
            pltpu.VMEM((2, TK // H, D), U32),
            pltpu.VMEM((2, 5, TK // 2 // H, D // 2), U32),
            pltpu.SemaphoreType.DMA((2, 2)),
            pltpu.VMEM((5, 7, D // 2 // H, D // 2), U32),
            pltpu.VMEM((2, 7, 16 * (-(-TQ // 32)) // H, D), U32),
            pltpu.SMEM((3,), jnp.int32),
        ],
        compiler_params=pltpu.CompilerParams(
            vmem_limit_bytes=100 * 1024 * 1024,
            disable_bounds_checks=True,
            disable_semaphore_checks=True,
        ),
    )(*ins)
    return out.reshape(B, T, D)
```

```python
import functools
import math

import jax
import jax.numpy as jnp
from jax import lax
import jax.experimental.pallas as pl
import jax.experimental.pallas.tpu as pltpu

LANES = 128
EPS = 1e-05
F32 = jnp.float32
BF16 = jnp.bfloat16
U32 = jnp.uint32
NT = (((1,), (1,)), ((), ()))
HALO = 16
H = 2


def _ln(x, eps):
    d = x.shape[-1]
    m = jnp.sum(x, axis=-1, keepdims=True) * (1.0 / d)
    xc = x - m
    v = jnp.sum(xc * xc, axis=-1, keepdims=True) * (1.0 / d)
    return xc * lax.rsqrt(v + eps)


def _gelu2(x):
    c1 = math.sqrt(2.0 / math.pi)
    c2 = c1 * 0.044715
    t = jnp.tanh(x * (c1 + c2 * (x * x)))
    return x + x * t


def _center(w):
    return w - jnp.sum(w, axis=0, keepdims=True) * (1.0 / w.shape[0])


def _pack(x):
    return pltpu.bitcast(x.astype(BF16), U32)


def _unpack(x):
    return pltpu.bitcast(x, BF16)


def _bits(x):
    return pltpu.bitcast(x, U32)


def _dot(a, b):
    return jnp.dot(a, b, preferred_element_type=F32)


def _dot_nt(a, b):
    return lax.dot_general(a, b, NT, preferred_element_type=F32)


def _split(v):
    return [v[:, c * LANES:(c + 1) * LANES] for c in range(v.shape[1] // LANES)]


def _aligned(i, n):
    return i if isinstance(i, int) else pl.multiple_of(i, n)


def _tie(flag, dep, val, n):
    if n == val.shape[0]:
        return jnp.where(flag, dep[0:n], val)
    return jnp.concatenate([jnp.where(flag, dep[0:n], val[0:n]), val[n:]], axis=0)


def _tie_bf16(flag, dep, val):
    head = _bits(val[0:16, 0:LANES])
    head = _unpack(jnp.where(flag, _bits(dep), head))
    top = jnp.concatenate([head, val[0:16, LANES:]], axis=1)
    return jnp.concatenate([top, val[16:, :]], axis=0)


def _tie_vregs(flag, deps, val, row, col):
    cast = _bits if val.dtype == U32 else (lambda v: v if v.dtype == F32 else pltpu.bitcast(v, F32))
    tiles = _split(val)
    t = tiles[col]
    n = 8 * len(deps)
    mid = jnp.where(flag, jnp.concatenate([cast(d) for d in deps], axis=0), t[row:row + n])
    tiles[col] = jnp.concatenate(([t[0:row]] if row else []) + [mid, t[row + n:]], axis=0)
    return jnp.concatenate(tiles, axis=1)


def _to_bf16(v):
    return _unpack(v) if v.dtype == U32 else v.astype(BF16)


def _paced(flag, src, span, val):
    rows = val.shape[0]
    rel = jnp.concatenate(
        [src[(r * span) % rows:(r * span) % rows + 8,
             ((r * span) // rows) * LANES:((r * span) // rows + 1) * LANES]
         for r in range(0, rows, 8)], axis=0)
    return jnp.concatenate([jnp.where(flag, rel, val[:, 0:LANES]), val[:, LANES:]], axis=1)


def _tokens(results):
    out = []
    for s in results:
        ncol = s.shape[1] // LANES
        step = 2 if ncol == 2 else 1
        out += [s[r:r + 8, c * LANES:(c + 1) * LANES] for c in range(0, ncol, step) for r in range(0, s.shape[0], 8)]
    return out


def _released(flag, toks, first, total, val, ntiles=1):
    n = val.shape[0] // 8
    rel = jnp.concatenate([toks[min(first + (i * total) // n, len(toks) - 1)] for i in range(n)], axis=0)
    if val.dtype == U32:
        rel = _bits(rel)
    tiles = _split(val)
    return jnp.concatenate([jnp.where(flag, rel, t) if c < ntiles else t for c, t in enumerate(tiles)], axis=1)


def _kernel(x_hbm, wq_hbm, wk_hbm, wv_hbm, wao_hbm, wup_hbm, dw_hbm, wdn_hbm, wm_hbm,
            o_hbm,
            x_s, wq_s, wk_s, wv_s, wao_s, wup_s, dw_s, wdn_s, wm_s, sems,
            xa_s, wa_s, wo_s, dwb_s, s_s, m_s, u_s, g_s, gn_s, acc_s, l_s, yc_s, vt_s, o_s, osems, tb_s, sx_s, st_s, wt_s, pl_s, z_s,
            *, B, T, D, K, TQ, TK, TP, FIN):
    NQ = T // TQ
    N = B * NQ
    NKV = TP // TK
    NC = D // LANES
    CPK = TK // LANES
    PAD = K // 2
    NQT = -(-TQ // LANES)
    NFULL = (T - (NKV - 1) * TK) // LANES
    TAIL = T % LANES

    def out_copy(blk):
        return pltpu.make_async_copy(o_s.at[blk % 2], o_hbm.at[pl.ds(_aligned(blk * TQ, 16), TQ), :],
                                     osems.at[blk % 2])

    def part_copy(blk, i):
        r0, r1 = FIN[i], FIN[i + 1]
        return pltpu.make_async_copy(o_s.at[blk % 2, pl.ds(r0, r1 - r0), :],
                                     o_hbm.at[pl.ds(blk * TQ + r0, r1 - r0), :], osems.at[2 + i])

    def keys(b, r0, n):
        return _unpack(xa_s[pl.ds(xrow(b * TP) + r0 // H, n // H), :])

    def tail_keys(b):
        return keys(b, T - TAIL, TAIL)

    DH = D // 2
    HR = 16 * (-(-TQ // 32))
    R2 = TQ - HR

    def key_tables(y):
        ev = jnp.concatenate([y[t * LANES:(t + 1) * LANES] for t in range(0, CPK, 2)], axis=0)
        od = jnp.concatenate([y[t * LANES:(t + 1) * LANES] for t in range(1, CPK, 2)], axis=0)
        e1, e2, o1, o2 = ev[:, 0:DH], ev[:, DH:], od[:, 0:DH], od[:, DH:]
        return [_pack(v) for v in (e1 + o2, o1 - o2, e2 - e1, e1 + o1, e2 + o2)]

    def row_operands(a, reused=False):
        a11, a12, a21, a22 = a[0:HR, 0:DH], a[0:HR, DH:], a[R2:TQ, 0:DH], a[R2:TQ, DH:]
        return {i: _pack(v) if reused else v
                for i, v in ((1, a11 + a22), (2, a21 + a22), (3, a11), (4, a22),
                             (5, a11 + a12), (6, a21 - a11), (7, a12 - a22))}

    ORDER = (4, 2, 1, 5, 3, 7, 6)
    TR = TK // 2 // H
    PX, PT = 0, 0

    def xrow(r):
        return PX + r // H if isinstance(r, int) else pl.multiple_of(z_s[3] + r // H, 8)

    def trow(blk, i):
        return PT + (blk * 5 + i) * TR if isinstance(blk, int) else pl.multiple_of(z_s[4] + (blk * 5 + i) * TR, 8)

    def weight_tables(mat, w):
        b11, b12, b21, b22 = w[0:DH, 0:DH], w[0:DH, DH:], w[DH:, 0:DH], w[DH:, DH:]
        for i, v in enumerate((b11 + b22, b11, b12 - b22, b21 - b11, b22, b11 + b12, b21 + b22)):
            wt_s[mat, i] = _pack(v)

    def combine(m):
        return {(0, 0): (m[1] + m[4] - m[5]) + m[7], (0, 1): m[3] + m[5],
                (1, 0): m[2] + m[4], (1, 1): (m[1] - m[2] + m[3]) + m[6]}

    def stack(top, bottom):
        return jnp.concatenate([top, bottom[HR - R2:]], axis=0)

    def project(lhs_list, mats, gate):
        m = {}
        for i in ORDER:
            l = jnp.concatenate([lhs[i] for lhs in lhs_list], axis=1)
            m[i] = gate(i, l, lambda v, i=i: _dot(v, _unpack(jnp.concatenate([wt_s[k, i - 1] for k in mats], axis=0))))
        c = combine(m)
        return jnp.concatenate([stack(c[0, 0], c[1, 0]), stack(c[0, 1], c[1, 1])], axis=1)

    def key_operand(b, j, npair, i):
        if i in (2, 5):
            base = xrow(b * TP) + j * TK // H
            parity, lo = (0, 0) if i == 2 else (1, DH)
            return _unpack(jnp.concatenate(
                [xa_s[pl.ds(base + (2 * p + parity) * LANES // H, LANES // H), lo:lo + DH] for p in range(npair)],
                axis=0))
        return _unpack(tb_s[pl.ds(trow(b * NKV, 0) + (j * 5 + {1: 0, 3: 1, 4: 2, 6: 3, 7: 4}[i]) * TR, npair * LANES // H), :])

    def pv_products(tiles, b, j, gate, pend):
        npair = len(tiles) // 2
        ev = jnp.concatenate(tiles[0:2 * npair:2], axis=1)
        od = jnp.concatenate(tiles[1:2 * npair:2], axis=1)
        a11, a12, a21, a22 = ev[0:HR], od[0:HR], ev[R2:TQ], od[R2:TQ]
        ops = {1: (a11 + a22, 1), 2: (a11, 7), 3: (a21 - a22, 2), 4: (a12 - a11, 5),
               5: (a22, 6), 6: (a11 + a21, 4), 7: (a12 + a22, 3)}
        n = {}
        if 0:
            w = npair * LANES
            for i in PVORD:
                pl_s[j % 2, i - 1, :, 0:w] = _pack(ops[i][0])
            if 0 == 1:
                pend.append(pl_s[z_s[0], 0, 0:8, 0:LANES])
            ops = {i: (pl_s[j % 2, i - 1, :, 0:w], ops[i][1]) for i in ops}
        for i in PVORD:
            l, k = ops[i]
            n[i] = gate(i, l, lambda v, k=k: _dot(v, key_operand(b, j, npair, k)),
                        2 if npair == 1 and n else 1)
        return n

    PVORD = (2, 5, 1, 3, 4, 6, 7)

    def qk_chunk2(lhs, q, b, j, gate, parts=None):
        last = j == NKV - 1
        last = last and 1
        npair = (NFULL if last else CPK) // 2
        m = {}
        for i in ORDER:
            m[i] = gate(i, lhs[i], lambda l, i=i: _dot_nt(l, key_operand(b, j, npair, i)), 2 if last and m else 1)
        c = combine(m)
        mx = None
        for t in range(CPK):
            if t < 2 * npair:
                cols = slice((t // 2) * LANES, (t // 2 + 1) * LANES)
                st = stack(c[0, t % 2][:, cols], c[1, t % 2][:, cols])
                if j == NKV - 1 and t == NFULL:
                    st = jnp.where(lax.broadcasted_iota(jnp.int32, st.shape, 1) < TAIL, st, -jnp.inf)
            elif t < NFULL:
                st = gate(0, q, lambda l: _dot_nt(l, keys(b, j * TK + t * LANES, LANES)))
            else:
                st = tail_tile(parts)
            s_s[j, :, t * LANES:(t + 1) * LANES] = st
            mx = st if mx is None else jnp.maximum(mx, st)
        return mx

    def tail_part(kt, q, n):
        qn = q[n * LANES:min((n + 1) * LANES, TQ), :]
        if qn.shape[0] < LANES:
            qn = jnp.concatenate([qn, jnp.zeros((LANES - qn.shape[0], D), BF16)], axis=0)
        return _dot_nt(kt, qn)

    def tail_tile(parts):
        fill = jnp.full((LANES - TAIL, LANES), -jnp.inf, F32)
        return jnp.concatenate([jnp.concatenate([p, fill], axis=0).T for p in parts], axis=0)[0:TQ, :]

    def qk_chunk(q, b, j, parts=None):
        last = j == NKV - 1
        s = _dot_nt(q, keys(b, j * TK, (NFULL if last else CPK) * LANES))
        mx = None
        for c in range(CPK):
            st = tail_tile(parts) if last and c == NFULL else s[:, c * LANES:(c + 1) * LANES]
            s_s[j, :, c * LANES:(c + 1) * LANES] = st
            mx = st if mx is None else jnp.maximum(mx, st)
        return s, mx

    def probs(j, m, ntiles):
        tiles = []
        lsum = None
        for c in range(ntiles):
            p = jnp.exp2(s_s[j, :, c * LANES:(c + 1) * LANES] - m)
            lsum = p if lsum is None else lsum + p
            tiles.append(p)
        return tiles, lsum

    def store_g(ref, row, g):
        for c in range(NC):
            ref[c, row:row + g.shape[0], :] = g[:, c * LANES:(c + 1) * LANES]

    def conv_rows(R, G, flag, prev=None, split2=False):
        rows = []
        for rr in range(0, R, G):
            cols = []
            for c in range(NC):
                acc = None
                acc2 = None
                for k in range(K):
                    gv = g_s[c, pl.ds(rr + HALO - PAD + k, G), :].reshape(G // 8, 8, LANES)
                    term = gv * dwb_s[k, :, c * LANES:(c + 1) * LANES][None]
                    if acc is None:
                        acc = term if prev is None else jnp.where(flag, prev, term)
                    elif split2 and k % 2 == 1:
                        acc2 = term if acc2 is None else acc2 + term
                    else:
                        acc = acc + term
                if acc2 is not None:
                    acc = acc + acc2
                prev = acc
                cols.append(acc.reshape(G, LANES))
            rows.append(jnp.concatenate(cols, axis=1))
        return jnp.concatenate(rows, axis=0)

    def pv_tail(pt, flag, start=None):
        lag, PG, PW = 5, 8, 1
        done = [] if start is None else [jnp.concatenate([start] * (PG // 8), axis=0)] * max(lag, PW)
        rows = []
        for r in range(0, TQ, PG):
            pr = pt[r:r + PG, :]
            if len(done) >= lag:
                pr = jnp.where(flag, done[-lag], pr)
            KG = 16
            cols = [None] * NC
            for k0 in range(0, TAIL, KG):
                if k0 and len(done) >= lag:
                    pr = jnp.where(flag, done[-lag], pt[r:r + PG, :])
                pb = [jnp.broadcast_to(pr[:, k:k + 1], (PG, LANES)) for k in range(k0, k0 + KG)]
                for c in range(NC):
                    acc = cols[c]
                    for k in range(k0, k0 + KG):
                        term = pb[k - k0] * vt_s[k:k + 1, c * LANES:(c + 1) * LANES]
                        if k == k0 and len(done) >= PW:
                            term = jnp.where(flag, done[-PW], term)
                        acc = term if acc is None else acc + term
                    done.append(acc)
                    cols[c] = acc
            rows.append(jnp.concatenate(cols, axis=1))
        return jnp.concatenate(rows, axis=0)

    def store_max(mx):
        m = jnp.max(mx, axis=-1, keepdims=True)
        if 1:
            m = m + jnp.log2(jnp.sum(jnp.exp2(mx - m), axis=-1, keepdims=True))
        m_s[...] = jnp.broadcast_to(m, (TQ, LANES))

    def first_step():
        C2 = NKV // 2

        def xrows(b, r0, r1):
            return x_hbm.at[pl.ds(b * T + r0, r1 - r0), :], x_s.at[pl.ds(b * TP + r0, r1 - r0), :]

        copies = {}
        plan = (
            ('wq', wq_hbm, wq_s), ('wk', wk_hbm, wk_s),
            ('xa',) + xrows(0, 0, TK), ('xb',) + xrows(0, TK, C2 * TK), ('xc',) + xrows(0, C2 * TK, T),
            ('wup', wup_hbm, wup_s), ('dw', dw_hbm, dw_s), ('xd',) + xrows(1, 0, TK),
            ('wv', wv_hbm, wv_s), ('wao', wao_hbm, wao_s), ('wdn', wdn_hbm, wdn_s), ('wm', wm_hbm, wm_s),
            ('xe1',) + xrows(1, TK, T),
        ) + tuple(('xe%d' % b,) + xrows(b, 0, T) for b in range(2, B))
        for i, (name, src, dst) in enumerate(plan):
            copies[name] = pltpu.make_async_copy(src, dst, sems.at[i])
            copies[name].start()

        z_s[0] = 0
        z_s[1] = 0
        z_s[2] = 0
        z_s[3] = PX
        z_s[4] = PT
        for b in range(B):
            x_s[b * TP + T:(b + 1) * TP, :] = jnp.zeros((TP - T, D), x_s.dtype)
        store_g(g_s, TQ, jnp.zeros((HALO, D), F32))
        acc_s[...] = jnp.zeros((TQ, D), F32)
        l_s[...] = jnp.zeros((TQ, LANES), F32)

        def ln_chunk(c, t=None, span=100):
            xv = x_s[c * TK:(c + 1) * TK, :].astype(F32)
            if t is not None:
                xv = _released(never, t, 0, len(t) * span // 100, xv)
            y = _ln(xv, EPS)
            xa_s[pl.ds(xrow(c * TK), TK // H), :] = _pack(y)
            for i, tbl in enumerate(key_tables(y)):
                tb_s[pl.ds(trow(c, i), TR), :] = tbl

        scale = float(D) ** (-0.5) * math.log2(math.e)
        DS = D // 2
        FL = 0
        copies['wq'].wait()
        copies['wk'].wait()
        m_lo = _dot_nt(wq_s[...], wk_s[0:DS, :])

        never = z_s[0] > 0
        zero = pl.multiple_of(z_s[0], 8)
        hist = []
        pend = []

        def gate(i, l, run, lag=1):
            if len(hist) >= lag:
                l = _tie_vregs(never, [hist[-lag][0:8, 0:LANES]], l, 0, 0)
            if pend:
                l = _tie_vregs(never, pend, l, 8, 0)
                del pend[:]
            hist.append(run(_to_bf16(l)))
            return hist[-1]

        copies['xa'].wait()
        wa_s[:, 0:DS] = _pack(_center(m_lo) * scale)
        wa_s[:, DS:D] = _pack(_center(_dot_nt(wq_s[...], wk_s[DS:D, :])) * scale)
        ln_chunk(0)
        q_raw = _dot(keys(0, 0, TQ), _unpack(wa_s[:, 0:D]))
        qp = _pack(q_raw)
        q = _unpack(qp)

        copies['xb'].wait()
        FS = 8
        if FS < NKV:
            lhs = row_operands(q_raw, True)
            lhs[3] = qp[0:HR // H, 0:DH]
            lhs[4] = qp[R2 // H:TQ // H, DH:]

        def qk(c, parts=None):
            n0 = len(hist)
            if c >= FS:
                mj = qk_chunk2(lhs, qp, 0, c, gate, parts)
            else:
                res = []
                gate(0, qp, lambda v: res.append(qk_chunk(v, 0, c, parts)) or res[0][0])
                mj = res[0][1]
            return mj, _tokens(hist[n0:]) if FL else None

        mx, t = qk(0)
        for c in range(1, C2):
            ln_chunk(c, t, FL)
            mj, t = qk(c)
            mx = jnp.maximum(mx, mj)

        for name in ('xc', 'wup', 'dw'):
            copies[name].wait()
        del hist[:]
        xq = xa_s[pl.ds(xrow(0), TQ // H), :]
        hg = gate(0, xq, lambda v: _dot(v, wup_s[:, D:2 * D]))
        hu = gate(0, xq, lambda v: _dot(v, wup_s[:, 0:D]))
        dwf = dw_s[...].astype(F32)
        for k in range(K):
            dwb_s[k] = jnp.broadcast_to(dwf[k:k + 1, :], (8, D))
        parts = None
        for c in range(C2, NKV):
            ln_chunk(c, (_tokens(hist) if 0 else None) if c == C2 else t, 0 if c == C2 else FL)
            if c == NKV - 1 and 1:
                kt = tail_keys(0)
                parts = [tail_part(kt, q, n) for n in range(NQT)]
            mj, t = qk(c, parts)
            mx = jnp.maximum(mx, mj)

        for name in ('xd', 'wv', 'wao', 'wdn', 'wm'):
            copies[name].wait()
        store_max(mx)
        wva_raw = _dot(wv_s[...], wao_s[...])
        t1 = _tokens([wva_raw])
        wdm = _dot(_tie_bf16(never, wva_raw[0:8, 0:LANES], wdn_s[...]), wm_s[D:2 * D, :])
        t2 = _tokens([wdm])
        t12 = t1 + t2
        n12 = len(t12)

        def rel(v, lo, hi, nt=NC):
            return _released(never, t12, n12 * lo // 100, n12 * (hi - lo) // 100, v, nt)

        store_g(gn_s, HALO, _ln(_gelu2(rel(hg, 0, 30)), 4.0 * EPS))
        u_s[...] = _gelu2(rel(hu, 30, 60))
        y = _ln(rel(x_s[TP:TP + TK, :].astype(F32), 0, 50, 1), EPS)
        sx_s[...] = _pack(y)
        for i, tbl in enumerate(key_tables(y)):
            st_s[i * TR:(i + 1) * TR, :] = tbl
        weight_tables(0, rel(_unpack(wa_s[:, 0:D]).astype(F32), 50, 65))
        weight_tables(1, rel(wup_s[:, D:2 * D].astype(F32), 65, 80))
        weight_tables(2, rel(wup_s[:, 0:D].astype(F32), 80, 95))
        mean = jnp.sum(wva_raw, axis=0, keepdims=True) * (1.0 / D)
        wva = (_released(never, t2, 0, len(t2) * 3 // 4, wva_raw, NC) - mean).astype(BF16)
        wo_s[D // H:2 * D // H, :] = _pack(0.5 * wdm)
        deps = [wdm[0:8, LANES:2 * LANES], sx_s[pl.ds(zero, 8), 0:LANES], st_s[pl.ds(zero, 8), 0:LANES],
                gn_s[0, pl.ds(zero + HALO, 8), :], u_s[pl.ds(zero, 8), 0:LANES]]
        if 1:
            deps.append(wt_s[z_s[0], 0, 0:8, 0:LANES])
        for i, dep in enumerate(deps):
            wva = jnp.concatenate(([wva[0:16 * i]] if i else []) + [_tie_bf16(never, dep, wva[16 * i:])], axis=0)
        wvom = _dot(wva, wm_s[0:D, :])
        t3 = _tokens([wvom])
        weight_tables(4, _released(never, t3, 0, len(t3) // 2, 0.5 * wdm, NC))
        wo_s[0:D // H, :] = _pack(wvom)
        weight_tables(3, wvom)
        for b in range(1, B):
            copies['xe%d' % b].wait()

    def next_chunk(step):
        return jnp.minimum(step // NQ + 1, B - 1) * NKV + jnp.minimum(step % NQ, NKV - 1)

    def has_next(step):
        return jnp.logical_and(step // NQ + 1 < B, step % NQ < NKV)

    def main_step(step):
        ba = step // NQ
        ia = step % NQ
        sb = step - 1
        bb = sb // NQ
        seq_start = sb % NQ == 0
        for c in range(NC):
            g_s[c, 0:HALO, :] = jnp.where(seq_start, 0.0, g_s[c, TQ:TQ + HALO, :])
            g_s[c, HALO:HALO + TQ, :] = gn_s[c, HALO:HALO + TQ, :]
        never = z_s[0] > 0
        never2 = z_s[1] > 0
        never3 = z_s[2] > 0

        hist = []
        pend = []

        def gate(i, l, run, lag=1):
            if hist and (1 == 1 or i in (0, ORDER[0], PVORD[0]) or lag > 1):
                l = _tie_vregs(never3, [hist[-lag][0:8, 0:LANES]], l, 0, 0)
            if pend:
                l = _tie_vregs(never3, pend, l, 8, 0)
                del pend[:]
            hist.append(run(_to_bf16(l)))
            return hist[-1]

        def toks(i0, i1=None):
            return _tokens(hist[i0:i1])

        m_old = m_s[...]
        xq = xa_s[pl.ds(xrow(ba * TP + ia * TQ), TQ // H), :]
        if 1:
            xops = row_operands(_unpack(xq).astype(F32), True)
            xops[3] = xq[0:HR // H, 0:DH]
            xops[4] = xq[R2 // H:TQ // H, DH:]
            q_raw = project([xops], [0], gate)
            hg = project([xops], [1], gate)
            n_u = len(hist)
            hu = project([xops], [2], gate)
        else:
            q_raw = gate(0, xq, lambda v: _dot(v, _unpack(wa_s[:, 0:D])))
            hg = gate(0, xq, lambda v: _dot(v, _unpack(wa_s[:, 2 * D:3 * D])))
            n_u = len(hist)
            hu = gate(0, xq, lambda v: _dot(v, _unpack(wa_s[:, D:2 * D])))
        qp = _pack(q_raw)
        q = _unpack(qp)
        ptok = toks(0)
        NP = len(ptok)
        dst = jnp.where(has_next(sb), next_chunk(sb), B * NKV)
        i0, i1 = NP * 50 // 100, NP * 90 // 100
        im = i0 + (i1 - i0) * 4 // 9
        xa_s[pl.ds(xrow(dst * TK), TK // H), :] = _released(never, ptok, i0, im - i0, sx_s[...], NC)
        tb_s[pl.ds(trow(dst, 0), 5 * TR), :] = _released(never, ptok, im, i1 - im, st_s[...], 2)
        def make_g(rel1, rel2):
            gg = _gelu2(hg if rel1 is None else _released(never, rel1, 0, len(rel1), hg, NC))
            if rel2 is not None:
                gg = _released(never, rel2, 0, len(rel2) * 75 // 100, gg)
            g_new = _ln(gg, 4.0 * EPS)
            store_g(gn_s, HALO, g_new)
            store_g(g_s, HALO + TQ, jnp.where(ia == 0, 0.0, g_new[0:HALO, :]))

        def make_next(t, first, total):
            xv = x_s[pl.ds(pl.multiple_of(next_chunk(step) * TK, 16), TK), :].astype(F32)
            if total:
                xv = _released(never, t, len(t) * first // 100, len(t) * total // 100, xv)
            y = _ln(xv, EPS)
            sx_s[...] = _pack(y)
            for i, tbl in enumerate(key_tables(y)):
                st_s[i * TR:(i + 1) * TR, :] = tbl

        if 1 < 0:
            make_g(None, toks(n_u) if 75 else None)
        u_old = u_s[...]
        if 2 < 0:
            make_next(ptok, 0, 60)
        lhs = row_operands(q_raw, True)
        lhs[3] = qp[0:HR // H, 0:DH]
        lhs[4] = qp[R2 // H:TQ // H, DH:]
        l_acc = None
        if 0:
            vt_s[...] = tail_keys(bb).astype(F32)
            p_tail = jnp.exp2(s_s[NKV - 1, :, NFULL * LANES:(NFULL + 1) * LANES] - m_old)
            l_acc = p_tail
        mx = None
        mx_prev = None
        acc = None
        extra = None
        parts = []
        pv0 = None
        cstart = None
        for j in range(NKV):
            m_use = m_old if mx_prev is None else jnp.where(never, mx_prev, m_old)
            if j == 0 and 0:
                m_use = _released(never, ptok, NP * 50 // 100, NP * 0 // 100, m_old)
            if j >= 1 and 60 and (j == 1 or 60 > 0):
                t = toks(pv0, pv1)
                m_use = _released(never, t, 0, len(t) * abs(60) // 100, m_old)
            nt = NFULL if j == NKV - 1 and 0 else CPK
            tiles, l_new = probs(j, m_use, nt)
            l_acc = l_new if l_acc is None else l_acc + l_new
            tiles[0] = jnp.where(never2, l_acc, tiles[0])
            pv0 = len(hist)
            if 1:
                n = pv_products(tiles, bb, j, gate, pend)
                acc = n if acc is None else {i: acc[i] + n[i] for i in n}
                if nt % 2:
                    extra = gate(0, tiles[nt - 1],
                                 lambda v: _dot(v, keys(bb, j * TK + (nt - 1) * LANES, LANES)))
            else:
                o = gate(0, jnp.concatenate(tiles, axis=1),
                         lambda v: _dot(v, keys(bb, j * TK, nt * LANES)))
                acc = o if acc is None else acc + o
            pv1 = len(hist)
            if j == 3:
                t = toks(pv0)
                u_s[...] = _gelu2(_released(never, t, 0, len(t), hu, NC))
            if j == 7:
                pend += [sx_s[pl.ds(pl.multiple_of(z_s[0], 8), 8), 0:LANES], st_s[pl.ds(pl.multiple_of(z_s[0], 8), 8), 0:LANES]]
            if j == 6:
                pend.append(gn_s[0, pl.ds(pl.multiple_of(z_s[0] + HALO, 8), 8), :])
            if j < NQT and 1:
                t = toks(pv0)
                kt = _tie_bf16(never3, t[len(t) * 3 // 4], tail_keys(ba))
                parts.append(tail_part(kt, q, j))
            if 1 <= j <= NQT and 1:
                pend += [parts[j - 1][r:r + 8] for r in range(0, TAIL if 1 else 8, 8)]
            mx_prev = mx
            mj = qk_chunk2(lhs, qp, ba, j, gate, parts)
            mx = mj if mx is None else jnp.maximum(mx, mj)
            if j == 2:
                make_next(toks(pv0), 0, 60)
            if j == 1:
                make_g(toks(pv0, pv1), toks(pv1))
            if j == -1:
                cstart = jnp.broadcast_to(toks(pv0)[0][None], (16 // 8, 8, LANES))
        yc = u_old * conv_rows(TQ, 16, never, cstart)
        if 1:
            z = combine(acc)
            acc = jnp.concatenate([stack(z[0, 0], z[0, 1]), stack(z[1, 0], z[1, 1])], axis=1)
            if extra is not None:
                acc = acc + extra
        if 0:
            acc = acc + pv_tail(p_tail, never)
        l = jnp.sum(l_acc, axis=-1, keepdims=True)
        ya = acc * (1.0 / l)
        def staged(ops, slot, lo):
            if not 2:
                return ops
            for i in ORDER:
                pl_s[slot, i - 1, :, lo:lo + DH] = _pack(ops[i])
            if 2 == 1:
                pend.append(pl_s[z_s[0], 0, 0:8, 0:LANES])
            return {i: pl_s[slot, i - 1, :, lo:lo + DH] for i in ops}

        if 2 == 1:
            oc = staged(row_operands(yc), 0, DH)
            out = project([staged(row_operands(ya), 1, DH), oc], [3, 4], gate)
        elif 2 == 2:
            out = project([staged(row_operands(yc), 0, DH)], [4], gate)
            out = out + project([staged(row_operands(ya), 1, DH)], [3], gate)
        else:
            out = gate(0, ya, lambda v: _dot(v, _unpack(wo_s[0:D // H, :])))
            out = out + gate(0, yc, lambda v: _dot(v, _unpack(wo_s[D // H:2 * D // H, :])))
        xr = x_s[pl.ds(pl.multiple_of(bb * TP + (sb % NQ) * TQ, 16), TQ), :].astype(F32)
        o_s[sb % 2] = (xr + out).astype(o_s.dtype)
        store_max(mx)

    def last_step():
        bb = B - 1
        CPI = 2
        NIT = NKV // CPI
        RL = 16 * (TQ // (16 * NIT))
        never = z_s[0] > 0
        never2 = z_s[1] > 0
        for c in range(NC):
            gn_s[c, 0:HALO, :] = jnp.where(NQ == 1, 0.0, g_s[c, TQ:TQ + HALO, :])
        store_g(gn_s, HALO + TQ, jnp.zeros((HALO, D), F32))

        def loop(t, carry):
            r0 = pl.multiple_of(jnp.minimum(t * RL, TQ - RL), 16)
            for c in range(NC):
                g_s[c, 0:RL + 2 * HALO, :] = gn_s[c, pl.ds(r0, RL + 2 * HALO), :]
            yc = u_s[pl.ds(r0, RL), :] * conv_rows(RL, 8, never)
            yc_s[pl.ds(pl.multiple_of(r0 // H, 8), RL // H), :] = _pack(yc)
            acc = acc_s[...]
            l_acc = l_s[...]
            o = None
            for jj in range(CPI):
                j = t * CPI + jj
                tiles, l_new = probs(j, m_s[...], CPK)
                l_acc = l_acc + l_new
                tiles[0] = jnp.where(never2, l_acc, tiles[0])
                if o is not None:
                    tiles[1] = _tie(never, o[:, LANES:2 * LANES], tiles[1], 8)
                kj = xa_s[pl.ds(xrow(bb * TP + j * TK), TK // H), :]
                o = _dot(jnp.concatenate(tiles, axis=1).astype(BF16), _unpack(kj))
                acc = acc + o
            acc_s[...] = acc
            l_s[...] = l_acc
            return carry

        lax.fori_loop(0, NIT, loop, 0)
        r0 = NIT * RL
        for c in range(NC):
            g_s[c, 0:TQ - r0 + 2 * HALO, :] = gn_s[c, r0:TQ + 2 * HALO, :]
        yc_s[r0 // H:TQ // H, :] = _pack(u_s[r0:TQ, :] * conv_rows(TQ - r0, 16, never))
        never = z_s[0] > 0
        for i in range(len(FIN) - 1):
            r0, r1 = FIN[i], FIN[i + 1]
            l = jnp.sum(l_s[r0:r1, :], axis=-1, keepdims=True)
            ya = (acc_s[r0:r1, :] * (1.0 / l)).astype(BF16)
            out = _dot(_unpack(yc_s[r0 // H:r1 // H, :]), _unpack(wo_s[D // H:2 * D // H, :]))
            out = out + _dot(_tie_bf16(never, out[0:8, 0:LANES], ya), _unpack(wo_s[0:D // H, :]))
            xr = x_s[bb * TP + T - TQ + r0:bb * TP + T - TQ + r1, :].astype(F32)
            o_s[(N - 1) % 2, r0:r1, :] = (xr + out).astype(o_s.dtype)
            part_copy(N - 1, i).start()

    first_step()

    def step_fn(step, carry):
        main_step(step)
        out_copy(step - 1).start()

        @pl.when(step >= 2)
        def _():
            out_copy(step - 2).wait()

        return carry

    lax.fori_loop(1, N, step_fn, 0)
    last_step()
    out_copy(N - 2).wait()
    for i in range(len(FIN) - 1):
        part_copy(N - 1, i).wait()


@jax.jit
def pallas_standalone__conformer_family_branchformer__speech_kernel(
    x: jax.Array,
    w_q: jax.Array,
    w_k: jax.Array,
    w_v: jax.Array,
    w_ao: jax.Array,
    w_up: jax.Array,
    dw: jax.Array,
    w_dn: jax.Array,
    w_merge: jax.Array,
):
    B, T, D = x.shape
    K = dw.shape[0]
    TQ = 400
    TK = 512
    FIN = (0, 256, 352, TQ)
    TP = -(-T // TK) * TK
    NKV = TP // TK
    assert B >= 2 and T % TQ == 0 and D == TK and K // 2 < HALO
    assert NKV + 1 < T // TQ and NKV == 8 and T % LANES in (16, 32, 48, 64) and TP - T < LANES
    x2 = x.reshape(B * T, D)

    kern = functools.partial(_kernel, B=B, T=T, D=D, K=K, TQ=TQ, TK=TK, TP=TP, FIN=FIN)
    ins = (x2, w_q, w_k, w_v, w_ao, w_up, dw, w_dn, w_merge)
    out = pl.pallas_call(
        kern,
        in_specs=[pl.BlockSpec(memory_space=pl.ANY) for _ in ins],
        out_specs=pl.BlockSpec(memory_space=pl.ANY),
        out_shape=jax.ShapeDtypeStruct((B * T, D), x.dtype),
        scratch_shapes=[pltpu.VMEM((B * TP, D), x.dtype)] + [pltpu.VMEM(a.shape, a.dtype) for a in ins[1:]] + [
            pltpu.SemaphoreType.DMA((11 + B,)),
            pltpu.VMEM(((B * TP + TK) // H + 64, D), U32),
            pltpu.VMEM((D // H, D), U32),
            pltpu.VMEM((2 * D // H, D), U32),
            pltpu.VMEM((K, 8, D), F32),
            pltpu.VMEM((NKV, TQ, TK), F32),
            pltpu.VMEM((TQ, LANES), F32),
            pltpu.VMEM((TQ, D), F32),
            pltpu.VMEM((D // LANES, TQ + 2 * HALO, LANES), F32),
            pltpu.VMEM((D // LANES, TQ + 2 * HALO, LANES), F32),
            pltpu.VMEM((TQ, D), F32),
            pltpu.VMEM((TQ, LANES), F32),
            pltpu.VMEM((TQ // H, D), U32),
            pltpu.VMEM((T % LANES, D), F32),
            pltpu.VMEM((2, TQ, D), x.dtype),
            pltpu.SemaphoreType.DMA((1 + len(FIN),)),
            pltpu.VMEM(((B * NKV + 1) * 5 * (TK // 2 // H) + 64, D // 2), U32),
            pltpu.VMEM((TK // H, D), U32),
            pltpu.VMEM((5 * (TK // 2 // H), D // 2), U32),
            pltpu.VMEM((5, 7, D // 2 // H, D // 2), U32),
            pltpu.VMEM((2, 7, 16 * (-(-TQ // 32)) // H, D), U32),
            pltpu.SMEM((5,), jnp.int32),
        ],
        compiler_params=pltpu.CompilerParams(
            vmem_limit_bytes=100 * 1024 * 1024,
            disable_bounds_checks=True,
            disable_semaphore_checks=True,
        ),
    )(*ins)
    return out.reshape(B, T, D)
```

```python
import functools
import math

import jax
import jax.numpy as jnp
from jax import lax
import jax.experimental.pallas as pl
import jax.experimental.pallas.tpu as pltpu

TUNE = {'A': {'LAG': 3, 'INS0': 20, 'INS1': 90, 'LREL': 2, 'LW': 2, 'LNJ': 7, 'GREL': 0, 'GJ': -1, 'UREL': 6, 'EPV': 70, 'E0S': 0, 'E00': 65, 'MGP': 75, 'LSP': 60, 'OST': 0, 'TTC': 1, 'CG': 8, 'SOUT': 2},
        'B': {'LAG': 4, 'GREL': 2, 'GJ': -1, 'UREL': 4, 'EPV': 90, 'E0S': 60, 'E00': 30, 'MGP': 100, 'OST': 2, 'TTC': 1, 'CG': 8, 'SOUT': 1, 'XREL': 0},
        'C': {'LAG': 4, 'EPV': 80, 'OST': 0, 'CG': 16, 'SOUT': 2, 'CM': 1}}
LANES = 128
EPS = 1e-05
F32 = jnp.float32
BF16 = jnp.bfloat16
U32 = jnp.uint32
NT = (((1,), (1,)), ((), ()))
HALO = 16
H = 2


def _ln(x, eps):
    d = x.shape[-1]
    m = jnp.sum(x, axis=-1, keepdims=True) * (1.0 / d)
    xc = x - m
    v = jnp.sum(xc * xc, axis=-1, keepdims=True) * (1.0 / d)
    return xc * lax.rsqrt(v + eps)


def _gelu2(x):
    c1 = math.sqrt(2.0 / math.pi)
    c2 = c1 * 0.044715
    t = jnp.tanh(x * (c1 + c2 * (x * x)))
    return x + x * t


def _center(w):
    return w - jnp.sum(w, axis=0, keepdims=True) * (1.0 / w.shape[0])


def _pack(x):
    return pltpu.bitcast(x.astype(BF16), U32)


def _unpack(x):
    return pltpu.bitcast(x, BF16)


def _bits(x):
    return pltpu.bitcast(x, U32)


def _dot(a, b):
    return jnp.dot(a, b, preferred_element_type=F32)


def _dot_nt(a, b):
    return lax.dot_general(a, b, NT, preferred_element_type=F32)


def _split(v):
    return [v[:, c * LANES:(c + 1) * LANES] for c in range(v.shape[1] // LANES)]


def _aligned(i, n):
    return i if isinstance(i, int) else pl.multiple_of(i, n)


def _tie(flag, dep, val, n):
    if n == val.shape[0]:
        return jnp.where(flag, dep[0:n], val)
    return jnp.concatenate([jnp.where(flag, dep[0:n], val[0:n]), val[n:]], axis=0)


def _tie_bf16(flag, dep, val):
    head = _bits(val[0:16, 0:LANES])
    head = _unpack(jnp.where(flag, _bits(dep), head))
    top = jnp.concatenate([head, val[0:16, LANES:]], axis=1)
    return jnp.concatenate([top, val[16:, :]], axis=0)


def _tie_vregs(flag, deps, val, row, col):
    cast = _bits if val.dtype == U32 else (lambda v: v if v.dtype == F32 else pltpu.bitcast(v, F32))
    tiles = _split(val)
    t = tiles[col]
    n = 8 * len(deps)
    mid = jnp.where(flag, jnp.concatenate([cast(d) for d in deps], axis=0), t[row:row + n])
    tiles[col] = jnp.concatenate(([t[0:row]] if row else []) + [mid, t[row + n:]], axis=0)
    return jnp.concatenate(tiles, axis=1)


def _to_bf16(v):
    return _unpack(v) if v.dtype == U32 else v.astype(BF16)


def _paced(flag, src, span, val):
    rows = val.shape[0]
    rel = jnp.concatenate(
        [src[(r * span) % rows:(r * span) % rows + 8,
             ((r * span) // rows) * LANES:((r * span) // rows + 1) * LANES]
         for r in range(0, rows, 8)], axis=0)
    return jnp.concatenate([jnp.where(flag, rel, val[:, 0:LANES]), val[:, LANES:]], axis=1)


def _tokens(results):
    out = []
    for s in results:
        ncol = s.shape[1] // LANES
        step = 2 if ncol == 2 else 1
        out += [s[r:r + 8, c * LANES:(c + 1) * LANES] for c in range(0, ncol, step) for r in range(0, s.shape[0], 8)]
    return out


def _released(flag, toks, first, total, val, ntiles=1):
    n = val.shape[0] // 8
    rel = jnp.concatenate([toks[min(first + (i * total) // n, len(toks) - 1)] for i in range(n)], axis=0)
    if val.dtype == U32:
        rel = _bits(rel)
    tiles = _split(val)
    return jnp.concatenate([jnp.where(flag, rel, t) if c < ntiles else t for c, t in enumerate(tiles)], axis=1)


def _kernel(x_hbm, wq_hbm, wk_hbm, wv_hbm, wao_hbm, wup_hbm, dw_hbm, wdn_hbm, wm_hbm,
            o_hbm,
            x_s, wq_s, wk_s, wv_s, wao_s, wup_s, dw_s, wdn_s, wm_s, sems,
            xa_s, wa_s, dwb_s, s_s, m_s, u_s, g_s, gn_s, o_s, osems, tb_s, sx_s, st_s, wt_s, pl_s, z_s,
            *, B, T, D, K, TQ, TK, TP, U, UR):
    NQ = T // TQ
    N = B * NQ
    NKV = TP // TK
    NC = D // LANES
    CPK = TK // LANES
    PAD = K // 2
    NQT = -(-TQ // LANES)
    NFULL = (T - (NKV - 1) * TK) // LANES
    TAIL = T % LANES

    def keys(b, r0, n):
        return _unpack(xa_s[pl.ds(xrow(b * TP) + r0 // H, n // H), :])

    def tail_keys(b):
        return keys(b, T - TAIL, TAIL)

    DH = D // 2
    HR = 16 * (-(-TQ // 32))
    R2 = TQ - HR

    def key_tables(y):
        nt = y.shape[0] // LANES
        ev = jnp.concatenate([y[t * LANES:(t + 1) * LANES] for t in range(0, nt, 2)], axis=0)
        od = jnp.concatenate([y[t * LANES:(t + 1) * LANES] for t in range(1, nt, 2)], axis=0)
        e1, e2, o1, o2 = ev[:, 0:DH], ev[:, DH:], od[:, 0:DH], od[:, DH:]
        return [_pack(v) for v in (e1 + o2, o1 - o2, e2 - e1, e1 + o1, e2 + o2)]

    def row_operands(a, reused=False):
        a11, a12, a21, a22 = a[0:HR, 0:DH], a[0:HR, DH:], a[R2:TQ, 0:DH], a[R2:TQ, DH:]
        return {i: _pack(v) if reused else v
                for i, v in ((1, a11 + a22), (2, a21 + a22), (3, a11), (4, a22),
                             (5, a11 + a12), (6, a21 - a11), (7, a12 - a22))}

    ORDER = (4, 2, 1, 5, 3, 7, 6)
    TR = TK // 2 // H
    PX, PT = 0, 0

    def xrow(r):
        return PX + r // H if isinstance(r, int) else pl.multiple_of(z_s[3] + r // H, 8)

    def trow(blk, i):
        return PT + (blk * 5 + i) * TR if isinstance(blk, int) else pl.multiple_of(z_s[4] + (blk * 5 + i) * TR, 8)

    def weight_tables(mat, w):
        b11, b12, b21, b22 = w[0:DH, 0:DH], w[0:DH, DH:], w[DH:, 0:DH], w[DH:, DH:]
        for i, v in enumerate((b11 + b22, b11, b12 - b22, b21 - b11, b22, b11 + b12, b21 + b22)):
            wt_s[mat, i] = _pack(v)

    def combine(m):
        return {(0, 0): (m[1] + m[4] - m[5]) + m[7], (0, 1): m[3] + m[5],
                (1, 0): m[2] + m[4], (1, 1): (m[1] - m[2] + m[3]) + m[6]}

    def stack(top, bottom):
        return jnp.concatenate([top, bottom[HR - R2:]], axis=0)

    def project(lhs_list, mats, gate):
        m = {}
        for i in ORDER:
            l = jnp.concatenate([lhs[i] for lhs in lhs_list], axis=1)
            m[i] = gate(i, l, lambda v, i=i: _dot(v, _unpack(jnp.concatenate([wt_s[k, i - 1] for k in mats], axis=0))))
        c = combine(m)
        return jnp.concatenate([stack(c[0, 0], c[1, 0]), stack(c[0, 1], c[1, 1])], axis=1)

    def key_operand(b, j, npair, i):
        if i in (2, 5):
            base = xrow(b * TP) + j * TK // H
            parity, lo = (0, 0) if i == 2 else (1, DH)
            return _unpack(jnp.concatenate(
                [xa_s[pl.ds(base + (2 * p + parity) * LANES // H, LANES // H), lo:lo + DH] for p in range(npair)],
                axis=0))
        return _unpack(tb_s[pl.ds(trow(b * NKV, 0) + (j * 5 + {1: 0, 3: 1, 4: 2, 6: 3, 7: 4}[i]) * TR, npair * LANES // H), :])

    def pv_products(tiles, b, j, gate, pend):
        npair = len(tiles) // 2
        ev = jnp.concatenate(tiles[0:2 * npair:2], axis=1)
        od = jnp.concatenate(tiles[1:2 * npair:2], axis=1)
        a11, a12, a21, a22 = ev[0:HR], od[0:HR], ev[R2:TQ], od[R2:TQ]
        ops = {1: (a11 + a22, 1), 2: (a11, 7), 3: (a21 - a22, 2), 4: (a12 - a11, 5),
               5: (a22, 6), 6: (a11 + a21, 4), 7: (a12 + a22, 3)}
        n = {}
        for i in PVORD:
            l, k = ops[i]
            n[i] = gate(i, l, lambda v, k=k: _dot(v, key_operand(b, j, npair, k)),
                        2 if npair == 1 and n else 1)
        return n

    PVORD = (2, 5, 1, 3, 4, 6, 7)

    def qk_chunk2(lhs, q, b, j, gate, parts=None):
        last = j == NKV - 1
        last = last and 1
        npair = (NFULL if last else CPK) // 2
        m = {}
        for i in ORDER:
            m[i] = gate(i, lhs[i], lambda l, i=i: _dot_nt(l, key_operand(b, j, npair, i)), 2 if last and m else 1)
        c = combine(m)
        mx = None
        for t in range(CPK):
            if t < 2 * npair:
                cols = slice((t // 2) * LANES, (t // 2 + 1) * LANES)
                st = stack(c[0, t % 2][:, cols], c[1, t % 2][:, cols])
                if j == NKV - 1 and t == NFULL:
                    st = jnp.where(lax.broadcasted_iota(jnp.int32, st.shape, 1) < TAIL, st, -jnp.inf)
            elif t < NFULL:
                st = gate(0, q, lambda l: _dot_nt(l, keys(b, j * TK + t * LANES, LANES)))
            else:
                st = tail_tile(parts)
            s_s[j, :, t * LANES:(t + 1) * LANES] = st
            mx = st if mx is None else jnp.maximum(mx, st)
        return mx

    def tail_part(kt, q, n):
        qn = q[n * LANES:min((n + 1) * LANES, TQ), :]
        if qn.shape[0] < LANES:
            qn = jnp.concatenate([qn, jnp.zeros((LANES - qn.shape[0], D), BF16)], axis=0)
        return _dot_nt(kt, qn)

    def tail_tile(parts):
        fill = jnp.full((LANES - TAIL, LANES), -jnp.inf, F32)
        return jnp.concatenate([jnp.concatenate([p, fill], axis=0).T for p in parts], axis=0)[0:TQ, :]

    def qk_chunk(q, b, j, parts=None):
        last = j == NKV - 1
        s = _dot_nt(q, keys(b, j * TK, (NFULL if last else CPK) * LANES))
        mx = None
        for c in range(CPK):
            st = tail_tile(parts) if last and c == NFULL else s[:, c * LANES:(c + 1) * LANES]
            s_s[j, :, c * LANES:(c + 1) * LANES] = st
            mx = st if mx is None else jnp.maximum(mx, st)
        return s, mx

    def probs(j, m, ntiles):
        tiles = []
        lsum = None
        for c in range(ntiles):
            p = jnp.exp2(s_s[j, :, c * LANES:(c + 1) * LANES] - m)
            lsum = p if lsum is None else lsum + p
            tiles.append(p)
        return tiles, lsum

    def store_g(ref, row, g):
        for c in range(NC):
            ref[c, row:row + g.shape[0], :] = g[:, c * LANES:(c + 1) * LANES]

    def conv_rows(g_w, R, G, flag, prev=None, split2=False):
        rows = []
        for rr in range(0, R, G):
            cols = []
            for c in range(NC):
                acc = None
                acc2 = None
                for k in range(K):
                    gv = g_w[c, pl.ds(rr + HALO - PAD + k, G), :].reshape(G // 8, 8, LANES)
                    term = gv * dwb_s[k, :, c * LANES:(c + 1) * LANES][None]
                    if acc is None:
                        acc = term if prev is None else jnp.where(flag, prev, term)
                    elif split2 and k % 2 == 1:
                        acc2 = term if acc2 is None else acc2 + term
                    else:
                        acc = acc + term
                if acc2 is not None:
                    acc = acc + acc2
                prev = acc
                cols.append(acc.reshape(G, LANES))
            rows.append(jnp.concatenate(cols, axis=1))
        return jnp.concatenate(rows, axis=0)

    def conv_unit(g_w, rr, c, G, flag, tok):
        acc = None
        for k in range(K):
            gv = g_w[c, pl.ds(rr + HALO - PAD + k, G), :].reshape(G // 8, 8, LANES)
            term = gv * dwb_s[k, :, c * LANES:(c + 1) * LANES][None]
            acc = jnp.where(flag, tok[None], term) if acc is None else acc + term
        return acc.reshape(G, LANES)

    def store_max(mx):
        m = jnp.max(mx, axis=-1, keepdims=True)
        if 1:
            m = m + jnp.log2(jnp.sum(jnp.exp2(mx - m), axis=-1, keepdims=True))
        m_s[...] = jnp.broadcast_to(m, (TQ, LANES))

    NU = TP // UR
    UT = UR // 2 // H

    def next_unit(step):
        return jnp.minimum(step // NQ + 1, B - 1) * NU + jnp.minimum(step % NQ, NU - 1)

    def has_next(step):
        return jnp.logical_and(step // NQ + 1 < B, step % NQ < NU)

    def stage(y):
        sx_s[...] = _pack(y)
        for i, tbl in enumerate(key_tables(y)):
            st_s[i * UT:(i + 1) * UT, :] = tbl

    def first_step():
        C2 = NKV // 2

        def xrows(b, r0, r1):
            return x_hbm.at[pl.ds(b * T + r0, r1 - r0), :], x_s.at[pl.ds(b * TP + r0, r1 - r0), :]

        copies = {}
        plan = (
            ('wq', wq_hbm, wq_s), ('wk', wk_hbm, wk_s),
            ('xa',) + xrows(0, 0, TK), ('xb',) + xrows(0, TK, C2 * TK), ('xc',) + xrows(0, C2 * TK, T),
            ('wup', wup_hbm, wup_s), ('dw', dw_hbm, dw_s), ('xd',) + xrows(1, 0, UR),
            ('wv', wv_hbm, wv_s), ('wao', wao_hbm, wao_s), ('wdn', wdn_hbm, wdn_s), ('wm', wm_hbm, wm_s),
            ('xe1',) + xrows(1, UR, T),
        ) + tuple(('xe%d' % b,) + xrows(b, 0, T) for b in range(2, B))
        for i, (name, src, dst) in enumerate(plan):
            copies[name] = pltpu.make_async_copy(src, dst, sems.at[i])
            copies[name].start()

        z_s[0] = 0
        z_s[1] = 0
        z_s[2] = 0
        z_s[3] = PX
        z_s[4] = PT
        for b in range(B):
            x_s[b * TP + T:(b + 1) * TP, :] = jnp.zeros((TP - T, D), x_s.dtype)
        store_g(g_s.at[0], TQ, jnp.zeros((HALO, D), F32))

        def ln_chunk(c, t=None, span=100):
            xv = x_s[c * TK:(c + 1) * TK, :].astype(F32)
            if t is not None:
                xv = _released(never, t, 0, len(t) * span // 100, xv)
            y = _ln(xv, EPS)
            xa_s[pl.ds(xrow(c * TK), TK // H), :] = _pack(y)
            for i, tbl in enumerate(key_tables(y)):
                tb_s[pl.ds(trow(c, i), TR), :] = tbl

        scale = float(D) ** (-0.5) * math.log2(math.e)
        DS = D // 2
        FL = 0
        copies['wq'].wait()
        copies['wk'].wait()
        m_lo = _dot_nt(wq_s[...], wk_s[0:DS, :])

        never = z_s[0] > 0
        zero = pl.multiple_of(z_s[0], 8)
        hist = []
        pend = []

        def gate(i, l, run, lag=1):
            if len(hist) >= lag:
                l = _tie_vregs(never, [hist[-lag][0:8, 0:LANES]], l, 0, 0)
            if pend:
                l = _tie_vregs(never, pend, l, 8, 0)
                del pend[:]
            hist.append(run(_to_bf16(l)))
            return hist[-1]

        copies['xa'].wait()
        wa_s[:, 0:DS] = _pack(_center(m_lo) * scale)
        wa_s[:, DS:D] = _pack(_center(_dot_nt(wq_s[...], wk_s[DS:D, :])) * scale)
        ln_chunk(0)
        q_raw = _dot(keys(0, 0, TQ), _unpack(wa_s[:, 0:D]))
        qp = _pack(q_raw)
        q = _unpack(qp)

        copies['xb'].wait()
        FS = 8
        if FS < NKV:
            lhs = row_operands(q_raw, True)
            lhs[3] = qp[0:HR // H, 0:DH]
            lhs[4] = qp[R2 // H:TQ // H, DH:]

        def qk(c, parts=None):
            n0 = len(hist)
            if c >= FS:
                mj = qk_chunk2(lhs, qp, 0, c, gate, parts)
            else:
                res = []
                gate(0, qp, lambda v: res.append(qk_chunk(v, 0, c, parts)) or res[0][0])
                mj = res[0][1]
            return mj, _tokens(hist[n0:]) if FL else None

        mx, t = qk(0)
        for c in range(1, C2):
            ln_chunk(c, t, FL)
            mj, t = qk(c)
            mx = jnp.maximum(mx, mj)

        for name in ('xc', 'wup', 'dw'):
            copies[name].wait()
        del hist[:]
        xq = xa_s[pl.ds(xrow(0), TQ // H), :]
        hg = gate(0, xq, lambda v: _dot(v, wup_s[:, D:2 * D]))
        hu = gate(0, xq, lambda v: _dot(v, wup_s[:, 0:D]))
        dwf = dw_s[...].astype(F32)
        for k in range(K):
            dwb_s[k] = jnp.broadcast_to(dwf[k:k + 1, :], (8, D))
        parts = None
        for c in range(C2, NKV):
            ln_chunk(c, (_tokens(hist) if 0 else None) if c == C2 else t, 0 if c == C2 else FL)
            if c == NKV - 1:
                kt = tail_keys(0)
                parts = [tail_part(kt, q, n) for n in range(NQT)]
            mj, t = qk(c, parts)
            mx = jnp.maximum(mx, mj)

        for name in ('xd', 'wv', 'wao', 'wdn', 'wm'):
            copies[name].wait()
        store_max(mx)
        wva_raw = _dot(wv_s[...], wao_s[...])
        t1 = _tokens([wva_raw])
        wdm = _dot(_tie_bf16(never, wva_raw[0:8, 0:LANES], wdn_s[...]), wm_s[D:2 * D, :])
        t2 = _tokens([wdm])
        t12 = t1 + t2
        n12 = len(t12)

        def rel(v, lo, hi, nt=NC):
            return _released(never, t12, n12 * lo // 100, n12 * (hi - lo) // 100, v, nt)

        store_g(gn_s, 0, _ln(_gelu2(rel(hg, 0, 30)), 4.0 * EPS))
        u_s[...] = _gelu2(rel(hu, 30, 60))
        stage(_ln(rel(x_s[TP:TP + UR, :].astype(F32), 0, 50, 1), EPS))
        weight_tables(0, rel(_unpack(wa_s[:, 0:D]).astype(F32), 50, 65))
        weight_tables(1, rel(wup_s[:, D:2 * D].astype(F32), 65, 80))
        weight_tables(2, rel(wup_s[:, 0:D].astype(F32), 80, 95))
        mean = jnp.sum(wva_raw, axis=0, keepdims=True) * (1.0 / D)
        wva = (_released(never, t2, 0, len(t2) * 3 // 4, wva_raw, NC) - mean).astype(BF16)
        deps = [wdm[0:8, LANES:2 * LANES], sx_s[pl.ds(zero, 8), 0:LANES], st_s[pl.ds(zero, 8), 0:LANES],
                gn_s[0, pl.ds(zero, 8), :], u_s[pl.ds(zero, 8), 0:LANES]]
        if 1:
            deps.append(wt_s[z_s[0], 0, 0:8, 0:LANES])
        for i, dep in enumerate(deps):
            wva = jnp.concatenate(([wva[0:16 * i]] if i else []) + [_tie_bf16(never, dep, wva[16 * i:])], axis=0)
        wvom = _dot(wva, wm_s[0:D, :])
        t3 = _tokens([wvom])
        weight_tables(4, _released(never, t3, 0, len(t3) // 2, 0.5 * wdm, NC))
        weight_tables(3, wvom)
        for b in range(1, B):
            copies['xe%d' % b].wait()

    def sub_step(step, hist, w, slot, ba, bb, keep_next, P, do_a=True):
        sb = step - 1
        ia, ib = step - ba * NQ, sb - bb * NQ

        def KP(k, d):
            return TUNE[P].get(k, d)
        never = z_s[0] > 0
        never2 = z_s[1] > 0
        never3 = z_s[2] > 0
        g_w, g_prev = g_s.at[w[0]], g_s.at[w[1]]
        for c in range(NC):
            g_w[c, 0:HALO, :] = jnp.where(ib == 0, 0.0, g_prev[c, TQ:TQ + HALO, :])
            g_w[c, HALO:HALO + TQ, :] = gn_s[c]
        pend = []
        h0 = len(hist)

        def gate(i, l, run, lag=1):
            lag = lag * KP('LAG', 2)
            if len(hist) >= lag:
                l = _tie_vregs(never3, [hist[-lag][0:8, 0:LANES]], l, 0, 0)
            if pend:
                l = _tie_vregs(never3, pend, l, 8, 0)
                del pend[:]
            hist.append(run(_to_bf16(l)))
            return hist[-1]

        def toks(i0, i1=None):
            return _tokens(hist[i0:i1])

        m_old = m_s[...]
        u_old = u_s[...]
        if do_a:
            xq = xa_s[pl.ds(xrow(ba * TP + ia * TQ), TQ // H), :]
            xf = _unpack(xq).astype(F32)
            if h0 and KP('XREL', 50):
                t = toks(h0 - 14)
                xf = _released(never, t, 0, len(t) * KP('XREL', 50) // 100, xf, NC)
            xops = row_operands(xf, True)
            xops[3] = xq[0:HR // H, 0:DH]
            xops[4] = xq[R2 // H:TQ // H, DH:]
            q_raw = project([xops], [0], gate)
            hg = project([xops], [1], gate)
            hu = project([xops], [2], gate)
            qp = _pack(q_raw)
            q = _unpack(qp)
            ptok = toks(h0)
            NP = len(ptok)
            lhs = row_operands(q_raw, True)
            lhs[3] = qp[0:HR // H, 0:DH]
            lhs[4] = qp[R2 // H:TQ // H, DH:]
        else:
            store_g(g_w, HALO + TQ, jnp.zeros((HALO, D), F32))
        if keep_next:
            dst = jnp.where(has_next(sb), next_unit(sb), B * NU)
            i0, i1 = NP * KP('INS0', 35) // 100, NP * KP('INS1', 90) // 100
            im = i0 + (i1 - i0) * 4 // 9
            xa_s[pl.ds(xrow(dst * UR), UR // H), :] = _released(never, ptok, i0, im - i0, sx_s[...], NC)
            tbl = _released(never, ptok, im, i1 - im, st_s[...], 2)
            upc = TK // UR
            tbase = trow(dst // upc, 0) + (dst % upc) * UT
            for i in range(5):
                tb_s[pl.ds(pl.multiple_of(tbase + i * TR, 8), UT), :] = tbl[i * UT:(i + 1) * UT]

        CM = KP('CM', 0)
        CG = KP('CG', 8)
        C0, C1, CD = KP('C0', 0), KP('C1', 6), KP('CD', 2)
        units = [(rr, c) for rr in range(0, TQ, CG) for c in range(NC)]
        conv = {}
        due = {}

        def conv_slice(j, t):
            if not C0 <= j < C1:
                return
            lo, hi = (len(units) * (j - C0)) // (C1 - C0), (len(units) * (j + 1 - C0)) // (C1 - C0)
            for n, (rr, c) in enumerate(units[lo:hi]):
                tok = t[(n * len(t) * KP('CSP', 100) // 100) // (hi - lo)]
                if KP('CCH', 0) and n >= KP('CCH', 0):
                    tok = conv[units[lo + n - KP('CCH', 0)]][0:8]
                conv[rr, c] = conv_unit(g_w, rr, c, CG, never, tok)
                if CD and (not KP('CCH', 0) or n >= hi - lo - KP('CCH', 0)):
                    due.setdefault(j + CD, []).extend(conv[rr, c][r:r + 8] for r in range(0, CG, 8))

        l_acc = None
        mx = None
        acc = None
        parts = []
        pv0 = pv1 = None
        starts = []
        for j in range(NKV):
            m_use = m_old
            if j == 0 and do_a and KP('E0S', 60):
                m_use = _released(never, ptok, NP * KP('E00', 50) // 100, NP * KP('E0S', 60) // 100, m_old)
            if j >= (1 if do_a else 2):
                t = toks(pv0, pv1) if do_a else toks(pv0 - 7, pv0)
                m_use = _released(never, t, 0, len(t) * KP('EPV', 80) // 100, m_old)
            tiles, l_new = probs(j, m_use, CPK)
            l_acc = l_new if l_acc is None else l_acc + l_new
            tiles[0] = jnp.where(never2, l_acc, tiles[0])
            for i0 in range(0, len(due.get(j, [])), TQ // 8):
                d = due[j][i0:i0 + TQ // 8]
                k = 1 + i0 // (TQ // 8)
                tiles[k] = _tie(never3, jnp.concatenate(d, axis=0), tiles[k], 8 * len(d))
            pv0 = len(hist)
            starts.append(pv0)
            n = pv_products(tiles, bb, j, gate, pend)
            acc = n if acc is None else {i: acc[i] + n[i] for i in n}
            pv1 = len(hist)
            if not do_a:
                if CM:
                    conv_slice(j, toks(pv0))
                continue
            if j == KP('UREL', 4):
                t = toks(pv0)
                u_s[...] = _gelu2(_released(never, t, 0, len(t), hu, NC))
            if j == KP('LNJ', 6) and keep_next:
                pend += [sx_s[pl.ds(pl.multiple_of(z_s[0], 8), 8), 0:LANES],
                         st_s[pl.ds(pl.multiple_of(z_s[0], 8), 8), 0:LANES]]
            if j == KP('GJ', 6):
                pend.append(gn_s[0, pl.ds(pl.multiple_of(z_s[0], 8), 8), :])
            if j < NQT:
                t = toks(pv0)
                kt = _tie_bf16(never3, t[len(t) * KP('TTC', 3) // 4], tail_keys(ba))
                parts.append(tail_part(kt, q, j))
            if 1 <= j <= NQT:
                pend.append(parts[j - 1][0:8])
            mj = qk_chunk2(lhs, qp, ba, j, gate, parts)
            mx = mj if mx is None else jnp.maximum(mx, mj)
            if j == KP('LREL', 2) and keep_next:
                xv = x_s[pl.ds(pl.multiple_of(next_unit(step) * UR, 16), UR), :].astype(F32)
                t = toks(starts[max(j + 1 - KP('LW', 1), 0)])
                stage(_ln(_released(never, t, 0, len(t) * KP('LSP', 60) // 100, xv), EPS))
            if j == KP('GREL', 1):
                t1, t2 = toks(pv0, pv1), toks(pv1)
                gg = _gelu2(_released(never, t1, 0, len(t1), hg, NC))
                g_new = _ln(_released(never, t2, 0, len(t2) * KP('MGP', 100) // 100, gg), 4.0 * EPS)
                store_g(gn_s, 0, g_new)
                store_g(g_w, HALO + TQ, jnp.where(ia == 0, 0.0, g_new[0:HALO, :]))
            if CM:
                conv_slice(j, toks(pv0))
        cstart = None
        if h0 and KP('CST', 0):
            cstart = jnp.broadcast_to(hist[h0 + KP('CS0', 0)][None, 0:8, 0:LANES], (KP('CG', 8) // 8, 8, LANES))
        if CM:
            yc = u_old * jnp.concatenate([jnp.concatenate([conv[rr, c] for c in range(NC)], axis=1)
                                          for rr in range(0, TQ, CG)], axis=0)
        else:
            yc = u_old * conv_rows(g_w, TQ, KP('CG', 8), never, cstart)
        z = combine(acc)
        acc = jnp.concatenate([stack(z[0, 0], z[0, 1]), stack(z[1, 0], z[1, 1])], axis=1)
        ya = acc * (1.0 / jnp.sum(l_acc, axis=-1, keepdims=True))

        def staged(ops, k):
            if not KP('OST', 2):
                return ops
            for i in ORDER:
                pl_s[k, i - 1] = _pack(ops[i])
            return {i: pl_s[k, i - 1] for i in ops}

        if KP('SOUT', 1) == 1:
            oc = staged(row_operands(yc), 0)
            out = project([staged(row_operands(ya), 1), oc], [3, 4], gate)
        else:
            out = project([staged(row_operands(yc), 0)], [4], gate)
            out = out + project([staged(row_operands(ya), 1)], [3], gate)
        xr = x_s[pl.ds(_aligned(bb * TP + ib * TQ, 16), TQ), :].astype(F32)
        o_s[slot] = (xr + out).astype(o_s.dtype)
        if do_a:
            store_max(mx)

    def out_copy(blk, slot):
        return pltpu.make_async_copy(o_s.at[slot], o_hbm.at[pl.ds(_aligned(blk * TQ, 16), TQ), :], osems.at[slot])

    first_step()

    def iteration0(step, carry):
        sub_step(step, [], (0, 0), (step - 1) % 2, step // NQ, 0, True, 'A')
        out_copy(step - 1, (step - 1) % 2).start()

        @pl.when(step >= 2)
        def _():
            out_copy(step - 2, step % 2).wait()

        return carry

    lax.fori_loop(1, NQ + 1, iteration0, 0)
    out_copy(NQ - 1, (NQ - 1) % 2).wait()

    NIT = (NQ - 1) // U

    def iteration1(it, carry):
        hist = []
        for u in range(U):
            step = NQ + 1 + it * U + u
            sub_step(step, hist, ((u + 1) % U, u), (it % 2) * U + u, 1, 1, False, 'B')
            out_copy(step - 1, (it % 2) * U + u).start()

        @pl.when(it >= 1)
        def _():
            for u in range(U):
                out_copy(NQ + (it - 1) * U + u, ((it - 1) % 2) * U + u).wait()

        return carry

    lax.fori_loop(0, NIT, iteration1, 0)
    sub_step(N, [], (1 % U, 0), (NIT % 2) * U, 1, 1, False, 'C', do_a=False)
    out_copy(N - 1, (NIT % 2) * U).start()
    for u in range(U):
        out_copy(NQ + (NIT - 1) * U + u, ((NIT - 1) % 2) * U + u).wait()
    out_copy(N - 1, (NIT % 2) * U).wait()


@jax.jit
def pallas_standalone__conformer_family_branchformer__speech_kernel(
    x: jax.Array,
    w_q: jax.Array,
    w_k: jax.Array,
    w_v: jax.Array,
    w_ao: jax.Array,
    w_up: jax.Array,
    dw: jax.Array,
    w_dn: jax.Array,
    w_merge: jax.Array,
):
    B, T, D = x.shape
    K = dw.shape[0]
    TQ = 160
    TK = 512
    U = 2
    TP = -(-T // TK) * TK
    UR = 256
    NKV = TP // TK
    assert B == 2 and (T // TQ - 1) % U == 0 and T % TQ == 0 and D == TK and K // 2 < HALO
    assert TP // UR + 1 < T // TQ and NKV == 8 and T % LANES in (16, 32, 48, 64) and TP - T < LANES
    x2 = x.reshape(B * T, D)

    kern = functools.partial(_kernel, B=B, T=T, D=D, K=K, TQ=TQ, TK=TK, TP=TP, U=U, UR=UR)
    ins = (x2, w_q, w_k, w_v, w_ao, w_up, dw, w_dn, w_merge)
    out = pl.pallas_call(
        kern,
        in_specs=[pl.BlockSpec(memory_space=pl.ANY) for _ in ins],
        out_specs=pl.BlockSpec(memory_space=pl.ANY),
        out_shape=jax.ShapeDtypeStruct((B * T, D), x.dtype),
        scratch_shapes=[pltpu.VMEM((B * TP, D), x.dtype)] + [pltpu.VMEM(a.shape, a.dtype) for a in ins[1:]] + [
            pltpu.SemaphoreType.DMA((11 + B,)),
            pltpu.VMEM(((B * TP + TK) // H + 64, D), U32),
            pltpu.VMEM((D // H, D), U32),
            pltpu.VMEM((K, 8, D), F32),
            pltpu.VMEM((NKV, TQ, TK), F32),
            pltpu.VMEM((TQ, LANES), F32),
            pltpu.VMEM((TQ, D), F32),
            pltpu.VMEM((U, D // LANES, TQ + 2 * HALO, LANES), F32),
            pltpu.VMEM((D // LANES, TQ, LANES), F32),
            pltpu.VMEM((2 * U, TQ, D), x.dtype),
            pltpu.SemaphoreType.DMA((2 * U,)),
            pltpu.VMEM(((B * NKV + 1) * 5 * (TK // 2 // H) + 64, D // 2), U32),
            pltpu.VMEM((UR // H, D), U32),
            pltpu.VMEM((5 * (UR // 2 // H), D // 2), U32),
            pltpu.VMEM((5, 7, D // 2 // H, D // 2), U32),
            pltpu.VMEM((2, 7, 16 * (-(-TQ // 32)) // H, D // 2), U32),
            pltpu.SMEM((5,), jnp.int32),
        ],
        compiler_params=pltpu.CompilerParams(
            vmem_limit_bytes=100 * 1024 * 1024,
            disable_bounds_checks=True,
            disable_semaphore_checks=True,
        ),
    )(*ins)
    return out.reshape(B, T, D)
```

```python
import functools
import math

import jax
import jax.numpy as jnp
from jax import lax
import jax.experimental.pallas as pl
import jax.experimental.pallas.tpu as pltpu

LANES = 128
EPS = 1e-05
F32 = jnp.float32
BF16 = jnp.bfloat16
U32 = jnp.uint32
NT = (((1,), (1,)), ((), ()))
HALO = 16
H = 2

SCHEME = (
    ('...-++..', '...+............', '-+.....+'),
    ('.+-.....', '.........-......', '.++..++.'),
    ('+...--..', '.+..+.......+...', '-+..-...'),
    ('.+.-.-.+', '...-...+....+...', '.-.+....'),
    ('.....+..', '.+...-+......-..', '.....-..'),
    ('+...-...', '+.-.-.......-...', '....-...'),
    ('--.+....', '...-........+...', '+-.+....'),
    ('..+...-.', '......+.-.+-....', '..+.....'),
    ('..-+....', '...........+....', '..--....'),
    ('-.....+.', '..+.....+.......', '..-.+...'),
    ('....+.-.', '..+.............', '....+.+.'),
    ('+.-.....', '........+.......', '-.-.....'),
    ('...-....', '...-.......-.-.-', '...+...+'),
    ('++..--..', '...-+.......+...', '+-......'),
    ('......+.', '..-......+-...-.', '..-...-.'),
    ('-.......', '++......+...+...', '-...-...'),
    ('-....-.+', '............+...', '.+.-+...'),
    ('.-+..+-.', '......+.........', '.....++.'),
    ('.-......', '...+--.-.-..-...', '.+......'),
    ('...-.-.+', '...+...-.....+..', '.-.+...+'),
    ('....--..', '.+..............', '+-..+-..'),
    ('...+...-', '...+...-......+-', '.......+'),
    ('...-..+.', '...........-..-.', '..+....-'),
    ('.-+...-.', '......-..-......', '..+..++.'),
    ('......+-', '..............+.', '......--'),
    ('.....-.+', '.............+..', '.+.-.+.-'),
)

_BASE = dict(lag=8, stride=4, q_end=70, e0=(45, 85), e1=(0, 100), s_end=60, s_due=(10, -1), p_due=True,
             g_at=2, g=(50, 90), u_at=3, u_end=30, out_split=False)
TUNE = {
    'seq0': dict(_BASE, q_end=30, e0=(30, 92), s_due=(5, 10), u_at=0, u_end=60),
    'seq1': _BASE,
    'last': dict(_BASE, lag=10, e1=(20, 80), p_due=False, out_split=True),
}

class _Forms:
    def __init__(self, rows):
        self.n = len(rows[0])
        forms = [{j: 1 if ch == '+' else -1 for j, ch in enumerate(r) if ch != '.'} for r in rows]
        self.steps = []
        while True:
            count = {}
            seen = set()
            for f in forms:
                items = sorted(f.items())
                key = tuple((j, v * items[0][1]) for j, v in items)
                if key not in seen:
                    seen.add(key)
                    for a in range(len(items)):
                        for b in range(a + 1, len(items)):
                            pair = (items[a][0], items[b][0], items[a][1] * items[b][1])
                            count[pair] = count.get(pair, 0) + 1
            if not count:
                break
            j, k, sg = max(count, key=count.get)
            new = self.n + len(self.steps)
            self.steps.append((j, k, sg))
            for f in forms:
                if j in f and k in f and f[j] * f[k] == sg:
                    f[new] = f.pop(j)
                    f.pop(k)
        self.node = [next(iter(f)) for f in forms]
        self.sign = [next(iter(f.values())) for f in forms]

    def expand(self, blocks):
        nodes = list(blocks)
        for j, k, sg in self.steps:
            nodes.append(nodes[j] + nodes[k] if sg > 0 else nodes[j] - nodes[k])
        return [nodes[i] for i in self.node]

    def contract(self, prods, signs, order):
        acc = {}

        def add(i, v, s):
            if i not in acc:
                acc[i] = (v, s)
            else:
                w, t = acc[i]
                acc[i] = (w + v, s) if s == t else ((w - v, 1) if t > 0 else (v - w, 1))

        for r in order:
            if self.node[r] >= self.n:
                add(self.node[r], prods[r], self.sign[r] * signs[r])
        for i in reversed(range(len(self.steps))):
            j, k, sg = self.steps[i]
            v, s = acc[self.n + i]
            add(j, v, s)
            add(k, v, s * sg)
        for r in order:
            if self.node[r] < self.n:
                add(self.node[r], prods[r], self.sign[r] * signs[r])
        return [acc[j][0] if acc[j][1] > 0 else -acc[j][0] for j in range(self.n)]


FU, FV, FW = (_Forms([t[i] for t in SCHEME]) for i in range(3))
NPROD = len(SCHEME)
TABLED = [r for r in range(NPROD) if FV.node[r] >= FV.n]


def _ln(x, eps):
    d = x.shape[-1]
    m = jnp.sum(x, axis=-1, keepdims=True) * (1.0 / d)
    xc = x - m
    v = jnp.sum(xc * xc, axis=-1, keepdims=True) * (1.0 / d)
    return xc * lax.rsqrt(v + eps)


def _gelu2(x):
    c1 = math.sqrt(2.0 / math.pi)
    c2 = c1 * 0.044715
    t = jnp.tanh(x * (c1 + c2 * (x * x)))
    return x + x * t


def _center(w):
    return w - jnp.sum(w, axis=0, keepdims=True) * (1.0 / w.shape[0])


def _pack(x):
    return pltpu.bitcast(x.astype(BF16), U32)


def _unpack(x):
    return pltpu.bitcast(x, BF16)


def _bits(x):
    return pltpu.bitcast(x, U32)


def _to_bf16(v):
    return _unpack(v) if v.dtype == U32 else v.astype(BF16)


def _dot(a, b):
    return jnp.dot(a, b, preferred_element_type=F32)


def _dot_nt(a, b):
    return lax.dot_general(a, b, NT, preferred_element_type=F32)


def _split(v):
    return [v[:, c * LANES:(c + 1) * LANES] for c in range(v.shape[1] // LANES)]


def _aligned(i, n):
    return i if isinstance(i, int) else pl.multiple_of(i, n)


def _tie_bf16(flag, dep, val):
    head = _bits(val[0:16, 0:LANES])
    head = _unpack(jnp.where(flag, _bits(dep), head))
    top = jnp.concatenate([head, val[0:16, LANES:]], axis=1)
    return jnp.concatenate([top, val[16:, :]], axis=0)


def _tie(flag, deps, val, row):
    cast = _bits if val.dtype == U32 else (lambda v: v if v.dtype == F32 else pltpu.bitcast(v, F32))
    tiles = _split(val)
    t = tiles[0]
    end = row + 8 * len(deps)
    mid = jnp.where(flag, jnp.concatenate([cast(d) for d in deps], axis=0), t[row:end])
    tiles[0] = jnp.concatenate(([t[0:row]] if row else []) + [mid] + ([t[end:]] if end < t.shape[0] else []),
                               axis=0)
    return jnp.concatenate(tiles, axis=1)


def _released(flag, toks, lo, hi, val, ntiles=1):
    first, total = len(toks) * lo // 100, len(toks) * (hi - lo) // 100
    n = val.shape[0] // 8
    rel = jnp.concatenate([toks[min(first + (i * total) // n, len(toks) - 1)] for i in range(n)], axis=0)
    tiles = _split(val)
    return jnp.concatenate([jnp.where(flag, rel, t) if c < ntiles else t for c, t in enumerate(tiles)], axis=1)


def _kernel(x_hbm, wq_hbm, wk_hbm, wv_hbm, wao_hbm, wup_hbm, dw_hbm, wdn_hbm, wm_hbm,
            o_hbm,
            x_s, wq_s, wk_s, wv_s, wao_s, wup_s, dw_s, wdn_s, wm_s, sems,
            xa0_s, xa1_s, wa_s, dwb_s, s_s, m_s, u_s, g_s, gn_s, o_s, osems,
            tb0_s, tb1_s, wt_s, po_s, xo_s, qo_s, z_s,
            *, B, T, D, K, TQ, TK, TP, UR):
    NQ = T // TQ
    N = B * NQ
    NKV = TP // TK
    NC = D // LANES
    CPK = TK // LANES
    PAD = K // 2
    NQT = -(-TQ // LANES)
    NFULL = (T - (NKV - 1) * TK) // LANES
    TAIL = T % LANES
    HR = TQ // 2
    TR = LANES // H
    G = 4
    NU = TP // UR
    UP = UR // CPK
    UT = UP // H
    ORDER = sorted(range(NPROD), key=lambda r: (FW.node[r] < FW.n, FU.node[r]))
    PORDER = sorted(range(NPROD), key=lambda r: FU.node[r] < FU.n)
    SUV = [FU.sign[r] * FV.sign[r] for r in range(NPROD)]
    SWV = [FW.sign[r] * FV.sign[r] for r in range(NPROD)]
    xa_s, tb_s = (xa0_s, xa1_s), (tb0_s, tb1_s)

    def blocks_of(a):
        return [a[h * HR:(h + 1) * HR, c * LANES:(c + 1) * LANES] for h in range(2) for c in range(NC)]

    def unblock(bl):
        return jnp.concatenate([jnp.concatenate(bl[h * NC:(h + 1) * NC], axis=1) for h in range(2)], axis=0)

    def key_tables(y):
        n = y.shape[0] // CPK
        ops = FV.expand([y[t * n:(t + 1) * n, d * LANES:(d + 1) * LANES] for d in range(NC) for t in range(CPK)])
        return _pack(jnp.concatenate([ops[r] for r in TABLED], axis=1))

    def weight_tables(mat, w):
        ops = FV.expand([w[d * LANES:(d + 1) * LANES, t * LANES:(t + 1) * LANES]
                         for d in range(NC) for t in range(NC)])
        wt_s[mat * TR:(mat + 1) * TR, :] = _pack(jnp.concatenate(ops, axis=1))

    def fence(ref):
        return ref[pl.ds(pl.multiple_of(z_s[0], 8), 8), 0:LANES]

    def staged_operands(ref, a, which):
        ops = FU.expand(blocks_of(a))
        ref[:, 0:len(which) * LANES] = _pack(jnp.concatenate([ops[r] for r in which], axis=1))
        done = fence(ref)
        return {r: ref[:, k * LANES:(k + 1) * LANES] for k, r in enumerate(which)}, done

    def key_operand(b, g, r):
        i = FV.node[r]
        if i < FV.n:
            d, t = i // CPK, i % CPK
            parts = [xa_s[b][pl.ds((j * TK + t * LANES) // H, TR), d * LANES:(d + 1) * LANES]
                     for j in range(g * G, (g + 1) * G)]
        else:
            k = TABLED.index(r)
            parts = [tb_s[b][j * TR:(j + 1) * TR, k * LANES:(k + 1) * LANES] for j in range(g * G, (g + 1) * G)]
        return _unpack(jnp.concatenate(parts, axis=0))

    def store_g(ref, row, g):
        for c in range(NC):
            ref[c, row:row + g.shape[0], :] = g[:, c * LANES:(c + 1) * LANES]

    def conv(flag):
        prev = None
        rows = []
        for rr in range(0, TQ, 16):
            cols = []
            for c in range(NC):
                acc = None
                for k in range(K):
                    gv = g_s[c, pl.ds(rr + HALO - PAD + k, 16), :].reshape(2, 8, LANES)
                    term = gv * dwb_s[k, :, c * LANES:(c + 1) * LANES][None]
                    if acc is None:
                        acc = term if prev is None else jnp.where(flag, prev, term)
                    else:
                        acc = acc + term
                prev = acc
                cols.append(acc.reshape(16, LANES))
            rows.append(jnp.concatenate(cols, axis=1))
        return jnp.concatenate(rows, axis=0)

    def store_max(mx):
        m = jnp.max(mx, axis=-1, keepdims=True)
        m = m + jnp.log2(jnp.sum(jnp.exp2(mx - m), axis=-1, keepdims=True))
        m_s[...] = jnp.broadcast_to(m, (TQ, LANES))

    def rest_copy():
        return pltpu.make_async_copy(x_hbm.at[pl.ds(T + TK, T - TK), :], x_s.at[pl.ds(TP + TK, T - TK), :],
                                     sems.at[13])

    def out_copy(blk):
        return pltpu.make_async_copy(o_s.at[blk % 2], o_hbm.at[pl.ds(_aligned(blk * TQ, 16), TQ), :],
                                     osems.at[blk % 2])

    def first_step():
        C1, C2 = 4, 6

        def xrows(b, r0, r1):
            return x_hbm.at[pl.ds(b * T + r0, r1 - r0), :], x_s.at[pl.ds(b * TP + r0, r1 - r0), :]

        copies = {}
        plan = (
            ('wq', wq_hbm, wq_s), ('wk', wk_hbm, wk_s),
            ('xa',) + xrows(0, 0, TK), ('xb',) + xrows(0, TK, C1 * TK), ('xc',) + xrows(0, C1 * TK, C2 * TK),
            ('xd',) + xrows(0, C2 * TK, T), ('wv', wv_hbm, wv_s), ('wao', wao_hbm, wao_s),
            ('wup', wup_hbm, wup_s), ('dw', dw_hbm, dw_s), ('wdn', wdn_hbm, wdn_s), ('wm', wm_hbm, wm_s),
            ('xe',) + xrows(1, 0, TK),
        )
        for i, (name, src, dst) in enumerate(plan):
            copies[name] = pltpu.make_async_copy(src, dst, sems.at[i])
            copies[name].start()
        rest_copy().start()

        z_s[0] = 0
        z_s[1] = 0
        z_s[2] = 0
        for b in range(B):
            x_s[b * TP + T:(b + 1) * TP, :] = jnp.zeros((TP - T, D), x_s.dtype)
        store_g(g_s, TQ, jnp.zeros((HALO, D), F32))

        def keys(r0, n):
            return _unpack(xa0_s[r0 // H:(r0 + n) // H, :])

        def ln_chunk(c):
            y = _ln(x_s[c * TK:(c + 1) * TK, :].astype(F32), EPS)
            xa0_s[c * TK // H:(c + 1) * TK // H, :] = _pack(y)
            tb0_s[c * TR:(c + 1) * TR, :] = key_tables(y)

        scale = float(D) ** (-0.5) * math.log2(math.e)
        DS = D // 2
        copies['wq'].wait()
        copies['wk'].wait()
        m_lo = _dot_nt(wq_s[...], wk_s[0:DS, :])

        never = z_s[0] > 0
        zero = pl.multiple_of(z_s[0], 8)

        def after(prev, l):
            return _unpack(l if prev is None else _tie(never, [prev[0:8, 0:LANES]], l, 0))

        copies['xa'].wait()
        wa_s[:, 0:DS] = _pack(_center(m_lo) * scale)
        wa_s[:, DS:D] = _pack(_center(_dot_nt(wq_s[...], wk_s[DS:D, :])) * scale)
        ln_chunk(0)
        qp = _pack(_dot(keys(0, TQ), _unpack(wa_s[:, 0:D])))
        q = _unpack(qp)

        def tail_parts():
            kt = keys(T - TAIL, TAIL)
            parts = []
            for n in range(NQT):
                qn = q[n * LANES:min((n + 1) * LANES, TQ), :]
                if qn.shape[0] < LANES:
                    qn = jnp.concatenate([qn, jnp.zeros((LANES - qn.shape[0], D), BF16)], axis=0)
                parts.append(_dot_nt(kt, qn))
            return parts

        def logits(c, prev, mx):
            last = c == NKV - 1
            parts = tail_parts() if last else None
            s = _dot_nt(after(prev, qp), keys(c * TK, (NFULL if last else CPK) * LANES))
            mc = None
            for t in range(CPK):
                if last and t == NFULL:
                    fill = jnp.full((LANES - TAIL, LANES), -jnp.inf, F32)
                    st = jnp.concatenate([jnp.concatenate([p, fill], axis=0).T for p in parts], axis=0)[0:TQ, :]
                else:
                    st = s[:, t * LANES:(t + 1) * LANES]
                s_s[c, :, t * LANES:(t + 1) * LANES] = st
                mc = st if mc is None else jnp.maximum(mc, st)
            return s, mc if mx is None else jnp.maximum(mx, mc)

        copies['xb'].wait()
        prev, mx = logits(0, None, None)
        for c in range(1, C1):
            ln_chunk(c)
            prev, mx = logits(c, prev, mx)

        copies['xc'].wait()
        prev = None
        for c in range(C1, C2):
            ln_chunk(c)
            prev, mx = logits(c, prev, mx)

        for name in ('xd', 'wv', 'wao'):
            copies[name].wait()
        wva_raw = _dot(wv_s[...], wao_s[...])
        mean = jnp.sum(wva_raw, axis=0, keepdims=True) * (1.0 / D)
        prev = wva_raw
        for c in range(C2, NKV):
            ln_chunk(c)
            prev, mx = logits(c, prev, mx)

        for name in ('wup', 'dw'):
            copies[name].wait()
        store_max(mx)
        xq = xa0_s[0:TQ // H, :]
        hg = _dot(after(None, xq), wup_s[:, D:2 * D])
        hu = _dot(after(hg, xq), wup_s[:, 0:D])
        dwf = dw_s[...].astype(F32)
        for k in range(K):
            dwb_s[k] = jnp.broadcast_to(dwf[k:k + 1, :], (8, D))
        wva = (wva_raw - mean).astype(BF16)

        def tokens(res):
            return [res[r:r + 8, c * LANES:(c + 1) * LANES] for c in range(NC) for r in range(0, D, 8)]

        for name in ('wdn', 'wm'):
            copies[name].wait()
        wvom = _dot(wva, wm_s[0:D, :])
        t1 = tokens(wvom)
        store_g(gn_s, 0, _ln(_gelu2(_released(never, t1, 0, 40, hg, NC)), 4.0 * EPS))
        u_s[...] = _gelu2(_released(never, t1, 0, 40, hu, NC))
        weight_tables(0, _released(never, t1, 0, 90, _unpack(wa_s[:, 0:D]).astype(F32), NC))
        weight_tables(1, _released(never, t1, 0, 90, wup_s[:, D:2 * D].astype(F32), NC))
        weight_tables(2, _released(never, t1, 30, 90, wup_s[:, 0:D].astype(F32), NC))
        wdn = wdn_s[...]
        deps = [wvom[0:8, LANES:2 * LANES], gn_s[0, pl.ds(zero, 8), :], u_s[pl.ds(zero, 8), 0:LANES],
                wt_s[pl.ds(zero, 8), 0:LANES]]
        for i, dep in enumerate(deps):
            wdn = jnp.concatenate(([wdn[0:16 * i]] if i else []) + [_tie_bf16(never, dep, wdn[16 * i:])], axis=0)
        wdm = _dot(wdn, wm_s[D:2 * D, :])
        weight_tables(3, _released(never, tokens(wdm), 0, 50, wvom, NC))
        weight_tables(4, 0.5 * wdm)
        copies['xe'].wait()

    def step_body(step, ba, bb, tune, normalise=False, do_a=True):
        sb = step - 1
        ia, ib = step - ba * NQ, sb - bb * NQ
        never = z_s[0] > 0
        never2 = z_s[1] > 0
        never3 = z_s[2] > 0
        for c in range(NC):
            g_s[c, 0:HALO, :] = jnp.where(ib == 0, 0.0, g_s[c, TQ:TQ + HALO, :])
            g_s[c, HALO:HALO + TQ, :] = gn_s[c]
        hist = []
        pend = []
        later = []

        def matmul(l, tiles, run):
            back = 0
            for res, n in reversed(hist):
                back += n
                if back >= tune['lag']:
                    l = _tie(never3, [res[0:8, 0:LANES]], l, 0)
                    break
            while later and later[0][0] <= len(hist) and len(pend) < 4:
                pend.append(later.pop(0)[1])
            if pend:
                l = _tie(never3, pend, l, 8)
                del pend[:]
            hist.append((run(_to_bf16(l)), tiles))
            return hist[-1][0]

        def toks(i0):
            return [res[r:r + 8, 0:LANES] for res, n in hist[i0:] for r in range(0, HR, 8 * (4 // n))]

        def rel2(v, t, lo, hi):
            return jnp.concatenate([_released(never, t, lo, hi, v[0:HR]), _released(never, t, lo, hi, v[HR:])],
                                   axis=0)

        def project(ops, mats, axis):
            m = [None] * NPROD
            for r in ORDER:
                m[r] = matmul(ops[r], len(mats), lambda v, r=r: _dot(v, _unpack(jnp.concatenate(
                    [wt_s[k * TR:(k + 1) * TR, r * LANES:(r + 1) * LANES] for k in mats], axis=axis))))
            return m

        def combine(prods, t=None, lo=0, hi=0):
            if t is not None:
                prods = list(prods)
                for r in ORDER[::tune['stride']]:
                    prods[r] = _released(never, t, lo, hi, prods[r])
            return unblock(FW.contract(prods, SUV, ORDER))

        m_old = m_s[...]
        u_old = u_s[...]
        if do_a:
            xq = xa_s[ba][pl.ds(_aligned(ia * (TQ // H), 8), TQ // H), :]
            xops, _ = staged_operands(xo_s, _unpack(xq).astype(F32),
                                      [r for r in range(NPROD) if FU.node[r] >= FU.n])
            for r in range(NPROD):
                i = FU.node[r]
                if i < FU.n:
                    xops[r] = xq[(i // NC) * HR // H:(i // NC + 1) * HR // H, (i % NC) * LANES:(i % NC + 1) * LANES]
            qm = project(xops, [0], 1)
            gm = project(xops, [1, 2], 1)
            q_raw = combine(qm, toks(NPROD), 0, tune['q_end'])
            qops, done = staged_operands(qo_s, q_raw, list(range(NPROD)))
            pend.append(done)
        else:
            store_g(g_s, HALO + TQ, jnp.zeros((HALO, D), F32))
        state = {'l': None, 'acc': None, 'mx': None}

        def probabilities(g, t, lo, hi):
            for jj in range(G):
                j = g * G + jj
                m = m_old if t is None else rel2(m_old, t, lo + (hi - lo) * jj // G, lo + (hi - lo) * (jj + 1) // G)
                tiles = []
                lsum = None
                for c in range(CPK):
                    p = jnp.exp2(s_s[j, :, c * LANES:(c + 1) * LANES] - m)
                    lsum = p if lsum is None else lsum + p
                    tiles.append(p)
                state['l'] = lsum if state['l'] is None else state['l'] + lsum
                tiles[0] = jnp.where(never2, state['l'], tiles[0])
                w = jnp.concatenate(FW.expand(blocks_of(jnp.concatenate(tiles, axis=1))), axis=1)
                po_s[j * HR // H:(j + 1) * HR // H, :] = _pack(w)
            return fence(po_s)

        def store_logits(g, m, t):
            for jj in range(G):
                j = g * G + jj
                s = combine([v[:, jj * LANES:(jj + 1) * LANES] for v in m], t,
                            tune['s_end'] * jj // G, tune['s_end'] * (jj + 1) // G)
                for c, st in enumerate(_split(s)):
                    if j == NKV - 1 and c == NFULL:
                        st = jnp.where(lax.broadcasted_iota(jnp.int32, st.shape, 1) < TAIL, st, -jnp.inf)
                    s_s[j, :, c * LANES:(c + 1) * LANES] = st
                    state['mx'] = st if state['mx'] is None else jnp.maximum(state['mx'], st)

        def side_work(phase, t):
            if phase == tune['g_at']:
                gg = _gelu2(combine([v[:, 0:LANES] for v in gm], t, 0, tune['g'][0]))
                g_new = _ln(rel2(gg, t, *tune['g']), 4.0 * EPS)
                store_g(gn_s, 0, g_new)
                store_g(g_s, HALO + TQ, jnp.where(ia == 0, 0.0, g_new[0:HALO, :]))
            if phase == tune['u_at']:
                u_s[...] = _gelu2(combine([v[:, LANES:] for v in gm], t, 0, tune['u_end']))
            if phase == 3 and normalise:
                unit = jnp.minimum(step - 1, NU - 1)
                c0, h = unit // (TK // UR), unit % (TK // UR)
                xv = [x_s[pl.ds(pl.multiple_of(TP + c0 * TK + k * LANES + h * UP, 16), UP), :].astype(F32)
                      for k in range(CPK)]
                y = _ln(jnp.concatenate([_released(never, t, 50, 80, v) for v in xv], axis=0), EPS)
                for k in range(CPK):
                    row = pl.multiple_of((c0 * TK + k * LANES) // H + h * UT, 8)
                    xa1_s[pl.ds(row, UT), :] = _pack(y[k * UP:(k + 1) * UP])
                tb1_s[pl.ds(pl.multiple_of(c0 * TR + h * UT, 8), UT), :] = key_tables(y)

        ready = None
        for g in range(NKV // G):
            if do_a:
                start = len(hist)
                sm = [None] * NPROD
                for r in ORDER:
                    sm[r] = matmul(qops[r], G, lambda v, r=r: _dot_nt(v, key_operand(ba, g, r)))
            if g == 0:
                ready = probabilities(0, toks(0) if do_a else None, *tune['e0'])
            if do_a:
                side_work(2 * g, toks(start))
            if tune['p_due']:
                pend.append(ready)
            start = len(hist)
            n = [None] * NPROD
            for r in PORDER:
                l = jnp.concatenate([po_s[j * HR // H:(j + 1) * HR // H, r * LANES:(r + 1) * LANES]
                                     for j in range(g * G, (g + 1) * G)], axis=1)
                n[r] = matmul(l, G, lambda v, r=r: _dot(v, key_operand(bb, g, r)))
            state['acc'] = n if state['acc'] is None else [x + y for x, y in zip(state['acc'], n)]
            t = toks(start)
            if do_a:
                store_logits(g, sm, t)
                if tune['s_due'][g] >= 0:
                    later.extend((len(hist) + tune['s_due'][g], state['mx'][r:r + 8]) for r in range(0, TQ, 8))
            if (g + 1) * G < NKV:
                ready = probabilities(g + 1, t, *tune['e1'])
            if do_a:
                side_work(2 * g + 1, t)
        yc = u_old * conv(never)
        ya = unblock(FU.contract(state['acc'], SWV, PORDER)) * (1.0 / jnp.sum(state['l'], axis=-1, keepdims=True))
        if tune['out_split']:
            om = project(FU.expand(blocks_of(yc)), [4], 0)
            om = [x + y for x, y in zip(om, project(FU.expand(blocks_of(ya)), [3], 0))]
        else:
            om = project([jnp.concatenate(p, axis=1)
                          for p in zip(FU.expand(blocks_of(ya)), FU.expand(blocks_of(yc)))], [3, 4], 0)
        out = combine(om)
        xr = x_s[pl.ds(_aligned(bb * TP + ib * TQ, 16), TQ), :].astype(F32)
        o_s[sb % 2] = (xr + out).astype(o_s.dtype)
        if do_a:
            store_max(state['mx'])
        out_copy(sb).start()

    def iteration0(step, carry):
        step_body(step, 0, 0, TUNE['seq0'], normalise=True)

        @pl.when(step >= 2)
        def _():
            out_copy(step - 2).wait()

        @pl.when(step == 1)
        def _():
            rest_copy().wait()

        return carry

    def iteration1(step, carry):
        step_body(step, 1, 1, TUNE['seq1'])
        out_copy(step - 2).wait()
        return carry

    first_step()
    lax.fori_loop(1, NQ, iteration0, 0)
    step_body(NQ + z_s[0], 1, 0, TUNE['seq1'])
    out_copy(NQ - 2).wait()
    lax.fori_loop(NQ + 1, N, iteration1, 0)
    step_body(N, 1, 1, TUNE['last'], do_a=False)
    out_copy(N - 2).wait()
    out_copy(N - 1).wait()


@jax.jit
def pallas_standalone__conformer_family_branchformer__speech_kernel(
    x: jax.Array,
    w_q: jax.Array,
    w_k: jax.Array,
    w_v: jax.Array,
    w_ao: jax.Array,
    w_up: jax.Array,
    dw: jax.Array,
    w_dn: jax.Array,
    w_merge: jax.Array,
):
    B, T, D = x.shape
    K = dw.shape[0]
    TQ = 160
    TK = 512
    TP = -(-T // TK) * TK
    UR = 256
    NKV = TP // TK
    assert B == 2 and T % TQ == 0 and TQ % 32 == 0 and D == TK == 4 * LANES and K // 2 < HALO
    assert TP // UR < T // TQ and NKV == 8 and T % LANES in (16, 32, 48, 64) and TP - T < LANES
    x2 = x.reshape(B * T, D)

    kern = functools.partial(_kernel, B=B, T=T, D=D, K=K, TQ=TQ, TK=TK, TP=TP, UR=UR)
    ins = (x2, w_q, w_k, w_v, w_ao, w_up, dw, w_dn, w_merge)
    out = pl.pallas_call(
        kern,
        in_specs=[pl.BlockSpec(memory_space=pl.ANY) for _ in ins],
        out_specs=pl.BlockSpec(memory_space=pl.ANY),
        out_shape=jax.ShapeDtypeStruct((B * T, D), x.dtype),
        scratch_shapes=[pltpu.VMEM((B * TP, D), x.dtype)] + [pltpu.VMEM(a.shape, a.dtype) for a in ins[1:]] + [
            pltpu.SemaphoreType.DMA((14,)),
            pltpu.VMEM((TP // H, D), U32),
            pltpu.VMEM((TP // H, D), U32),
            pltpu.VMEM((D // H, D), U32),
            pltpu.VMEM((K, 8, D), F32),
            pltpu.VMEM((NKV, TQ, TK), F32),
            pltpu.VMEM((TQ, LANES), F32),
            pltpu.VMEM((TQ, D), F32),
            pltpu.VMEM((D // LANES, TQ + 2 * HALO, LANES), F32),
            pltpu.VMEM((D // LANES, TQ, LANES), F32),
            pltpu.VMEM((2, TQ, D), x.dtype),
            pltpu.SemaphoreType.DMA((2,)),
            pltpu.VMEM((NKV * LANES // H, len(TABLED) * LANES), U32),
            pltpu.VMEM((NKV * LANES // H, len(TABLED) * LANES), U32),
            pltpu.VMEM((5 * LANES // H, NPROD * LANES), U32),
            pltpu.VMEM((NKV * TQ // 2 // H, NPROD * LANES), U32),
            pltpu.VMEM((TQ // 2 // H, NPROD * LANES), U32),
            pltpu.VMEM((TQ // 2 // H, NPROD * LANES), U32),
            pltpu.SMEM((3,), jnp.int32),
        ],
        compiler_params=pltpu.CompilerParams(
            vmem_limit_bytes=100 * 1024 * 1024,
            disable_bounds_checks=True,
            disable_semaphore_checks=True,
        ),
    )(*ins)
    return out.reshape(B, T, D)
```

```python
import functools
import math

import jax
import jax.numpy as jnp
from jax import lax
import jax.experimental.pallas as pl
import jax.experimental.pallas.tpu as pltpu

LANES = 128
EPS = 1e-05
F32 = jnp.float32
BF16 = jnp.bfloat16
U32 = jnp.uint32
NT = (((1,), (1,)), ((), ()))
HALO = 16
H = 2

SCHEME = (
    ('...-++..', '...+............', '-+.....+'),
    ('.+-.....', '.........-......', '.++..++.'),
    ('+...--..', '.+..+.......+...', '-+..-...'),
    ('.+.-.-.+', '...-...+....+...', '.-.+....'),
    ('.....+..', '.+...-+......-..', '.....-..'),
    ('+...-...', '+.-.-.......-...', '....-...'),
    ('--.+....', '...-........+...', '+-.+....'),
    ('..+...-.', '......+.-.+-....', '..+.....'),
    ('..-+....', '...........+....', '..--....'),
    ('-.....+.', '..+.....+.......', '..-.+...'),
    ('....+.-.', '..+.............', '....+.+.'),
    ('+.-.....', '........+.......', '-.-.....'),
    ('...-....', '...-.......-.-.-', '...+...+'),
    ('++..--..', '...-+.......+...', '+-......'),
    ('......+.', '..-......+-...-.', '..-...-.'),
    ('-.......', '++......+...+...', '-...-...'),
    ('-....-.+', '............+...', '.+.-+...'),
    ('.-+..+-.', '......+.........', '.....++.'),
    ('.-......', '...+--.-.-..-...', '.+......'),
    ('...-.-.+', '...+...-.....+..', '.-.+...+'),
    ('....--..', '.+..............', '+-..+-..'),
    ('...+...-', '...+...-......+-', '.......+'),
    ('...-..+.', '...........-..-.', '..+....-'),
    ('.-+...-.', '......-..-......', '..+..++.'),
    ('......+-', '..............+.', '......--'),
    ('.....-.+', '.............+..', '.+.-.+.-'),
)

_BASE = dict(lag=8, stride=3, q_end=60, e0=(45, 85), e1=(0, 100), s_end=60, s_due=(5, 10), p_due=True,
             g_at=2, g=(50, 90), u_at=3, u_end=20, out_split=False)
TUNE = {
    'seq0': dict(_BASE, stride=4, q_end=50, e0=(30, 92), e1=(10, 100), s_due=(5, 10), u_at=0, u_end=60),
    'seq1': _BASE,
    'last': dict(_BASE, lag=10, e1=(20, 80), p_due=False, out_split=True),
}


class _Forms:
    def __init__(self, rows):
        self.n = len(rows[0])
        forms = [{j: 1 if ch == '+' else -1 for j, ch in enumerate(r) if ch != '.'} for r in rows]
        self.steps = []
        while True:
            count = {}
            seen = set()
            for f in forms:
                items = sorted(f.items())
                key = tuple((j, v * items[0][1]) for j, v in items)
                if key not in seen:
                    seen.add(key)
                    for a in range(len(items)):
                        for b in range(a + 1, len(items)):
                            pair = (items[a][0], items[b][0], items[a][1] * items[b][1])
                            count[pair] = count.get(pair, 0) + 1
            if not count:
                break
            j, k, sg = max(count, key=count.get)
            new = self.n + len(self.steps)
            self.steps.append((j, k, sg))
            for f in forms:
                if j in f and k in f and f[j] * f[k] == sg:
                    f[new] = f.pop(j)
                    f.pop(k)
        self.node = [next(iter(f)) for f in forms]
        self.sign = [next(iter(f.values())) for f in forms]

    def expand(self, blocks):
        nodes = list(blocks)
        for j, k, sg in self.steps:
            nodes.append(nodes[j] + nodes[k] if sg > 0 else nodes[j] - nodes[k])
        return [nodes[i] for i in self.node]

    def contract(self, prods, signs, order):
        acc = {}

        def add(i, v, s):
            if i not in acc:
                acc[i] = (v, s)
            else:
                w, t = acc[i]
                acc[i] = (w + v, s) if s == t else ((w - v, 1) if t > 0 else (v - w, 1))

        for r in order:
            if self.node[r] >= self.n:
                add(self.node[r], prods[r], self.sign[r] * signs[r])
        for i in reversed(range(len(self.steps))):
            j, k, sg = self.steps[i]
            v, s = acc[self.n + i]
            add(j, v, s)
            add(k, v, s * sg)
        for r in order:
            if self.node[r] < self.n:
                add(self.node[r], prods[r], self.sign[r] * signs[r])
        return [acc[j][0] if acc[j][1] > 0 else -acc[j][0] for j in range(self.n)]


FU, FV, FW = (_Forms([t[i] for t in SCHEME]) for i in range(3))
NPROD = len(SCHEME)
TABLED = [r for r in range(NPROD) if FV.node[r] >= FV.n]


def _ln(x, eps):
    d = x.shape[-1]
    m = jnp.sum(x, axis=-1, keepdims=True) * (1.0 / d)
    xc = x - m
    v = jnp.sum(xc * xc, axis=-1, keepdims=True) * (1.0 / d)
    return xc * lax.rsqrt(v + eps)


def _gelu2(x):
    c1 = math.sqrt(2.0 / math.pi)
    c2 = c1 * 0.044715
    t = jnp.tanh(x * (c1 + c2 * (x * x)))
    return x + x * t


def _center(w):
    return w - jnp.sum(w, axis=0, keepdims=True) * (1.0 / w.shape[0])


def _pack(x):
    return pltpu.bitcast(x.astype(BF16), U32)


def _unpack(x):
    return pltpu.bitcast(x, BF16)


def _bits(x):
    return pltpu.bitcast(x, U32)


def _to_bf16(v):
    return _unpack(v) if v.dtype == U32 else v.astype(BF16)


def _dot(a, b):
    return jnp.dot(a, b, preferred_element_type=F32)


def _dot_nt(a, b):
    return lax.dot_general(a, b, NT, preferred_element_type=F32)


def _split(v):
    return [v[:, c * LANES:(c + 1) * LANES] for c in range(v.shape[1] // LANES)]


def _aligned(i, n):
    return i if isinstance(i, int) else pl.multiple_of(i, n)


def _tie_bf16(flag, dep, val):
    head = _bits(val[0:16, 0:LANES])
    head = _unpack(jnp.where(flag, _bits(dep), head))
    top = jnp.concatenate([head, val[0:16, LANES:]], axis=1)
    return jnp.concatenate([top, val[16:, :]], axis=0)


def _tie(flag, deps, val, row):
    cast = _bits if val.dtype == U32 else (lambda v: v if v.dtype == F32 else pltpu.bitcast(v, F32))
    tiles = _split(val)
    t = tiles[0]
    end = row + 8 * len(deps)
    mid = jnp.where(flag, jnp.concatenate([cast(d) for d in deps], axis=0), t[row:end])
    tiles[0] = jnp.concatenate(([t[0:row]] if row else []) + [mid] + ([t[end:]] if end < t.shape[0] else []),
                               axis=0)
    return jnp.concatenate(tiles, axis=1)


def _released(flag, toks, lo, hi, val, ntiles=1):
    first, total = len(toks) * lo // 100, len(toks) * (hi - lo) // 100
    n = val.shape[0] // 8
    rel = jnp.concatenate([toks[min(first + (i * total) // n, len(toks) - 1)] for i in range(n)], axis=0)
    tiles = _split(val)
    return jnp.concatenate([jnp.where(flag, rel, t) if c < ntiles else t for c, t in enumerate(tiles)], axis=1)


def _kernel(x_hbm, wq_hbm, wk_hbm, wv_hbm, wao_hbm, wup_hbm, dw_hbm, wdn_hbm, wm_hbm,
            o_hbm,
            x_s, wq_s, wk_s, wv_s, wao_s, wup_s, dw_s, wdn_s, wm_s, sems,
            xa0_s, xa1_s, wa_s, dwb_s, s_s, m_s, u_s, g_s, gn_s, o_s, osems,
            tb0_s, tb1_s, wt_s, po_s, xo_s, qo_s, z_s,
            *, B, T, D, K, TQ, TK, TP, UR):
    NQ = T // TQ
    N = B * NQ
    NKV = TP // TK
    NC = D // LANES
    CPK = TK // LANES
    PAD = K // 2
    NQT = -(-TQ // LANES)
    NFULL = (T - (NKV - 1) * TK) // LANES
    TAIL = T % LANES
    HR = TQ // 2
    TR = LANES // H
    G = 4
    UP = UR // CPK
    UPC = -(-LANES // UP)
    NU = NKV * UPC
    UT = UP // H
    ORDER = [15, 12, 14, 10, 23, 18, 6, 17, 16, 1, 22, 0, 25, 2, 11, 3, 8, 13, 9, 19, 20, 24, 4, 5, 7, 21]
    PORDER = sorted(range(NPROD), key=lambda r: FU.node[r] < FU.n)
    SUV = [FU.sign[r] * FV.sign[r] for r in range(NPROD)]
    SWV = [FW.sign[r] * FV.sign[r] for r in range(NPROD)]
    xa_s, tb_s = (xa0_s, xa1_s), (tb0_s, tb1_s)

    def blocks_of(a):
        return [a[h * HR:(h + 1) * HR, c * LANES:(c + 1) * LANES] for h in range(2) for c in range(NC)]

    def unblock(bl):
        return jnp.concatenate([jnp.concatenate(bl[h * NC:(h + 1) * NC], axis=1) for h in range(2)], axis=0)

    def key_tables(y):
        n = y.shape[0] // CPK
        ops = FV.expand([y[t * n:(t + 1) * n, d * LANES:(d + 1) * LANES] for d in range(NC) for t in range(CPK)])
        return _pack(jnp.concatenate([ops[r] for r in TABLED], axis=1))

    def weight_tables(mat, w):
        ops = FV.expand([w[d * LANES:(d + 1) * LANES, t * LANES:(t + 1) * LANES]
                         for d in range(NC) for t in range(NC)])
        wt_s[mat * TR:(mat + 1) * TR, :] = _pack(jnp.concatenate(ops, axis=1))

    def fence(ref):
        return ref[pl.ds(pl.multiple_of(z_s[0], 8), 8), 0:LANES]

    def staged_operands(ref, a, which):
        ops = FU.expand(blocks_of(a))
        ref[:, 0:len(which) * LANES] = _pack(jnp.concatenate([ops[r] for r in which], axis=1))
        done = fence(ref)
        return {r: ref[:, k * LANES:(k + 1) * LANES] for k, r in enumerate(which)}, done

    def key_operand(b, g, r):
        i = FV.node[r]
        if i < FV.n:
            d, t = i // CPK, i % CPK
            parts = [xa_s[b][pl.ds((j * TK + t * LANES) // H, TR), d * LANES:(d + 1) * LANES]
                     for j in range(g * G, (g + 1) * G)]
        else:
            k = TABLED.index(r)
            parts = [tb_s[b][j * TR:(j + 1) * TR, k * LANES:(k + 1) * LANES] for j in range(g * G, (g + 1) * G)]
        return _unpack(jnp.concatenate(parts, axis=0))

    def store_g(ref, row, g):
        for c in range(NC):
            ref[c, row:row + g.shape[0], :] = g[:, c * LANES:(c + 1) * LANES]

    def conv(flag):
        prev = None
        rows = []
        for rr in range(0, TQ, 16):
            cols = []
            for c in range(NC):
                acc = None
                for k in range(K):
                    gv = g_s[c, pl.ds(rr + HALO - PAD + k, 16), :].reshape(2, 8, LANES)
                    term = gv * dwb_s[k, :, c * LANES:(c + 1) * LANES][None]
                    if acc is None:
                        acc = term if prev is None else jnp.where(flag, prev, term)
                    else:
                        acc = acc + term
                prev = acc
                cols.append(acc.reshape(16, LANES))
            rows.append(jnp.concatenate(cols, axis=1))
        return jnp.concatenate(rows, axis=0)

    def store_max(mx):
        m = jnp.max(mx, axis=-1, keepdims=True)
        m = m + jnp.log2(jnp.sum(jnp.exp2(mx - m), axis=-1, keepdims=True))
        m_s[...] = jnp.broadcast_to(m, (TQ, LANES))

    def rest_copy():
        return pltpu.make_async_copy(x_hbm.at[pl.ds(T + TK, T - TK), :], x_s.at[pl.ds(TP + TK, T - TK), :],
                                     sems.at[13])

    def out_copy(blk):
        return pltpu.make_async_copy(o_s.at[blk % 2], o_hbm.at[pl.ds(_aligned(blk * TQ, 16), TQ), :],
                                     osems.at[blk % 2])

    def first_step():
        C1, C2 = 3, 6

        def xrows(b, r0, r1):
            return x_hbm.at[pl.ds(b * T + r0, r1 - r0), :], x_s.at[pl.ds(b * TP + r0, r1 - r0), :]

        copies = {}
        plan = (
            ('wq', wq_hbm, wq_s), ('wk', wk_hbm, wk_s),
            ('xa',) + xrows(0, 0, TK), ('xb',) + xrows(0, TK, C1 * TK), ('xc',) + xrows(0, C1 * TK, C2 * TK),
            ('xd',) + xrows(0, C2 * TK, T), ('wv', wv_hbm, wv_s), ('wao', wao_hbm, wao_s),
            ('wup', wup_hbm, wup_s), ('dw', dw_hbm, dw_s), ('wdn', wdn_hbm, wdn_s), ('wm', wm_hbm, wm_s),
            ('xe',) + xrows(1, 0, TK),
        )
        for i, (name, src, dst) in enumerate(plan):
            copies[name] = pltpu.make_async_copy(src, dst, sems.at[i])
            copies[name].start()
        rest_copy().start()

        z_s[0] = 0
        z_s[1] = 0
        z_s[2] = 0
        for b in range(B):
            x_s[b * TP + T:(b + 1) * TP, :] = jnp.zeros((TP - T, D), x_s.dtype)
        store_g(g_s, TQ, jnp.zeros((HALO, D), F32))

        def keys(r0, n):
            return _unpack(xa0_s[r0 // H:(r0 + n) // H, :])

        def ln_chunk(c):
            y = _ln(x_s[c * TK:(c + 1) * TK, :].astype(F32), EPS)
            xa0_s[c * TK // H:(c + 1) * TK // H, :] = _pack(y)
            tb0_s[c * TR:(c + 1) * TR, :] = key_tables(y)

        scale = float(D) ** (-0.5) * math.log2(math.e)
        DS = D // 2
        copies['wq'].wait()
        copies['wk'].wait()
        m_lo = _dot_nt(wq_s[...], wk_s[0:DS, :])

        never = z_s[0] > 0
        zero = pl.multiple_of(z_s[0], 8)

        def after(prev, l):
            return _unpack(l if prev is None else _tie(never, [prev[0:8, 0:LANES]], l, 0))

        copies['xa'].wait()
        wa_s[:, 0:DS] = _pack(_center(m_lo) * scale)
        wa_s[:, DS:D] = _pack(_center(_dot_nt(wq_s[...], wk_s[DS:D, :])) * scale)
        ln_chunk(0)
        qp = _pack(_dot(keys(0, TQ), _unpack(wa_s[:, 0:D])))
        q = _unpack(qp)

        def tail_parts():
            kt = keys(T - TAIL, TAIL)
            parts = []
            for n in range(NQT):
                qn = q[n * LANES:min((n + 1) * LANES, TQ), :]
                if qn.shape[0] < LANES:
                    qn = jnp.concatenate([qn, jnp.zeros((LANES - qn.shape[0], D), BF16)], axis=0)
                parts.append(_dot_nt(kt, qn))
            return parts

        def logits(c, prev, mx):
            last = c == NKV - 1
            parts = tail_parts() if last else None
            s = _dot_nt(after(prev, qp), keys(c * TK, (NFULL if last else CPK) * LANES))
            mc = None
            for t in range(CPK):
                if last and t == NFULL:
                    fill = jnp.full((LANES - TAIL, LANES), -jnp.inf, F32)
                    st = jnp.concatenate([jnp.concatenate([p, fill], axis=0).T for p in parts], axis=0)[0:TQ, :]
                else:
                    st = s[:, t * LANES:(t + 1) * LANES]
                s_s[c, :, t * LANES:(t + 1) * LANES] = st
                mc = st if mc is None else jnp.maximum(mc, st)
            return s, mc if mx is None else jnp.maximum(mx, mc)

        copies['xb'].wait()
        prev, mx = logits(0, None, None)
        for c in range(1, C1):
            ln_chunk(c)
            prev, mx = logits(c, prev, mx)

        copies['xc'].wait()
        prev = None
        for c in range(C1, C2):
            ln_chunk(c)
            prev, mx = logits(c, prev, mx)

        for name in ('xd', 'wv', 'wao'):
            copies[name].wait()
        wva_raw = _dot(wv_s[...], wao_s[...])
        mean = jnp.sum(wva_raw, axis=0, keepdims=True) * (1.0 / D)
        prev = wva_raw
        for c in range(C2, NKV):
            ln_chunk(c)
            prev, mx = logits(c, prev, mx)

        for name in ('wup', 'dw'):
            copies[name].wait()
        store_max(mx)
        xq = xa0_s[0:TQ // H, :]
        hg = _dot(after(None, xq), wup_s[:, D:2 * D])
        hu = _dot(after(hg, xq), wup_s[:, 0:D])
        dwf = dw_s[...].astype(F32)
        for k in range(K):
            dwb_s[k] = jnp.broadcast_to(dwf[k:k + 1, :], (8, D))
        wva = (wva_raw - mean).astype(BF16)
        weight_tables(0, _unpack(wa_s[:, 0:D]).astype(F32))

        def tokens(res):
            return [res[r:r + 8, c * LANES:(c + 1) * LANES] for c in range(NC) for r in range(0, D, 8)]

        for name in ('wdn', 'wm'):
            copies[name].wait()
        wvom = _dot(wva, wm_s[0:D, :])
        t1 = tokens(wvom)
        store_g(gn_s, 0, _ln(_gelu2(_released(never, t1, 0, 40, hg, NC)), 4.0 * EPS))
        u_s[...] = _gelu2(_released(never, t1, 0, 40, hu, NC))
        weight_tables(1, _released(never, t1, 0, 90, wup_s[:, D:2 * D].astype(F32), NC))
        weight_tables(2, _released(never, t1, 30, 90, wup_s[:, 0:D].astype(F32), NC))
        wdn = wdn_s[...]
        deps = [wvom[0:8, LANES:2 * LANES], gn_s[0, pl.ds(zero, 8), :], u_s[pl.ds(zero, 8), 0:LANES],
                wt_s[pl.ds(zero, 8), 0:LANES]]
        for i, dep in enumerate(deps):
            wdn = jnp.concatenate(([wdn[0:16 * i]] if i else []) + [_tie_bf16(never, dep, wdn[16 * i:])], axis=0)
        wdm = _dot(wdn, wm_s[D:2 * D, :])
        weight_tables(3, _released(never, tokens(wdm), 0, 50, wvom, NC))
        weight_tables(4, 0.5 * wdm)
        copies['xe'].wait()

    def step_body(step, ba, bb, tune, normalise=False, do_a=True):
        sb = step - 1
        ia, ib = step - ba * NQ, sb - bb * NQ
        never = z_s[0] > 0
        never2 = z_s[1] > 0
        never3 = z_s[2] > 0
        for c in range(NC):
            g_s[c, 0:HALO, :] = jnp.where(ib == 0, 0.0, g_s[c, TQ:TQ + HALO, :])
            g_s[c, HALO:HALO + TQ, :] = gn_s[c]
        hist = []
        pend = []
        later = []

        def matmul(l, tiles, run):
            back = 0
            for res, n in reversed(hist):
                back += n
                if back >= tune['lag']:
                    l = _tie(never3, [res[0:8, 0:LANES]], l, 0)
                    break
            while later and later[0][0] <= len(hist) and len(pend) < 4:
                pend.append(later.pop(0)[1])
            if pend:
                l = _tie(never3, pend, l, 8)
                del pend[:]
            hist.append((run(_to_bf16(l)), tiles))
            return hist[-1][0]

        def toks(i0):
            return [res[r:r + 8, 0:LANES] for res, n in hist[i0:] for r in range(0, HR, 8 * (4 // n))]

        def rel2(v, t, lo, hi):
            return jnp.concatenate([_released(never, t, lo, hi, v[0:HR]), _released(never, t, lo, hi, v[HR:])],
                                   axis=0)

        def project(ops, mats, axis):
            m = [None] * NPROD
            for r in ORDER:
                m[r] = matmul(ops[r], len(mats), lambda v, r=r: _dot(v, _unpack(jnp.concatenate(
                    [wt_s[k * TR:(k + 1) * TR, r * LANES:(r + 1) * LANES] for k in mats], axis=axis))))
            return m

        def combine(prods, t=None, lo=0, hi=0):
            if t is not None:
                prods = list(prods)
                for r in ORDER[::tune['stride']]:
                    prods[r] = _released(never, t, lo, hi, prods[r])
            return unblock(FW.contract(prods, SUV, ORDER))

        m_old = m_s[...]
        u_old = u_s[...]
        if do_a:
            xq = xa_s[ba][pl.ds(_aligned(ia * (TQ // H), 8), TQ // H), :]
            xops, _ = staged_operands(xo_s, _unpack(xq).astype(F32),
                                      [r for r in range(NPROD) if FU.node[r] >= FU.n])
            for r in range(NPROD):
                i = FU.node[r]
                if i < FU.n:
                    xops[r] = xq[(i // NC) * HR // H:(i // NC + 1) * HR // H, (i % NC) * LANES:(i % NC + 1) * LANES]
            qm = project(xops, [0], 1)
            gm = project(xops, [1, 2], 1)
            q_raw = combine(qm, toks(NPROD), 0, tune['q_end'])
            qops, done = staged_operands(qo_s, q_raw, list(range(NPROD)))
            pend.append(done)
        else:
            store_g(g_s, HALO + TQ, jnp.zeros((HALO, D), F32))
        state = {'l': None, 'acc': None, 'mx': None}

        def probabilities(g, t, lo, hi):
            for jj in range(G):
                j = g * G + jj
                m = m_old if t is None else rel2(m_old, t, lo + (hi - lo) * jj // G, lo + (hi - lo) * (jj + 1) // G)
                tiles = []
                lsum = None
                for c in range(CPK):
                    p = jnp.exp2(s_s[j, :, c * LANES:(c + 1) * LANES] - m)
                    lsum = p if lsum is None else lsum + p
                    tiles.append(p)
                state['l'] = lsum if state['l'] is None else state['l'] + lsum
                tiles[0] = jnp.where(never2, state['l'], tiles[0])
                w = jnp.concatenate(FW.expand(blocks_of(jnp.concatenate(tiles, axis=1))), axis=1)
                po_s[j * HR // H:(j + 1) * HR // H, :] = _pack(w)
            return fence(po_s)

        def store_logits(g, m, t):
            for jj in range(G):
                j = g * G + jj
                s = combine([v[:, jj * LANES:(jj + 1) * LANES] for v in m], t,
                            tune['s_end'] * jj // G, tune['s_end'] * (jj + 1) // G)
                for c, st in enumerate(_split(s)):
                    if j == NKV - 1 and c == NFULL:
                        st = jnp.where(lax.broadcasted_iota(jnp.int32, st.shape, 1) < TAIL, st, -jnp.inf)
                    s_s[j, :, c * LANES:(c + 1) * LANES] = st
                    state['mx'] = st if state['mx'] is None else jnp.maximum(state['mx'], st)

        def side_work(phase, t):
            if phase == tune['g_at']:
                gg = _gelu2(combine([v[:, 0:LANES] for v in gm], t, 0, tune['g'][0]))
                g_new = _ln(rel2(gg, t, *tune['g']), 4.0 * EPS)
                store_g(gn_s, 0, g_new)
                store_g(g_s, HALO + TQ, jnp.where(ia == 0, 0.0, g_new[0:HALO, :]))
            if phase == tune['u_at']:
                u_s[...] = _gelu2(combine([v[:, LANES:] for v in gm], t, 0, tune['u_end']))
            if phase == 3 and normalise:
                unit = jnp.minimum(step - 1, NU - 1)
                c0, r0 = unit // UPC, jnp.minimum((unit % UPC) * UP, LANES - UP)
                xv = [x_s[pl.ds(pl.multiple_of(TP + c0 * TK + k * LANES + r0, 16), UP), :].astype(F32)
                      for k in range(CPK)]
                y = _ln(jnp.concatenate([_released(never, t, 50, 80, v) for v in xv], axis=0), EPS)
                for k in range(CPK):
                    row = pl.multiple_of((c0 * TK + k * LANES + r0) // H, 8)
                    xa1_s[pl.ds(row, UT), :] = _pack(y[k * UP:(k + 1) * UP])
                tb1_s[pl.ds(pl.multiple_of(c0 * TR + r0 // H, 8), UT), :] = key_tables(y)

        ready = None
        for g in range(NKV // G):
            if do_a:
                start = len(hist)
                sm = [None] * NPROD
                for r in ORDER:
                    sm[r] = matmul(qops[r], G, lambda v, r=r: _dot_nt(v, key_operand(ba, g, r)))
            if g == 0:
                ready = probabilities(0, toks(0) if do_a else None, *tune['e0'])
            if do_a:
                side_work(2 * g, toks(start))
            if tune['p_due']:
                pend.append(ready)
            start = len(hist)
            n = [None] * NPROD
            for r in PORDER:
                l = jnp.concatenate([po_s[j * HR // H:(j + 1) * HR // H, r * LANES:(r + 1) * LANES]
                                     for j in range(g * G, (g + 1) * G)], axis=1)
                n[r] = matmul(l, G, lambda v, r=r: _dot(v, key_operand(bb, g, r)))
            state['acc'] = n if state['acc'] is None else [x + y for x, y in zip(state['acc'], n)]
            t = toks(start)
            if do_a:
                store_logits(g, sm, t)
                if tune['s_due'][g] >= 0:
                    later.extend((len(hist) + tune['s_due'][g], state['mx'][r:r + 8]) for r in range(0, TQ, 8))
            if (g + 1) * G < NKV:
                ready = probabilities(g + 1, t, *tune['e1'])
            if do_a:
                side_work(2 * g + 1, t)
        yc = u_old * conv(never)
        ya = unblock(FU.contract(state['acc'], SWV, PORDER)) * (1.0 / jnp.sum(state['l'], axis=-1, keepdims=True))
        if tune['out_split']:
            om = project(FU.expand(blocks_of(yc)), [4], 0)
            om = [x + y for x, y in zip(om, project(FU.expand(blocks_of(ya)), [3], 0))]
        else:
            om = project([jnp.concatenate(p, axis=1)
                          for p in zip(FU.expand(blocks_of(ya)), FU.expand(blocks_of(yc)))], [3, 4], 0)
        out = combine(om)
        xr = x_s[pl.ds(_aligned(bb * TP + ib * TQ, 16), TQ), :].astype(F32)
        o_s[sb % 2] = (xr + out).astype(o_s.dtype)
        if do_a:
            store_max(state['mx'])
        out_copy(sb).start()

    def iteration0(step, carry):
        step_body(step, 0, 0, TUNE['seq0'], normalise=True)

        @pl.when(step >= 2)
        def _():
            out_copy(step - 2).wait()

        @pl.when(step == 1)
        def _():
            rest_copy().wait()

        return carry

    def iteration1(step, carry):
        step_body(step, 1, 1, TUNE['seq1'])
        out_copy(step - 2).wait()
        return carry

    first_step()
    lax.fori_loop(1, NQ, iteration0, 0)
    step_body(NQ + z_s[0], 1, 0, TUNE['seq1'])
    out_copy(NQ - 2).wait()
    lax.fori_loop(NQ + 1, N, iteration1, 0)
    step_body(N, 1, 1, TUNE['last'], do_a=False)
    out_copy(N - 2).wait()
    out_copy(N - 1).wait()


@jax.jit
def pallas_standalone__conformer_family_branchformer__speech_kernel(
    x: jax.Array,
    w_q: jax.Array,
    w_k: jax.Array,
    w_v: jax.Array,
    w_ao: jax.Array,
    w_up: jax.Array,
    dw: jax.Array,
    w_dn: jax.Array,
    w_merge: jax.Array,
):
    B, T, D = x.shape
    K = dw.shape[0]
    TQ = 160
    TK = 512
    TP = -(-T // TK) * TK
    UR = 192
    NKV = TP // TK
    assert B == 2 and T % TQ == 0 and TQ % 32 == 0 and D == TK == 4 * LANES and K // 2 < HALO
    assert NKV * -(-TK // UR) < T // TQ and UR % 64 == 0 and NKV == 8 and T % LANES in (16, 32, 48, 64) and TP - T < LANES
    x2 = x.reshape(B * T, D)

    kern = functools.partial(_kernel, B=B, T=T, D=D, K=K, TQ=TQ, TK=TK, TP=TP, UR=UR)
    ins = (x2, w_q, w_k, w_v, w_ao, w_up, dw, w_dn, w_merge)
    out = pl.pallas_call(
        kern,
        in_specs=[pl.BlockSpec(memory_space=pl.ANY) for _ in ins],
        out_specs=pl.BlockSpec(memory_space=pl.ANY),
        out_shape=jax.ShapeDtypeStruct((B * T, D), x.dtype),
        scratch_shapes=[pltpu.VMEM((B * TP, D), x.dtype)] + [pltpu.VMEM(a.shape, a.dtype) for a in ins[1:]] + [
            pltpu.SemaphoreType.DMA((14,)),
            pltpu.VMEM((TP // H, D), U32),
            pltpu.VMEM((TP // H, D), U32),
            pltpu.VMEM((D // H, D), U32),
            pltpu.VMEM((K, 8, D), F32),
            pltpu.VMEM((NKV, TQ, TK), F32),
            pltpu.VMEM((TQ, LANES), F32),
            pltpu.VMEM((TQ, D), F32),
            pltpu.VMEM((D // LANES, TQ + 2 * HALO, LANES), F32),
            pltpu.VMEM((D // LANES, TQ, LANES), F32),
            pltpu.VMEM((2, TQ, D), x.dtype),
            pltpu.SemaphoreType.DMA((2,)),
            pltpu.VMEM((NKV * LANES // H, len(TABLED) * LANES), U32),
            pltpu.VMEM((NKV * LANES // H, len(TABLED) * LANES), U32),
            pltpu.VMEM((5 * LANES // H, NPROD * LANES), U32),
            pltpu.VMEM((NKV * TQ // 2 // H, NPROD * LANES), U32),
            pltpu.VMEM((TQ // 2 // H, NPROD * LANES), U32),
            pltpu.VMEM((TQ // 2 // H, NPROD * LANES), U32),
            pltpu.SMEM((3,), jnp.int32),
        ],
        compiler_params=pltpu.CompilerParams(
            vmem_limit_bytes=100 * 1024 * 1024,
            disable_bounds_checks=True,
            disable_semaphore_checks=True,
        ),
    )(*ins)
    return out.reshape(B, T, D)
```

```python
import functools
import math

import jax
import jax.numpy as jnp
from jax import lax
import jax.experimental.pallas as pl
import jax.experimental.pallas.tpu as pltpu

LANES = 128
EPS = 1e-05
F32 = jnp.float32
BF16 = jnp.bfloat16
U32 = jnp.uint32
NT = (((1,), (1,)), ((), ()))
HALO = 16
H = 2

SCHEME = (
    ('...-++..', '...+............', '-+.....+'),
    ('.+-.....', '.........-......', '.++..++.'),
    ('+...--..', '.+..+.......+...', '-+..-...'),
    ('.+.-.-.+', '...-...+....+...', '.-.+....'),
    ('.....+..', '.+...-+......-..', '.....-..'),
    ('+...-...', '+.-.-.......-...', '....-...'),
    ('--.+....', '...-........+...', '+-.+....'),
    ('..+...-.', '......+.-.+-....', '..+.....'),
    ('..-+....', '...........+....', '..--....'),
    ('-.....+.', '..+.....+.......', '..-.+...'),
    ('....+.-.', '..+.............', '....+.+.'),
    ('+.-.....', '........+.......', '-.-.....'),
    ('...-....', '...-.......-.-.-', '...+...+'),
    ('++..--..', '...-+.......+...', '+-......'),
    ('......+.', '..-......+-...-.', '..-...-.'),
    ('-.......', '++......+...+...', '-...-...'),
    ('-....-.+', '............+...', '.+.-+...'),
    ('.-+..+-.', '......+.........', '.....++.'),
    ('.-......', '...+--.-.-..-...', '.+......'),
    ('...-.-.+', '...+...-.....+..', '.-.+...+'),
    ('....--..', '.+..............', '+-..+-..'),
    ('...+...-', '...+...-......+-', '.......+'),
    ('...-..+.', '...........-..-.', '..+....-'),
    ('.-+...-.', '......-..-......', '..+..++.'),
    ('......+-', '..............+.', '......--'),
    ('.....-.+', '.............+..', '.+.-.+.-'),
)

_BASE = dict(lag=8, stride=3, q_end=60, e0=(45, 85), e1=(0, 100), s_end=60, s_due=(5, 10), p_due=True,
             g_at=2, g=(50, 90), u_at=3, u_end=20, out_split=False)
TUNE = {
    'seq0': dict(_BASE, stride=4, q_end=50, e0=(30, 92), e1=(10, 100), s_due=(5, 10), u_at=0, u_end=60),
    'seq1': _BASE,
    'last': dict(_BASE, lag=10, e1=(20, 80), p_due=False, out_split=True),
}


class _Forms:
    def __init__(self, rows):
        self.n = len(rows[0])
        forms = [{j: 1 if ch == '+' else -1 for j, ch in enumerate(r) if ch != '.'} for r in rows]
        self.steps = []
        while True:
            count = {}
            seen = set()
            for f in forms:
                items = sorted(f.items())
                key = tuple((j, v * items[0][1]) for j, v in items)
                if key not in seen:
                    seen.add(key)
                    for a in range(len(items)):
                        for b in range(a + 1, len(items)):
                            pair = (items[a][0], items[b][0], items[a][1] * items[b][1])
                            count[pair] = count.get(pair, 0) + 1
            if not count:
                break
            j, k, sg = max(count, key=count.get)
            new = self.n + len(self.steps)
            self.steps.append((j, k, sg))
            for f in forms:
                if j in f and k in f and f[j] * f[k] == sg:
                    f[new] = f.pop(j)
                    f.pop(k)
        self.node = [next(iter(f)) for f in forms]
        self.sign = [next(iter(f.values())) for f in forms]

    def expand(self, blocks):
        nodes = list(blocks)
        for j, k, sg in self.steps:
            nodes.append(nodes[j] + nodes[k] if sg > 0 else nodes[j] - nodes[k])
        return [nodes[i] for i in self.node]

    def contract(self, prods, signs, order):
        acc = {}

        def add(i, v, s):
            if i not in acc:
                acc[i] = (v, s)
            else:
                w, t = acc[i]
                acc[i] = (w + v, s) if s == t else ((w - v, 1) if t > 0 else (v - w, 1))

        for r in order:
            if self.node[r] >= self.n:
                add(self.node[r], prods[r], self.sign[r] * signs[r])
        for i in reversed(range(len(self.steps))):
            j, k, sg = self.steps[i]
            v, s = acc[self.n + i]
            add(j, v, s)
            add(k, v, s * sg)
        for r in order:
            if self.node[r] < self.n:
                add(self.node[r], prods[r], self.sign[r] * signs[r])
        return [acc[j][0] if acc[j][1] > 0 else -acc[j][0] for j in range(self.n)]


FU, FV, FW = (_Forms([t[i] for t in SCHEME]) for i in range(3))
NPROD = len(SCHEME)
TABLED = [r for r in range(NPROD) if FV.node[r] >= FV.n]


def _ln(x, eps):
    d = x.shape[-1]
    m = jnp.sum(x, axis=-1, keepdims=True) * (1.0 / d)
    xc = x - m
    v = jnp.sum(xc * xc, axis=-1, keepdims=True) * (1.0 / d)
    return xc * lax.rsqrt(v + eps)


def _gelu2(x):
    c1 = math.sqrt(2.0 / math.pi)
    c2 = c1 * 0.044715
    t = jnp.tanh(x * (c1 + c2 * (x * x)))
    return x + x * t


def _center(w):
    return w - jnp.sum(w, axis=0, keepdims=True) * (1.0 / w.shape[0])


def _pack(x):
    return pltpu.bitcast(x.astype(BF16), U32)


def _unpack(x):
    return pltpu.bitcast(x, BF16)


def _bits(x):
    return pltpu.bitcast(x, U32)


def _to_bf16(v):
    return _unpack(v) if v.dtype == U32 else v.astype(BF16)


def _dot(a, b):
    return jnp.dot(a, b, preferred_element_type=F32)


def _dot_nt(a, b):
    return lax.dot_general(a, b, NT, preferred_element_type=F32)


def _split(v):
    return [v[:, c * LANES:(c + 1) * LANES] for c in range(v.shape[1] // LANES)]


def _aligned(i, n):
    return i if isinstance(i, int) else pl.multiple_of(i, n)


def _tie_bf16(flag, dep, val):
    head = _bits(val[0:16, 0:LANES])
    head = _unpack(jnp.where(flag, _bits(dep), head))
    top = jnp.concatenate([head, val[0:16, LANES:]], axis=1)
    return jnp.concatenate([top, val[16:, :]], axis=0)


def _tie(flag, deps, val, row):
    cast = _bits if val.dtype == U32 else (lambda v: v if v.dtype == F32 else pltpu.bitcast(v, F32))
    tiles = _split(val)
    t = tiles[0]
    end = row + 8 * len(deps)
    mid = jnp.where(flag, jnp.concatenate([cast(d) for d in deps], axis=0), t[row:end])
    tiles[0] = jnp.concatenate(([t[0:row]] if row else []) + [mid] + ([t[end:]] if end < t.shape[0] else []),
                               axis=0)
    return jnp.concatenate(tiles, axis=1)


def _released(flag, toks, lo, hi, val, ntiles=1):
    first, total = len(toks) * lo // 100, len(toks) * (hi - lo) // 100
    n = val.shape[0] // 8
    rel = jnp.concatenate([toks[min(first + (i * total) // n, len(toks) - 1)] for i in range(n)], axis=0)
    tiles = _split(val)
    return jnp.concatenate([jnp.where(flag, rel, t) if c < ntiles else t for c, t in enumerate(tiles)], axis=1)


def _kernel(x_hbm, wq_hbm, wk_hbm, wv_hbm, wao_hbm, wup_hbm, dw_hbm, wdn_hbm, wm_hbm,
            o_hbm,
            x_s, wq_s, wk_s, wv_s, wao_s, wup_s, dw_s, wdn_s, wm_s, sems,
            xa0_s, xa1_s, wa_s, dwb_s, s_s, m_s, u_s, g_s, gn_s, o_s, osem,
            tb0_s, tb1_s, wt_s, po_s, xo_s, qo_s, z_s,
            *, B, T, D, K, TQ, TK, TP, UR):
    NQ = T // TQ
    N = B * NQ
    NKV = TP // TK
    NC = D // LANES
    CPK = TK // LANES
    PAD = K // 2
    NQT = -(-TQ // LANES)
    NFULL = (T - (NKV - 1) * TK) // LANES
    TAIL = T % LANES
    HR = TQ // 2
    TR = LANES // H
    G = 4
    UP = UR // CPK
    UPC = -(-LANES // UP)
    NU = NKV * UPC
    UT = UP // H
    ORDER = [15, 12, 14, 10, 23, 18, 6, 17, 16, 1, 22, 0, 25, 2, 11, 3, 8, 13, 9, 19, 20, 24, 4, 5, 7, 21]
    PORDER = sorted(range(NPROD), key=lambda r: FU.node[r] < FU.n)
    SUV = [FU.sign[r] * FV.sign[r] for r in range(NPROD)]
    SWV = [FW.sign[r] * FV.sign[r] for r in range(NPROD)]
    xa_s, tb_s = (xa0_s, xa1_s), (tb0_s, tb1_s)

    def blocks_of(a):
        return [a[h * HR:(h + 1) * HR, c * LANES:(c + 1) * LANES] for h in range(2) for c in range(NC)]

    def unblock(bl):
        return jnp.concatenate([jnp.concatenate(bl[h * NC:(h + 1) * NC], axis=1) for h in range(2)], axis=0)

    def key_tables(y):
        n = y.shape[0] // CPK
        ops = FV.expand([y[t * n:(t + 1) * n, d * LANES:(d + 1) * LANES] for d in range(NC) for t in range(CPK)])
        return _pack(jnp.concatenate([ops[r] for r in TABLED], axis=1))

    def weight_tables(mat, w):
        ops = FV.expand([w[d * LANES:(d + 1) * LANES, t * LANES:(t + 1) * LANES]
                         for d in range(NC) for t in range(NC)])
        wt_s[mat * TR:(mat + 1) * TR, :] = _pack(jnp.concatenate(ops, axis=1))

    def fence(ref):
        return ref[pl.ds(pl.multiple_of(z_s[0], 8), 8), 0:LANES]

    def staged_operands(ref, a, which):
        ops = FU.expand(blocks_of(a))
        ref[:, 0:len(which) * LANES] = _pack(jnp.concatenate([ops[r] for r in which], axis=1))
        done = fence(ref)
        return {r: ref[:, k * LANES:(k + 1) * LANES] for k, r in enumerate(which)}, done

    def key_operand(b, g, r):
        i = FV.node[r]
        if i < FV.n:
            d, t = i // CPK, i % CPK
            parts = [xa_s[b][pl.ds((j * TK + t * LANES) // H, TR), d * LANES:(d + 1) * LANES]
                     for j in range(g * G, (g + 1) * G)]
        else:
            k = TABLED.index(r)
            parts = [tb_s[b][j * TR:(j + 1) * TR, k * LANES:(k + 1) * LANES] for j in range(g * G, (g + 1) * G)]
        return _unpack(jnp.concatenate(parts, axis=0))

    def store_g(ref, row, g):
        for c in range(NC):
            ref[c, row:row + g.shape[0], :] = g[:, c * LANES:(c + 1) * LANES]

    def conv(flag):
        prev = None
        rows = []
        for rr in range(0, TQ, 16):
            cols = []
            for c in range(NC):
                acc = None
                for k in range(K):
                    gv = g_s[c, pl.ds(rr + HALO - PAD + k, 16), :].reshape(2, 8, LANES)
                    term = gv * dwb_s[k, :, c * LANES:(c + 1) * LANES][None]
                    if acc is None:
                        acc = term if prev is None else jnp.where(flag, prev, term)
                    else:
                        acc = acc + term
                prev = acc
                cols.append(acc.reshape(16, LANES))
            rows.append(jnp.concatenate(cols, axis=1))
        return jnp.concatenate(rows, axis=0)

    def store_max(mx):
        m = jnp.max(mx, axis=-1, keepdims=True)
        m = m + jnp.log2(jnp.sum(jnp.exp2(mx - m), axis=-1, keepdims=True))
        m_s[...] = jnp.broadcast_to(m, (TQ, LANES))

    def rest_copy():
        return pltpu.make_async_copy(x_hbm.at[pl.ds(T + TK, T - TK), :], x_s.at[pl.ds(TP + TK, T - TK), :],
                                     sems.at[13])

    def out_copy(blk):
        rows = pl.ds(_aligned(blk * TQ, 16), TQ)
        return pltpu.make_async_copy(o_s.at[rows, :], o_hbm.at[rows, :], osem)

    def first_step():
        C1, C2 = 3, 6

        def xrows(b, r0, r1):
            return x_hbm.at[pl.ds(b * T + r0, r1 - r0), :], x_s.at[pl.ds(b * TP + r0, r1 - r0), :]

        copies = {}
        plan = (
            ('wq', wq_hbm, wq_s), ('wk', wk_hbm, wk_s),
            ('xa',) + xrows(0, 0, TK), ('xb',) + xrows(0, TK, C1 * TK), ('xc',) + xrows(0, C1 * TK, C2 * TK),
            ('xd',) + xrows(0, C2 * TK, T), ('wv', wv_hbm, wv_s), ('wao', wao_hbm, wao_s),
            ('wup', wup_hbm, wup_s), ('dw', dw_hbm, dw_s), ('wdn', wdn_hbm, wdn_s), ('wm', wm_hbm, wm_s),
            ('xe',) + xrows(1, 0, TK),
        )
        for i, (name, src, dst) in enumerate(plan):
            copies[name] = pltpu.make_async_copy(src, dst, sems.at[i])
            copies[name].start()
        rest_copy().start()

        z_s[0] = 0
        z_s[1] = 0
        z_s[2] = 0
        for b in range(B):
            x_s[b * TP + T:(b + 1) * TP, :] = jnp.zeros((TP - T, D), x_s.dtype)
        store_g(g_s, TQ, jnp.zeros((HALO, D), F32))

        def keys(r0, n):
            return _unpack(xa0_s[r0 // H:(r0 + n) // H, :])

        def ln_chunk(c):
            y = _ln(x_s[c * TK:(c + 1) * TK, :].astype(F32), EPS)
            xa0_s[c * TK // H:(c + 1) * TK // H, :] = _pack(y)
            tb0_s[c * TR:(c + 1) * TR, :] = key_tables(y)

        scale = float(D) ** (-0.5) * math.log2(math.e)
        DS = D // 2
        copies['wq'].wait()
        copies['wk'].wait()
        m_lo = _dot_nt(wq_s[...], wk_s[0:DS, :])

        never = z_s[0] > 0
        zero = pl.multiple_of(z_s[0], 8)

        def after(prev, l):
            return _unpack(l if prev is None else _tie(never, [prev[0:8, 0:LANES]], l, 0))

        copies['xa'].wait()
        wa_s[:, 0:DS] = _pack(_center(m_lo) * scale)
        wa_s[:, DS:D] = _pack(_center(_dot_nt(wq_s[...], wk_s[DS:D, :])) * scale)
        ln_chunk(0)
        qp = _pack(_dot(keys(0, TQ), _unpack(wa_s[:, 0:D])))
        q = _unpack(qp)

        def tail_parts():
            kt = keys(T - TAIL, TAIL)
            parts = []
            for n in range(NQT):
                qn = q[n * LANES:min((n + 1) * LANES, TQ), :]
                if qn.shape[0] < LANES:
                    qn = jnp.concatenate([qn, jnp.zeros((LANES - qn.shape[0], D), BF16)], axis=0)
                parts.append(_dot_nt(kt, qn))
            return parts

        def logits(c, prev, mx):
            last = c == NKV - 1
            parts = tail_parts() if last else None
            s = _dot_nt(after(prev, qp), keys(c * TK, (NFULL if last else CPK) * LANES))
            mc = None
            for t in range(CPK):
                if last and t == NFULL:
                    fill = jnp.full((LANES - TAIL, LANES), -jnp.inf, F32)
                    st = jnp.concatenate([jnp.concatenate([p, fill], axis=0).T for p in parts], axis=0)[0:TQ, :]
                else:
                    st = s[:, t * LANES:(t + 1) * LANES]
                s_s[c, :, t * LANES:(t + 1) * LANES] = st
                mc = st if mc is None else jnp.maximum(mc, st)
            return s, mc if mx is None else jnp.maximum(mx, mc)

        copies['xb'].wait()
        prev, mx = logits(0, None, None)
        for c in range(1, C1):
            ln_chunk(c)
            prev, mx = logits(c, prev, mx)

        copies['xc'].wait()
        prev = None
        for c in range(C1, C2):
            ln_chunk(c)
            prev, mx = logits(c, prev, mx)

        for name in ('xd', 'wv', 'wao'):
            copies[name].wait()
        wva_raw = _dot(wv_s[...], wao_s[...])
        mean = jnp.sum(wva_raw, axis=0, keepdims=True) * (1.0 / D)
        prev = wva_raw
        for c in range(C2, NKV):
            ln_chunk(c)
            prev, mx = logits(c, prev, mx)

        for name in ('wup', 'dw'):
            copies[name].wait()
        store_max(mx)
        xq = xa0_s[0:TQ // H, :]
        hg = _dot(after(None, xq), wup_s[:, D:2 * D])
        hu = _dot(after(hg, xq), wup_s[:, 0:D])
        dwf = dw_s[...].astype(F32)
        for k in range(K):
            dwb_s[k] = jnp.broadcast_to(dwf[k:k + 1, :], (8, D))
        wva = (wva_raw - mean).astype(BF16)
        weight_tables(0, _unpack(wa_s[:, 0:D]).astype(F32))

        def tokens(res):
            return [res[r:r + 8, c * LANES:(c + 1) * LANES] for c in range(NC) for r in range(0, D, 8)]

        for name in ('wdn', 'wm'):
            copies[name].wait()
        wvom = _dot(wva, wm_s[0:D, :])
        t1 = tokens(wvom)
        store_g(gn_s, 0, _ln(_gelu2(_released(never, t1, 0, 40, hg, NC)), 4.0 * EPS))
        u_s[...] = _gelu2(_released(never, t1, 0, 40, hu, NC))
        weight_tables(1, _released(never, t1, 0, 90, wup_s[:, D:2 * D].astype(F32), NC))
        weight_tables(2, _released(never, t1, 30, 90, wup_s[:, 0:D].astype(F32), NC))
        wdn = wdn_s[...]
        deps = [wvom[0:8, LANES:2 * LANES], gn_s[0, pl.ds(zero, 8), :], u_s[pl.ds(zero, 8), 0:LANES],
                wt_s[pl.ds(zero, 8), 0:LANES]]
        for i, dep in enumerate(deps):
            wdn = jnp.concatenate(([wdn[0:16 * i]] if i else []) + [_tie_bf16(never, dep, wdn[16 * i:])], axis=0)
        wdm = _dot(wdn, wm_s[D:2 * D, :])
        weight_tables(3, _released(never, tokens(wdm), 0, 50, wvom, NC))
        weight_tables(4, 0.5 * wdm)
        copies['xe'].wait()

    def step_body(step, ba, bb, tune, normalise=False, do_a=True):
        sb = step - 1
        ia, ib = step - ba * NQ, sb - bb * NQ
        never = z_s[0] > 0
        never2 = z_s[1] > 0
        never3 = z_s[2] > 0
        for c in range(NC):
            g_s[c, 0:HALO, :] = jnp.where(ib == 0, 0.0, g_s[c, TQ:TQ + HALO, :])
            g_s[c, HALO:HALO + TQ, :] = gn_s[c]
        hist = []
        pend = []
        later = []

        def matmul(l, tiles, run):
            back = 0
            for res, n in reversed(hist):
                back += n
                if back >= tune['lag']:
                    l = _tie(never3, [res[0:8, 0:LANES]], l, 0)
                    break
            while later and later[0][0] <= len(hist) and len(pend) < 4:
                pend.append(later.pop(0)[1])
            if pend:
                l = _tie(never3, pend, l, 8)
                del pend[:]
            hist.append((run(_to_bf16(l)), tiles))
            return hist[-1][0]

        def toks(i0):
            return [res[r:r + 8, 0:LANES] for res, n in hist[i0:] for r in range(0, HR, 8 * (4 // n))]

        def rel2(v, t, lo, hi):
            return jnp.concatenate([_released(never, t, lo, hi, v[0:HR]), _released(never, t, lo, hi, v[HR:])],
                                   axis=0)

        def project(ops, mats, axis):
            m = [None] * NPROD
            for r in ORDER:
                m[r] = matmul(ops[r], len(mats), lambda v, r=r: _dot(v, _unpack(jnp.concatenate(
                    [wt_s[k * TR:(k + 1) * TR, r * LANES:(r + 1) * LANES] for k in mats], axis=axis))))
            return m

        def combine(prods, t=None, lo=0, hi=0):
            if t is not None:
                prods = list(prods)
                for r in ORDER[::tune['stride']]:
                    prods[r] = _released(never, t, lo, hi, prods[r])
            return unblock(FW.contract(prods, SUV, ORDER))

        m_old = m_s[...]
        u_old = u_s[...]
        if do_a:
            xq = xa_s[ba][pl.ds(_aligned(ia * (TQ // H), 8), TQ // H), :]
            xops, _ = staged_operands(xo_s, _unpack(xq).astype(F32),
                                      [r for r in range(NPROD) if FU.node[r] >= FU.n])
            for r in range(NPROD):
                i = FU.node[r]
                if i < FU.n:
                    xops[r] = xq[(i // NC) * HR // H:(i // NC + 1) * HR // H, (i % NC) * LANES:(i % NC + 1) * LANES]
            qm = project(xops, [0], 1)
            gm = project(xops, [1, 2], 1)
            q_raw = combine(qm, toks(NPROD), 0, tune['q_end'])
            qops, done = staged_operands(qo_s, q_raw, list(range(NPROD)))
            pend.append(done)
        else:
            store_g(g_s, HALO + TQ, jnp.zeros((HALO, D), F32))
        state = {'l': None, 'acc': None, 'mx': None}

        def probabilities(g, t, lo, hi):
            for jj in range(G):
                j = g * G + jj
                m = m_old if t is None else rel2(m_old, t, lo + (hi - lo) * jj // G, lo + (hi - lo) * (jj + 1) // G)
                tiles = []
                lsum = None
                for c in range(CPK):
                    p = jnp.exp2(s_s[j, :, c * LANES:(c + 1) * LANES] - m)
                    lsum = p if lsum is None else lsum + p
                    tiles.append(p)
                state['l'] = lsum if state['l'] is None else state['l'] + lsum
                tiles[0] = jnp.where(never2, state['l'], tiles[0])
                w = jnp.concatenate(FW.expand(blocks_of(jnp.concatenate(tiles, axis=1))), axis=1)
                po_s[j * HR // H:(j + 1) * HR // H, :] = _pack(w)
            return fence(po_s)

        def store_logits(g, m, t):
            for jj in range(G):
                j = g * G + jj
                s = combine([v[:, jj * LANES:(jj + 1) * LANES] for v in m], t,
                            tune['s_end'] * jj // G, tune['s_end'] * (jj + 1) // G)
                for c, st in enumerate(_split(s)):
                    if j == NKV - 1 and c == NFULL:
                        st = jnp.where(lax.broadcasted_iota(jnp.int32, st.shape, 1) < TAIL, st, -jnp.inf)
                    s_s[j, :, c * LANES:(c + 1) * LANES] = st
                    state['mx'] = st if state['mx'] is None else jnp.maximum(state['mx'], st)

        def side_work(phase, t):
            if phase == tune['g_at']:
                gg = _gelu2(combine([v[:, 0:LANES] for v in gm], t, 0, tune['g'][0]))
                g_new = _ln(rel2(gg, t, *tune['g']), 4.0 * EPS)
                store_g(gn_s, 0, g_new)
                store_g(g_s, HALO + TQ, jnp.where(ia == 0, 0.0, g_new[0:HALO, :]))
            if phase == tune['u_at']:
                u_s[...] = _gelu2(combine([v[:, LANES:] for v in gm], t, 0, tune['u_end']))
            if phase == 3 and normalise:
                unit = jnp.minimum(step - 1, NU - 1)
                c0, r0 = unit // UPC, jnp.minimum((unit % UPC) * UP, LANES - UP)
                xv = [x_s[pl.ds(pl.multiple_of(TP + c0 * TK + k * LANES + r0, 16), UP), :].astype(F32)
                      for k in range(CPK)]
                y = _ln(jnp.concatenate([_released(never, t, 50, 80, v) for v in xv], axis=0), EPS)
                for k in range(CPK):
                    row = pl.multiple_of((c0 * TK + k * LANES + r0) // H, 8)
                    xa1_s[pl.ds(row, UT), :] = _pack(y[k * UP:(k + 1) * UP])
                tb1_s[pl.ds(pl.multiple_of(c0 * TR + r0 // H, 8), UT), :] = key_tables(y)

        ready = None
        for g in range(NKV // G):
            if do_a:
                start = len(hist)
                sm = [None] * NPROD
                for r in ORDER:
                    sm[r] = matmul(qops[r], G, lambda v, r=r: _dot_nt(v, key_operand(ba, g, r)))
            if g == 0:
                ready = probabilities(0, toks(0) if do_a else None, *tune['e0'])
            if do_a:
                side_work(2 * g, toks(start))
            if tune['p_due']:
                pend.append(ready)
            start = len(hist)
            n = [None] * NPROD
            for r in PORDER:
                l = jnp.concatenate([po_s[j * HR // H:(j + 1) * HR // H, r * LANES:(r + 1) * LANES]
                                     for j in range(g * G, (g + 1) * G)], axis=1)
                n[r] = matmul(l, G, lambda v, r=r: _dot(v, key_operand(bb, g, r)))
            state['acc'] = n if state['acc'] is None else [x + y for x, y in zip(state['acc'], n)]
            t = toks(start)
            if do_a:
                store_logits(g, sm, t)
                if tune['s_due'][g] >= 0:
                    later.extend((len(hist) + tune['s_due'][g], state['mx'][r:r + 8]) for r in range(0, TQ, 8))
            if (g + 1) * G < NKV:
                ready = probabilities(g + 1, t, *tune['e1'])
            if do_a:
                side_work(2 * g + 1, t)
        yc = u_old * conv(never)
        ya = unblock(FU.contract(state['acc'], SWV, PORDER)) * (1.0 / jnp.sum(state['l'], axis=-1, keepdims=True))
        if tune['out_split']:
            om = project(FU.expand(blocks_of(yc)), [4], 0)
            om = [x + y for x, y in zip(om, project(FU.expand(blocks_of(ya)), [3], 0))]
        else:
            om = project([jnp.concatenate(p, axis=1)
                          for p in zip(FU.expand(blocks_of(ya)), FU.expand(blocks_of(yc)))], [3, 4], 0)
        out = combine(om)
        xr = x_s[pl.ds(_aligned(bb * TP + ib * TQ, 16), TQ), :].astype(F32)
        o_s[pl.ds(_aligned(sb * TQ, 16), TQ), :] = (xr + out).astype(o_s.dtype)
        if do_a:
            store_max(state['mx'])
        out_copy(sb).start()

    def iteration0(step, carry):
        step_body(step, 0, 0, TUNE['seq0'], normalise=True)

        @pl.when(step == 1)
        def _():
            rest_copy().wait()

        return carry

    def iteration1(step, carry):
        step_body(step, 1, 1, TUNE['seq1'])
        return carry

    first_step()
    lax.fori_loop(1, NQ, iteration0, 0)
    step_body(NQ + z_s[0], 1, 0, TUNE['seq1'])
    lax.fori_loop(NQ + 1, N, iteration1, 0)
    step_body(N, 1, 1, TUNE['last'], do_a=False)
    pltpu.make_async_copy(o_s, o_hbm, osem).wait()


@jax.jit
def pallas_standalone__conformer_family_branchformer__speech_kernel(
    x: jax.Array,
    w_q: jax.Array,
    w_k: jax.Array,
    w_v: jax.Array,
    w_ao: jax.Array,
    w_up: jax.Array,
    dw: jax.Array,
    w_dn: jax.Array,
    w_merge: jax.Array,
):
    B, T, D = x.shape
    K = dw.shape[0]
    TQ = 160
    TK = 512
    TP = -(-T // TK) * TK
    UR = 192
    NKV = TP // TK
    assert B == 2 and T % TQ == 0 and TQ % 32 == 0 and D == TK == 4 * LANES and K // 2 < HALO
    assert NKV * -(-TK // UR) < T // TQ and UR % 64 == 0 and NKV == 8 and T % LANES in (16, 32, 48, 64) and TP - T < LANES
    x2 = x.reshape(B * T, D)

    kern = functools.partial(_kernel, B=B, T=T, D=D, K=K, TQ=TQ, TK=TK, TP=TP, UR=UR)
    ins = (x2, w_q, w_k, w_v, w_ao, w_up, dw, w_dn, w_merge)
    out = pl.pallas_call(
        kern,
        in_specs=[pl.BlockSpec(memory_space=pl.ANY) for _ in ins],
        out_specs=pl.BlockSpec(memory_space=pl.ANY),
        out_shape=jax.ShapeDtypeStruct((B * T, D), x.dtype),
        scratch_shapes=[pltpu.VMEM((B * TP, D), x.dtype)] + [pltpu.VMEM(a.shape, a.dtype) for a in ins[1:]] + [
            pltpu.SemaphoreType.DMA((14,)),
            pltpu.VMEM((TP // H, D), U32),
            pltpu.VMEM((TP // H, D), U32),
            pltpu.VMEM((D // H, D), U32),
            pltpu.VMEM((K, 8, D), F32),
            pltpu.VMEM((NKV, TQ, TK), F32),
            pltpu.VMEM((TQ, LANES), F32),
            pltpu.VMEM((TQ, D), F32),
            pltpu.VMEM((D // LANES, TQ + 2 * HALO, LANES), F32),
            pltpu.VMEM((D // LANES, TQ, LANES), F32),
            pltpu.VMEM((B * T, D), x.dtype),
            pltpu.SemaphoreType.DMA(()),
            pltpu.VMEM((NKV * LANES // H, len(TABLED) * LANES), U32),
            pltpu.VMEM((NKV * LANES // H, len(TABLED) * LANES), U32),
            pltpu.VMEM((5 * LANES // H, NPROD * LANES), U32),
            pltpu.VMEM((NKV * TQ // 2 // H, NPROD * LANES), U32),
            pltpu.VMEM((TQ // 2 // H, NPROD * LANES), U32),
            pltpu.VMEM((TQ // 2 // H, NPROD * LANES), U32),
            pltpu.SMEM((3,), jnp.int32),
        ],
        compiler_params=pltpu.CompilerParams(
            vmem_limit_bytes=100 * 1024 * 1024,
            disable_bounds_checks=True,
            disable_semaphore_checks=True,
        ),
    )(*ins)
    return out.reshape(B, T, D)
```

```python
import functools
import math

import jax
import jax.numpy as jnp
from jax import lax
import jax.experimental.pallas as pl
import jax.experimental.pallas.tpu as pltpu

LANES = 128
EPS = 1e-05
F32 = jnp.float32
BF16 = jnp.bfloat16
U32 = jnp.uint32
NT = (((1,), (1,)), ((), ()))
HALO = 16
H = 2

SCHEME = (
    ('...-++..', '...+............', '-+.....+'),
    ('.+-.....', '.........-......', '.++..++.'),
    ('+...--..', '.+..+.......+...', '-+..-...'),
    ('.+.-.-.+', '...-...+....+...', '.-.+....'),
    ('.....+..', '.+...-+......-..', '.....-..'),
    ('+...-...', '+.-.-.......-...', '....-...'),
    ('--.+....', '...-........+...', '+-.+....'),
    ('..+...-.', '......+.-.+-....', '..+.....'),
    ('..-+....', '...........+....', '..--....'),
    ('-.....+.', '..+.....+.......', '..-.+...'),
    ('....+.-.', '..+.............', '....+.+.'),
    ('+.-.....', '........+.......', '-.-.....'),
    ('...-....', '...-.......-.-.-', '...+...+'),
    ('++..--..', '...-+.......+...', '+-......'),
    ('......+.', '..-......+-...-.', '..-...-.'),
    ('-.......', '++......+...+...', '-...-...'),
    ('-....-.+', '............+...', '.+.-+...'),
    ('.-+..+-.', '......+.........', '.....++.'),
    ('.-......', '...+--.-.-..-...', '.+......'),
    ('...-.-.+', '...+...-.....+..', '.-.+...+'),
    ('....--..', '.+..............', '+-..+-..'),
    ('...+...-', '...+...-......+-', '.......+'),
    ('...-..+.', '...........-..-.', '..+....-'),
    ('.-+...-.', '......-..-......', '..+..++.'),
    ('......+-', '..............+.', '......--'),
    ('.....-.+', '.............+..', '.+.-.+.-'),
)

_BASE = dict(lag=8, stride=3, q_end=60, e0=(45, 85), e1=(0, 100), s_end=60, s_due=(5, 10), p_due=True,
             g_at=2, g=(50, 90), u_at=3, u_end=20, out_split=False)
TUNE = {
    'seq0': dict(_BASE, stride=4, q_end=50, e0=(30, 92), e1=(10, 100), s_due=(5, 10), u_at=0, u_end=60),
    'seq1': _BASE,
    'last': dict(_BASE, lag=10, e1=(20, 80), p_due=False, out_split=True),
}


class _Forms:
    def __init__(self, rows):
        self.n = len(rows[0])
        forms = [{j: 1 if ch == '+' else -1 for j, ch in enumerate(r) if ch != '.'} for r in rows]
        self.steps = []
        while True:
            count = {}
            seen = set()
            for f in forms:
                items = sorted(f.items())
                key = tuple((j, v * items[0][1]) for j, v in items)
                if key not in seen:
                    seen.add(key)
                    for a in range(len(items)):
                        for b in range(a + 1, len(items)):
                            pair = (items[a][0], items[b][0], items[a][1] * items[b][1])
                            count[pair] = count.get(pair, 0) + 1
            if not count:
                break
            j, k, sg = max(count, key=count.get)
            new = self.n + len(self.steps)
            self.steps.append((j, k, sg))
            for f in forms:
                if j in f and k in f and f[j] * f[k] == sg:
                    f[new] = f.pop(j)
                    f.pop(k)
        self.node = [next(iter(f)) for f in forms]
        self.sign = [next(iter(f.values())) for f in forms]

    def expand(self, blocks):
        nodes = list(blocks)
        for j, k, sg in self.steps:
            nodes.append(nodes[j] + nodes[k] if sg > 0 else nodes[j] - nodes[k])
        return [nodes[i] for i in self.node]

    def contract(self, prods, signs, order):
        acc = {}

        def add(i, v, s):
            if i not in acc:
                acc[i] = (v, s)
            else:
                w, t = acc[i]
                acc[i] = (w + v, s) if s == t else ((w - v, 1) if t > 0 else (v - w, 1))

        for r in order:
            if self.node[r] >= self.n:
                add(self.node[r], prods[r], self.sign[r] * signs[r])
        for i in reversed(range(len(self.steps))):
            j, k, sg = self.steps[i]
            v, s = acc[self.n + i]
            add(j, v, s)
            add(k, v, s * sg)
        for r in order:
            if self.node[r] < self.n:
                add(self.node[r], prods[r], self.sign[r] * signs[r])
        return [acc[j][0] if acc[j][1] > 0 else -acc[j][0] for j in range(self.n)]


FU, FV, FW = (_Forms([t[i] for t in SCHEME]) for i in range(3))
NPROD = len(SCHEME)
TABLED = [r for r in range(NPROD) if FV.node[r] >= FV.n]


def _ln(x, eps):
    d = x.shape[-1]
    m = jnp.sum(x, axis=-1, keepdims=True) * (1.0 / d)
    xc = x - m
    v = jnp.sum(xc * xc, axis=-1, keepdims=True) * (1.0 / d)
    return xc * lax.rsqrt(v + eps)


def _gelu2(x):
    c1 = math.sqrt(2.0 / math.pi)
    c2 = c1 * 0.044715
    t = jnp.tanh(x * (c1 + c2 * (x * x)))
    return x + x * t


def _center(w):
    return w - jnp.sum(w, axis=0, keepdims=True) * (1.0 / w.shape[0])


def _pack(x):
    return pltpu.bitcast(x.astype(BF16), U32)


def _unpack(x):
    return pltpu.bitcast(x, BF16)


def _bits(x):
    return pltpu.bitcast(x, U32)


def _to_bf16(v):
    return _unpack(v) if v.dtype == U32 else v.astype(BF16)


def _dot(a, b):
    return jnp.dot(a, b, preferred_element_type=F32)


def _dot_nt(a, b):
    return lax.dot_general(a, b, NT, preferred_element_type=F32)


def _split(v):
    return [v[:, c * LANES:(c + 1) * LANES] for c in range(v.shape[1] // LANES)]


def _aligned(i, n):
    return i if isinstance(i, int) else pl.multiple_of(i, n)


def _tie_bf16(flag, dep, val):
    head = _bits(val[0:16, 0:LANES])
    head = _unpack(jnp.where(flag, _bits(dep), head))
    top = jnp.concatenate([head, val[0:16, LANES:]], axis=1)
    return jnp.concatenate([top, val[16:, :]], axis=0)


def _tie(flag, deps, val, row):
    cast = _bits if val.dtype == U32 else (lambda v: v if v.dtype == F32 else pltpu.bitcast(v, F32))
    tiles = _split(val)
    t = tiles[0]
    end = row + 8 * len(deps)
    mid = jnp.where(flag, jnp.concatenate([cast(d) for d in deps], axis=0), t[row:end])
    tiles[0] = jnp.concatenate(([t[0:row]] if row else []) + [mid] + ([t[end:]] if end < t.shape[0] else []),
                               axis=0)
    return jnp.concatenate(tiles, axis=1)


def _released(flag, toks, lo, hi, val, ntiles=1):
    first, total = len(toks) * lo // 100, len(toks) * (hi - lo) // 100
    n = val.shape[0] // 8
    rel = jnp.concatenate([toks[min(first + (i * total) // n, len(toks) - 1)] for i in range(n)], axis=0)
    tiles = _split(val)
    return jnp.concatenate([jnp.where(flag, rel, t) if c < ntiles else t for c, t in enumerate(tiles)], axis=1)


def _kernel(x_hbm, wq_hbm, wk_hbm, wv_hbm, wao_hbm, wup_hbm, dw_hbm, wdn_hbm, wm_hbm,
            o_hbm,
            x_s, wq_s, wk_s, wv_s, wao_s, wup_s, dw_s, wdn_s, wm_s, sems,
            xa0_s, xa1_s, wa_s, dwb_s, s_s, m_s, u_s, g_s, gn_s, o_s, osem,
            tb0_s, tb1_s, wt_s, po_s, xo_s, qo_s, z_s,
            *, B, T, D, K, TQ, TK, TP, UR):
    NQ = T // TQ
    N = B * NQ
    NKV = TP // TK
    NC = D // LANES
    CPK = TK // LANES
    PAD = K // 2
    NQT = -(-TQ // LANES)
    NFULL = (T - (NKV - 1) * TK) // LANES
    TAIL = T % LANES
    HR = TQ // 2
    TR = LANES // H
    G = 4
    UP = UR // CPK
    UPC = -(-LANES // UP)
    NU = NKV * UPC
    UT = UP // H
    ORDER = [15, 12, 14, 10, 23, 18, 6, 17, 16, 1, 22, 0, 25, 2, 11, 3, 8, 13, 9, 19, 20, 24, 4, 5, 7, 21]
    PORDER = sorted(range(NPROD), key=lambda r: FU.node[r] < FU.n)
    SUV = [FU.sign[r] * FV.sign[r] for r in range(NPROD)]
    SWV = [FW.sign[r] * FV.sign[r] for r in range(NPROD)]
    xa_s, tb_s = (xa0_s, xa1_s), (tb0_s, tb1_s)

    def blocks_of(a):
        return [a[h * HR:(h + 1) * HR, c * LANES:(c + 1) * LANES] for h in range(2) for c in range(NC)]

    def unblock(bl):
        return jnp.concatenate([jnp.concatenate(bl[h * NC:(h + 1) * NC], axis=1) for h in range(2)], axis=0)

    def key_tables(y):
        n = y.shape[0] // CPK
        ops = FV.expand([y[t * n:(t + 1) * n, d * LANES:(d + 1) * LANES] for d in range(NC) for t in range(CPK)])
        return _pack(jnp.concatenate([ops[r] for r in TABLED], axis=1))

    def weight_tables(mat, w):
        ops = FV.expand([w[d * LANES:(d + 1) * LANES, t * LANES:(t + 1) * LANES]
                         for d in range(NC) for t in range(NC)])
        wt_s[mat * TR:(mat + 1) * TR, :] = _pack(jnp.concatenate(ops, axis=1))

    def fence(ref):
        return ref[pl.ds(pl.multiple_of(z_s[0], 8), 8), 0:LANES]

    def staged_operands(ref, a, which):
        ops = FU.expand(blocks_of(a))
        ref[:, 0:len(which) * LANES] = _pack(jnp.concatenate([ops[r] for r in which], axis=1))
        done = fence(ref)
        return {r: ref[:, k * LANES:(k + 1) * LANES] for k, r in enumerate(which)}, done

    def key_operand(b, g, r):
        i = FV.node[r]
        if i < FV.n:
            d, t = i // CPK, i % CPK
            parts = [xa_s[b][pl.ds((j * TK + t * LANES) // H, TR), d * LANES:(d + 1) * LANES]
                     for j in range(g * G, (g + 1) * G)]
        else:
            k = TABLED.index(r)
            parts = [tb_s[b][j * TR:(j + 1) * TR, k * LANES:(k + 1) * LANES] for j in range(g * G, (g + 1) * G)]
        return _unpack(jnp.concatenate(parts, axis=0))

    def store_g(ref, row, g):
        for c in range(NC):
            ref[c, row:row + g.shape[0], :] = g[:, c * LANES:(c + 1) * LANES]

    def conv(flag):
        prev = None
        rows = []
        for rr in range(0, TQ, 16):
            cols = []
            for c in range(NC):
                acc = None
                for k in range(K):
                    gv = g_s[c, pl.ds(rr + HALO - PAD + k, 16), :].reshape(2, 8, LANES)
                    term = gv * dwb_s[k, :, c * LANES:(c + 1) * LANES][None]
                    if acc is None:
                        acc = term if prev is None else jnp.where(flag, prev, term)
                    else:
                        acc = acc + term
                prev = acc
                cols.append(acc.reshape(16, LANES))
            rows.append(jnp.concatenate(cols, axis=1))
        return jnp.concatenate(rows, axis=0)

    def store_max(mx):
        m = jnp.max(mx, axis=-1, keepdims=True)
        m = m + jnp.log2(jnp.sum(jnp.exp2(mx - m), axis=-1, keepdims=True))
        m_s[...] = jnp.broadcast_to(m, (TQ, LANES))

    def rest_copy():
        return pltpu.make_async_copy(x_hbm.at[pl.ds(T + TK, T - TK), :], x_s.at[pl.ds(TP + TK, T - TK), :],
                                     sems.at[14])

    def out_copy(blk):
        rows = pl.ds(_aligned(blk * TQ, 16), TQ)
        return pltpu.make_async_copy(o_s.at[rows, :], o_hbm.at[rows, :], osem)

    def first_step():
        C1, C2 = 3, 6

        def xrows(b, r0, r1):
            return x_hbm.at[pl.ds(b * T + r0, r1 - r0), :], x_s.at[pl.ds(b * TP + r0, r1 - r0), :]

        copies = {}
        plan = (
            ('wq', wq_hbm, wq_s), ('wk', wk_hbm, wk_s),
            ('xa',) + xrows(0, 0, TK), ('xb',) + xrows(0, TK, C1 * TK), ('xc',) + xrows(0, C1 * TK, C2 * TK),
            ('xd',) + xrows(0, C2 * TK, T), ('wv', wv_hbm, wv_s), ('wao', wao_hbm, wao_s),
            ('wm1', wm_hbm.at[pl.ds(0, D), :], wm_s.at[pl.ds(0, D), :]), ('wup', wup_hbm, wup_s), ('dw', dw_hbm, dw_s),
            ('wdn', wdn_hbm, wdn_s), ('wm2', wm_hbm.at[pl.ds(D, D), :], wm_s.at[pl.ds(D, D), :]),
            ('xe',) + xrows(1, 0, TK),
        )
        for i, (name, src, dst) in enumerate(plan):
            copies[name] = pltpu.make_async_copy(src, dst, sems.at[i])
            copies[name].start()
        rest_copy().start()

        z_s[0] = 0
        z_s[1] = 0
        z_s[2] = 0
        for b in range(B):
            x_s[b * TP + T:(b + 1) * TP, :] = jnp.zeros((TP - T, D), x_s.dtype)
        store_g(g_s, TQ, jnp.zeros((HALO, D), F32))

        def keys(r0, n):
            return _unpack(xa0_s[r0 // H:(r0 + n) // H, :])

        def ln_chunk(c):
            y = _ln(x_s[c * TK:(c + 1) * TK, :].astype(F32), EPS)
            xa0_s[c * TK // H:(c + 1) * TK // H, :] = _pack(y)
            tb0_s[c * TR:(c + 1) * TR, :] = key_tables(y)

        scale = float(D) ** (-0.5) * math.log2(math.e)
        DS = D // 2
        copies['wq'].wait()
        copies['wk'].wait()
        m_lo = _dot_nt(wq_s[...], wk_s[0:DS, :])

        never = z_s[0] > 0
        zero = pl.multiple_of(z_s[0], 8)

        def after(prev, l):
            return _unpack(l if prev is None else _tie(never, [prev[0:8, 0:LANES]], l, 0))

        copies['xa'].wait()
        wa_s[:, 0:DS] = _pack(_center(m_lo) * scale)
        wa_s[:, DS:D] = _pack(_center(_dot_nt(wq_s[...], wk_s[DS:D, :])) * scale)
        ln_chunk(0)
        qp = _pack(_dot(keys(0, TQ), _unpack(wa_s[:, 0:D])))
        q = _unpack(qp)

        def tail_parts():
            kt = keys(T - TAIL, TAIL)
            parts = []
            for n in range(NQT):
                qn = q[n * LANES:min((n + 1) * LANES, TQ), :]
                if qn.shape[0] < LANES:
                    qn = jnp.concatenate([qn, jnp.zeros((LANES - qn.shape[0], D), BF16)], axis=0)
                parts.append(_dot_nt(kt, qn))
            return parts

        def logits(c, prev, mx):
            last = c == NKV - 1
            parts = tail_parts() if last else None
            s = _dot_nt(after(prev, qp), keys(c * TK, (NFULL if last else CPK) * LANES))
            mc = None
            for t in range(CPK):
                if last and t == NFULL:
                    fill = jnp.full((LANES - TAIL, LANES), -jnp.inf, F32)
                    st = jnp.concatenate([jnp.concatenate([p, fill], axis=0).T for p in parts], axis=0)[0:TQ, :]
                else:
                    st = s[:, t * LANES:(t + 1) * LANES]
                s_s[c, :, t * LANES:(t + 1) * LANES] = st
                mc = st if mc is None else jnp.maximum(mc, st)
            return s, mc if mx is None else jnp.maximum(mx, mc)

        copies['xb'].wait()
        prev, mx = logits(0, None, None)
        for c in range(1, C1):
            ln_chunk(c)
            prev, mx = logits(c, prev, mx)

        copies['xc'].wait()
        prev = None
        for c in range(C1, C2):
            ln_chunk(c)
            prev, mx = logits(c, prev, mx)

        for name in ('xd', 'wv', 'wao'):
            copies[name].wait()
        wva_raw = _dot(wv_s[...], wao_s[...])
        mean = jnp.sum(wva_raw, axis=0, keepdims=True) * (1.0 / D)
        prev = wva_raw
        for c in range(C2, NKV):
            ln_chunk(c)
            prev, mx = logits(c, prev, mx)

        def tokens(res):
            return [res[r:r + 8, c * LANES:(c + 1) * LANES] for c in range(NC) for r in range(0, res.shape[0], 8)]

        def rel(t, lo, hi, v):
            return _released(never, t, lo, hi, v, NC)

        for name in ('wm1', 'wup', 'dw'):
            copies[name].wait()
        store_max(mx)
        xq = xa0_s[0:TQ // H, :]
        hg = _dot(after(None, xq), wup_s[:, D:2 * D])
        hu = _dot(after(hg, xq), wup_s[:, 0:D])
        dwf = dw_s[...].astype(F32)
        for k in range(K):
            dwb_s[k] = jnp.broadcast_to(dwf[k:k + 1, :], (8, D))
        wva = (wva_raw - mean).astype(BF16)
        wvom = _dot(_tie_bf16(never, hu[0:8, 0:LANES], wva), wm_s[0:D, :])
        t1 = tokens(hg) + tokens(hu) + tokens(wvom)
        weight_tables(0, rel(t1, 0, 60, _unpack(wa_s[:, 0:D]).astype(F32)))
        weight_tables(1, rel(t1, 0, 70, wup_s[:, D:2 * D].astype(F32)))
        weight_tables(2, rel(t1, 60, 95, wup_s[:, 0:D].astype(F32)))

        for name in ('wdn', 'wm2'):
            copies[name].wait()
        wdm = _dot(wdn_s[...], wm_s[D:2 * D, :])
        t2 = tokens(wdm)
        store_g(gn_s, 0, _ln(_gelu2(rel(t2, 0, 40, hg)), 4.0 * EPS))
        u_s[...] = _gelu2(rel(t2, 0, 40, hu))
        weight_tables(3, rel(t2, 20, 80, wvom))
        weight_tables(4, 0.5 * wdm)
        copies['xe'].wait()

    def step_body(step, ba, bb, tune, normalise=False, do_a=True):
        sb = step - 1
        ia, ib = step - ba * NQ, sb - bb * NQ
        never = z_s[0] > 0
        never2 = z_s[1] > 0
        never3 = z_s[2] > 0
        for c in range(NC):
            g_s[c, 0:HALO, :] = jnp.where(ib == 0, 0.0, g_s[c, TQ:TQ + HALO, :])
            g_s[c, HALO:HALO + TQ, :] = gn_s[c]
        hist = []
        pend = []
        later = []

        def matmul(l, tiles, run):
            back = 0
            for res, n in reversed(hist):
                back += n
                if back >= tune['lag']:
                    l = _tie(never3, [res[0:8, 0:LANES]], l, 0)
                    break
            while later and later[0][0] <= len(hist) and len(pend) < 4:
                pend.append(later.pop(0)[1])
            if pend:
                l = _tie(never3, pend, l, 8)
                del pend[:]
            hist.append((run(_to_bf16(l)), tiles))
            return hist[-1][0]

        def toks(i0):
            return [res[r:r + 8, 0:LANES] for res, n in hist[i0:] for r in range(0, HR, 8 * (4 // n))]

        def rel2(v, t, lo, hi):
            return jnp.concatenate([_released(never, t, lo, hi, v[0:HR]), _released(never, t, lo, hi, v[HR:])],
                                   axis=0)

        def project(ops, mats, axis):
            m = [None] * NPROD
            for r in ORDER:
                m[r] = matmul(ops[r], len(mats), lambda v, r=r: _dot(v, _unpack(jnp.concatenate(
                    [wt_s[k * TR:(k + 1) * TR, r * LANES:(r + 1) * LANES] for k in mats], axis=axis))))
            return m

        def combine(prods, t=None, lo=0, hi=0):
            if t is not None:
                prods = list(prods)
                for r in ORDER[::tune['stride']]:
                    prods[r] = _released(never, t, lo, hi, prods[r])
            return unblock(FW.contract(prods, SUV, ORDER))

        m_old = m_s[...]
        u_old = u_s[...]
        if do_a:
            xq = xa_s[ba][pl.ds(_aligned(ia * (TQ // H), 8), TQ // H), :]
            xops, _ = staged_operands(xo_s, _unpack(xq).astype(F32),
                                      [r for r in range(NPROD) if FU.node[r] >= FU.n])
            for r in range(NPROD):
                i = FU.node[r]
                if i < FU.n:
                    xops[r] = xq[(i // NC) * HR // H:(i // NC + 1) * HR // H, (i % NC) * LANES:(i % NC + 1) * LANES]
            qm = project(xops, [0], 1)
            gm = project(xops, [1, 2], 1)
            q_raw = combine(qm, toks(NPROD), 0, tune['q_end'])
            qops, done = staged_operands(qo_s, q_raw, list(range(NPROD)))
            pend.append(done)
        else:
            store_g(g_s, HALO + TQ, jnp.zeros((HALO, D), F32))
        state = {'l': None, 'acc': None, 'mx': None}

        def probabilities(g, t, lo, hi):
            for jj in range(G):
                j = g * G + jj
                m = m_old if t is None else rel2(m_old, t, lo + (hi - lo) * jj // G, lo + (hi - lo) * (jj + 1) // G)
                tiles = []
                lsum = None
                for c in range(CPK):
                    p = jnp.exp2(s_s[j, :, c * LANES:(c + 1) * LANES] - m)
                    lsum = p if lsum is None else lsum + p
                    tiles.append(p)
                state['l'] = lsum if state['l'] is None else state['l'] + lsum
                tiles[0] = jnp.where(never2, state['l'], tiles[0])
                w = jnp.concatenate(FW.expand(blocks_of(jnp.concatenate(tiles, axis=1))), axis=1)
                po_s[j * HR // H:(j + 1) * HR // H, :] = _pack(w)
            return fence(po_s)

        def store_logits(g, m, t):
            for jj in range(G):
                j = g * G + jj
                s = combine([v[:, jj * LANES:(jj + 1) * LANES] for v in m], t,
                            tune['s_end'] * jj // G, tune['s_end'] * (jj + 1) // G)
                for c, st in enumerate(_split(s)):
                    if j == NKV - 1 and c == NFULL:
                        st = jnp.where(lax.broadcasted_iota(jnp.int32, st.shape, 1) < TAIL, st, -jnp.inf)
                    s_s[j, :, c * LANES:(c + 1) * LANES] = st
                    state['mx'] = st if state['mx'] is None else jnp.maximum(state['mx'], st)

        def side_work(phase, t):
            if phase == tune['g_at']:
                gg = _gelu2(combine([v[:, 0:LANES] for v in gm], t, 0, tune['g'][0]))
                g_new = _ln(rel2(gg, t, *tune['g']), 4.0 * EPS)
                store_g(gn_s, 0, g_new)
                store_g(g_s, HALO + TQ, jnp.where(ia == 0, 0.0, g_new[0:HALO, :]))
            if phase == tune['u_at']:
                u_s[...] = _gelu2(combine([v[:, LANES:] for v in gm], t, 0, tune['u_end']))
            if phase == 3 and normalise:
                unit = jnp.minimum(step - 1, NU - 1)
                c0, r0 = unit // UPC, jnp.minimum((unit % UPC) * UP, LANES - UP)
                xv = [x_s[pl.ds(pl.multiple_of(TP + c0 * TK + k * LANES + r0, 16), UP), :].astype(F32)
                      for k in range(CPK)]
                y = _ln(jnp.concatenate([_released(never, t, 50, 80, v) for v in xv], axis=0), EPS)
                for k in range(CPK):
                    row = pl.multiple_of((c0 * TK + k * LANES + r0) // H, 8)
                    xa1_s[pl.ds(row, UT), :] = _pack(y[k * UP:(k + 1) * UP])
                tb1_s[pl.ds(pl.multiple_of(c0 * TR + r0 // H, 8), UT), :] = key_tables(y)

        ready = None
        for g in range(NKV // G):
            if do_a:
                start = len(hist)
                sm = [None] * NPROD
                for r in ORDER:
                    sm[r] = matmul(qops[r], G, lambda v, r=r: _dot_nt(v, key_operand(ba, g, r)))
            if g == 0:
                ready = probabilities(0, toks(0) if do_a else None, *tune['e0'])
            if do_a:
                side_work(2 * g, toks(start))
            if tune['p_due']:
                pend.append(ready)
            start = len(hist)
            n = [None] * NPROD
            for r in PORDER:
                l = jnp.concatenate([po_s[j * HR // H:(j + 1) * HR // H, r * LANES:(r + 1) * LANES]
                                     for j in range(g * G, (g + 1) * G)], axis=1)
                n[r] = matmul(l, G, lambda v, r=r: _dot(v, key_operand(bb, g, r)))
            state['acc'] = n if state['acc'] is None else [x + y for x, y in zip(state['acc'], n)]
            t = toks(start)
            if do_a:
                store_logits(g, sm, t)
                if tune['s_due'][g] >= 0:
                    later.extend((len(hist) + tune['s_due'][g], state['mx'][r:r + 8]) for r in range(0, TQ, 8))
            if (g + 1) * G < NKV:
                ready = probabilities(g + 1, t, *tune['e1'])
            if do_a:
                side_work(2 * g + 1, t)
        yc = u_old * conv(never)
        ya = unblock(FU.contract(state['acc'], SWV, PORDER)) * (1.0 / jnp.sum(state['l'], axis=-1, keepdims=True))
        if tune['out_split']:
            om = project(FU.expand(blocks_of(yc)), [4], 0)
            om = [x + y for x, y in zip(om, project(FU.expand(blocks_of(ya)), [3], 0))]
        else:
            om = project([jnp.concatenate(p, axis=1)
                          for p in zip(FU.expand(blocks_of(ya)), FU.expand(blocks_of(yc)))], [3, 4], 0)
        out = combine(om)
        xr = x_s[pl.ds(_aligned(bb * TP + ib * TQ, 16), TQ), :].astype(F32)
        o_s[pl.ds(_aligned(sb * TQ, 16), TQ), :] = (xr + out).astype(o_s.dtype)
        if do_a:
            store_max(state['mx'])
        out_copy(sb).start()

    def iteration0(step, carry):
        step_body(step, 0, 0, TUNE['seq0'], normalise=True)

        @pl.when(step == 1)
        def _():
            rest_copy().wait()

        return carry

    def iteration1(step, carry):
        step_body(step, 1, 1, TUNE['seq1'])
        return carry

    first_step()
    lax.fori_loop(1, NQ, iteration0, 0)
    step_body(NQ + z_s[0], 1, 0, TUNE['seq1'])
    lax.fori_loop(NQ + 1, N, iteration1, 0)
    step_body(N, 1, 1, TUNE['last'], do_a=False)
    pltpu.make_async_copy(o_s, o_hbm, osem).wait()


@jax.jit
def pallas_standalone__conformer_family_branchformer__speech_kernel(
    x: jax.Array,
    w_q: jax.Array,
    w_k: jax.Array,
    w_v: jax.Array,
    w_ao: jax.Array,
    w_up: jax.Array,
    dw: jax.Array,
    w_dn: jax.Array,
    w_merge: jax.Array,
):
    B, T, D = x.shape
    K = dw.shape[0]
    TQ = 160
    TK = 512
    TP = -(-T // TK) * TK
    UR = 192
    NKV = TP // TK
    assert B == 2 and T % TQ == 0 and TQ % 32 == 0 and D == TK == 4 * LANES and K // 2 < HALO
    assert NKV * -(-TK // UR) < T // TQ and UR % 64 == 0 and NKV == 8 and T % LANES in (16, 32, 48, 64) and TP - T < LANES
    x2 = x.reshape(B * T, D)

    kern = functools.partial(_kernel, B=B, T=T, D=D, K=K, TQ=TQ, TK=TK, TP=TP, UR=UR)
    ins = (x2, w_q, w_k, w_v, w_ao, w_up, dw, w_dn, w_merge)
    out = pl.pallas_call(
        kern,
        in_specs=[pl.BlockSpec(memory_space=pl.ANY) for _ in ins],
        out_specs=pl.BlockSpec(memory_space=pl.ANY),
        out_shape=jax.ShapeDtypeStruct((B * T, D), x.dtype),
        scratch_shapes=[pltpu.VMEM((B * TP, D), x.dtype)] + [pltpu.VMEM(a.shape, a.dtype) for a in ins[1:]] + [
            pltpu.SemaphoreType.DMA((15,)),
            pltpu.VMEM((TP // H, D), U32),
            pltpu.VMEM((TP // H, D), U32),
            pltpu.VMEM((D // H, D), U32),
            pltpu.VMEM((K, 8, D), F32),
            pltpu.VMEM((NKV, TQ, TK), F32),
            pltpu.VMEM((TQ, LANES), F32),
            pltpu.VMEM((TQ, D), F32),
            pltpu.VMEM((D // LANES, TQ + 2 * HALO, LANES), F32),
            pltpu.VMEM((D // LANES, TQ, LANES), F32),
            pltpu.VMEM((B * T, D), x.dtype),
            pltpu.SemaphoreType.DMA(()),
            pltpu.VMEM((NKV * LANES // H, len(TABLED) * LANES), U32),
            pltpu.VMEM((NKV * LANES // H, len(TABLED) * LANES), U32),
            pltpu.VMEM((5 * LANES // H, NPROD * LANES), U32),
            pltpu.VMEM((NKV * TQ // 2 // H, NPROD * LANES), U32),
            pltpu.VMEM((TQ // 2 // H, NPROD * LANES), U32),
            pltpu.VMEM((TQ // 2 // H, NPROD * LANES), U32),
            pltpu.SMEM((3,), jnp.int32),
        ],
        compiler_params=pltpu.CompilerParams(
            vmem_limit_bytes=100 * 1024 * 1024,
            disable_bounds_checks=True,
            disable_semaphore_checks=True,
        ),
    )(*ins)
    return out.reshape(B, T, D)
```

```python
import functools
import math

import jax
import jax.numpy as jnp
from jax import lax
import jax.experimental.pallas as pl
import jax.experimental.pallas.tpu as pltpu

LANES = 128
EPS = 1e-05
F32 = jnp.float32
BF16 = jnp.bfloat16
U32 = jnp.uint32
NT = (((1,), (1,)), ((), ()))
HALO = 16
H = 2

SCHEME = (
    ('...-++..', '...+............', '-+.....+'),
    ('.+-.....', '.........-......', '.++..++.'),
    ('+...--..', '.+..+.......+...', '-+..-...'),
    ('.+.-.-.+', '...-...+....+...', '.-.+....'),
    ('.....+..', '.+...-+......-..', '.....-..'),
    ('+...-...', '+.-.-.......-...', '....-...'),
    ('--.+....', '...-........+...', '+-.+....'),
    ('..+...-.', '......+.-.+-....', '..+.....'),
    ('..-+....', '...........+....', '..--....'),
    ('-.....+.', '..+.....+.......', '..-.+...'),
    ('....+.-.', '..+.............', '....+.+.'),
    ('+.-.....', '........+.......', '-.-.....'),
    ('...-....', '...-.......-.-.-', '...+...+'),
    ('++..--..', '...-+.......+...', '+-......'),
    ('......+.', '..-......+-...-.', '..-...-.'),
    ('-.......', '++......+...+...', '-...-...'),
    ('-....-.+', '............+...', '.+.-+...'),
    ('.-+..+-.', '......+.........', '.....++.'),
    ('.-......', '...+--.-.-..-...', '.+......'),
    ('...-.-.+', '...+...-.....+..', '.-.+...+'),
    ('....--..', '.+..............', '+-..+-..'),
    ('...+...-', '...+...-......+-', '.......+'),
    ('...-..+.', '...........-..-.', '..+....-'),
    ('.-+...-.', '......-..-......', '..+..++.'),
    ('......+-', '..............+.', '......--'),
    ('.....-.+', '.............+..', '.+.-.+.-'),
)

_BASE = dict(lag=8, stride=3, q_end=60, e0=(45, 85), e1=(0, 100), s_end=60, s_due=(5, 10), p_due=True,
             g_at=2, g=(50, 90), u_at=3, u_end=20, out_split=False)
TUNE = {
    'seq0': dict(_BASE, stride=4, q_end=50, e0=(30, 92), e1=(10, 100), s_due=(5, 10), u_at=0, u_end=60),
    'seq1': _BASE,
    'last': dict(_BASE, lag=10, e1=(20, 80), p_due=False, out_split=True),
}


class _Forms:
    def __init__(self, rows):
        self.n = len(rows[0])
        forms = [{j: 1 if ch == '+' else -1 for j, ch in enumerate(r) if ch != '.'} for r in rows]
        self.steps = []
        while True:
            count = {}
            seen = set()
            for f in forms:
                items = sorted(f.items())
                key = tuple((j, v * items[0][1]) for j, v in items)
                if key not in seen:
                    seen.add(key)
                    for a in range(len(items)):
                        for b in range(a + 1, len(items)):
                            pair = (items[a][0], items[b][0], items[a][1] * items[b][1])
                            count[pair] = count.get(pair, 0) + 1
            if not count:
                break
            j, k, sg = max(count, key=count.get)
            new = self.n + len(self.steps)
            self.steps.append((j, k, sg))
            for f in forms:
                if j in f and k in f and f[j] * f[k] == sg:
                    f[new] = f.pop(j)
                    f.pop(k)
        self.node = [next(iter(f)) for f in forms]
        self.sign = [next(iter(f.values())) for f in forms]

    def expand(self, blocks):
        nodes = list(blocks)
        for j, k, sg in self.steps:
            nodes.append(nodes[j] + nodes[k] if sg > 0 else nodes[j] - nodes[k])
        return [nodes[i] for i in self.node]

    def contract(self, prods, signs, order):
        acc = {}

        def add(i, v, s):
            if i not in acc:
                acc[i] = (v, s)
            else:
                w, t = acc[i]
                acc[i] = (w + v, s) if s == t else ((w - v, 1) if t > 0 else (v - w, 1))

        for r in order:
            if self.node[r] >= self.n:
                add(self.node[r], prods[r], self.sign[r] * signs[r])
        for i in reversed(range(len(self.steps))):
            j, k, sg = self.steps[i]
            v, s = acc[self.n + i]
            add(j, v, s)
            add(k, v, s * sg)
        for r in order:
            if self.node[r] < self.n:
                add(self.node[r], prods[r], self.sign[r] * signs[r])
        return [acc[j][0] if acc[j][1] > 0 else -acc[j][0] for j in range(self.n)]


FU, FV, FW = (_Forms([t[i] for t in SCHEME]) for i in range(3))
NPROD = len(SCHEME)
TABLED = [r for r in range(NPROD) if FV.node[r] >= FV.n]


def _ln(x, eps):
    d = x.shape[-1]
    m = jnp.sum(x, axis=-1, keepdims=True) * (1.0 / d)
    xc = x - m
    v = jnp.sum(xc * xc, axis=-1, keepdims=True) * (1.0 / d)
    return xc * lax.rsqrt(v + eps)


def _gelu2(x):
    c1 = math.sqrt(2.0 / math.pi)
    c2 = c1 * 0.044715
    t = jnp.tanh(x * (c1 + c2 * (x * x)))
    return x + x * t


def _center(w):
    return w - jnp.sum(w, axis=0, keepdims=True) * (1.0 / w.shape[0])


def _pack(x):
    return pltpu.bitcast(x.astype(BF16), U32)


def _unpack(x):
    return pltpu.bitcast(x, BF16)


def _bits(x):
    return pltpu.bitcast(x, U32)


def _to_bf16(v):
    return _unpack(v) if v.dtype == U32 else v.astype(BF16)


def _dot(a, b):
    return jnp.dot(a, b, preferred_element_type=F32)


def _dot_nt(a, b):
    return lax.dot_general(a, b, NT, preferred_element_type=F32)


def _split(v):
    return [v[:, c * LANES:(c + 1) * LANES] for c in range(v.shape[1] // LANES)]


def _aligned(i, n):
    return i if isinstance(i, int) else pl.multiple_of(i, n)


def _tie_bf16(flag, dep, val):
    head = _bits(val[0:16, 0:LANES])
    head = _unpack(jnp.where(flag, _bits(dep), head))
    top = jnp.concatenate([head, val[0:16, LANES:]], axis=1)
    return jnp.concatenate([top, val[16:, :]], axis=0)


def _tie(flag, deps, val, row):
    cast = _bits if val.dtype == U32 else (lambda v: v if v.dtype == F32 else pltpu.bitcast(v, F32))
    tiles = _split(val)
    t = tiles[0]
    end = row + 8 * len(deps)
    mid = jnp.where(flag, jnp.concatenate([cast(d) for d in deps], axis=0), t[row:end])
    tiles[0] = jnp.concatenate(([t[0:row]] if row else []) + [mid] + ([t[end:]] if end < t.shape[0] else []),
                               axis=0)
    return jnp.concatenate(tiles, axis=1)


def _released(flag, toks, lo, hi, val, ntiles=1):
    first, total = len(toks) * lo // 100, len(toks) * (hi - lo) // 100
    n = val.shape[0] // 8
    rel = jnp.concatenate([toks[min(first + (i * total) // n, len(toks) - 1)] for i in range(n)], axis=0)
    tiles = _split(val)
    return jnp.concatenate([jnp.where(flag, rel, t) if c < ntiles else t for c, t in enumerate(tiles)], axis=1)


def _kernel(x_hbm, wq_hbm, wk_hbm, wv_hbm, wao_hbm, wup_hbm, dw_hbm, wdn_hbm, wm_hbm,
            o_hbm,
            x_s, wq_s, wk_s, wv_s, wao_s, wup_s, dw_s, wdn_s, wm_s, sems,
            xa0_s, xa1_s, wa_s, dwb_s, s_s, m_s, u_s, g_s, gn_s, o_s, osem,
            tb0_s, tb1_s, wt_s, po_s, xo_s, qo_s, z_s,
            *, B, T, D, K, TQ, TK, TP, UR):
    NQ = T // TQ
    N = B * NQ
    NKV = TP // TK
    NC = D // LANES
    CPK = TK // LANES
    PAD = K // 2
    NQT = -(-TQ // LANES)
    NFULL = (T - (NKV - 1) * TK) // LANES
    TAIL = T % LANES
    HR = TQ // 2
    TR = LANES // H
    TW = len(TABLED) * LANES
    G = 4
    UP = UR // CPK
    UPC = -(-LANES // UP)
    NU = NKV * UPC
    UT = UP // H
    ORDER = [15, 12, 14, 10, 23, 18, 6, 17, 16, 1, 22, 0, 25, 2, 11, 3, 8, 13, 9, 19, 20, 24, 4, 5, 7, 21]
    PORDER = sorted(range(NPROD), key=lambda r: FU.node[r] < FU.n)
    SUV = [FU.sign[r] * FV.sign[r] for r in range(NPROD)]
    SWV = [FW.sign[r] * FV.sign[r] for r in range(NPROD)]
    xa_s, tb_s = (xa0_s, xa1_s), (tb0_s, tb1_s)

    def blocks_of(a):
        return [a[h * HR:(h + 1) * HR, c * LANES:(c + 1) * LANES] for h in range(2) for c in range(NC)]

    def unblock(bl):
        return jnp.concatenate([jnp.concatenate(bl[h * NC:(h + 1) * NC], axis=1) for h in range(2)], axis=0)

    def key_tables(y):
        n = y.shape[0] // CPK
        ops = FV.expand([y[t * n:(t + 1) * n, d * LANES:(d + 1) * LANES] for d in range(NC) for t in range(CPK)])
        return _pack(jnp.concatenate([ops[r] for r in TABLED], axis=1))

    def weight_tables(mat, w):
        ops = FV.expand([w[d * LANES:(d + 1) * LANES, t * LANES:(t + 1) * LANES]
                         for d in range(NC) for t in range(NC)])
        wt_s[mat * TR:(mat + 1) * TR, :] = _pack(jnp.concatenate(ops, axis=1))

    def fence(ref):
        return ref[pl.ds(pl.multiple_of(z_s[0], 8), 8), 0:LANES]

    def staged_operands(ref, a, which):
        ops = FU.expand(blocks_of(a))
        ref[:, 0:len(which) * LANES] = _pack(jnp.concatenate([ops[r] for r in which], axis=1))
        done = fence(ref)
        return {r: ref[:, k * LANES:(k + 1) * LANES] for k, r in enumerate(which)}, done

    def key_operand(b, g, r):
        i = FV.node[r]
        if i < FV.n:
            d, t = i // CPK, i % CPK
            parts = [xa_s[b][pl.ds((j * TK + t * LANES) // H, TR), d * LANES:(d + 1) * LANES]
                     for j in range(g * G, (g + 1) * G)]
        else:
            k = TABLED.index(r)
            parts = [tb_s[b][j * TR:(j + 1) * TR, k * LANES:(k + 1) * LANES] for j in range(g * G, (g + 1) * G)]
        return _unpack(jnp.concatenate(parts, axis=0))

    def store_g(ref, row, g):
        for c in range(NC):
            ref[c, row:row + g.shape[0], :] = g[:, c * LANES:(c + 1) * LANES]

    def conv(flag):
        prev = None
        rows = []
        for rr in range(0, TQ, 16):
            cols = []
            for c in range(NC):
                acc = None
                for k in range(K):
                    gv = g_s[c, pl.ds(rr + HALO - PAD + k, 16), :].reshape(2, 8, LANES)
                    term = gv * dwb_s[k, :, c * LANES:(c + 1) * LANES][None]
                    if acc is None:
                        acc = term if prev is None else jnp.where(flag, prev, term)
                    else:
                        acc = acc + term
                prev = acc
                cols.append(acc.reshape(16, LANES))
            rows.append(jnp.concatenate(cols, axis=1))
        return jnp.concatenate(rows, axis=0)

    def store_max(mx):
        m = jnp.max(mx, axis=-1, keepdims=True)
        m = m + jnp.log2(jnp.sum(jnp.exp2(mx - m), axis=-1, keepdims=True))
        m_s[...] = jnp.broadcast_to(m, (TQ, LANES))

    def rest_copy():
        return pltpu.make_async_copy(x_hbm.at[pl.ds(T + TK, T - TK), :], x_s.at[pl.ds(TP + TK, T - TK), :],
                                     sems.at[14])

    def out_copy(blk):
        rows = pl.ds(_aligned(blk * TQ, 16), TQ)
        return pltpu.make_async_copy(o_s.at[rows, :], o_hbm.at[rows, :], osem)

    def first_step():
        C1, C2 = 3, 6

        def xrows(b, r0, r1):
            return x_hbm.at[pl.ds(b * T + r0, r1 - r0), :], x_s.at[pl.ds(b * TP + r0, r1 - r0), :]

        copies = {}
        plan = (
            ('wq', wq_hbm, wq_s), ('wk', wk_hbm, wk_s),
            ('xa',) + xrows(0, 0, TK), ('xb',) + xrows(0, TK, C1 * TK), ('xc',) + xrows(0, C1 * TK, C2 * TK),
            ('xd',) + xrows(0, C2 * TK, T), ('wv', wv_hbm, wv_s), ('wao', wao_hbm, wao_s),
            ('wm1', wm_hbm.at[pl.ds(0, D), :], wm_s.at[pl.ds(0, D), :]), ('wup', wup_hbm, wup_s), ('dw', dw_hbm, dw_s),
            ('wdn', wdn_hbm, wdn_s), ('wm2', wm_hbm.at[pl.ds(D, D), :], wm_s.at[pl.ds(D, D), :]),
            ('xe',) + xrows(1, 0, TK),
        )
        for i, (name, src, dst) in enumerate(plan):
            copies[name] = pltpu.make_async_copy(src, dst, sems.at[i])
            copies[name].start()
        rest_copy().start()

        z_s[0] = 0
        z_s[1] = 0
        z_s[2] = 0
        for b in range(B):
            x_s[b * TP + T:(b + 1) * TP, :] = jnp.zeros((TP - T, D), x_s.dtype)
        store_g(g_s, TQ, jnp.zeros((HALO, D), F32))

        def keys(r0, n):
            return _unpack(xa0_s[r0 // H:(r0 + n) // H, 0:D])

        def ln_chunk(c):
            y = _ln(x_s[c * TK:(c + 1) * TK, :].astype(F32), EPS)
            xa0_s[c * TK // H:(c + 1) * TK // H, 0:D] = _pack(y)
            tb0_s[c * TR:(c + 1) * TR, 0:TW] = key_tables(y)

        scale = float(D) ** (-0.5) * math.log2(math.e)
        DS = D // 2
        copies['wq'].wait()
        copies['wk'].wait()
        m_lo = _dot_nt(wq_s[...], wk_s[0:DS, :])

        never = z_s[0] > 0

        def after(prev, l):
            return _unpack(l if prev is None else _tie(never, [prev[0:8, 0:LANES]], l, 0))

        copies['xa'].wait()
        wa_s[:, 0:DS] = _pack(_center(m_lo) * scale)
        wa_s[:, DS:D] = _pack(_center(_dot_nt(wq_s[...], wk_s[DS:D, :])) * scale)
        ln_chunk(0)
        qp = _pack(_dot(keys(0, TQ), _unpack(wa_s[:, 0:D])))
        q = _unpack(qp)

        def tail_parts():
            kt = keys(T - TAIL, TAIL)
            parts = []
            for n in range(NQT):
                qn = q[n * LANES:min((n + 1) * LANES, TQ), :]
                if qn.shape[0] < LANES:
                    qn = jnp.concatenate([qn, jnp.zeros((LANES - qn.shape[0], D), BF16)], axis=0)
                parts.append(_dot_nt(kt, qn))
            return parts

        def logits(c, prev, mx):
            last = c == NKV - 1
            parts = tail_parts() if last else None
            s = _dot_nt(after(prev, qp), keys(c * TK, (NFULL if last else CPK) * LANES))
            mc = None
            for t in range(CPK):
                if last and t == NFULL:
                    fill = jnp.full((LANES - TAIL, LANES), -jnp.inf, F32)
                    st = jnp.concatenate([jnp.concatenate([p, fill], axis=0).T for p in parts], axis=0)[0:TQ, :]
                else:
                    st = s[:, t * LANES:(t + 1) * LANES]
                s_s[c, :, t * LANES:(t + 1) * LANES] = st
                mc = st if mc is None else jnp.maximum(mc, st)
            return s, mc if mx is None else jnp.maximum(mx, mc)

        copies['xb'].wait()
        prev, mx = logits(0, None, None)
        for c in range(1, C1):
            ln_chunk(c)
            prev, mx = logits(c, prev, mx)

        copies['xc'].wait()
        prev = None
        for c in range(C1, C2):
            ln_chunk(c)
            prev, mx = logits(c, prev, mx)

        for name in ('xd', 'wv', 'wao'):
            copies[name].wait()
        wva_raw = _dot(wv_s[...], wao_s[...])
        mean = jnp.sum(wva_raw, axis=0, keepdims=True) * (1.0 / D)
        prev = wva_raw
        for c in range(C2, NKV):
            ln_chunk(c)
            prev, mx = logits(c, prev, mx)

        def tokens(res):
            return [res[r:r + 8, c * LANES:(c + 1) * LANES] for c in range(NC) for r in range(0, res.shape[0], 8)]

        def rel(t, lo, hi, v):
            return _released(never, t, lo, hi, v, NC)

        for name in ('wm1', 'wup', 'dw'):
            copies[name].wait()
        store_max(mx)
        xq = xa0_s[0:TQ // H, 0:D]
        hg = _dot(after(None, xq), wup_s[:, D:2 * D])
        hu = _dot(after(hg, xq), wup_s[:, 0:D])
        dwf = dw_s[...].astype(F32)
        for k in range(K):
            dwb_s[k] = jnp.broadcast_to(dwf[k:k + 1, :], (8, D))
        wva = (wva_raw - mean).astype(BF16)
        wvom = _dot(_tie_bf16(never, hu[0:8, 0:LANES], wva), wm_s[0:D, :])
        t1 = tokens(hg) + tokens(hu) + tokens(wvom)
        weight_tables(0, rel(t1, 0, 60, _unpack(wa_s[:, 0:D]).astype(F32)))
        weight_tables(1, rel(t1, 0, 70, wup_s[:, D:2 * D].astype(F32)))
        weight_tables(2, rel(t1, 60, 95, wup_s[:, 0:D].astype(F32)))

        for name in ('wdn', 'wm2'):
            copies[name].wait()
        wdm = _dot(wdn_s[...], wm_s[D:2 * D, :])
        t2 = tokens(wdm)
        store_g(gn_s, 0, _ln(_gelu2(rel(t2, 0, 40, hg)), 4.0 * EPS))
        u_s[...] = _gelu2(rel(t2, 0, 40, hu))
        weight_tables(3, rel(t2, 20, 80, wvom))
        weight_tables(4, 0.5 * wdm)
        copies['xe'].wait()

    def step_body(step, ba, bb, tune, normalise=False, do_a=True):
        sb = step - 1
        ia, ib = step - ba * NQ, sb - bb * NQ
        never = z_s[0] > 0
        never2 = z_s[1] > 0
        never3 = z_s[2] > 0
        for c in range(NC):
            g_s[c, 0:HALO, :] = jnp.where(ib == 0, 0.0, g_s[c, TQ:TQ + HALO, :])
            g_s[c, HALO:HALO + TQ, :] = gn_s[c]
        hist = []
        pend = []
        later = []

        def matmul(l, tiles, run):
            back = 0
            for res, n in reversed(hist):
                back += n
                if back >= tune['lag']:
                    l = _tie(never3, [res[0:8, 0:LANES]], l, 0)
                    break
            while later and later[0][0] <= len(hist) and len(pend) < 4:
                pend.append(later.pop(0)[1])
            if pend:
                l = _tie(never3, pend, l, 8)
                del pend[:]
            hist.append((run(_to_bf16(l)), tiles))
            return hist[-1][0]

        def toks(i0):
            return [res[r:r + 8, 0:LANES] for res, n in hist[i0:] for r in range(0, HR, 8 * (4 // n))]

        def rel2(v, t, lo, hi):
            return jnp.concatenate([_released(never, t, lo, hi, v[0:HR]), _released(never, t, lo, hi, v[HR:])],
                                   axis=0)

        def project(ops, mats, axis):
            m = [None] * NPROD
            for r in ORDER:
                m[r] = matmul(ops[r], len(mats), lambda v, r=r: _dot(v, _unpack(jnp.concatenate(
                    [wt_s[k * TR:(k + 1) * TR, r * LANES:(r + 1) * LANES] for k in mats], axis=axis))))
            return m

        def combine(prods, t=None, lo=0, hi=0):
            if t is not None:
                prods = list(prods)
                for r in ORDER[::tune['stride']]:
                    prods[r] = _released(never, t, lo, hi, prods[r])
            return unblock(FW.contract(prods, SUV, ORDER))

        m_old = m_s[...]
        u_old = u_s[...]
        if do_a:
            xq = xa_s[ba][pl.ds(_aligned(ia * (TQ // H), 8), TQ // H), 0:D]
            xops, _ = staged_operands(xo_s, _unpack(xq).astype(F32),
                                      [r for r in range(NPROD) if FU.node[r] >= FU.n])
            for r in range(NPROD):
                i = FU.node[r]
                if i < FU.n:
                    xops[r] = xq[(i // NC) * HR // H:(i // NC + 1) * HR // H, (i % NC) * LANES:(i % NC + 1) * LANES]
            qm = project(xops, [0], 1)
            gm = project(xops, [1, 2], 1)
            q_raw = combine(qm, toks(NPROD), 0, tune['q_end'])
            qops, done = staged_operands(qo_s, q_raw, list(range(NPROD)))
            pend.append(done)
        else:
            store_g(g_s, HALO + TQ, jnp.zeros((HALO, D), F32))
        state = {'l': None, 'acc': None, 'mx': None}

        def probabilities(g, t, lo, hi):
            for jj in range(G):
                j = g * G + jj
                m = m_old if t is None else rel2(m_old, t, lo + (hi - lo) * jj // G, lo + (hi - lo) * (jj + 1) // G)
                tiles = []
                lsum = None
                for c in range(CPK):
                    p = jnp.exp2(s_s[j, :, c * LANES:(c + 1) * LANES] - m)
                    lsum = p if lsum is None else lsum + p
                    tiles.append(p)
                state['l'] = lsum if state['l'] is None else state['l'] + lsum
                tiles[0] = jnp.where(never2, state['l'], tiles[0])
                w = jnp.concatenate(FW.expand(blocks_of(jnp.concatenate(tiles, axis=1))), axis=1)
                po_s[j * HR // H:(j + 1) * HR // H, :] = _pack(w)
            return fence(po_s)

        def store_logits(g, m, t):
            for jj in range(G):
                j = g * G + jj
                s = combine([v[:, jj * LANES:(jj + 1) * LANES] for v in m], t,
                            tune['s_end'] * jj // G, tune['s_end'] * (jj + 1) // G)
                for c, st in enumerate(_split(s)):
                    if j == NKV - 1 and c == NFULL:
                        st = jnp.where(lax.broadcasted_iota(jnp.int32, st.shape, 1) < TAIL, st, -jnp.inf)
                    s_s[j, :, c * LANES:(c + 1) * LANES] = st
                    state['mx'] = st if state['mx'] is None else jnp.maximum(state['mx'], st)

        def side_work(phase, t):
            if phase == tune['g_at']:
                gg = _gelu2(combine([v[:, 0:LANES] for v in gm], t, 0, tune['g'][0]))
                g_new = _ln(rel2(gg, t, *tune['g']), 4.0 * EPS)
                store_g(gn_s, 0, g_new)
                store_g(g_s, HALO + TQ, jnp.where(ia == 0, 0.0, g_new[0:HALO, :]))
            if phase == tune['u_at']:
                u_s[...] = _gelu2(combine([v[:, LANES:] for v in gm], t, 0, tune['u_end']))
            if phase == 3 and normalise:
                unit = jnp.minimum(step - 1, NU - 1)
                c0, r0 = unit // UPC, jnp.minimum((unit % UPC) * UP, LANES - UP)
                xv = [x_s[pl.ds(pl.multiple_of(TP + c0 * TK + k * LANES + r0, 16), UP), :].astype(F32)
                      for k in range(CPK)]
                y = _ln(jnp.concatenate([_released(never, t, 50, 80, v) for v in xv], axis=0), EPS)
                for k in range(CPK):
                    row = pl.multiple_of((c0 * TK + k * LANES + r0) // H, 8)
                    xa1_s[pl.ds(row, UT), 0:D] = _pack(y[k * UP:(k + 1) * UP])
                tb1_s[pl.ds(pl.multiple_of(c0 * TR + r0 // H, 8), UT), 0:TW] = key_tables(y)

        ready = None
        for g in range(NKV // G):
            if do_a:
                start = len(hist)
                sm = [None] * NPROD
                for r in ORDER:
                    sm[r] = matmul(qops[r], G, lambda v, r=r: _dot_nt(v, key_operand(ba, g, r)))
            if g == 0:
                ready = probabilities(0, toks(0) if do_a else None, *tune['e0'])
            if do_a:
                side_work(2 * g, toks(start))
            if tune['p_due']:
                pend.append(ready)
            start = len(hist)
            n = [None] * NPROD
            for r in PORDER:
                l = jnp.concatenate([po_s[j * HR // H:(j + 1) * HR // H, r * LANES:(r + 1) * LANES]
                                     for j in range(g * G, (g + 1) * G)], axis=1)
                n[r] = matmul(l, G, lambda v, r=r: _dot(v, key_operand(bb, g, r)))
            state['acc'] = n if state['acc'] is None else [x + y for x, y in zip(state['acc'], n)]
            t = toks(start)
            if do_a:
                store_logits(g, sm, t)
                if tune['s_due'][g] >= 0:
                    later.extend((len(hist) + tune['s_due'][g], state['mx'][r:r + 8]) for r in range(0, TQ, 8))
            if (g + 1) * G < NKV:
                ready = probabilities(g + 1, t, *tune['e1'])
            if do_a:
                side_work(2 * g + 1, t)
        yc = u_old * conv(never)
        ya = unblock(FU.contract(state['acc'], SWV, PORDER)) * (1.0 / jnp.sum(state['l'], axis=-1, keepdims=True))
        if tune['out_split']:
            om = project(FU.expand(blocks_of(yc)), [4], 0)
            om = [x + y for x, y in zip(om, project(FU.expand(blocks_of(ya)), [3], 0))]
        else:
            om = project([jnp.concatenate(p, axis=1)
                          for p in zip(FU.expand(blocks_of(ya)), FU.expand(blocks_of(yc)))], [3, 4], 0)
        out = combine(om)
        xr = x_s[pl.ds(_aligned(bb * TP + ib * TQ, 16), TQ), :].astype(F32)
        o_s[pl.ds(_aligned(sb * TQ, 16), TQ), :] = (xr + out).astype(o_s.dtype)
        if do_a:
            store_max(state['mx'])
        out_copy(sb).start()

    def iteration0(step, carry):
        step_body(step, 0, 0, TUNE['seq0'], normalise=True)

        @pl.when(step == 1)
        def _():
            rest_copy().wait()

        return carry

    def iteration1(step, carry):
        step_body(step, 1, 1, TUNE['seq1'])
        return carry

    first_step()
    lax.fori_loop(1, NQ, iteration0, 0)
    step_body(NQ + z_s[0], 1, 0, TUNE['seq1'])
    lax.fori_loop(NQ + 1, N, iteration1, 0)
    step_body(N, 1, 1, TUNE['last'], do_a=False)
    pltpu.make_async_copy(o_s, o_hbm, osem).wait()


@jax.jit
def pallas_standalone__conformer_family_branchformer__speech_kernel(
    x: jax.Array,
    w_q: jax.Array,
    w_k: jax.Array,
    w_v: jax.Array,
    w_ao: jax.Array,
    w_up: jax.Array,
    dw: jax.Array,
    w_dn: jax.Array,
    w_merge: jax.Array,
):
    B, T, D = x.shape
    K = dw.shape[0]
    TQ = 160
    TK = 512
    TP = -(-T // TK) * TK
    UR = 192
    NKV = TP // TK
    assert B == 2 and T % TQ == 0 and TQ % 32 == 0 and D == TK == 4 * LANES and K // 2 < HALO
    assert NKV * -(-TK // UR) < T // TQ and UR % 64 == 0 and NKV == 8 and T % LANES in (16, 32, 48, 64) and TP - T < LANES
    x2 = x.reshape(B * T, D)

    kern = functools.partial(_kernel, B=B, T=T, D=D, K=K, TQ=TQ, TK=TK, TP=TP, UR=UR)
    ins = (x2, w_q, w_k, w_v, w_ao, w_up, dw, w_dn, w_merge)
    out = pl.pallas_call(
        kern,
        in_specs=[pl.BlockSpec(memory_space=pl.ANY) for _ in ins],
        out_specs=pl.BlockSpec(memory_space=pl.ANY),
        out_shape=jax.ShapeDtypeStruct((B * T, D), x.dtype),
        scratch_shapes=[pltpu.VMEM((B * TP, D), x.dtype)] + [pltpu.VMEM(a.shape, a.dtype) for a in ins[1:]] + [
            pltpu.SemaphoreType.DMA((15,)),
            pltpu.VMEM((TP // H, D + 2 * LANES), U32),
            pltpu.VMEM((TP // H, D + 2 * LANES), U32),
            pltpu.VMEM((D // H, D), U32),
            pltpu.VMEM((K, 8, D), F32),
            pltpu.VMEM((NKV, TQ, TK), F32),
            pltpu.VMEM((TQ, LANES), F32),
            pltpu.VMEM((TQ, D), F32),
            pltpu.VMEM((D // LANES, TQ + 2 * HALO, LANES), F32),
            pltpu.VMEM((D // LANES, TQ, LANES), F32),
            pltpu.VMEM((B * T, D), x.dtype),
            pltpu.SemaphoreType.DMA(()),
            pltpu.VMEM((NKV * LANES // H, (len(TABLED) + 1) * LANES), U32),
            pltpu.VMEM((NKV * LANES // H, (len(TABLED) + 1) * LANES), U32),
            pltpu.VMEM((5 * LANES // H, NPROD * LANES), U32),
            pltpu.VMEM((NKV * TQ // 2 // H, NPROD * LANES), U32),
            pltpu.VMEM((TQ // 2 // H, NPROD * LANES), U32),
            pltpu.VMEM((TQ // 2 // H, NPROD * LANES), U32),
            pltpu.SMEM((3,), jnp.int32),
        ],
        compiler_params=pltpu.CompilerParams(
            vmem_limit_bytes=100 * 1024 * 1024,
            disable_bounds_checks=True,
            disable_semaphore_checks=True,
        ),
    )(*ins)
    return out.reshape(B, T, D)
```

```python
import functools
import math

import jax
import jax.numpy as jnp
from jax import lax
import jax.experimental.pallas as pl
import jax.experimental.pallas.tpu as pltpu

LANES = 128
EPS = 1e-05
F32 = jnp.float32
BF16 = jnp.bfloat16
U32 = jnp.uint32
NT = (((1,), (1,)), ((), ()))
HALO = 16
H = 2

SCHEME = (
    ('...-++..', '...+............', '-+.....+'),
    ('.+-.....', '.........-......', '.++..++.'),
    ('+...--..', '.+..+.......+...', '-+..-...'),
    ('.+.-.-.+', '...-...+....+...', '.-.+....'),
    ('.....+..', '.+...-+......-..', '.....-..'),
    ('+...-...', '+.-.-.......-...', '....-...'),
    ('--.+....', '...-........+...', '+-.+....'),
    ('..+...-.', '......+.-.+-....', '..+.....'),
    ('..-+....', '...........+....', '..--....'),
    ('-.....+.', '..+.....+.......', '..-.+...'),
    ('....+.-.', '..+.............', '....+.+.'),
    ('+.-.....', '........+.......', '-.-.....'),
    ('...-....', '...-.......-.-.-', '...+...+'),
    ('++..--..', '...-+.......+...', '+-......'),
    ('......+.', '..-......+-...-.', '..-...-.'),
    ('-.......', '++......+...+...', '-...-...'),
    ('-....-.+', '............+...', '.+.-+...'),
    ('.-+..+-.', '......+.........', '.....++.'),
    ('.-......', '...+--.-.-..-...', '.+......'),
    ('...-.-.+', '...+...-.....+..', '.-.+...+'),
    ('....--..', '.+..............', '+-..+-..'),
    ('...+...-', '...+...-......+-', '.......+'),
    ('...-..+.', '...........-..-.', '..+....-'),
    ('.-+...-.', '......-..-......', '..+..++.'),
    ('......+-', '..............+.', '......--'),
    ('.....-.+', '.............+..', '.+.-.+.-'),
)

_BASE = dict(order=[15, 12, 14, 10, 23, 18, 6, 17, 16, 1, 22, 0, 25, 2, 11, 3, 8, 13, 9, 19, 20, 24, 4, 5, 7, 21],
             lag=8, stride=3, q_end=60, e0=(45, 85), e1=(0, 100), s_end=60, s_due=(5, 10), p_due=True,
             g_at=2, g=(50, 90), u_at=3, u_end=20, out_split=False)
TUNE = {
    'seq0': dict(_BASE, order=[15, 12, 14, 0, 8, 4, 11, 13, 17, 1, 3, 18, 16, 25, 6, 9, 22, 2, 23, 20, 19, 10, 24, 5, 7, 21],
                 lag=9, stride=4, q_end=70, e0=(30, 92), e1=(10, 100), s_due=(5, -1), u_at=0, u_end=60),
    'seq1': dict(_BASE, order=[15, 12, 14, 10, 4, 13, 22, 0, 9, 20, 18, 11, 25, 3, 8, 24, 6, 2, 1, 17, 19, 23, 16, 5, 7, 21],
                 lag=9, q_end=70, s_end=70, s_due=(0, -1)),
    'last': dict(_BASE, lag=10, e1=(20, 80), p_due=False, out_split=True),
}


class _Forms:
    def __init__(self, rows):
        self.n = len(rows[0])
        forms = [{j: 1 if ch == '+' else -1 for j, ch in enumerate(r) if ch != '.'} for r in rows]
        self.steps = []
        while True:
            count = {}
            seen = set()
            for f in forms:
                items = sorted(f.items())
                key = tuple((j, v * items[0][1]) for j, v in items)
                if key not in seen:
                    seen.add(key)
                    for a in range(len(items)):
                        for b in range(a + 1, len(items)):
                            pair = (items[a][0], items[b][0], items[a][1] * items[b][1])
                            count[pair] = count.get(pair, 0) + 1
            if not count:
                break
            j, k, sg = max(count, key=count.get)
            new = self.n + len(self.steps)
            self.steps.append((j, k, sg))
            for f in forms:
                if j in f and k in f and f[j] * f[k] == sg:
                    f[new] = f.pop(j)
                    f.pop(k)
        self.node = [next(iter(f)) for f in forms]
        self.sign = [next(iter(f.values())) for f in forms]

    def expand(self, blocks):
        nodes = list(blocks)
        for j, k, sg in self.steps:
            nodes.append(nodes[j] + nodes[k] if sg > 0 else nodes[j] - nodes[k])
        return [nodes[i] for i in self.node]

    def contract(self, prods, signs, order):
        acc = {}

        def add(i, v, s):
            if i not in acc:
                acc[i] = (v, s)
            else:
                w, t = acc[i]
                acc[i] = (w + v, s) if s == t else ((w - v, 1) if t > 0 else (v - w, 1))

        for r in order:
            if self.node[r] >= self.n:
                add(self.node[r], prods[r], self.sign[r] * signs[r])
        for i in reversed(range(len(self.steps))):
            j, k, sg = self.steps[i]
            v, s = acc[self.n + i]
            add(j, v, s)
            add(k, v, s * sg)
        for r in order:
            if self.node[r] < self.n:
                add(self.node[r], prods[r], self.sign[r] * signs[r])
        return [acc[j][0] if acc[j][1] > 0 else -acc[j][0] for j in range(self.n)]


FU, FV, FW = (_Forms([t[i] for t in SCHEME]) for i in range(3))
NPROD = len(SCHEME)
TABLED = [r for r in range(NPROD) if FV.node[r] >= FV.n]


def _ln(x, eps):
    d = x.shape[-1]
    m = jnp.sum(x, axis=-1, keepdims=True) * (1.0 / d)
    xc = x - m
    v = jnp.sum(xc * xc, axis=-1, keepdims=True) * (1.0 / d)
    return xc * lax.rsqrt(v + eps)


def _gelu2(x):
    c1 = math.sqrt(2.0 / math.pi)
    c2 = c1 * 0.044715
    t = jnp.tanh(x * (c1 + c2 * (x * x)))
    return x + x * t


def _center(w):
    return w - jnp.sum(w, axis=0, keepdims=True) * (1.0 / w.shape[0])


def _pack(x):
    return pltpu.bitcast(x.astype(BF16), U32)


def _unpack(x):
    return pltpu.bitcast(x, BF16)


def _bits(x):
    return pltpu.bitcast(x, U32)


def _to_bf16(v):
    return _unpack(v) if v.dtype == U32 else v.astype(BF16)


def _dot(a, b):
    return jnp.dot(a, b, preferred_element_type=F32)


def _dot_nt(a, b):
    return lax.dot_general(a, b, NT, preferred_element_type=F32)


def _split(v):
    return [v[:, c * LANES:(c + 1) * LANES] for c in range(v.shape[1] // LANES)]


def _aligned(i, n):
    return i if isinstance(i, int) else pl.multiple_of(i, n)


def _tie_bf16(flag, dep, val):
    head = _bits(val[0:16, 0:LANES])
    head = _unpack(jnp.where(flag, _bits(dep), head))
    top = jnp.concatenate([head, val[0:16, LANES:]], axis=1)
    return jnp.concatenate([top, val[16:, :]], axis=0)


def _tie(flag, deps, val, row):
    cast = _bits if val.dtype == U32 else (lambda v: v if v.dtype == F32 else pltpu.bitcast(v, F32))
    tiles = _split(val)
    t = tiles[0]
    end = row + 8 * len(deps)
    mid = jnp.where(flag, jnp.concatenate([cast(d) for d in deps], axis=0), t[row:end])
    tiles[0] = jnp.concatenate(([t[0:row]] if row else []) + [mid] + ([t[end:]] if end < t.shape[0] else []),
                               axis=0)
    return jnp.concatenate(tiles, axis=1)


def _released(flag, toks, lo, hi, val, ntiles=1):
    first, total = len(toks) * lo // 100, len(toks) * (hi - lo) // 100
    n = val.shape[0] // 8
    rel = jnp.concatenate([toks[min(first + (i * total) // n, len(toks) - 1)] for i in range(n)], axis=0)
    tiles = _split(val)
    return jnp.concatenate([jnp.where(flag, rel, t) if c < ntiles else t for c, t in enumerate(tiles)], axis=1)


def _kernel(x_hbm, wq_hbm, wk_hbm, wv_hbm, wao_hbm, wup_hbm, dw_hbm, wdn_hbm, wm_hbm,
            o_hbm,
            x_s, wq_s, wk_s, wv_s, wao_s, wup_s, dw_s, wdn_s, wm_s, sems,
            xa0_s, xa1_s, wa_s, dwb_s, s_s, m_s, u_s, g_s, gn_s, o_s, osem,
            tb0_s, tb1_s, wt_s, po_s, xo_s, qo_s, z_s,
            *, B, T, D, K, TQ, TK, TP, UR):
    NQ = T // TQ
    N = B * NQ
    NKV = TP // TK
    NC = D // LANES
    CPK = TK // LANES
    PAD = K // 2
    NQT = -(-TQ // LANES)
    NFULL = (T - (NKV - 1) * TK) // LANES
    TAIL = T % LANES
    HR = TQ // 2
    TR = LANES // H
    TW = len(TABLED) * LANES
    G = 4
    UP = UR // CPK
    UPC = -(-LANES // UP)
    NU = NKV * UPC
    UT = UP // H
    PORDER = sorted(range(NPROD), key=lambda r: FU.node[r] < FU.n)
    SUV = [FU.sign[r] * FV.sign[r] for r in range(NPROD)]
    SWV = [FW.sign[r] * FV.sign[r] for r in range(NPROD)]
    xa_s, tb_s = (xa0_s, xa1_s), (tb0_s, tb1_s)

    def blocks_of(a):
        return [a[h * HR:(h + 1) * HR, c * LANES:(c + 1) * LANES] for h in range(2) for c in range(NC)]

    def unblock(bl):
        return jnp.concatenate([jnp.concatenate(bl[h * NC:(h + 1) * NC], axis=1) for h in range(2)], axis=0)

    def key_tables(y):
        n = y.shape[0] // CPK
        ops = FV.expand([y[t * n:(t + 1) * n, d * LANES:(d + 1) * LANES] for d in range(NC) for t in range(CPK)])
        return _pack(jnp.concatenate([ops[r] for r in TABLED], axis=1))

    def weight_tables(mat, w):
        ops = FV.expand([w[d * LANES:(d + 1) * LANES, t * LANES:(t + 1) * LANES]
                         for d in range(NC) for t in range(NC)])
        wt_s[mat * TR:(mat + 1) * TR, :] = _pack(jnp.concatenate(ops, axis=1))

    def fence(ref):
        return ref[pl.ds(pl.multiple_of(z_s[0], 8), 8), 0:LANES]

    def staged_operands(ref, a, which):
        ops = FU.expand(blocks_of(a))
        ref[:, 0:len(which) * LANES] = _pack(jnp.concatenate([ops[r] for r in which], axis=1))
        done = fence(ref)
        return {r: ref[:, k * LANES:(k + 1) * LANES] for k, r in enumerate(which)}, done

    def key_operand(b, g, r):
        i = FV.node[r]
        if i < FV.n:
            d, t = i // CPK, i % CPK
            parts = [xa_s[b][pl.ds((j * TK + t * LANES) // H, TR), d * LANES:(d + 1) * LANES]
                     for j in range(g * G, (g + 1) * G)]
        else:
            k = TABLED.index(r)
            parts = [tb_s[b][j * TR:(j + 1) * TR, k * LANES:(k + 1) * LANES] for j in range(g * G, (g + 1) * G)]
        return _unpack(jnp.concatenate(parts, axis=0))

    def store_g(ref, row, g):
        for c in range(NC):
            ref[c, row:row + g.shape[0], :] = g[:, c * LANES:(c + 1) * LANES]

    def conv(flag):
        prev = None
        rows = []
        for rr in range(0, TQ, 16):
            cols = []
            for c in range(NC):
                acc = None
                for k in range(K):
                    gv = g_s[c, pl.ds(rr + HALO - PAD + k, 16), :].reshape(2, 8, LANES)
                    term = gv * dwb_s[k, :, c * LANES:(c + 1) * LANES][None]
                    if acc is None:
                        acc = term if prev is None else jnp.where(flag, prev, term)
                    else:
                        acc = acc + term
                prev = acc
                cols.append(acc.reshape(16, LANES))
            rows.append(jnp.concatenate(cols, axis=1))
        return jnp.concatenate(rows, axis=0)

    def store_max(mx):
        m = jnp.max(mx, axis=-1, keepdims=True)
        m = m + jnp.log2(jnp.sum(jnp.exp2(mx - m), axis=-1, keepdims=True))
        m_s[...] = jnp.broadcast_to(m, (TQ, LANES))

    def rest_copy():
        return pltpu.make_async_copy(x_hbm.at[pl.ds(T + TK, T - TK), :], x_s.at[pl.ds(TP + TK, T - TK), :],
                                     sems.at[14])

    def out_copy(blk):
        rows = pl.ds(_aligned(blk * TQ, 16), TQ)
        return pltpu.make_async_copy(o_s.at[rows, :], o_hbm.at[rows, :], osem)

    def first_step():
        C1, C2 = 3, 6

        def xrows(b, r0, r1):
            return x_hbm.at[pl.ds(b * T + r0, r1 - r0), :], x_s.at[pl.ds(b * TP + r0, r1 - r0), :]

        copies = {}
        plan = (
            ('wq', wq_hbm, wq_s), ('wk', wk_hbm, wk_s),
            ('xa',) + xrows(0, 0, TK), ('xb',) + xrows(0, TK, C1 * TK), ('xc',) + xrows(0, C1 * TK, C2 * TK),
            ('xd',) + xrows(0, C2 * TK, T), ('wv', wv_hbm, wv_s), ('wao', wao_hbm, wao_s),
            ('wm1', wm_hbm.at[pl.ds(0, D), :], wm_s.at[pl.ds(0, D), :]), ('wup', wup_hbm, wup_s), ('dw', dw_hbm, dw_s),
            ('wdn', wdn_hbm, wdn_s), ('wm2', wm_hbm.at[pl.ds(D, D), :], wm_s.at[pl.ds(D, D), :]),
            ('xe',) + xrows(1, 0, TK),
        )
        for i, (name, src, dst) in enumerate(plan):
            copies[name] = pltpu.make_async_copy(src, dst, sems.at[i])
            copies[name].start()
        rest_copy().start()

        z_s[0] = 0
        z_s[1] = 0
        z_s[2] = 0
        for b in range(B):
            x_s[b * TP + T:(b + 1) * TP, :] = jnp.zeros((TP - T, D), x_s.dtype)
        store_g(g_s, TQ, jnp.zeros((HALO, D), F32))

        def keys(r0, n):
            return _unpack(xa0_s[r0 // H:(r0 + n) // H, 0:D])

        def ln_chunk(c):
            y = _ln(x_s[c * TK:(c + 1) * TK, :].astype(F32), EPS)
            xa0_s[c * TK // H:(c + 1) * TK // H, 0:D] = _pack(y)
            tb0_s[c * TR:(c + 1) * TR, 0:TW] = key_tables(y)

        scale = float(D) ** (-0.5) * math.log2(math.e)
        DS = D // 2
        copies['wq'].wait()
        copies['wk'].wait()
        m_lo = _dot_nt(wq_s[...], wk_s[0:DS, :])

        never = z_s[0] > 0

        def after(prev, l):
            return _unpack(l if prev is None else _tie(never, [prev[0:8, 0:LANES]], l, 0))

        copies['xa'].wait()
        wa_s[:, 0:DS] = _pack(_center(m_lo) * scale)
        wa_s[:, DS:D] = _pack(_center(_dot_nt(wq_s[...], wk_s[DS:D, :])) * scale)
        ln_chunk(0)
        qp = _pack(_dot(keys(0, TQ), _unpack(wa_s[:, 0:D])))
        q = _unpack(qp)

        def tail_parts():
            kt = keys(T - TAIL, TAIL)
            parts = []
            for n in range(NQT):
                qn = q[n * LANES:min((n + 1) * LANES, TQ), :]
                if qn.shape[0] < LANES:
                    qn = jnp.concatenate([qn, jnp.zeros((LANES - qn.shape[0], D), BF16)], axis=0)
                parts.append(_dot_nt(kt, qn))
            return parts

        def logits(c, prev, mx):
            last = c == NKV - 1
            parts = tail_parts() if last else None
            s = _dot_nt(after(prev, qp), keys(c * TK, (NFULL if last else CPK) * LANES))
            mc = None
            for t in range(CPK):
                if last and t == NFULL:
                    fill = jnp.full((LANES - TAIL, LANES), -jnp.inf, F32)
                    st = jnp.concatenate([jnp.concatenate([p, fill], axis=0).T for p in parts], axis=0)[0:TQ, :]
                else:
                    st = s[:, t * LANES:(t + 1) * LANES]
                s_s[c, :, t * LANES:(t + 1) * LANES] = st
                mc = st if mc is None else jnp.maximum(mc, st)
            return s, mc if mx is None else jnp.maximum(mx, mc)

        copies['xb'].wait()
        prev, mx = logits(0, None, None)
        for c in range(1, C1):
            ln_chunk(c)
            prev, mx = logits(c, prev, mx)

        copies['xc'].wait()
        prev = None
        for c in range(C1, C2):
            ln_chunk(c)
            prev, mx = logits(c, prev, mx)

        for name in ('xd', 'wv', 'wao'):
            copies[name].wait()
        wva_raw = _dot(wv_s[...], wao_s[...])
        mean = jnp.sum(wva_raw, axis=0, keepdims=True) * (1.0 / D)
        prev = wva_raw
        for c in range(C2, NKV):
            ln_chunk(c)
            prev, mx = logits(c, prev, mx)

        def tokens(res):
            return [res[r:r + 8, c * LANES:(c + 1) * LANES] for c in range(NC) for r in range(0, res.shape[0], 8)]

        def rel(t, lo, hi, v):
            return _released(never, t, lo, hi, v, NC)

        for name in ('wm1', 'wup', 'dw'):
            copies[name].wait()
        store_max(mx)
        xq = xa0_s[0:TQ // H, 0:D]
        hg = _dot(after(None, xq), wup_s[:, D:2 * D])
        hu = _dot(after(hg, xq), wup_s[:, 0:D])
        dwf = dw_s[...].astype(F32)
        for k in range(K):
            dwb_s[k] = jnp.broadcast_to(dwf[k:k + 1, :], (8, D))
        wva = (wva_raw - mean).astype(BF16)
        wvom = _dot(_tie_bf16(never, hu[0:8, 0:LANES], wva), wm_s[0:D, :])
        t1 = tokens(hg) + tokens(hu) + tokens(wvom)
        weight_tables(0, rel(t1, 0, 60, _unpack(wa_s[:, 0:D]).astype(F32)))
        weight_tables(1, rel(t1, 0, 70, wup_s[:, D:2 * D].astype(F32)))
        weight_tables(2, rel(t1, 60, 95, wup_s[:, 0:D].astype(F32)))

        for name in ('wdn', 'wm2'):
            copies[name].wait()
        wdm = _dot(wdn_s[...], wm_s[D:2 * D, :])
        t2 = tokens(wdm)
        store_g(gn_s, 0, _ln(_gelu2(rel(t2, 0, 40, hg)), 4.0 * EPS))
        u_s[...] = _gelu2(rel(t2, 0, 40, hu))
        weight_tables(3, rel(t2, 20, 80, wvom))
        weight_tables(4, 0.5 * wdm)
        copies['xe'].wait()

    def step_body(step, ba, bb, tune, normalise=False, do_a=True):
        sb = step - 1
        ia, ib = step - ba * NQ, sb - bb * NQ
        ORDER = tune['order']
        never = z_s[0] > 0
        never2 = z_s[1] > 0
        never3 = z_s[2] > 0
        for c in range(NC):
            g_s[c, 0:HALO, :] = jnp.where(ib == 0, 0.0, g_s[c, TQ:TQ + HALO, :])
            g_s[c, HALO:HALO + TQ, :] = gn_s[c]
        hist = []
        pend = []
        later = []

        def matmul(l, tiles, run):
            back = 0
            for res, n in reversed(hist):
                back += n
                if back >= tune['lag']:
                    l = _tie(never3, [res[0:8, 0:LANES]], l, 0)
                    break
            while later and later[0][0] <= len(hist) and len(pend) < 4:
                pend.append(later.pop(0)[1])
            if pend:
                l = _tie(never3, pend, l, 8)
                del pend[:]
            hist.append((run(_to_bf16(l)), tiles))
            return hist[-1][0]

        def toks(i0):
            return [res[r:r + 8, 0:LANES] for res, n in hist[i0:] for r in range(0, HR, 8 * (4 // n))]

        def rel2(v, t, lo, hi):
            return jnp.concatenate([_released(never, t, lo, hi, v[0:HR]), _released(never, t, lo, hi, v[HR:])],
                                   axis=0)

        def project(ops, mats, axis):
            m = [None] * NPROD
            for r in ORDER:
                m[r] = matmul(ops[r], len(mats), lambda v, r=r: _dot(v, _unpack(jnp.concatenate(
                    [wt_s[k * TR:(k + 1) * TR, r * LANES:(r + 1) * LANES] for k in mats], axis=axis))))
            return m

        def combine(prods, t=None, lo=0, hi=0):
            if t is not None:
                prods = list(prods)
                for r in ORDER[::tune['stride']]:
                    prods[r] = _released(never, t, lo, hi, prods[r])
            return unblock(FW.contract(prods, SUV, ORDER))

        m_old = m_s[...]
        u_old = u_s[...]
        if do_a:
            xq = xa_s[ba][pl.ds(_aligned(ia * (TQ // H), 8), TQ // H), 0:D]
            xops, _ = staged_operands(xo_s, _unpack(xq).astype(F32),
                                      [r for r in range(NPROD) if FU.node[r] >= FU.n])
            for r in range(NPROD):
                i = FU.node[r]
                if i < FU.n:
                    xops[r] = xq[(i // NC) * HR // H:(i // NC + 1) * HR // H, (i % NC) * LANES:(i % NC + 1) * LANES]
            qm = project(xops, [0], 1)
            gm = project(xops, [1, 2], 1)
            q_raw = combine(qm, toks(NPROD), 0, tune['q_end'])
            qops, done = staged_operands(qo_s, q_raw, list(range(NPROD)))
            pend.append(done)
        else:
            store_g(g_s, HALO + TQ, jnp.zeros((HALO, D), F32))
        state = {'l': None, 'acc': None, 'mx': None}

        def probabilities(g, t, lo, hi):
            for jj in range(G):
                j = g * G + jj
                m = m_old if t is None else rel2(m_old, t, lo + (hi - lo) * jj // G, lo + (hi - lo) * (jj + 1) // G)
                tiles = []
                lsum = None
                for c in range(CPK):
                    p = jnp.exp2(s_s[j, :, c * LANES:(c + 1) * LANES] - m)
                    lsum = p if lsum is None else lsum + p
                    tiles.append(p)
                state['l'] = lsum if state['l'] is None else state['l'] + lsum
                tiles[0] = jnp.where(never2, state['l'], tiles[0])
                w = jnp.concatenate(FW.expand(blocks_of(jnp.concatenate(tiles, axis=1))), axis=1)
                po_s[j * HR // H:(j + 1) * HR // H, :] = _pack(w)
            return fence(po_s)

        def store_logits(g, m, t):
            for jj in range(G):
                j = g * G + jj
                s = combine([v[:, jj * LANES:(jj + 1) * LANES] for v in m], t,
                            tune['s_end'] * jj // G, tune['s_end'] * (jj + 1) // G)
                for c, st in enumerate(_split(s)):
                    if j == NKV - 1 and c == NFULL:
                        st = jnp.where(lax.broadcasted_iota(jnp.int32, st.shape, 1) < TAIL, st, -jnp.inf)
                    s_s[j, :, c * LANES:(c + 1) * LANES] = st
                    state['mx'] = st if state['mx'] is None else jnp.maximum(state['mx'], st)

        def side_work(phase, t):
            if phase == tune['g_at']:
                gg = _gelu2(combine([v[:, 0:LANES] for v in gm], t, 0, tune['g'][0]))
                g_new = _ln(rel2(gg, t, *tune['g']), 4.0 * EPS)
                store_g(gn_s, 0, g_new)
                store_g(g_s, HALO + TQ, jnp.where(ia == 0, 0.0, g_new[0:HALO, :]))
            if phase == tune['u_at']:
                u_s[...] = _gelu2(combine([v[:, LANES:] for v in gm], t, 0, tune['u_end']))
            if phase == 3 and normalise:
                unit = jnp.minimum(step - 1, NU - 1)
                c0, r0 = unit // UPC, jnp.minimum((unit % UPC) * UP, LANES - UP)
                xv = [x_s[pl.ds(pl.multiple_of(TP + c0 * TK + k * LANES + r0, 16), UP), :].astype(F32)
                      for k in range(CPK)]
                y = _ln(jnp.concatenate([_released(never, t, 50, 80, v) for v in xv], axis=0), EPS)
                for k in range(CPK):
                    row = pl.multiple_of((c0 * TK + k * LANES + r0) // H, 8)
                    xa1_s[pl.ds(row, UT), 0:D] = _pack(y[k * UP:(k + 1) * UP])
                tb1_s[pl.ds(pl.multiple_of(c0 * TR + r0 // H, 8), UT), 0:TW] = key_tables(y)

        ready = None
        for g in range(NKV // G):
            if do_a:
                start = len(hist)
                sm = [None] * NPROD
                for r in ORDER:
                    sm[r] = matmul(qops[r], G, lambda v, r=r: _dot_nt(v, key_operand(ba, g, r)))
            if g == 0:
                ready = probabilities(0, toks(0) if do_a else None, *tune['e0'])
            if do_a:
                side_work(2 * g, toks(start))
            if tune['p_due']:
                pend.append(ready)
            start = len(hist)
            n = [None] * NPROD
            for r in PORDER:
                l = jnp.concatenate([po_s[j * HR // H:(j + 1) * HR // H, r * LANES:(r + 1) * LANES]
                                     for j in range(g * G, (g + 1) * G)], axis=1)
                n[r] = matmul(l, G, lambda v, r=r: _dot(v, key_operand(bb, g, r)))
            state['acc'] = n if state['acc'] is None else [x + y for x, y in zip(state['acc'], n)]
            t = toks(start)
            if do_a:
                store_logits(g, sm, t)
                if tune['s_due'][g] >= 0:
                    later.extend((len(hist) + tune['s_due'][g], state['mx'][r:r + 8]) for r in range(0, TQ, 8))
            if (g + 1) * G < NKV:
                ready = probabilities(g + 1, t, *tune['e1'])
            if do_a:
                side_work(2 * g + 1, t)
        yc = u_old * conv(never)
        ya = unblock(FU.contract(state['acc'], SWV, PORDER)) * (1.0 / jnp.sum(state['l'], axis=-1, keepdims=True))
        if tune['out_split']:
            om = project(FU.expand(blocks_of(yc)), [4], 0)
            om = [x + y for x, y in zip(om, project(FU.expand(blocks_of(ya)), [3], 0))]
        else:
            om = project([jnp.concatenate(p, axis=1)
                          for p in zip(FU.expand(blocks_of(ya)), FU.expand(blocks_of(yc)))], [3, 4], 0)
        out = combine(om)
        xr = x_s[pl.ds(_aligned(bb * TP + ib * TQ, 16), TQ), :].astype(F32)
        o_s[pl.ds(_aligned(sb * TQ, 16), TQ), :] = (xr + out).astype(o_s.dtype)
        if do_a:
            store_max(state['mx'])
        out_copy(sb).start()

    def iteration0(step, carry):
        step_body(step, 0, 0, TUNE['seq0'], normalise=True)

        @pl.when(step == 1)
        def _():
            rest_copy().wait()

        return carry

    def iteration1(step, carry):
        step_body(step, 1, 1, TUNE['seq1'])
        return carry

    first_step()
    lax.fori_loop(1, NQ, iteration0, 0)
    step_body(NQ + z_s[0], 1, 0, TUNE['seq1'])
    lax.fori_loop(NQ + 1, N, iteration1, 0)
    step_body(N, 1, 1, TUNE['last'], do_a=False)
    pltpu.make_async_copy(o_s, o_hbm, osem).wait()


@jax.jit
def pallas_standalone__conformer_family_branchformer__speech_kernel(
    x: jax.Array,
    w_q: jax.Array,
    w_k: jax.Array,
    w_v: jax.Array,
    w_ao: jax.Array,
    w_up: jax.Array,
    dw: jax.Array,
    w_dn: jax.Array,
    w_merge: jax.Array,
):
    B, T, D = x.shape
    K = dw.shape[0]
    TQ = 160
    TK = 512
    TP = -(-T // TK) * TK
    UR = 192
    NKV = TP // TK
    assert B == 2 and T % TQ == 0 and TQ % 32 == 0 and D == TK == 4 * LANES and K // 2 < HALO
    assert NKV * -(-TK // UR) < T // TQ and UR % 64 == 0 and NKV == 8 and T % LANES in (16, 32, 48, 64) and TP - T < LANES
    x2 = x.reshape(B * T, D)

    kern = functools.partial(_kernel, B=B, T=T, D=D, K=K, TQ=TQ, TK=TK, TP=TP, UR=UR)
    ins = (x2, w_q, w_k, w_v, w_ao, w_up, dw, w_dn, w_merge)
    out = pl.pallas_call(
        kern,
        in_specs=[pl.BlockSpec(memory_space=pl.ANY) for _ in ins],
        out_specs=pl.BlockSpec(memory_space=pl.ANY),
        out_shape=jax.ShapeDtypeStruct((B * T, D), x.dtype),
        scratch_shapes=[pltpu.VMEM((B * TP, D), x.dtype)] + [pltpu.VMEM(a.shape, a.dtype) for a in ins[1:]] + [
            pltpu.SemaphoreType.DMA((15,)),
            pltpu.VMEM((TP // H, D + 2 * LANES), U32),
            pltpu.VMEM((TP // H, D + 2 * LANES), U32),
            pltpu.VMEM((D // H, D), U32),
            pltpu.VMEM((K, 8, D), F32),
            pltpu.VMEM((NKV, TQ, TK), F32),
            pltpu.VMEM((TQ, LANES), F32),
            pltpu.VMEM((TQ, D), F32),
            pltpu.VMEM((D // LANES, TQ + 2 * HALO, LANES), F32),
            pltpu.VMEM((D // LANES, TQ, LANES), F32),
            pltpu.VMEM((B * T, D), x.dtype),
            pltpu.SemaphoreType.DMA(()),
            pltpu.VMEM((NKV * LANES // H, (len(TABLED) + 1) * LANES), U32),
            pltpu.VMEM((NKV * LANES // H, (len(TABLED) + 1) * LANES), U32),
            pltpu.VMEM((5 * LANES // H, NPROD * LANES), U32),
            pltpu.VMEM((NKV * TQ // 2 // H, NPROD * LANES), U32),
            pltpu.VMEM((TQ // 2 // H, NPROD * LANES), U32),
            pltpu.VMEM((TQ // 2 // H, NPROD * LANES), U32),
            pltpu.SMEM((3,), jnp.int32),
        ],
        compiler_params=pltpu.CompilerParams(
            vmem_limit_bytes=100 * 1024 * 1024,
            disable_bounds_checks=True,
            disable_semaphore_checks=True,
        ),
    )(*ins)
    return out.reshape(B, T, D)
```

```python
import functools
import math

import jax
import jax.numpy as jnp
from jax import lax
import jax.experimental.pallas as pl
import jax.experimental.pallas.tpu as pltpu

LANES = 128
EPS = 1e-05
F32 = jnp.float32
BF16 = jnp.bfloat16
U32 = jnp.uint32
NT = (((1,), (1,)), ((), ()))
HALO = 16
H = 2

SCHEME = (
    ('...-++..', '...+............', '-+.....+'),
    ('.+-.....', '.........-......', '.++..++.'),
    ('+...--..', '.+..+.......+...', '-+..-...'),
    ('.+.-.-.+', '...-...+....+...', '.-.+....'),
    ('.....+..', '.+...-+......-..', '.....-..'),
    ('+...-...', '+.-.-.......-...', '....-...'),
    ('--.+....', '...-........+...', '+-.+....'),
    ('..+...-.', '......+.-.+-....', '..+.....'),
    ('..-+....', '...........+....', '..--....'),
    ('-.....+.', '..+.....+.......', '..-.+...'),
    ('....+.-.', '..+.............', '....+.+.'),
    ('+.-.....', '........+.......', '-.-.....'),
    ('...-....', '...-.......-.-.-', '...+...+'),
    ('++..--..', '...-+.......+...', '+-......'),
    ('......+.', '..-......+-...-.', '..-...-.'),
    ('-.......', '++......+...+...', '-...-...'),
    ('-....-.+', '............+...', '.+.-+...'),
    ('.-+..+-.', '......+.........', '.....++.'),
    ('.-......', '...+--.-.-..-...', '.+......'),
    ('...-.-.+', '...+...-.....+..', '.-.+...+'),
    ('....--..', '.+..............', '+-..+-..'),
    ('...+...-', '...+...-......+-', '.......+'),
    ('...-..+.', '...........-..-.', '..+....-'),
    ('.-+...-.', '......-..-......', '..+..++.'),
    ('......+-', '..............+.', '......--'),
    ('.....-.+', '.............+..', '.+.-.+.-'),
)

_BASE = dict(order=[15, 12, 14, 10, 23, 18, 6, 17, 16, 1, 22, 0, 25, 2, 11, 3, 8, 13, 9, 19, 20, 24, 4, 5, 7, 21],
             lag=8, stride=3, q_end=60, e0=(45, 85), e1=(0, 100), s_end=60, s_due=(5, 10), p_due=True,
             g_at=2, g=(50, 90), u_at=3, u_end=20, out_split=False)
TUNE = {
    'seq0': dict(_BASE, order=[15, 12, 14, 0, 8, 4, 11, 13, 17, 1, 3, 18, 16, 25, 6, 9, 22, 2, 23, 20, 19, 10, 24, 5, 7, 21],
                 lag=9, stride=4, q_end=70, e0=(30, 92), e1=(10, 100), s_due=(5, -1), u_at=0, u_end=60),
    'seq1': dict(_BASE, order=[15, 12, 14, 10, 4, 13, 22, 0, 9, 20, 18, 11, 25, 3, 8, 24, 6, 2, 1, 17, 19, 23, 16, 5, 7, 21],
                 lag=9, q_end=70, s_end=70, s_due=(0, -1)),
    'last': dict(_BASE, lag=10, e1=(20, 80), p_due=False, out_split=True),
}


class _Forms:
    def __init__(self, rows):
        self.n = len(rows[0])
        forms = [{j: 1 if ch == '+' else -1 for j, ch in enumerate(r) if ch != '.'} for r in rows]
        self.steps = []
        while True:
            count = {}
            seen = set()
            for f in forms:
                items = sorted(f.items())
                key = tuple((j, v * items[0][1]) for j, v in items)
                if key not in seen:
                    seen.add(key)
                    for a in range(len(items)):
                        for b in range(a + 1, len(items)):
                            pair = (items[a][0], items[b][0], items[a][1] * items[b][1])
                            count[pair] = count.get(pair, 0) + 1
            if not count:
                break
            j, k, sg = max(count, key=count.get)
            new = self.n + len(self.steps)
            self.steps.append((j, k, sg))
            for f in forms:
                if j in f and k in f and f[j] * f[k] == sg:
                    f[new] = f.pop(j)
                    f.pop(k)
        self.node = [next(iter(f)) for f in forms]
        self.sign = [next(iter(f.values())) for f in forms]

    def expand(self, blocks):
        nodes = list(blocks)
        for j, k, sg in self.steps:
            nodes.append(nodes[j] + nodes[k] if sg > 0 else nodes[j] - nodes[k])
        return [nodes[i] for i in self.node]

    def contract(self, prods, signs, order):
        acc = {}

        def add(i, v, s):
            if i not in acc:
                acc[i] = (v, s)
            else:
                w, t = acc[i]
                acc[i] = (w + v, s) if s == t else ((w - v, 1) if t > 0 else (v - w, 1))

        for r in order:
            if self.node[r] >= self.n:
                add(self.node[r], prods[r], self.sign[r] * signs[r])
        for i in reversed(range(len(self.steps))):
            j, k, sg = self.steps[i]
            v, s = acc[self.n + i]
            add(j, v, s)
            add(k, v, s * sg)
        for r in order:
            if self.node[r] < self.n:
                add(self.node[r], prods[r], self.sign[r] * signs[r])
        return [acc[j][0] if acc[j][1] > 0 else -acc[j][0] for j in range(self.n)]


FU, FV, FW = (_Forms([t[i] for t in SCHEME]) for i in range(3))
NPROD = len(SCHEME)
TABLED = [r for r in range(NPROD) if FV.node[r] >= FV.n]


def _ln(x, eps):
    d = x.shape[-1]
    m = jnp.sum(x, axis=-1, keepdims=True) * (1.0 / d)
    xc = x - m
    v = jnp.sum(xc * xc, axis=-1, keepdims=True) * (1.0 / d)
    return xc * lax.rsqrt(v + eps)


def _gelu2(x):
    c1 = math.sqrt(2.0 / math.pi)
    c2 = c1 * 0.044715
    t = jnp.tanh(x * (c1 + c2 * (x * x)))
    return x + x * t


def _center(w):
    return w - jnp.sum(w, axis=0, keepdims=True) * (1.0 / w.shape[0])


def _pack(x):
    return pltpu.bitcast(x.astype(BF16), U32)


def _unpack(x):
    return pltpu.bitcast(x, BF16)


def _bits(x):
    return pltpu.bitcast(x, U32)


def _to_bf16(v):
    return _unpack(v) if v.dtype == U32 else v.astype(BF16)


def _dot(a, b):
    return jnp.dot(a, b, preferred_element_type=F32)


def _dot_nt(a, b):
    return lax.dot_general(a, b, NT, preferred_element_type=F32)


def _split(v):
    return [v[:, c * LANES:(c + 1) * LANES] for c in range(v.shape[1] // LANES)]


def _aligned(i, n):
    return i if isinstance(i, int) else pl.multiple_of(i, n)


def _tie_bf16(flag, dep, val):
    head = _bits(val[0:16, 0:LANES])
    head = _unpack(jnp.where(flag, _bits(dep), head))
    top = jnp.concatenate([head, val[0:16, LANES:]], axis=1)
    return jnp.concatenate([top, val[16:, :]], axis=0)


def _tie(flag, deps, val, row):
    cast = _bits if val.dtype == U32 else (lambda v: v if v.dtype == F32 else pltpu.bitcast(v, F32))
    tiles = _split(val)
    t = tiles[0]
    end = row + 8 * len(deps)
    mid = jnp.where(flag, jnp.concatenate([cast(d) for d in deps], axis=0), t[row:end])
    tiles[0] = jnp.concatenate(([t[0:row]] if row else []) + [mid] + ([t[end:]] if end < t.shape[0] else []),
                               axis=0)
    return jnp.concatenate(tiles, axis=1)


def _released(flag, toks, lo, hi, val, ntiles=1):
    first, total = len(toks) * lo // 100, len(toks) * (hi - lo) // 100
    n = val.shape[0] // 8
    rel = jnp.concatenate([toks[min(first + (i * total) // n, len(toks) - 1)] for i in range(n)], axis=0)
    tiles = _split(val)
    return jnp.concatenate([jnp.where(flag, rel, t) if c < ntiles else t for c, t in enumerate(tiles)], axis=1)


def _kernel(x_hbm, wq_hbm, wk_hbm, wv_hbm, wao_hbm, wup_hbm, dw_hbm, wdn_hbm, wm_hbm,
            o_hbm,
            x_s, wq_s, wk_s, wv_s, wao_s, wup_s, dw_s, wdn_s, wm_s, sems,
            xa0_s, xa1_s, wa_s, dwb_s, s_s, m_s, u_s, g_s, gn_s, o_s, osem,
            tb0_s, tb1_s, wt_s, po_s, xo_s, qo_s, z_s,
            *, B, T, D, K, TQ, TK, TP, UR):
    NQ = T // TQ
    N = B * NQ
    NKV = TP // TK
    NC = D // LANES
    CPK = TK // LANES
    PAD = K // 2
    NQT = -(-TQ // LANES)
    NFULL = (T - (NKV - 1) * TK) // LANES
    TAIL = T % LANES
    HR = TQ // 2
    TR = LANES // H
    TW = len(TABLED) * LANES
    G = 4
    UP = UR // CPK
    UPC = -(-LANES // UP)
    NU = NKV * UPC
    UT = UP // H
    PORDER = sorted(range(NPROD), key=lambda r: FU.node[r] < FU.n)
    SUV = [FU.sign[r] * FV.sign[r] for r in range(NPROD)]
    SWV = [FW.sign[r] * FV.sign[r] for r in range(NPROD)]
    xa_s, tb_s = (xa0_s, xa1_s), (tb0_s, tb1_s)

    def blocks_of(a):
        return [a[h * HR:(h + 1) * HR, c * LANES:(c + 1) * LANES] for h in range(2) for c in range(NC)]

    def unblock(bl):
        return jnp.concatenate([jnp.concatenate(bl[h * NC:(h + 1) * NC], axis=1) for h in range(2)], axis=0)

    def key_tables(y):
        n = y.shape[0] // CPK
        ops = FV.expand([y[t * n:(t + 1) * n, d * LANES:(d + 1) * LANES] for d in range(NC) for t in range(CPK)])
        return _pack(jnp.concatenate([ops[r] for r in TABLED], axis=1))

    def weight_tables(mat, w):
        ops = FV.expand([w[d * LANES:(d + 1) * LANES, t * LANES:(t + 1) * LANES]
                         for d in range(NC) for t in range(NC)])
        wt_s[mat * TR:(mat + 1) * TR, :] = _pack(jnp.concatenate(ops, axis=1))

    def fence(ref):
        return ref[pl.ds(pl.multiple_of(z_s[0], 8), 8), 0:LANES]

    def staged_operands(ref, a, which):
        ops = FU.expand(blocks_of(a))
        ref[:, 0:len(which) * LANES] = _pack(jnp.concatenate([ops[r] for r in which], axis=1))
        done = fence(ref)
        return {r: ref[:, k * LANES:(k + 1) * LANES] for k, r in enumerate(which)}, done

    def key_operand(b, g, r):
        i = FV.node[r]
        if i < FV.n:
            d, t = i // CPK, i % CPK
            parts = [xa_s[b][pl.ds((j * TK + t * LANES) // H, TR), d * LANES:(d + 1) * LANES]
                     for j in range(g * G, (g + 1) * G)]
        else:
            k = TABLED.index(r)
            parts = [tb_s[b][j * TR:(j + 1) * TR, k * LANES:(k + 1) * LANES] for j in range(g * G, (g + 1) * G)]
        return _unpack(jnp.concatenate(parts, axis=0))

    def store_g(ref, row, g):
        for c in range(NC):
            ref[c, row:row + g.shape[0], :] = g[:, c * LANES:(c + 1) * LANES]

    def conv(flag):
        taps = [[g_s[c, pl.ds(HALO - PAD + k, TQ), :] for k in range(K)] for c in range(NC)]
        wts = [dwb_s[k] for k in range(K)]
        prev = None
        rows = []
        for rr in range(0, TQ, 16):
            cols = []
            for c in range(NC):
                acc = None
                for k in range(K):
                    gv = taps[c][k][rr:rr + 16].reshape(2, 8, LANES)
                    term = gv * wts[k][None, :, c * LANES:(c + 1) * LANES]
                    if acc is None:
                        acc = term if prev is None else jnp.where(flag, prev, term)
                    else:
                        acc = acc + term
                prev = acc
                cols.append(acc.reshape(16, LANES))
            rows.append(jnp.concatenate(cols, axis=1))
        return jnp.concatenate(rows, axis=0)

    def store_max(mx):
        m = jnp.max(mx, axis=-1, keepdims=True)
        m = m + jnp.log2(jnp.sum(jnp.exp2(mx - m), axis=-1, keepdims=True))
        m_s[...] = jnp.broadcast_to(m, (TQ, LANES))

    def rest_copy():
        return pltpu.make_async_copy(x_hbm.at[pl.ds(T + TK, T - TK), :], x_s.at[pl.ds(TP + TK, T - TK), :],
                                     sems.at[14])

    def out_copy(blk):
        rows = pl.ds(_aligned(blk * TQ, 16), TQ)
        return pltpu.make_async_copy(o_s.at[rows, :], o_hbm.at[rows, :], osem)

    def first_step():
        C1, C2 = 3, 6

        def xrows(b, r0, r1):
            return x_hbm.at[pl.ds(b * T + r0, r1 - r0), :], x_s.at[pl.ds(b * TP + r0, r1 - r0), :]

        copies = {}
        plan = (
            ('wq', wq_hbm, wq_s), ('wk', wk_hbm, wk_s),
            ('xa',) + xrows(0, 0, TK), ('xb',) + xrows(0, TK, C1 * TK), ('xc',) + xrows(0, C1 * TK, C2 * TK),
            ('xd',) + xrows(0, C2 * TK, T), ('wv', wv_hbm, wv_s), ('wao', wao_hbm, wao_s),
            ('wm1', wm_hbm.at[pl.ds(0, D), :], wm_s.at[pl.ds(0, D), :]), ('wup', wup_hbm, wup_s), ('dw', dw_hbm, dw_s),
            ('wdn', wdn_hbm, wdn_s), ('wm2', wm_hbm.at[pl.ds(D, D), :], wm_s.at[pl.ds(D, D), :]),
            ('xe',) + xrows(1, 0, TK),
        )
        for i, (name, src, dst) in enumerate(plan):
            copies[name] = pltpu.make_async_copy(src, dst, sems.at[i])
            copies[name].start()
        rest_copy().start()

        z_s[0] = 0
        z_s[1] = 0
        z_s[2] = 0
        for b in range(B):
            x_s[b * TP + T:(b + 1) * TP, :] = jnp.zeros((TP - T, D), x_s.dtype)
        store_g(g_s, TQ, jnp.zeros((HALO, D), F32))

        def keys(r0, n):
            return _unpack(xa0_s[r0 // H:(r0 + n) // H, 0:D])

        def ln_chunk(c):
            y = _ln(x_s[c * TK:(c + 1) * TK, :].astype(F32), EPS)
            xa0_s[c * TK // H:(c + 1) * TK // H, 0:D] = _pack(y)
            tb0_s[c * TR:(c + 1) * TR, 0:TW] = key_tables(y)

        scale = float(D) ** (-0.5) * math.log2(math.e)
        DS = D // 2
        copies['wq'].wait()
        copies['wk'].wait()
        m_lo = _dot_nt(wq_s[...], wk_s[0:DS, :])

        never = z_s[0] > 0

        def after(prev, l):
            return _unpack(l if prev is None else _tie(never, [prev[0:8, 0:LANES]], l, 0))

        copies['xa'].wait()
        wa_s[:, 0:DS] = _pack(_center(m_lo) * scale)
        wa_s[:, DS:D] = _pack(_center(_dot_nt(wq_s[...], wk_s[DS:D, :])) * scale)
        ln_chunk(0)
        qp = _pack(_dot(keys(0, TQ), _unpack(wa_s[:, 0:D])))
        q = _unpack(qp)

        def tail_parts():
            kt = keys(T - TAIL, TAIL)
            parts = []
            for n in range(NQT):
                qn = q[n * LANES:min((n + 1) * LANES, TQ), :]
                if qn.shape[0] < LANES:
                    qn = jnp.concatenate([qn, jnp.zeros((LANES - qn.shape[0], D), BF16)], axis=0)
                parts.append(_dot_nt(kt, qn))
            return parts

        def logits(c, prev, mx):
            last = c == NKV - 1
            parts = tail_parts() if last else None
            s = _dot_nt(after(prev, qp), keys(c * TK, (NFULL if last else CPK) * LANES))
            mc = None
            for t in range(CPK):
                if last and t == NFULL:
                    fill = jnp.full((LANES - TAIL, LANES), -jnp.inf, F32)
                    st = jnp.concatenate([jnp.concatenate([p, fill], axis=0).T for p in parts], axis=0)[0:TQ, :]
                else:
                    st = s[:, t * LANES:(t + 1) * LANES]
                s_s[c, :, t * LANES:(t + 1) * LANES] = st
                mc = st if mc is None else jnp.maximum(mc, st)
            return s, mc if mx is None else jnp.maximum(mx, mc)

        copies['xb'].wait()
        prev, mx = logits(0, None, None)
        for c in range(1, C1):
            ln_chunk(c)
            prev, mx = logits(c, prev, mx)

        copies['xc'].wait()
        prev = None
        for c in range(C1, C2):
            ln_chunk(c)
            prev, mx = logits(c, prev, mx)

        for name in ('xd', 'wv', 'wao'):
            copies[name].wait()
        wva_raw = _dot(wv_s[...], wao_s[...])
        mean = jnp.sum(wva_raw, axis=0, keepdims=True) * (1.0 / D)
        prev = wva_raw
        for c in range(C2, NKV):
            ln_chunk(c)
            prev, mx = logits(c, prev, mx)

        def tokens(res):
            return [res[r:r + 8, c * LANES:(c + 1) * LANES] for c in range(NC) for r in range(0, res.shape[0], 8)]

        def rel(t, lo, hi, v):
            return _released(never, t, lo, hi, v, NC)

        for name in ('wm1', 'wup', 'dw'):
            copies[name].wait()
        store_max(mx)
        xq = xa0_s[0:TQ // H, 0:D]
        hg = _dot(after(None, xq), wup_s[:, D:2 * D])
        hu = _dot(after(hg, xq), wup_s[:, 0:D])
        dwf = dw_s[...].astype(F32)
        for k in range(K):
            dwb_s[k] = jnp.broadcast_to(dwf[k:k + 1, :], (8, D))
        wva = (wva_raw - mean).astype(BF16)
        wvom = _dot(_tie_bf16(never, hu[0:8, 0:LANES], wva), wm_s[0:D, :])
        t1 = tokens(hg) + tokens(hu) + tokens(wvom)
        weight_tables(0, rel(t1, 0, 60, _unpack(wa_s[:, 0:D]).astype(F32)))
        weight_tables(1, rel(t1, 0, 70, wup_s[:, D:2 * D].astype(F32)))
        weight_tables(2, rel(t1, 60, 95, wup_s[:, 0:D].astype(F32)))

        for name in ('wdn', 'wm2'):
            copies[name].wait()
        wdm = _dot(wdn_s[...], wm_s[D:2 * D, :])
        t2 = tokens(wdm)
        store_g(gn_s, 0, _ln(_gelu2(rel(t2, 0, 40, hg)), 4.0 * EPS))
        u_s[...] = _gelu2(rel(t2, 0, 40, hu))
        weight_tables(3, rel(t2, 20, 80, wvom))
        weight_tables(4, 0.5 * wdm)
        copies['xe'].wait()

    def step_body(step, ba, bb, tune, normalise=False, do_a=True):
        sb = step - 1
        ia, ib = step - ba * NQ, sb - bb * NQ
        ORDER = tune['order']
        never = z_s[0] > 0
        never2 = z_s[1] > 0
        never3 = z_s[2] > 0
        for c in range(NC):
            g_s[c, 0:HALO, :] = jnp.where(ib == 0, 0.0, g_s[c, TQ:TQ + HALO, :])
            g_s[c, HALO:HALO + TQ, :] = gn_s[c]
        hist = []
        pend = []
        later = []

        def matmul(l, tiles, run):
            back = 0
            for res, n in reversed(hist):
                back += n
                if back >= tune['lag']:
                    l = _tie(never3, [res[0:8, 0:LANES]], l, 0)
                    break
            while later and later[0][0] <= len(hist) and len(pend) < 4:
                pend.append(later.pop(0)[1])
            if pend:
                l = _tie(never3, pend, l, 8)
                del pend[:]
            hist.append((run(_to_bf16(l)), tiles))
            return hist[-1][0]

        def toks(i0):
            return [res[r:r + 8, 0:LANES] for res, n in hist[i0:] for r in range(0, HR, 8 * (4 // n))]

        def rel2(v, t, lo, hi):
            return jnp.concatenate([_released(never, t, lo, hi, v[0:HR]), _released(never, t, lo, hi, v[HR:])],
                                   axis=0)

        def project(ops, mats, axis):
            m = [None] * NPROD
            for r in ORDER:
                m[r] = matmul(ops[r], len(mats), lambda v, r=r: _dot(v, _unpack(jnp.concatenate(
                    [wt_s[k * TR:(k + 1) * TR, r * LANES:(r + 1) * LANES] for k in mats], axis=axis))))
            return m

        def combine(prods, t=None, lo=0, hi=0):
            if t is not None:
                prods = list(prods)
                for r in ORDER[::tune['stride']]:
                    prods[r] = _released(never, t, lo, hi, prods[r])
            return unblock(FW.contract(prods, SUV, ORDER))

        m_old = m_s[...]
        u_old = u_s[...]
        if do_a:
            xq = xa_s[ba][pl.ds(_aligned(ia * (TQ // H), 8), TQ // H), 0:D]
            xops, _ = staged_operands(xo_s, _unpack(xq).astype(F32),
                                      [r for r in range(NPROD) if FU.node[r] >= FU.n])
            for r in range(NPROD):
                i = FU.node[r]
                if i < FU.n:
                    xops[r] = xq[(i // NC) * HR // H:(i // NC + 1) * HR // H, (i % NC) * LANES:(i % NC + 1) * LANES]
            qm = project(xops, [0], 1)
            gm = project(xops, [1, 2], 1)
            q_raw = combine(qm, toks(NPROD), 0, tune['q_end'])
            qops, done = staged_operands(qo_s, q_raw, list(range(NPROD)))
            pend.append(done)
        else:
            store_g(g_s, HALO + TQ, jnp.zeros((HALO, D), F32))
        state = {'l': None, 'acc': None, 'mx': None}

        def probabilities(g, t, lo, hi):
            for jj in range(G):
                j = g * G + jj
                m = m_old if t is None else rel2(m_old, t, lo + (hi - lo) * jj // G, lo + (hi - lo) * (jj + 1) // G)
                tiles = []
                lsum = None
                for c in range(CPK):
                    p = jnp.exp2(s_s[j, :, c * LANES:(c + 1) * LANES] - m)
                    lsum = p if lsum is None else lsum + p
                    tiles.append(p)
                state['l'] = lsum if state['l'] is None else state['l'] + lsum
                tiles[0] = jnp.where(never2, state['l'], tiles[0])
                w = jnp.concatenate(FW.expand(blocks_of(jnp.concatenate(tiles, axis=1))), axis=1)
                po_s[j * HR // H:(j + 1) * HR // H, :] = _pack(w)
            return fence(po_s)

        def store_logits(g, m, t):
            for jj in range(G):
                j = g * G + jj
                s = combine([v[:, jj * LANES:(jj + 1) * LANES] for v in m], t,
                            tune['s_end'] * jj // G, tune['s_end'] * (jj + 1) // G)
                for c, st in enumerate(_split(s)):
                    if j == NKV - 1 and c == NFULL:
                        st = jnp.where(lax.broadcasted_iota(jnp.int32, st.shape, 1) < TAIL, st, -jnp.inf)
                    s_s[j, :, c * LANES:(c + 1) * LANES] = st
                    state['mx'] = st if state['mx'] is None else jnp.maximum(state['mx'], st)

        def side_work(phase, t):
            if phase == tune['g_at']:
                gg = _gelu2(combine([v[:, 0:LANES] for v in gm], t, 0, tune['g'][0]))
                g_new = _ln(rel2(gg, t, *tune['g']), 4.0 * EPS)
                store_g(gn_s, 0, g_new)
                store_g(g_s, HALO + TQ, jnp.where(ia == 0, 0.0, g_new[0:HALO, :]))
            if phase == tune['u_at']:
                u_s[...] = _gelu2(combine([v[:, LANES:] for v in gm], t, 0, tune['u_end']))
            if phase == 3 and normalise:
                unit = jnp.minimum(step - 1, NU - 1)
                c0, r0 = unit // UPC, jnp.minimum((unit % UPC) * UP, LANES - UP)
                xv = [x_s[pl.ds(pl.multiple_of(TP + c0 * TK + k * LANES + r0, 16), UP), :].astype(F32)
                      for k in range(CPK)]
                y = _ln(jnp.concatenate([_released(never, t, 50, 80, v) for v in xv], axis=0), EPS)
                for k in range(CPK):
                    row = pl.multiple_of((c0 * TK + k * LANES + r0) // H, 8)
                    xa1_s[pl.ds(row, UT), 0:D] = _pack(y[k * UP:(k + 1) * UP])
                tb1_s[pl.ds(pl.multiple_of(c0 * TR + r0 // H, 8), UT), 0:TW] = key_tables(y)

        ready = None
        for g in range(NKV // G):
            if do_a:
                start = len(hist)
                sm = [None] * NPROD
                for r in ORDER:
                    sm[r] = matmul(qops[r], G, lambda v, r=r: _dot_nt(v, key_operand(ba, g, r)))
            if g == 0:
                ready = probabilities(0, toks(0) if do_a else None, *tune['e0'])
            if do_a:
                side_work(2 * g, toks(start))
            if tune['p_due']:
                pend.append(ready)
            start = len(hist)
            n = [None] * NPROD
            for r in PORDER:
                l = jnp.concatenate([po_s[j * HR // H:(j + 1) * HR // H, r * LANES:(r + 1) * LANES]
                                     for j in range(g * G, (g + 1) * G)], axis=1)
                n[r] = matmul(l, G, lambda v, r=r: _dot(v, key_operand(bb, g, r)))
            state['acc'] = n if state['acc'] is None else [x + y for x, y in zip(state['acc'], n)]
            t = toks(start)
            if do_a:
                store_logits(g, sm, t)
                if tune['s_due'][g] >= 0:
                    later.extend((len(hist) + tune['s_due'][g], state['mx'][r:r + 8]) for r in range(0, TQ, 8))
            if (g + 1) * G < NKV:
                ready = probabilities(g + 1, t, *tune['e1'])
            if do_a:
                side_work(2 * g + 1, t)
        yc = u_old * conv(never)
        ya = unblock(FU.contract(state['acc'], SWV, PORDER)) * (1.0 / jnp.sum(state['l'], axis=-1, keepdims=True))
        if tune['out_split']:
            om = project(FU.expand(blocks_of(yc)), [4], 0)
            om = [x + y for x, y in zip(om, project(FU.expand(blocks_of(ya)), [3], 0))]
        else:
            om = project([jnp.concatenate(p, axis=1)
                          for p in zip(FU.expand(blocks_of(ya)), FU.expand(blocks_of(yc)))], [3, 4], 0)
        out = combine(om)
        xr = x_s[pl.ds(_aligned(bb * TP + ib * TQ, 16), TQ), :].astype(F32)
        o_s[pl.ds(_aligned(sb * TQ, 16), TQ), :] = (xr + out).astype(o_s.dtype)
        if do_a:
            store_max(state['mx'])
        out_copy(sb).start()

    def iteration0(step, carry):
        step_body(step, 0, 0, TUNE['seq0'], normalise=True)

        @pl.when(step == 1)
        def _():
            rest_copy().wait()

        return carry

    def iteration1(step, carry):
        step_body(step, 1, 1, TUNE['seq1'])
        return carry

    first_step()
    lax.fori_loop(1, NQ, iteration0, 0)
    step_body(NQ + z_s[0], 1, 0, TUNE['seq1'])
    lax.fori_loop(NQ + 1, N, iteration1, 0)
    step_body(N, 1, 1, TUNE['last'], do_a=False)
    pltpu.make_async_copy(o_s, o_hbm, osem).wait()


@jax.jit
def pallas_standalone__conformer_family_branchformer__speech_kernel(
    x: jax.Array,
    w_q: jax.Array,
    w_k: jax.Array,
    w_v: jax.Array,
    w_ao: jax.Array,
    w_up: jax.Array,
    dw: jax.Array,
    w_dn: jax.Array,
    w_merge: jax.Array,
):
    B, T, D = x.shape
    K = dw.shape[0]
    TQ = 160
    TK = 512
    TP = -(-T // TK) * TK
    UR = 192
    NKV = TP // TK
    assert B == 2 and T % TQ == 0 and TQ % 32 == 0 and D == TK == 4 * LANES and K // 2 < HALO
    assert NKV * -(-TK // UR) < T // TQ and UR % 64 == 0 and NKV == 8 and T % LANES in (16, 32, 48, 64) and TP - T < LANES
    x2 = x.reshape(B * T, D)

    kern = functools.partial(_kernel, B=B, T=T, D=D, K=K, TQ=TQ, TK=TK, TP=TP, UR=UR)
    ins = (x2, w_q, w_k, w_v, w_ao, w_up, dw, w_dn, w_merge)
    out = pl.pallas_call(
        kern,
        in_specs=[pl.BlockSpec(memory_space=pl.ANY) for _ in ins],
        out_specs=pl.BlockSpec(memory_space=pl.ANY),
        out_shape=jax.ShapeDtypeStruct((B * T, D), x.dtype),
        scratch_shapes=[pltpu.VMEM((B * TP, D), x.dtype)] + [pltpu.VMEM(a.shape, a.dtype) for a in ins[1:]] + [
            pltpu.SemaphoreType.DMA((15,)),
            pltpu.VMEM((TP // H, D + 2 * LANES), U32),
            pltpu.VMEM((TP // H, D + 2 * LANES), U32),
            pltpu.VMEM((D // H, D), U32),
            pltpu.VMEM((K, 8, D), F32),
            pltpu.VMEM((NKV, TQ, TK), F32),
            pltpu.VMEM((TQ, LANES), F32),
            pltpu.VMEM((TQ, D), F32),
            pltpu.VMEM((D // LANES, TQ + 2 * HALO, LANES), F32),
            pltpu.VMEM((D // LANES, TQ, LANES), F32),
            pltpu.VMEM((B * T, D), x.dtype),
            pltpu.SemaphoreType.DMA(()),
            pltpu.VMEM((NKV * LANES // H, (len(TABLED) + 1) * LANES), U32),
            pltpu.VMEM((NKV * LANES // H, (len(TABLED) + 1) * LANES), U32),
            pltpu.VMEM((5 * LANES // H, NPROD * LANES), U32),
            pltpu.VMEM((NKV * TQ // 2 // H, NPROD * LANES), U32),
            pltpu.VMEM((TQ // 2 // H, NPROD * LANES), U32),
            pltpu.VMEM((TQ // 2 // H, NPROD * LANES), U32),
            pltpu.SMEM((3,), jnp.int32),
        ],
        compiler_params=pltpu.CompilerParams(
            vmem_limit_bytes=100 * 1024 * 1024,
            disable_bounds_checks=True,
            disable_semaphore_checks=True,
        ),
    )(*ins)
    return out.reshape(B, T, D)
```
